```python
import jax
import jax.numpy as jnp

def _softmax(x, axis=-1):
    return jax.nn.softmax(x, axis=axis)
def _gelu(x):
    return jax.nn.gelu(x, approximate=True)
def _silu(x):
    return jax.nn.silu(x)
def _sigmoid(x):
    return jax.nn.sigmoid(x)
def _layernorm(x, axis=-1, eps=1e-5):
    m = jnp.mean(x, axis=axis, keepdims=True)
    v = jnp.var(x, axis=axis, keepdims=True)
    return (x - m) / jnp.sqrt(v + eps)
def _scatter_add(tgt, idx, src, axis=0):
    return tgt.at[idx].add(src)
def _segment_sum(src, seg, n):
    return jax.ops.segment_sum(src, seg, n)
class _Rng:
    def __init__(self, key):
        self._k = key
    def _next(self):
        self._k, sub = jax.random.split(self._k)
        return sub
    def normal(self, shape):
        return jax.random.normal(self._next(), shape, dtype=jnp.bfloat16)
    def randint(self, lo, hi, shape):
        return jax.random.randint(self._next(), shape, lo, hi, dtype=jnp.int32)
    def uniform(self, shape, lo=0.0, hi=1.0):
        return jax.random.uniform(self._next(), shape, jnp.bfloat16, lo, hi)
    def permutation(self, n):
        return jax.random.permutation(self._next(), n)


kernel_name = 'recurrent_scan__linear_kernel_hedgehog__moe_arch_mod__prompt'

def setup_inputs():
    _rng = _Rng(jax.random.key(int.from_bytes(__import__("os").urandom(4), "little")))
    _w = (lambda a: (lambda t: t.astype(jnp.bfloat16) if jnp.issubdtype(t.dtype, jnp.floating) else t)(jnp.asarray(a)))
    def _A_setup():
        B, S, D, H = 1, 2048, 1024, 32
        Dh = D // H
        return {
            "x": _w((lambda *s: _rng.normal(s) * 0.05)(B, S, D)),
            "wqkv": _w((lambda *s: _rng.normal(s) * 0.05)(D, 3 * D)),
            "w_phi": _w((lambda *s: _rng.normal(s) * 0.05)(H, Dh, Dh) * (Dh ** -0.5)),
            "wo": _w((lambda *s: _rng.normal(s) * 0.05)(D, D)),
        }
    _A_in = _A_setup()

    def _B_setup():
        B, S, D, F, C = 1, 2048, 1024, 3584, 1
        return {
            "x": _w((lambda *s: _rng.normal(s) * 0.05)(B, S, D)),
            "w_r": _w((lambda *s: _rng.normal(s) * 0.05)(D)),
            "w_gate": _w((lambda *s: _rng.normal(s) * 0.05)(D, F)),
            "w_up": _w((lambda *s: _rng.normal(s) * 0.05)(D, F)),
            "w_down": _w((lambda *s: _rng.normal(s) * 0.05)(F, D)),
        }
    _B_in = _B_setup()

    return {
        "A_x": _A_in["x"],
        "A_wqkv": _A_in["wqkv"],
        "A_w_phi": _A_in["w_phi"],
        "A_wo": _A_in["wo"],
        "B_x": _B_in["x"],
        "B_w_r": _B_in["w_r"],
        "B_w_gate": _B_in["w_gate"],
        "B_w_up": _B_in["w_up"],
        "B_w_down": _B_in["w_down"],
    }

def reference(A_x, A_wqkv, A_w_phi, A_wo, B_x, B_w_r, B_w_gate, B_w_up, B_w_down):
    def _A_ref(x, wqkv, w_phi, wo):
        B, S, D = x.shape
        H = 32; Dh = D // H
        qkv = (lambda x, *d: x.transpose(*d))((x @ wqkv).reshape(B, S, 3, H, Dh), 2, 0, 3, 1, 4)
        q, k, v = qkv[0], qkv[1], qkv[2]
        pq = jnp.einsum("bhsd,hdf->bhsf", q, w_phi)
        pk = jnp.einsum("bhsd,hdf->bhsf", k, w_phi)
        phi_q = jnp.concatenate([_softmax(pq, axis=-1), _softmax(-pq, axis=-1)], axis=-1)
        phi_k = jnp.concatenate([_softmax(pk, axis=-1), _softmax(-pk, axis=-1)], axis=-1)
        kv = jnp.einsum("bhsf,bhsd->bhfd", phi_k, v)
        z  = jnp.einsum("bhsf->bhf", phi_k)
        num = jnp.einsum("bhqf,bhfd->bhqd", phi_q, kv)
        den = jnp.einsum("bhqf,bhf->bhq", phi_q, z)[..., None] + 1e-6
        o = num / den
        return (lambda x, *d: x.transpose(*d))(o, 0, 2, 1, 3).reshape(B, S, D) @ wo

    def _B_ref(x, w_r, w_gate, w_up, w_down):
        B, S, D = x.shape
        C = 1
        r = x @ w_r
        idx = jnp.argsort(-r, axis=-1)[:, :C]
        idx_e = jnp.repeat(idx.reshape(B, C, 1), D, axis=2)
        x_sel = jnp.take_along_axis(x, idx_e, axis=1)
        g = _silu(x_sel @ w_gate)
        u = x_sel @ w_up
        y = (g * u) @ w_down
        r_sel = _sigmoid(jnp.take_along_axis(r, idx, axis=1))
        y = y * r_sel.reshape(B, C, 1)
        b_off = (jnp.arange(B) * S).reshape(B, 1)
        flat_idx = (idx + b_off).reshape(B * C)
        zero = (x * 0.0).reshape(B * S, D)
        upd = _scatter_add(zero, flat_idx, y.reshape(B * C, D), axis=0)
        return x + upd.reshape(B, S, D)

    x = A_x
    xn = _layernorm(x, axis=-1)
    s = _A_ref(xn, A_wqkv, A_w_phi, A_wo)
    g = _silu(_B_ref(xn, B_w_r, B_w_gate, B_w_up, B_w_down))
    return x + s * g
```

```python
import functools
import math

import numpy as np

import jax
import jax.numpy as jnp
from jax import lax
import jax.experimental.pallas as pl
import jax.experimental.pallas.tpu as pltpu

S, D, H, DH, F = 2048, 1024, 32, 32, 3584
LOG2E = math.log2(math.e)
EPS_BF16 = float(np.float32(1e-5).astype(jnp.bfloat16))
NT_DIMS = (((1,), (1,)), ((), ()))
f32, bf16 = jnp.float32, jnp.bfloat16


def _dot_nt(a, b):
    return lax.dot_general(a, b, NT_DIMS, preferred_element_type=f32)


def _dot(a, b):
    return jnp.dot(a, b, preferred_element_type=f32)


def _dual_softmax(p):
    t = p.shape[-1]
    p3 = p.reshape(8, 8, t)

    def allred(v, op):
        v = op(v, pltpu.roll(v, 4, 0))
        return op(v, pltpu.roll(v, 2, 0))

    mx = allred(jnp.max(p3, axis=0), jnp.maximum)
    mn = allred(jnp.min(p3, axis=0), jnp.minimum)
    ep = jnp.exp2(p3 - mx[None])
    en = jnp.exp2(mn[None] - p3)
    sp = allred(jnp.sum(ep, axis=0), jnp.add)
    sn = allred(jnp.sum(en, axis=0), jnp.add)
    return ep * (1.0 / sp)[None], en * (1.0 / sn)[None]


def make_kernel(T=512, FC=512):
    NTILE = S // T
    NG = 8
    A_ROWS = 2 * D + 16

    def kernel(x_hbm, wqkv_hbm, wphi_hbm, wo_hbm, wr_hbm, wg_hbm, wu_hbm, wd_hbm,
               out_hbm,
               x_v, xn_v, wqkv_v, wphi_v, wr_v, a1_v, aq_v, wo_v, wg_v, wu_v, wd_v,
               kv_acc, z_acc, kvb_v, r_v, o_v, y_v, out_v,
               sem_x, sem_w, sem_s, sem_f, sem_o):
        def cp_x(i):
            return pltpu.make_async_copy(x_hbm.at[pl.ds(i * T, T)], x_v.at[pl.ds(i * T, T)], sem_x.at[i])

        def cp_w(j):
            return pltpu.make_async_copy(wqkv_hbm.at[:, pl.ds(j * D, D)], wqkv_v.at[j], sem_w.at[j])

        cp_phi = pltpu.make_async_copy(wphi_hbm, wphi_v, sem_s.at[0])
        cp_wr = pltpu.make_async_copy(wr_hbm, wr_v, sem_s.at[1])
        cp_wo = pltpu.make_async_copy(wo_hbm, wo_v, sem_s.at[2])
        cp_g = pltpu.make_async_copy(wg_hbm, wg_v, sem_f.at[0])
        cp_u = pltpu.make_async_copy(wu_hbm, wu_v, sem_f.at[1])
        cp_d = pltpu.make_async_copy(wd_hbm, wd_v, sem_f.at[2])

        def cp_o(k, t):
            return pltpu.make_async_copy(out_v.at[pl.ds(t * T, T)], out_hbm.at[pl.ds(t * T, T)], sem_o.at[k])

        cp_phi.start()
        cp_wr.start()
        cp_w(1).start()
        cp_x(0).start()
        cp_w(2).start()

        def blockdiag(g):
            rho = lax.broadcasted_iota(jnp.int32, (128, DH), 0)
            fi = lax.broadcasted_iota(jnp.int32, (128, DH), 1)
            sel = (((rho % 64) // 8) * 4 + (rho % 8) // 2 == fi).astype(bf16)
            w = wphi_v[pl.ds(g * 128, 128), :]
            full = _dot_nt(sel, w)
            rho = lax.broadcasted_iota(jnp.int32, (128, 128), 0)
            c = lax.broadcasted_iota(jnp.int32, (128, 128), 1)
            keep = (rho // 64) * 2 + rho % 2 == c // DH
            return jnp.where(keep, full, 0.0).astype(bf16)

        def fold(j, g, lmat):
            w = wqkv_v[j, :, pl.ds(g * 128, 128)]
            return (_dot_nt(lmat, w) * LOG2E).astype(bf16)

        def layernorm(t):
            rows = pl.ds(pl.multiple_of(t * T, T), T)
            x = x_v[rows, :].astype(f32)
            m = jnp.sum(x, axis=-1, keepdims=True) * (1.0 / D)
            c = x - m
            v = jnp.sum(c * c, axis=-1, keepdims=True) * (1.0 / D)
            mb = m.astype(bf16).astype(f32)
            vb = (v.astype(bf16) .astype(f32) + EPS_BF16).astype(bf16).astype(f32)
            sd = jnp.sqrt(vb).astype(bf16).astype(f32)
            xn_v[rows, :] = ((x - mb) * (1.0 / sd)).astype(bf16)

        cp_phi.wait()
        cp_wr.wait()
        w8 = wr_v[...].astype(f32)
        wrow = jnp.concatenate([w8[j:j + 1, :] for j in range(8)], axis=1)
        a1_v[pl.ds(2 * D, 16), :] = jnp.broadcast_to(wrow, (16, D)).astype(bf16)
        kv_acc[...] = jnp.zeros(kv_acc.shape, f32)
        z_acc[...] = jnp.zeros(z_acc.shape, f32)
        lmats = [blockdiag(g) for g in range(NG)]
        cp_w(1).wait()
        cp_w(0).start()
        for g in range(NG):
            a1_v[pl.ds(g * 256, 128), :] = fold(1, g, lmats[g])
        cp_x(0).wait()
        for i in range(1, NTILE):
            cp_x(i).start()
        layernorm(0)
        cp_w(2).wait()
        cp_wo.start()
        for g in range(NG):
            a1_v[pl.ds(g * 256 + 128, 128), :] = wqkv_v[2, :, pl.ds(g * 128, 128)].T
        cp_w(0).wait()
        cp_g.start()
        cp_u.start()
        cp_d.start()
        for g in range(NG):
            aq_v[pl.ds(g * 128, 128), :] = fold(0, g, lmats[g])

        def p1_mm(t, g):
            rows = pl.ds(pl.multiple_of(t * T, T), T)
            n = 256 + (16 if g == NG - 1 else 0)
            return _dot_nt(a1_v[pl.ds(g * 256, n), :], xn_v[rows, :])

        def p1_post(t, g, raw):
            if g == NG - 1:
                r_v[t] = raw[256:264, :]
            for pr in range(2):
                ep, en = _dual_softmax(raw[pr * 64:(pr + 1) * 64, :])
                phi = jnp.concatenate([ep.reshape(64, T), en.reshape(64, T)], axis=0)
                zs = phi[:, 0:128]
                for c in range(1, T // 128):
                    zs = zs + phi[:, c * 128:(c + 1) * 128]
                z_acc[2 * g + pr] += zs
                vt = raw[128 + pr * 64:128 + (pr + 1) * 64, :].astype(bf16)
                kv_acc[2 * g + pr] += _dot_nt(vt, phi.astype(bf16))

        def p1_body(t, carry):
            @pl.when(t + 1 < NTILE)
            def _():
                cp_x(t + 1).wait()
            raw = p1_mm(t, 0)
            for g in range(NG):
                nxt = p1_mm(t, g + 1) if g + 1 < NG else None
                if g == 0:
                    layernorm(jnp.minimum(t + 1, NTILE - 1))
                p1_post(t, g, raw)
                raw = nxt
            return carry

        lax.fori_loop(0, NTILE, p1_body, 0)

        d_i = lax.broadcasted_iota(jnp.int32, (64, 128), 0)
        c_i = lax.broadcasted_iota(jnp.int32, (64, 128), 1)
        keep_kv = d_i // DH == c_i % 2
        s_i = lax.broadcasted_iota(jnp.int32, (16, 128), 0)
        c2_i = lax.broadcasted_iota(jnp.int32, (16, 128), 1)
        keep_z = s_i // 8 == c2_i % 2
        for p in range(H // 2):
            kvb_v[p, pl.ds(0, 64), :] = jnp.where(keep_kv, kv_acc[p], 0.0).astype(bf16)
            zrow = jnp.sum(z_acc[p].T, axis=0, keepdims=True)
            kvb_v[p, pl.ds(64, 16), :] = jnp.where(keep_z, jnp.broadcast_to(zrow, (16, 128)), 0.0).astype(bf16)

        r = r_v[...].astype(bf16).astype(f32)
        r = jnp.where(r != r, -jnp.inf, r)
        tok = (lax.broadcasted_iota(jnp.int32, r.shape, 0) * T + lax.broadcasted_iota(jnp.int32, r.shape, 2))
        rmax = jnp.max(jnp.max(r, axis=0), axis=-1, keepdims=True)
        cand = jnp.where(r == rmax[None], tok, S).astype(f32)
        idx = jnp.min(jnp.min(cand, axis=0)).astype(jnp.int32)
        idx = jnp.clip(idx, 0, S - 1)
        gate = jax.nn.sigmoid(rmax[0:1, :])
        base = pl.multiple_of((idx // 16) * 16, 16)
        grp = xn_v[pl.ds(base, 16), :].astype(f32)
        row = lax.broadcasted_iota(jnp.int32, (16, D), 0)
        xsel = jnp.sum(jnp.where(row == idx - base, grp, 0.0), axis=0, keepdims=True)
        xsel = jnp.broadcast_to(xsel, (16, D)).astype(bf16)

        cp_g.wait()
        cp_u.wait()
        cp_d.wait()
        cp_wo.wait()
        gg = _dot(xsel, wg_v[...])
        uu = _dot(xsel, wu_v[...])
        hh = (gg * jax.nn.sigmoid(gg) * uu).astype(bf16)
        y_v[...] = _dot(hh, wd_v[...]) * gate

        def q_mm(t, g):
            rows = pl.ds(pl.multiple_of(t * T, T), T)
            return _dot_nt(aq_v[pl.ds(g * 256, 256), :], xn_v[rows, :])

        def q_post(slot, g, raw):
            for half in range(2):
                outs = []
                for pr in range(2):
                    p = 4 * g + 2 * half + pr
                    ep, en = _dual_softmax(raw[(2 * half + pr) * 64:(2 * half + pr + 1) * 64, :])
                    phi = jnp.concatenate([ep.reshape(64, T), en.reshape(64, T)], axis=0).astype(bf16)
                    nd = _dot(kvb_v[p], phi)
                    rd = 1.0 / (nd[64:80, :] + 1e-6)
                    outs.append((nd[0:32, :].reshape(4, 8, T) * rd[0:8, :][None]).reshape(32, T))
                    outs.append((nd[32:64, :].reshape(4, 8, T) * rd[8:16, :][None]).reshape(32, T))
                ot = jnp.concatenate(outs, axis=0).astype(bf16)
                o_v[slot, :, pl.ds((2 * g + half) * 128, 128)] = ot.T

        def out_part(t, slot, c):
            rows = pl.ds(pl.multiple_of(t * T, T), T)
            cols = pl.ds(c * 256, 256)
            s = _dot(o_v[slot], wo_v[:, cols])
            xg = xn_v[rows, cols].astype(f32)
            rid = lax.broadcasted_iota(jnp.int32, (T, 256), 0)
            xg = xg + jnp.where(rid == idx - t * T, y_v[0:1, cols], 0.0)
            h = 0.5 * xg
            g = h + h * jnp.tanh(h)
            out_v[rows, cols] = (x_v[rows, cols].astype(f32) + s * g).astype(bf16)

        raw = q_mm(0, 0)
        for g in range(4):
            nxt = q_mm(0, g + 1) if g < 3 else None
            q_post(0, g, raw)
            raw = nxt

        def p2_body(t, carry):
            slot = t % 2
            raw = q_mm(t, 0)
            for g in range(4):
                nxt = q_mm(t, g + 1) if g < 3 else None
                out_part(t - 1, 1 - slot, g)
                q_post(slot, g, raw)
                raw = nxt
            cp_o(t - 1, t - 1).start()
            return carry

        lax.fori_loop(1, NTILE, p2_body, 0)
        for g in range(4):
            out_part(NTILE - 1, (NTILE - 1) % 2, g)
        cp_o(NTILE - 1, NTILE - 1).start()
        for t in range(NTILE):
            cp_o(t, t).wait()

    scratch = [
        pltpu.VMEM((S, D), bf16),
        pltpu.VMEM((S, D), bf16),
        pltpu.VMEM((3, D, D), bf16),
        pltpu.VMEM((D, DH), bf16),
        pltpu.VMEM((8, 128), bf16),
        pltpu.VMEM((A_ROWS, D), bf16),
        pltpu.VMEM((D, D), bf16),
        pltpu.VMEM((D, D), bf16),
        pltpu.VMEM((D, F), bf16),
        pltpu.VMEM((D, F), bf16),
        pltpu.VMEM((F, D), bf16),
        pltpu.VMEM((H // 2, 64, 128), f32),
        pltpu.VMEM((H // 2, 128, 128), f32),
        pltpu.VMEM((H // 2, 80, 128), bf16),
        pltpu.VMEM((NTILE, 8, T), f32),
        pltpu.VMEM((2, T, D), bf16),
        pltpu.VMEM((16, D), f32),
        pltpu.VMEM((S, D), bf16),
        pltpu.SemaphoreType.DMA((NTILE,)),
        pltpu.SemaphoreType.DMA((3,)),
        pltpu.SemaphoreType.DMA((3,)),
        pltpu.SemaphoreType.DMA((3,)),
        pltpu.SemaphoreType.DMA((NTILE,)),
    ]

    def call(x, wqkv, wphi, wo, wr, wg, wu, wd):
        hbm = pl.BlockSpec(memory_space=pltpu.HBM)
        return pl.pallas_call(
            kernel,
            out_shape=jax.ShapeDtypeStruct((S, D), bf16),
            in_specs=[hbm] * 8,
            out_specs=hbm,
            scratch_shapes=scratch,
            compiler_params=pltpu.CompilerParams(vmem_limit_bytes=110 * 2**20),
            name="hedgehog",
        )(x, wqkv, wphi, wo, wr, wg, wu, wd)

    return call


@jax.jit
def pallas_recurrent_scan__linear_kernel_hedgehog__moe_arch_mod__prompt_kernel(
    A_x: jax.Array,
    A_wqkv: jax.Array,
    A_w_phi: jax.Array,
    A_wo: jax.Array,
    B_x: jax.Array,
    B_w_r: jax.Array,
    B_w_gate: jax.Array,
    B_w_up: jax.Array,
    B_w_down: jax.Array,
):
    del B_x
    out = make_kernel()(
        A_x.reshape(S, D), A_wqkv, A_w_phi.reshape(D, DH), A_wo,
        B_w_r.reshape(8, 128), B_w_gate, B_w_up, B_w_down)
    return out.reshape(1, S, D)
```

```python
import math
import contextlib

import numpy as np

import jax
import jax.numpy as jnp
from jax import lax
import jax.experimental.pallas as pl
import jax.experimental.pallas.tpu as pltpu

S, D, H, DH, F = 2048, 1024, 32, 32, 3584
T = 512
TH = T // 2
NTILE = S // T
NF = F // 128
WQ, WK, WV, WO = (S + T + j * D for j in range(4))
RR = 16
LOG2E = math.log2(math.e)
EPS_BF16 = float(np.float32(1e-5).astype(jnp.bfloat16))
NT_DIMS = (((1,), (1,)), ((), ()))
f32, bf16, i32, u32 = jnp.float32, jnp.bfloat16, jnp.int32, jnp.uint32


def _dot_nt(a, b):
    return lax.dot_general(a, b, NT_DIMS, preferred_element_type=f32)


def _dot(a, b):
    return jnp.dot(a, b, preferred_element_type=f32)


def _unpack(w):
    return [pltpu.unpack_elementwise(w, index=i, packed_dtype=bf16, unpacked_dtype=f32) for i in range(2)]


def _pack(even, odd):
    return pltpu.bitcast(pltpu.pack_elementwise([even, odd], packed_dtype=bf16), u32)


def _lhs_combos(a11, a12, a21, a22):
    return [a11 + a22, a21 + a22, a11, a22, a11 + a12, a21 - a11, a12 - a22]


def _rhs_combos(b11, b12, b21, b22):
    return [b11 + b22, b11, b12 - b22, b21 - b11, b22, b11 + b12, b21 + b22]


def _strassen(prod, emit):
    m1 = prod(0)
    yield
    m4 = prod(3)
    c11 = m1 + m4
    yield
    m5 = prod(4)
    c11 = c11 - m5
    yield
    emit(0, 0, c11 + prod(6))
    yield
    m3 = prod(2)
    emit(0, 1, m3 + m5)
    c22 = m1 + m3
    yield
    m2 = prod(1)
    emit(1, 0, m2 + m4)
    c22 = c22 - m2
    yield
    emit(1, 1, c22 + prod(5))
    yield


def _schedule(clock, *streams):
    events = []
    for order, (gen, n, a, b) in enumerate(streams):
        for k in range(n):
            events.append((a + (b - a) * k / n, order, k, gen))
    for when, _, _, gen in sorted(events, key=lambda e: e[:3]):
        clock[:] = [when]
        next(gen)


def _dual_softmax(p, zero=None):
    rows = [p[8 * j:8 * j + 8] for j in range(8)]
    if zero is not None:
        rows[0] = rows[0] + zero

    def reduce(vs, op):
        while len(vs) > 1:
            vs = [op(vs[i], vs[i + 1]) for i in range(0, len(vs), 2)]
        v = op(vs[0], pltpu.roll(vs[0], 4, 0))
        return op(v, pltpu.roll(v, 2, 0))

    mx, mn = reduce(rows, jnp.maximum), reduce(rows, jnp.minimum)
    ep = [jnp.exp2(v - mx) for v in rows]
    en = [jnp.exp2(mn - v) for v in rows]
    rp, rn = 1.0 / reduce(ep, jnp.add), 1.0 / reduce(en, jnp.add)
    return jnp.concatenate([v * rp for v in ep] + [v * rn for v in en], axis=0)


def make_kernel(FFN_SPLIT=(2, 8, 2), SA=(18, 14, 0, 0), SB=(0, 2, 14, 0), PEND=0.75, FLAGS=None,
                FPIN=True, FINE=True, SPIN=True, EPIN=True, EROWS=32, DMA_ORDER='a0 a1 a2 a3 k0 v0 k1 v1 k2 v2 v3 x1 f0 o0 x2 f1 o1 x3 f2 o2 x4 f3 o3 f4'.split(), PSLOT=(1, 3), A0=0.4, AEND=0.85, SCOPES=False, OTR=0, FSL=(2, 2, 2, 2)):

    stack = []
    def mark(name):
        if not SCOPES: return
        if stack: stack.pop().__exit__(None, None, None)
        if name:
            cm = jax.named_scope(name); cm.__enter__(); stack.append(cm)

    def kernel(x_hbm, wqkv_hbm, wphi_hbm, wo_hbm, wr_hbm, wg_hbm, wu_hbm, wd_hbm,
               out_hbm,
               in_v, st_v, xb_v, wphi_v, wr_v, lm_v, a_v, a12_v, wo_v, wg_v, wu_v, wd_v,
               kv_acc, z_acc, kvb_v, r_v, raw_v, oba_v, obb_v, part_v, xcol_v, y_acc, out_v, zero_s,
               sem_x, sem_w, sem_s, sem_o):
        def cp_x(r0, n, sem, src0=None):
            src0 = r0 if src0 is None else src0
            return pltpu.make_async_copy(x_hbm.at[pl.ds(src0, n)], in_v.at[pl.ds(r0, n)], sem_x.at[sem])

        def cp_x0(piece):
            return cp_x((piece % 2) * TH + (piece // 2) * (TH // 2), TH // 2, NTILE + 1 + piece)

        def cp_xt(t):
            return cp_x(pl.multiple_of(t * T, T), T, t, pl.multiple_of((t % NTILE) * T, T))

        def cp_w(j, c0, n, sem):
            src = wo_hbm.at[:, pl.ds(c0, n)] if j == 3 else wqkv_hbm.at[:, pl.ds(j * D + c0, n)]
            return pltpu.make_async_copy(src, in_v.at[pl.ds(WQ + j * D, D), pl.ds(c0, n)], sem_w.at[sem])

        def wait_group(base, g, sem):
            dst = in_v.at[pl.ds(pl.multiple_of(base, 128), D), pl.ds(pl.multiple_of(g * 128, 128), 128)]
            pltpu.make_async_copy(dst, dst, sem_w.at[sem]).wait()

        def cp_k(c):
            return cp_w(1, c * 256, 256, c)

        def cp_v(c):
            return cp_w(2, c * 256, 256, 4 + c)

        def cp_fold(t):
            j, groups = (1, (6, 7)) if t == 0 else (0, (t - 1, t + 3))
            return [cp_w(j, g * 128, 128, 8 + t) for g in groups]

        def cp_wo(t):
            g = (t // 2) * 4 + t % 2
            return [cp_w(3, g * 128, 128, 13 + t), cp_w(3, (g + 2) * 128, 128, 13 + t)]

        cp_phi = pltpu.make_async_copy(wphi_hbm, wphi_v, sem_s.at[0])
        cp_wr = pltpu.make_async_copy(wr_hbm, wr_v, sem_s.at[1])
        cp_ffn = [pltpu.make_async_copy(wg_hbm, wg_v, sem_s.at[2]),
                  pltpu.make_async_copy(wu_hbm, wu_v, sem_s.at[3]),
                  pltpu.make_async_copy(wd_hbm, wd_v, sem_s.at[4])]

        def cp_o(k, t):
            rows = pl.ds(pl.multiple_of(t * T, T), T)
            return pltpu.make_async_copy(out_v.at[rows], out_hbm.at[rows], sem_o.at[k])

        def cp_o_blk(t, blk):
            rows = pl.ds(pl.multiple_of(t * T + (blk % 2) * TH, TH), TH)
            cols = pl.ds((blk // 2) * 256, 256)
            return pltpu.make_async_copy(out_v.at[rows, cols], out_hbm.at[rows, cols], sem_o.at[NTILE - 1 + blk])

        cp_wr.start()
        cp_phi.start()
        for n, name in enumerate(DMA_ORDER):
            if n == 1:
                cp_wr.wait()
                cp_phi.wait()
            cps = {"a": cp_x0, "k": cp_k, "v": cp_v, "x": cp_xt, "f": cp_fold, "o": cp_wo}[name[0]](int(name[1]))
            for cp in cps if isinstance(cps, list) else [cps]:
                cp.start()

        last_product = []

        clock = [0.0]
        rate = [7]

        def pin(n=8):
            if not last_product:
                return jnp.zeros((n, 128), f32)
            q = min(int((clock[0] * rate[0]) % 1.0 * 64 + 1e-6), 63) if FINE else 0
            m = last_product[0][(q % 32) * 8:(q % 32) * 8 + 8, (q // 32) * 128:(q // 32) * 128 + 128]
            z = pltpu.bitcast(pltpu.bitcast(m, u32) & zero_s[0].astype(u32), f32)
            return z if n == 8 else jnp.concatenate([z] * (n // 8), axis=0)

        def as_bf16(w):
            return pltpu.bitcast(w, bf16)

        def words(ref, *idx):
            return pltpu.bitcast(ref[idx], u32)

        def feature_maps():
            def target(shape):
                s = lax.broadcasted_iota(i32, shape, 0)
                return (s // 16) * 16 + (s % 8) * 2 + (s // 8) % 2

            rho = target((128, DH))
            sel = (((rho % 64) // 8) * 4 + (rho % 8) // 2 == lax.broadcasted_iota(i32, (128, DH), 1)).astype(bf16)
            rho = target((128, 128))
            keep = (rho // 64) * 2 + rho % 2 == lax.broadcasted_iota(i32, (128, 128), 1) // DH
            for g in range(8):
                full = _dot_nt(sel, wphi_v[pl.ds(g * 128, 128), :])
                lm_v[g] = jnp.where(keep, full, 0.0).astype(bf16)

        def operand(chunk):
            if not isinstance(chunk, (int, jax.Array)):
                return chunk
            return a12_v.at[chunk - 1] if isinstance(chunk, int) and chunk in (1, 2) else a_v.at[chunk]

        def put_lhs(chunk, rows, cols, a11, a12, a21, a22):
            cmb = [_lhs_combos(a11[e], a12[e], a21[e], a22[e]) for e in range(2)]
            for i in range(7):
                operand(chunk)[i, rows, cols] = _pack(cmb[0][i], cmb[1][i])

        def w_blocks(base, top, bot, k):
            return [in_v[pl.ds(pl.multiple_of(base + kh * 512 + k * 128, 128), 128),
                         pl.ds(pl.multiple_of(g * 128, 128), 128)] for g in (top, bot) for kh in range(2)]

        def prep_fold(base, top, bot, chunk, row0):
            for k in range(4):
                blocks = [_dot_nt(lm_v[g], w) for g, w in zip((top, top, bot, bot), w_blocks(base, top, bot, k))]
                for j in range(8):
                    put_lhs(chunk, pl.ds(pl.multiple_of(row0 + 8 * j, 8), 8), pl.ds(k * 128, 128),
                            *[(p[16 * j:16 * j + 8] * LOG2E, p[16 * j + 8:16 * j + 16] * LOG2E) for p in blocks])
                yield

        def prep_transpose(base, top, bot, chunk, row0):
            for k in range(4):
                zero = pltpu.bitcast(pin(64), u32)
                blocks = [pltpu.bitcast(as_bf16(pltpu.bitcast(w, u32) | zero).T, u32)
                          for w in w_blocks(base, top, bot, k)]
                for j in range(8):
                    put_lhs(chunk, pl.ds(pl.multiple_of(row0 + 8 * j, 8), 8), pl.ds(k * 128, 128),
                            *[_unpack(w[8 * j:8 * j + 8]) for w in blocks])
                yield

        def prep_fold_later(t):
            start, u = t == 0, t - 1
            base, top, bot = jnp.where(start, WK, WQ), jnp.where(start, 6, u), jnp.where(start, 7, u + 4)
            wait_group(base, top, 8 + t)
            wait_group(base, bot, 8 + t)
            yield from prep_fold(base, top, bot, jnp.where(start, 3, 4 + u // 2), jnp.where(start, 0, (u % 2) * 64))

        def prep_wo(t):
            g = (t // 2) * 4 + t % 2
            wait_group(WO, g, 13 + t)
            wait_group(WO, g + 2, 13 + t)
            yield from prep_transpose(WO, g, g + 2, wo_v.at[t // 2], (t % 2) * 64)

        def x_words(r0, c0):
            return _unpack(words(in_v, pl.ds(r0, 16), pl.ds(c0, 128)))

        def ln_stats(t, st):
            for step in range(32):
                pos = (step % 2) * 16 + step // 2
                r0 = pl.multiple_of(t * T + pos * 16, 16)
                x0 = x_words(r0, 0)
                if last_product:
                    zero = pin()
                    x0 = [v + zero for v in x0]
                s1, s2 = [None, None], [None, None]
                for j in range(1, 8):
                    xj = x_words(r0, j * 128)
                    for e in range(2):
                        d = xj[e] - x0[e]
                        s1[e] = d if j == 1 else s1[e] + d
                        s2[e] = d * d if j == 1 else s2[e] + d * d
                for e in range(2):
                    lane_mean = x0[e] + s1[e] * 0.125
                    m = jnp.sum(lane_mean, axis=-1, keepdims=True) * (1.0 / 128)
                    dm = lane_mean - m
                    v = jnp.sum((s2[e] - s1[e] * s1[e] * 0.125) * 0.125 + dm * dm, axis=-1, keepdims=True) * (1.0 / 128)
                    mb = m.astype(bf16).astype(f32)
                    vb = (v.astype(bf16).astype(f32) + EPS_BF16).astype(bf16).astype(f32)
                    rs = 1.0 / jnp.sqrt(vb).astype(bf16).astype(f32)
                    st[0, pl.ds(e * TH + pos * 8, 8), :] = jnp.broadcast_to(mb, (8, 128))
                    st[1, pl.ds(e * TH + pos * 8, 8), :] = jnp.broadcast_to(rs, (8, 128))
                yield

        def ln_apply(t, st, xb):
            for step in range(16):
                r0 = [pl.multiple_of(t * T + hf * TH + step * 16 + zero_s[0], 16) for hf in range(2)]
                srow = [[pl.ds(e * TH + hf * (TH // 2) + step * 8, 8) for e in range(2)] for hf in range(2)]
                mb = [[st[0, srow[hf][e], :] for e in range(2)] for hf in range(2)]
                rs = [[st[1, srow[hf][e], :] for e in range(2)] for hf in range(2)]
                mb0 = mb
                for k in range(4):
                    if last_product:
                        zero = pin()
                        mb = [[v + zero for v in row] for row in mb0]
                    blk = [[x_words(r0[hf], kh * 512 + k * 128) for kh in range(2)] for hf in range(2)]
                    cmb = []
                    for e in range(2):
                        nb = [[(blk[hf][kh][e] - mb[hf][e]) * rs[hf][e] for kh in range(2)] for hf in range(2)]
                        cmb.append(_rhs_combos(nb[0][0], nb[1][0], nb[0][1], nb[1][1]))
                    for i in range(7):
                        xb[i, pl.ds(step * 8, 8), pl.ds(k * 128, 128)] = _pack(cmb[0][i], cmb[1][i])
                    yield

        def project(chunk, xb, res, router=None):
            extra = {}

            def prod(i):
                n = 128 + (RR // 2 if router is not None and i % 2 == 0 else 0)
                m = _dot_nt(as_bf16(operand(chunk)[i, pl.ds(0, n), :]), as_bf16(xb[i]))
                last_product[:] = [m]
                if n > 128:
                    extra[i] = m[256:264]
                return m[:256]

            def emit(a, b, val):
                if isinstance(res, list):
                    res[a][b] = val
                else:
                    res[a, b] = val
                if router is not None and a == 0:
                    r_v[router, :, pl.ds(b * TH, TH)] = (
                        extra[0] - extra[4] + extra[6] if b == 0 else extra[2] + extra[4])

            return _strassen(prod, emit)

        def raw_blk(res, a, r0, lane):
            b, c0 = lane // 2, (lane % 2) * 128
            if isinstance(res, list):
                return res[a][b][r0:r0 + 64, c0:c0 + 128]
            return res[a, b, pl.ds(r0, 64), pl.ds(c0, 128)]

        def kv_post(c, res):
            pending = None
            for a in range(2):
                for pr in range(2):
                    p = 4 * c + 2 * a + pr
                    phis, zs = [], None
                    for lane in range(4):
                        phi = _dual_softmax(raw_blk(res, a, pr * 64, lane), pin() if SPIN else None)
                        zs = phi if zs is None else zs + phi
                        phis.append(phi.astype(bf16))
                        if lane == 1 and pending:
                            kv_acc[pending[0]] += _dot_nt(pending[1], pending[2])
                        if lane == 3:
                            z_acc[p] += zs
                            vt = jnp.concatenate([raw_blk(res, a, 128 + pr * 64, l) for l in range(4)], axis=1)
                            pending = (p, vt.astype(bf16), jnp.concatenate(phis, axis=1))
                        yield
            yield
            kv_acc[pending[0]] += _dot_nt(pending[1], pending[2])
            yield

        def route():
            r = r_v[pl.ds(0, NTILE)].astype(bf16).astype(f32)
            r = jnp.where(r != r, -jnp.inf, r)
            tok = lax.broadcasted_iota(i32, r.shape, 0) * T + lax.broadcasted_iota(i32, r.shape, 2)
            rmax = jnp.max(jnp.max(r, axis=0), axis=-1, keepdims=True)
            cand = jnp.min(jnp.where(r == rmax[None], tok, S).astype(f32), axis=0)
            return jnp.clip(jnp.min(cand).astype(i32), 0, S - 1), rmax

        mark('s0_init')
        zero_s[0] = 0
        kv_acc[...] = jnp.zeros(kv_acc.shape, f32)
        z_acc[...] = jnp.zeros(z_acc.shape, f32)
        y_acc[...] = jnp.zeros(y_acc.shape, f32)
        r_v[...] = jnp.full(r_v.shape, -jnp.inf, f32)
        w8 = wr_v[...].astype(f32)
        wrow = jnp.broadcast_to(jnp.concatenate([w8[j:j + 1, :] for j in range(8)], axis=1), (RR // 2, D))
        none = [jnp.zeros((RR // 2, 512), f32)] * 2
        put_lhs(0, pl.ds(128, RR // 2), slice(None), [wrow[:, :512]] * 2, [wrow[:, 512:]] * 2, none, none)
        for i in range(7):
            a_v[4, i, pl.ds(128, RR // 2), :] = jnp.zeros((RR // 2, 512), u32)
        feature_maps()
        mark('s1_ln0')
        stats, apply = ln_stats(0, st_v.at[0]), ln_apply(0, st_v.at[0], xb_v.at[0])
        for half in range(2):
            cp_x0(2 * half).wait()
            cp_x0(2 * half + 1).wait()
            _schedule(clock, (stats, 16, 0.0, 1.0))
            _schedule(clock, (apply, 32, 0.0, 1.0))

        def prep_kv(c):
            cp_k(c).wait()
            yield from prep_fold(WK, 2 * c, 2 * c + 1, c, 0)
            cp_v(c).wait()
            yield from prep_transpose(WV, 2 * c, 2 * c + 1, c, 64)

        mark('s3_prep0')
        _schedule(clock, (prep_kv(0), 8, 0.0, 1.0))
        mark('s4_proj0')
        _schedule(clock, (project(0, xb_v.at[0], raw_v, router=0), 7, 0.0, 1.0),
                  (prep_kv(1), 8, 0.1, 0.5), (prep_kv(2), 8, 0.5, 1.0))
        cp_v(3).wait()
        _schedule(clock, (prep_transpose(WV, 6, 7, 3, 64), 4, 0.0, 1.0))

        def kv_tile(t, carry):
            last = t == NTILE - 1

            @pl.when(t == 0)
            def _():
                for cp in cp_ffn:
                    cp.start()

            first = (route()[0] // T + 1) % NTILE
            last_product[:] = []
            xb = xb_v.at[pl.ds(t, 2)]
            st = st_v.at[t + 1]

            def next_stats():
                cp_xt(t + 1).wait()
                yield from ln_stats(t + 1, st)

            stats, apply = next_stats(), ln_apply(t + 1, st, xb.at[1])
            fold, trans = prep_fold_later(t), prep_wo(t)
            res = raw_v
            for c in range(4):
                streams = [(kv_post(c, res), 18, 0.0, 1.0)]
                if c < 3:
                    res = [[None, None], [None, None]]
                    streams.append((project(c + 1, xb.at[0], res), 7, 0.0, 1.0))
                else:
                    streams.append((project(jnp.where(last, 4, 0), xb_v.at[jnp.where(last, first, t + 1)],
                                            raw_v, router=t + 1), 7, 0.0, 1.0))
                if c == PSLOT[0]:
                    streams.append((fold, 4, 0.1, 0.9))
                if c == PSLOT[1]:
                    streams.append((trans, 4, 0.1, 0.8))
                streams.append((stats, SA[c], A0 if c == 0 else 0.0, 1.0))
                streams.append((apply, 4 * SB[c], 0.07, AEND if c == 2 else 1.0))
                _schedule(clock, *streams)
            return carry

        mark('s6_phase1')
        lax.fori_loop(0, NTILE, kv_tile, 0)
        mark('s7_mid')
        last_product[:] = []
        _schedule(clock, (prep_fold_later(jnp.int32(NTILE)), 4, 0.0, 1.0))

        keep_kv = lax.broadcasted_iota(i32, (64, 128), 0) // DH == lax.broadcasted_iota(i32, (64, 128), 1) % 2
        keep_z = lax.broadcasted_iota(i32, (16, 128), 0) // 8 == lax.broadcasted_iota(i32, (16, 128), 1) % 2

        def finish_kv():
            for p in range(H // 2):
                kvb_v[p, pl.ds(0, 64), :] = jnp.where(keep_kv, kv_acc[p], 0.0).astype(bf16)
                zrow = jnp.sum(z_acc[p].T, axis=0, keepdims=True)
                kvb_v[p, pl.ds(64, 16), :] = jnp.where(keep_z, jnp.broadcast_to(zrow, (16, 128)), 0.0).astype(bf16)
                yield

        idx, rmax = route()
        first = (idx // T + 1) % NTILE
        base = pl.multiple_of((idx // 16) * 16, 16)
        srow = pl.multiple_of((idx % T) // 16 * 8, 8)
        grp = _unpack(words(in_v, pl.ds(base, 16), slice(None)))
        sub = lax.broadcasted_iota(i32, (8, D), 0)
        xsel = jnp.zeros((8, D), f32)
        for e in range(2):
            rows = pl.ds(pl.multiple_of(e * TH + srow, 8), 8)
            xn = (grp[e] - st_v[idx // T, 0, rows, 0:1]) * st_v[idx // T, 1, rows, 0:1]
            xsel = xsel + jnp.where(2 * sub + e == idx - base, xn, 0.0)
        xsel = jnp.sum(xsel, axis=0, keepdims=True).astype(bf16).astype(f32)
        for j in range(8):
            xcol_v[pl.ds(j * 128, 128), :] = jnp.broadcast_to(xsel[:, j * 128:(j + 1) * 128], (128, 128)).T
        for cp in cp_ffn:
            cp.wait()

        def ffn(f0, nf):
            for j in range(nf):
                cols = pl.ds(pl.multiple_of((f0 + j) * 128, 128), 128)
                accs = [jnp.zeros((8, 128), f32)] * 2
                for r in range(8):
                    rows = pl.ds(r * 128, 128)
                    xc = xcol_v[rows, :]
                    if FPIN:
                        zero = pin()
                    for a, w_v in enumerate((wg_v, wu_v)):
                        prod = w_v[rows, cols].astype(f32) * xc
                        acc = accs[a] + zero if FPIN else accs[a]
                        for q in range(16):
                            acc = acc + prod[8 * q:8 * q + 8]
                        accs[a] = acc
                    yield
                gate, up = [jnp.sum(acc, axis=0, keepdims=True) for acc in accs]
                hcol = jnp.broadcast_to(gate * jax.nn.sigmoid(gate) * up, (128, 128)).T
                for n in range(8):
                    ycols = pl.ds(n * 128, 128)
                    prod = wd_v[cols, ycols].astype(f32) * hcol
                    acc = y_acc[:, ycols] + pin() if FPIN else y_acc[:, ycols]
                    for q in range(16):
                        acc = acc + prod[8 * q:8 * q + 8]
                    y_acc[:, ycols] = acc
                    if n % 2 == 1:
                        yield

        def tile(j):
            return (first + j) % NTILE

        def q_post(c, res, ob):
            phis, nds, outs = {}, {}, {}
            for tick in range(40):
                step, lane = tick // 4, tick % 4
                if step < 8:
                    u, a, pr = step // 4, (step // 2) % 2, step % 2
                    phis.setdefault(step, []).append(_dual_softmax(
                        raw_blk(res, a, u * 128 + pr * 64, lane), pin() if SPIN else None).astype(bf16))
                if 1 <= step < 9 and lane == 1:
                    w = step - 1
                    pair = 2 * (2 * c + w // 4 + 4 * ((w // 2) % 2)) + w % 2
                    nds[step - 1] = _dot(kvb_v[pair], jnp.concatenate(phis.pop(step - 1), axis=1))
                if step >= 2 and lane == 0:
                    nd = nds.pop(step - 2)
                    rd = 1.0 / (nd[64:80, :] + 1e-6)
                    outs[step - 2] = jnp.concatenate(
                        [(nd[0:32, :].reshape(4, 8, T) * rd[0:8, :][None]).reshape(32, T),
                         (nd[32:64, :].reshape(4, 8, T) * rd[8:16, :][None]).reshape(32, T)], axis=0)
                    if (step - 2) % 4 == 3:
                        u = (step - 2) // 4
                        o1 = jnp.concatenate([outs.pop(4 * u), outs.pop(4 * u + 1)], axis=0)
                        o2 = jnp.concatenate([outs.pop(4 * u + 2), outs.pop(4 * u + 3)], axis=0)
                        cmb = _rhs_combos(o1[:, :TH], o1[:, TH:], o2[:, :TH], o2[:, TH:])
                        if OTR == 0:
                            for i in range(7):
                                ob[i, :, pl.ds(u * 128, 128)] = pltpu.bitcast(cmb[i].astype(bf16).T, u32)
                        else:
                            for b in range(2):
                                tr = pltpu.bitcast(jnp.concatenate(
                                    [v[:, b * 128:(b + 1) * 128] for v in cmb], axis=0).astype(bf16).T, u32)
                                for i in range(7):
                                    ob[i, pl.ds(b * 64, 64), pl.ds(u * 128, 128)] = tr[:, i * 128:(i + 1) * 128]
                yield

        def out_project(h, oba, obb, res, ks=(0, 1)):
            def prod(i):
                lhs = jnp.concatenate([(oba, obb)[k][i] for k in ks], axis=1)
                m = _dot_nt(as_bf16(lhs), as_bf16(wo_v[h, i, :, pl.ds(ks[0] * 256, len(ks) * 256)]))
                last_product[:] = [m]
                return m

            def emit(a, b, val):
                if isinstance(res, list):
                    res[a][b] = val
                else:
                    res[a, b] = val

            return _strassen(prod, emit)

        def epilogue(t, h, res, part=None, upd=None, done=None):
            n = EROWS
            for a in range(2):
                for b in range(2):
                    cols = pl.ds(h * 512 + a * 256, 256)
                    for q in range(TH // n):
                        r0 = pl.multiple_of(t * T + b * TH + q * n, n)
                        hx, xs = [], _unpack(words(in_v, pl.ds(r0, n), cols))
                        for e in range(2):
                            rows = pl.ds(e * TH + b * (TH // 2) + q * n // 2, n // 2)
                            mb, rs = st_v[t, 0, rows, :], st_v[t, 1, rows, :] * 0.5
                            if upd is None:
                                mb = mb + pin(n // 2)
                            v = (xs[e] - jnp.concatenate([mb, mb], axis=1)) * jnp.concatenate([rs, rs], axis=1)
                            if upd is not None:
                                rid = lax.broadcasted_iota(i32, (n // 2, 256), 0) * 2 + e
                                v = v + jnp.where(rid == idx - r0, upd[:, h * 512 + a * 256:h * 512 + (a + 1) * 256], 0.0)
                            hx.append(v + v * jnp.tanh(v))
                        g = as_bf16(_pack(hx[0], hx[1])).astype(f32)
                        s = res[a][b][q * n:(q + 1) * n]
                        if part is not None:
                            s = s + part[a, b, pl.ds(q * n, n), :]
                        out_v[pl.ds(r0, n), cols] = (in_v[pl.ds(r0, n), cols].astype(f32) + s * g).astype(bf16)
                        if done is not None and q == TH // n - 1:
                            done(4 * h + 2 * a + b)
                        yield

        NE = 4 * TH // EROWS
        mark('s8_q0')
        fa, fl, fb = FFN_SPLIT
        res0 = None
        _schedule(clock, (q_post(0, raw_v, oba_v.at[0]), 40, 0.02, PEND),
                  (project(5, xb_v.at[tile(0)], part_v.at[0]), 7, 0.0, 1.0),
                  (finish_kv(), 16, 0.0, 0.3),
                  (ffn(0, fa), 12 * fa, 0.2, 1.0))

        def q_tile(j, carry):
            last_product[:] = []
            oba = oba_v.at[pl.ds(j, 2)]
            obb = obb_v.at[zero_s[0]]
            xb = xb_v.at[tile(j + 1)]
            fg = ffn(fa + j * fl, fl)
            q0, o0, o1 = ([[None, None], [None, None]] for _ in range(3))
            _schedule(clock, (project(4, xb, q0), 7, 0.0, 1.0), (q_post(1, part_v.at[0], obb_v.at[0]), 40, 0.0, PEND),
                      (fg, 12 * FSL[0], 0.1, 1.0))
            _schedule(clock, (out_project(0, oba.at[0], obb, o0), 7, 0.0, 1.0), (q_post(0, q0, oba.at[1]), 40, 0.05, 1.0),
                      (fg, 12 * FSL[1], 0.1, 1.0))
            _schedule(clock, (out_project(1, oba.at[0], obb, o1), 7, 0.0, 1.0), (epilogue(tile(j), 0, o0), NE, 0.0, 1.0),
                      (fg, 12 * FSL[2], 0.1, 1.0))
            _schedule(clock, (project(5, xb, part_v.at[0]), 7, 0.0, 1.0), (epilogue(tile(j), 1, o1), NE, 0.0, 1.0),
                      (fg, 12 * FSL[3], 0.1, 0.9))
            cp_o(j, tile(j)).start()
            return carry

        mark('s9_phase2')
        lax.fori_loop(0, NTILE - 1, q_tile, 0)
        mark('sa_tail')

        j = NTILE - 1
        rate[0] = 14
        last_product[:] = []
        oba, obb = oba_v.at[j], obb_v.at[zero_s[0]]
        _schedule(clock, (out_project(0, oba, obb, part_v.at[1], (0,)), 7, 0.0, 0.5),
                  (out_project(1, oba, obb, part_v.at[2], (0,)), 7, 0.5, 1.0),
                  (q_post(1, part_v.at[0], obb_v.at[0]), 40, 0.0, PEND),
                  (ffn(fa + j * fl, fb), 12 * fb, 0.1, 0.8))
        upd = jnp.sum(y_acc[...], axis=0, keepdims=True) * (0.5 * jax.nn.sigmoid(rmax[0:1, :]))
        o0, o1 = ([[None, None], [None, None]] for _ in range(2))
        t = tile(j)
        send = lambda blk: cp_o_blk(t, blk).start()
        e0 = epilogue(t, 0, o0, part_v.at[1], upd, send)
        e1 = epilogue(t, 1, o1, part_v.at[2], upd, send)
        _schedule(clock, (out_project(0, oba, obb, o0, (1,)), 7, 0.0, 0.5),
                  (out_project(1, oba, obb, o1, (1,)), 7, 0.5, 1.0),
                  (e0, NE, 0.29, 0.57), (e1, NE, 0.79, 1.07))
        mark('sb_outdma')
        for k in range(NTILE - 1):
            cp_o(k, tile(k)).wait()
        for blk in range(8):
            cp_o_blk(t, blk).wait()
        mark(None)

    scratch = [
        pltpu.VMEM((S + T + 4 * D, D), bf16),
        pltpu.VMEM((NTILE + 1, 2, T, 128), f32),
        pltpu.VMEM((NTILE + 1, 7, TH // 2, 512), u32),
        pltpu.VMEM((D, DH), bf16),
        pltpu.VMEM((8, 128), bf16),
        pltpu.VMEM((8, 128, 128), bf16),
        pltpu.VMEM((6, 7, 128 + RR // 2, 512), u32),
        pltpu.VMEM((2, 7, 128, 512), u32),
        pltpu.VMEM((2, 7, 128, 512), u32),
        pltpu.VMEM((D, F), bf16),
        pltpu.VMEM((D, F), bf16),
        pltpu.VMEM((F, D), bf16),
        pltpu.VMEM((H // 2, 64, 128), f32),
        pltpu.VMEM((H // 2, 128, 128), f32),
        pltpu.VMEM((H // 2, 80, 128), bf16),
        pltpu.VMEM((NTILE + 1, 8, T), f32),
        pltpu.VMEM((2, 2, 256, TH), f32),
        pltpu.VMEM((NTILE, 7, TH // 2, 256), u32),
        pltpu.VMEM((2, 7, TH // 2, 256), u32),
        pltpu.VMEM((3, 2, 2, 256, 256), f32),
        pltpu.VMEM((D, 128), f32),
        pltpu.VMEM((8, D), f32),
        pltpu.VMEM((S, D), bf16),
        pltpu.SMEM((1,), i32),
        pltpu.SemaphoreType.DMA((NTILE + 5,)),
        pltpu.SemaphoreType.DMA((17,)),
        pltpu.SemaphoreType.DMA((5,)),
        pltpu.SemaphoreType.DMA((NTILE + 7,)),
    ]

    def call(x, wqkv, wphi, wo, wr, wg, wu, wd):
        hbm = pl.BlockSpec(memory_space=pltpu.HBM)
        return pl.pallas_call(
            kernel,
            out_shape=jax.ShapeDtypeStruct((S, D), bf16),
            in_specs=[hbm] * 8,
            out_specs=hbm,
            scratch_shapes=scratch,
            compiler_params=pltpu.CompilerParams(vmem_limit_bytes=120 * 2**20, flags=FLAGS),
            name="hedgehog",
        )(x, wqkv, wphi, wo, wr, wg, wu, wd)

    return call


@jax.jit
def pallas_recurrent_scan__linear_kernel_hedgehog__moe_arch_mod__prompt_kernel(
    A_x: jax.Array,
    A_wqkv: jax.Array,
    A_w_phi: jax.Array,
    A_wo: jax.Array,
    B_x: jax.Array,
    B_w_r: jax.Array,
    B_w_gate: jax.Array,
    B_w_up: jax.Array,
    B_w_down: jax.Array,
):
    del B_x
    out = make_kernel()(
        A_x.reshape(S, D), A_wqkv, A_w_phi.reshape(D, DH), A_wo,
        B_w_r.reshape(8, 128), B_w_gate, B_w_up, B_w_down)
    return out.reshape(1, S, D)
```

```python
import math
import contextlib

import numpy as np

import jax
import jax.numpy as jnp
from jax import lax
import jax.experimental.pallas as pl
import jax.experimental.pallas.tpu as pltpu

S, D, H, DH, F = 2048, 1024, 32, 32, 3584
T = 512
TH = T // 2
NTILE = S // T
NF = F // 128
FG = NF // NTILE
WQ, WK, WV, WO = (S + T + j * D for j in range(4))
RR = 16
LOG2E = math.log2(math.e)
EPS_BF16 = float(np.float32(1e-5).astype(jnp.bfloat16))
NT_DIMS = (((1,), (1,)), ((), ()))
f32, bf16, i32, u32 = jnp.float32, jnp.bfloat16, jnp.int32, jnp.uint32


def _dot_nt(a, b):
    return lax.dot_general(a, b, NT_DIMS, preferred_element_type=f32)


def _dot(a, b):
    return jnp.dot(a, b, preferred_element_type=f32)


def aligned(i, n):
    return i if isinstance(i, int) else pl.multiple_of(i, n)


def _recip(v):
    r = pl.reciprocal(v, approx=True)
    return r * (2.0 - v * r)


def _unpack(w):
    return [pltpu.unpack_elementwise(w, index=i, packed_dtype=bf16, unpacked_dtype=f32) for i in range(2)]


def _pack(even, odd):
    return pltpu.bitcast(pltpu.pack_elementwise([even, odd], packed_dtype=bf16), u32)


def _lhs_combos(a11, a12, a21, a22):
    return [a11 + a22, a21 + a22, a11, a22, a11 + a12, a21 - a11, a12 - a22]


def _rhs_combos(b11, b12, b21, b22):
    return [b11 + b22, b11, b12 - b22, b21 - b11, b22, b11 + b12, b21 + b22]


def _strassen(prod, emit):
    m1 = prod(0)
    yield
    m4 = prod(3)
    c11 = m1 + m4
    yield
    m5 = prod(4)
    c11 = c11 - m5
    yield
    emit(0, 0, c11 + prod(6))
    yield
    m3 = prod(2)
    emit(0, 1, m3 + m5)
    c22 = m1 + m3
    yield
    m2 = prod(1)
    emit(1, 0, m2 + m4)
    c22 = c22 - m2
    yield
    emit(1, 1, c22 + prod(5))
    yield


def _schedule(clock, *streams):
    events = []
    for order, (gen, n, a, b) in enumerate(streams):
        for k in range(n):
            events.append((a + (b - a) * k / n, order, k, gen))
    for when, _, _, gen in sorted(events, key=lambda e: e[:3]):
        clock[:] = [when]
        next(gen)


def _dual_softmax(p, zero=None):
    rows = [p[8 * j:8 * j + 8] for j in range(8)]
    if zero is not None:
        rows[0] = rows[0] + zero

    def reduce(vs, op):
        while len(vs) > 1:
            vs = [op(vs[i], vs[i + 1]) for i in range(0, len(vs), 2)]
        v = op(vs[0], pltpu.roll(vs[0], 4, 0))
        return op(v, pltpu.roll(v, 2, 0))

    mx, mn = reduce(rows, jnp.maximum), reduce(rows, jnp.minimum)
    ep = [jnp.exp2(v - mx) for v in rows]
    en = [jnp.exp2(mn - v) for v in rows]
    rp, rn = _recip(reduce(ep, jnp.add)), _recip(reduce(en, jnp.add))
    return jnp.concatenate([v * rp for v in ep] + [v * rn for v in en], axis=0)


def make_kernel(FL=9, W1=0.58, W2=0.15, W3=0.6, NOBC=True, DSLOT=3, SA=(32, 0), SB=(0, 16), SF=(3, 1), PEND=1.0, FLAGS=None,
                FPIN=True, FINE=True, SPIN=True, EPIN=True, EROWS=32, DMA_ORDER='a0 a1 a2 a3 k0 v0 k1 v1 k2 v2 k3 v3 x1 f0 x2 f1 o0 o1 x3 f2 o2 o3 x4 f3'.split(), PSLOT=(1, 3), A0=0.55, AEND=0.85, SCOPES=False, OTR=0, FSL=(14, 18, 38, 38)):

    stack = []
    def mark(name):
        if not SCOPES: return
        if stack: stack.pop().__exit__(None, None, None)
        if name:
            cm = jax.named_scope(name); cm.__enter__(); stack.append(cm)

    def kernel(x_hbm, wqkv_hbm, wphi_hbm, wo_hbm, wr_hbm, wg_hbm, wu_hbm, wd_hbm,
               out_hbm,
               in_v, st_v, xb_v, wphi_v, wr_v, lm_v, a_v, a23_v, wo_v, wg_v, wu_v, wd_v,
               kv_acc, z_acc, kvb_v, r_v, raw_v, phi_v, oba_v, obb_v, part_v, xcol_v, y_acc, out_v, zero_s,
               sem_x, sem_w, sem_s, sem_f, sem_o):
        def cp_x(r0, n, sem, src0=None):
            src0 = r0 if src0 is None else src0
            return pltpu.make_async_copy(x_hbm.at[pl.ds(src0, n)], in_v.at[pl.ds(r0, n)], sem_x.at[sem])

        def cp_x0(piece):
            return cp_x((piece % 2) * TH + (piece // 2) * (TH // 2), TH // 2, 0 if piece < 2 else NTILE + 1)

        def cp_xt(t):
            return cp_x(pl.multiple_of(t * T, T), T, t, pl.multiple_of((t % NTILE) * T, T))

        def cp_w(j, c0, n, sem):
            src = wo_hbm.at[:, pl.ds(c0, n)] if j == 3 else wqkv_hbm.at[:, pl.ds(aligned(j * D + c0, 128), n)]
            return pltpu.make_async_copy(src, in_v.at[pl.ds(WQ + j * D, D), pl.ds(c0, n)], sem_w.at[sem])

        def cp_k(c):
            return cp_w(1, c * 256, 256, c)

        def cp_v(c):
            return cp_w(2, c * 256, 256, c if c else 4)

        def cp_fold(t):
            return [cp_w(0, aligned(g * 128, 128), 128, 5 + t) for g in (t, t + 4)]

        def cp_wo(u):
            g = (u // 2) * 4 + u % 2
            return [cp_w(3, aligned(c * 128, 128), 128, 9 + u // 2) for c in (g, g + 2)]

        cp_phi = pltpu.make_async_copy(wphi_hbm, wphi_v, sem_s.at[0])
        cp_wr = pltpu.make_async_copy(wr_hbm, wr_v, sem_s.at[0])
        def cp_ffn(g):
            cps = []
            for j in range(FG):
                cols = pl.ds(aligned((g * FG + j) * 128, 128), 128)
                for src, dst in ((wg_hbm, wg_v), (wu_hbm, wu_v)):
                    cps.append(pltpu.make_async_copy(src.at[:, cols], dst.at[g * FG + j], sem_f.at[g]))
            rows = pl.ds(aligned(g * FG * 128, 128), FG * 128)
            for n in range(D // 128):
                cps.append(pltpu.make_async_copy(wd_hbm.at[rows, pl.ds(n * 128, 128)], wd_v.at[n, rows], sem_f.at[g]))
            return cps

        def cp_o(k, t):
            rows = pl.ds(pl.multiple_of(t * T, T), T)
            return pltpu.make_async_copy(out_v.at[rows], out_hbm.at[rows], sem_o.at[0])

        def cp_o_blk(t, blk):
            rows = pl.ds(pl.multiple_of(t * T + (blk % 2) * TH, TH), TH)
            cols = pl.ds((blk // 2) * 256, 256)
            return pltpu.make_async_copy(out_v.at[rows, cols], out_hbm.at[rows, cols], sem_o.at[0])

        cp_wr.start()
        cp_phi.start()
        for n, name in enumerate(DMA_ORDER):
            if n == 1:
                cp_wr.wait()
                cp_phi.wait()
            cps = {"a": cp_x0, "k": cp_k, "v": cp_v, "x": cp_xt, "f": cp_fold, "o": cp_wo}[name[0]](int(name[1]))
            for cp in cps if isinstance(cps, list) else [cps]:
                cp.start()

        last_product = []

        clock = [0.0]
        rate = [7]

        def pin(n=8):
            if not last_product:
                return jnp.zeros((n, 128), f32)
            q = min(int((clock[0] * rate[0]) % 1.0 * 64 + 1e-6), 63) if FINE else 0
            m = last_product[0][(q % 32) * 8:(q % 32) * 8 + 8, (q // 32) * 128:(q // 32) * 128 + 128]
            z = pltpu.bitcast(pltpu.bitcast(m, u32) & zero_s[0].astype(u32), f32)
            return z if n == 8 else jnp.concatenate([z] * (n // 8), axis=0)

        def as_bf16(w):
            return pltpu.bitcast(w, bf16)

        def words(ref, *idx):
            return pltpu.bitcast(ref[idx], u32)

        def feature_maps():
            def target(shape):
                s = lax.broadcasted_iota(i32, shape, 0)
                return (s // 16) * 16 + (s % 8) * 2 + (s // 8) % 2

            rho = target((128, DH))
            sel = (((rho % 64) // 8) * 4 + (rho % 8) // 2 == lax.broadcasted_iota(i32, (128, DH), 1)).astype(bf16)
            rho = target((128, 128))
            keep = (rho // 64) * 2 + rho % 2 == lax.broadcasted_iota(i32, (128, 128), 1) // DH
            for g in range(8):
                full = _dot_nt(sel, wphi_v[pl.ds(g * 128, 128), :])
                lm_v[g] = jnp.where(keep, full, 0.0).astype(bf16)

        def operand(chunk):
            if isinstance(chunk, int):
                return a_v.at[chunk] if chunk < 2 else a23_v.at[chunk - 2]
            return chunk

        def put_lhs(chunk, rows, cols, a11, a12, a21, a22):
            cmb = [_lhs_combos(a11[e], a12[e], a21[e], a22[e]) for e in range(2)]
            for i in range(7):
                operand(chunk)[i, rows, cols] = _pack(cmb[0][i], cmb[1][i])

        def w_blocks(base, top, bot, k):
            return [in_v[pl.ds(aligned(base + kh * 512 + k * 128, 128), 128),
                         pl.ds(aligned(g * 128, 128), 128)] for g in (top, bot) for kh in range(2)]

        def prep_fold(base, top, bot, chunk, row0):
            for k in range(4):
                blocks = [_dot_nt(lm_v[g], w) for g, w in zip((top, top, bot, bot), w_blocks(base, top, bot, k))]
                for j in range(8):
                    put_lhs(chunk, pl.ds(aligned(row0 + 8 * j, 8), 8), pl.ds(k * 128, 128),
                            *[(p[16 * j:16 * j + 8] * LOG2E, p[16 * j + 8:16 * j + 16] * LOG2E) for p in blocks])
                yield

        def prep_transpose(base, top, bot, chunk, row0):
            for k in range(4):
                zero = pltpu.bitcast(pin(64), u32)
                blocks = [pltpu.bitcast(as_bf16(pltpu.bitcast(w, u32) | zero).T, u32)
                          for w in w_blocks(base, top, bot, k)]
                for j in range(8):
                    put_lhs(chunk, pl.ds(aligned(row0 + 8 * j, 8), 8), pl.ds(k * 128, 128),
                            *[_unpack(w[8 * j:8 * j + 8]) for w in blocks])
                yield

        def prep_q(u):
            return prep_fold(WQ, u, u + 4, a_v.at[2 + u // 2], (u % 2) * 64)

        def prep_wo(u, base=WO):
            g = (u // 2) * 4 + u % 2
            return prep_transpose(base, g, g + 2, wo_v.at[u // 2], (u % 2) * 64)

        def x_words(r0, c0):
            return _unpack(words(in_v, pl.ds(r0, 16), pl.ds(c0, 128)))

        def ln_stats(t, st):
            for step in range(32):
                pos = (step % 2) * 16 + step // 2
                r0 = pl.multiple_of(t * T + pos * 16, 16)
                x0 = x_words(r0, 0)
                if last_product:
                    zero = pin()
                    x0 = [v + zero for v in x0]
                s1, s2 = [None, None], [None, None]
                for j in range(1, 8):
                    xj = x_words(r0, j * 128)
                    for e in range(2):
                        d = xj[e] - x0[e]
                        s1[e] = d if j == 1 else s1[e] + d
                        s2[e] = d * d if j == 1 else s2[e] + d * d
                for e in range(2):
                    lane_mean = x0[e] + s1[e] * 0.125
                    m = jnp.sum(lane_mean, axis=-1, keepdims=True) * (1.0 / 128)
                    dm = lane_mean - m
                    v = jnp.sum((s2[e] - s1[e] * s1[e] * 0.125) * 0.125 + dm * dm, axis=-1, keepdims=True) * (1.0 / 128)
                    mb = m.astype(bf16).astype(f32)
                    vb = (v.astype(bf16).astype(f32) + EPS_BF16).astype(bf16).astype(f32)
                    rs = 1.0 / jnp.sqrt(vb).astype(bf16).astype(f32)
                    st[0, pl.ds(pos * 16 + e, 8, stride=2), :] = jnp.broadcast_to(mb, (8, 128))
                    st[1, pl.ds(pos * 16 + e, 8, stride=2), :] = jnp.broadcast_to(rs, (8, 128))
                yield

        def ln_apply(t, st, xb):
            for step in range(16):
                r0 = [pl.multiple_of(t * T + hf * TH + step * 16 + zero_s[0], 16) for hf in range(2)]
                srow = [[pl.ds(hf * TH + step * 16 + e, 8, stride=2) for e in range(2)] for hf in range(2)]
                mb = [[st[0, srow[hf][e], :] for e in range(2)] for hf in range(2)]
                rs = [[st[1, srow[hf][e], :] for e in range(2)] for hf in range(2)]
                mb0 = mb
                for k in range(4):
                    if last_product:
                        zero = pin()
                        mb = [[v + zero for v in row] for row in mb0]
                    blk = [[x_words(r0[hf], kh * 512 + k * 128) for kh in range(2)] for hf in range(2)]
                    cmb = []
                    for e in range(2):
                        nb = [[(blk[hf][kh][e] - mb[hf][e]) * rs[hf][e] for kh in range(2)] for hf in range(2)]
                        cmb.append(_rhs_combos(nb[0][0], nb[1][0], nb[0][1], nb[1][1]))
                    for i in range(7):
                        xb[i, pl.ds(step * 8, 8), pl.ds(k * 128, 128)] = _pack(cmb[0][i], cmb[1][i])
                    yield

        def project(chunk, xb, res, router=None, keep=None):
            extra = {}

            def prod(i):
                n = 128 + (RR // 2 if router is not None and i % 2 == 0 else 0)
                m = _dot_nt(as_bf16(operand(chunk)[i, pl.ds(0, n), :]), as_bf16(xb[i]))
                last_product[:] = [m]
                if n > 128:
                    extra[i] = m[256:264]
                return m[:256]

            def emit(a, b, val):
                if isinstance(res, list):
                    res[a][b] = val
                else:
                    res[a, b] = val
                if keep is not None:
                    keep[a, b, pl.ds(128, 128), :] = val[128:]
                if router is not None and a == 0:
                    r_v[router, :, pl.ds(b * TH, TH)] = (
                        extra[0] - extra[4] + extra[6] if b == 0 else extra[2] + extra[4])

            return _strassen(prod, emit)

        def raw_blk(res, a, r0, lane):
            b, c0 = lane // 2, (lane % 2) * 128
            if isinstance(res, list):
                return res[a][b][r0:r0 + 64, c0:c0 + 128]
            return res[a, b, pl.ds(r0, 64), pl.ds(c0, 128)]

        keep_kv = lax.broadcasted_iota(i32, (64, 128), 0) // DH == lax.broadcasted_iota(i32, (64, 128), 1) % 2
        keep_z = lax.broadcasted_iota(i32, (16, 128), 0) // 8 == lax.broadcasted_iota(i32, (16, 128), 1) % 2

        def kv_post(c, res, keep=None):
            def accumulate(p, vt, phi):
                kv = kv_acc[p] + _dot_nt(vt, phi)
                kv_acc[p] = kv
                kvb_v[p, pl.ds(0, 64), :] = jnp.where(keep_kv, kv, 0.0).astype(bf16)

            pending = None
            for a in range(2):
                for pr in range(2):
                    p = 4 * c + 2 * a + pr
                    phis, zs = [], z_acc[p]
                    for lane in range(4):
                        phi = _dual_softmax(raw_blk(res, a, pr * 64, lane), pin())
                        zs = zs + phi
                        phis.append(phi.astype(bf16))
                        if keep is not None:
                            keep[2 * a + pr, :, pl.ds(lane * 128, 128)] = pltpu.bitcast(phis[-1], u32)
                        if lane == 1 and pending:
                            accumulate(*pending)
                        if lane == 3:
                            z_acc[p] = zs
                            zrow = jnp.broadcast_to(jnp.sum(zs.T, axis=0, keepdims=True), (16, 128))
                            kvb_v[p, pl.ds(64, 16), :] = jnp.where(keep_z, zrow, 0.0).astype(bf16)
                            vt = jnp.concatenate([raw_blk(res, a, 128 + pr * 64, l) for l in range(4)], axis=1)
                            pending = (p, vt.astype(bf16), jnp.concatenate(phis, axis=1))
                        yield
            yield
            accumulate(*pending)
            yield

        def route():
            r = r_v[pl.ds(0, NTILE)].astype(bf16).astype(f32)
            r = jnp.where(r != r, -jnp.inf, r)
            tok = lax.broadcasted_iota(i32, r.shape, 0) * T + lax.broadcasted_iota(i32, r.shape, 2)
            rmax = jnp.max(jnp.max(r, axis=0), axis=-1, keepdims=True)
            cand = jnp.min(jnp.where(r == rmax[None], tok, S).astype(f32), axis=0)
            return jnp.clip(jnp.min(cand).astype(i32), 0, S - 1), rmax

        def routed_token(idx):
            base = pl.multiple_of((idx // 16) * 16, 16)
            rows = pl.ds(pl.multiple_of(base % T, 16), 16)
            xn = (in_v[pl.ds(base, 16), :].astype(f32) - st_v[idx // T, 0, rows, 0:1]) * st_v[idx // T, 1, rows, 0:1]
            xsel = jnp.where(lax.broadcasted_iota(i32, (16, D), 0) == idx - base, xn, 0.0)
            xsel = jnp.sum(xsel, axis=0, keepdims=True).astype(bf16).astype(f32)
            for j in range(8):
                row = xsel[:, j * 128:(j + 1) * 128] + pin()
                xcol_v[pl.ds(j * 128, 128), :] = jnp.concatenate([row] * 16, axis=0).T
                yield

        mark('s0_init')
        zero_s[0] = 0
        kv_acc[...] = jnp.zeros(kv_acc.shape, f32)
        z_acc[...] = jnp.zeros(z_acc.shape, f32)
        y_acc[...] = jnp.zeros(y_acc.shape, f32)
        r_v[...] = jnp.full(r_v.shape, -jnp.inf, f32)
        w8 = wr_v[...].astype(f32)
        wrow = jnp.broadcast_to(jnp.concatenate([w8[j:j + 1, :] for j in range(8)], axis=1), (RR // 2, D))
        none = [jnp.zeros((RR // 2, 512), f32)] * 2
        put_lhs(0, pl.ds(128, RR // 2), slice(None), [wrow[:, :512]] * 2, [wrow[:, 512:]] * 2, none, none)
        for i in range(7):
            a_v[2, i, pl.ds(128, RR // 2), :] = jnp.zeros((RR // 2, 512), u32)
        feature_maps()
        mark('s1_ln0')
        stats, apply = ln_stats(0, st_v.at[0]), ln_apply(0, st_v.at[0], xb_v.at[0])
        for half in range(2):
            cp_x0(2 * half).wait()
            cp_x0(2 * half + 1).wait()
            _schedule(clock, (stats, 16, 0.0, 1.0))
            _schedule(clock, (apply, 32, 0.0, 1.0))

        def prep_kv(c):
            cp_k(c).wait()
            if c:
                cp_v(c).wait()
            yield from prep_fold(WK, 2 * c, 2 * c + 1, c, 0)
            if not c:
                cp_v(c).wait()
            yield from prep_transpose(WV, 2 * c, 2 * c + 1, c, 64)

        mark('s3_prep0')
        _schedule(clock, (prep_kv(0), 8, 0.0, 1.0))
        mark('s4_proj0')
        _schedule(clock, (project(0, xb_v.at[0], raw_v.at[0], router=0), 7, 0.0, 1.0),
                  (prep_kv(1), 8, W1, 1.0))
        _schedule(clock, (project(1, xb_v.at[0], raw_v.at[1]), 7, 0.0, 1.0),
                  (kv_post(0, raw_v.at[zero_s[0]]), 18, 0.0, 1.0), (prep_kv(2), 8, W2, W3), (prep_kv(3), 8, W3, 1.0))

        def kv_tile(t, idx):
            last = t == NTILE - 1
            for cp in cp_fold(t) + [cp_xt(t + 1)]:
                cp.wait()

            @pl.when(jnp.logical_and(t > 0, t < 3))
            def _():
                for cp in cp_wo(2 * t - 2) + cp_wo(2 * t - 1):
                    cp.wait()

            if not NOBC:
                for g in range(NTILE):
                    @pl.when(t == g)
                    def _():
                        for cp in cp_ffn(g):
                            cp.start()

            last_product[:] = []
            idx = route()[0]
            xb, st = xb_v.at[pl.ds(t, 2)], st_v.at[t + 1]
            stats, apply = ln_stats(t + 1, st), ln_apply(t + 1, st, xb.at[1])
            fold = prep_q(t)
            trans = [prep_wo(2 * ((t + 1) % 2) + u, jnp.where(t == 0, WV, WO)) for u in range(2)]

            def fetch_ffn():
                for cp in cp_ffn(t):
                    cp.start()
                    yield

            c2, c3, c0 = ([[None, None], [None, None]] for _ in range(3))
            _schedule(clock, (project(2, xb.at[0], c2), 7, 0.0, 1.0), (kv_post(1, raw_v.at[1]), 18, 0.0, 1.0),
                      (stats, SA[0], 0.0, 1.0), (apply, 4 * SB[0], 0.07, 1.0), (fold, SF[0], 0.1, 0.9),
                      (fetch_ffn(), 2 * FG + 8 if NOBC else 0, 0.05, 0.95))
            _schedule(clock, (project(3, xb.at[0], c3), 7, 0.0, 1.0), (kv_post(2, c2), 18, 0.0, 1.0),
                      (stats, SA[1], 0.0, 0.5), (apply, 4 * SB[1], 0.03, AEND), (fold, SF[1], 0.1, 0.8))
            xb = xb_v.at[jnp.where(last, (idx // T + 1) % NTILE, t + 1)]
            chunk = jnp.where(last, 2, 0)
            _schedule(clock, (project(a_v.at[chunk], xb, c0, router=t + 1, keep=raw_v.at[0]), 7, 0.0, 1.0),
                      (kv_post(3, c3), 18, 0.0, 1.0), (trans[0], 4, 0.1, 0.9), (routed_token(idx), 8, 0.0, 1.0))
            _schedule(clock, (project(a_v.at[chunk + 1], xb, raw_v.at[1]), 7, 0.0, 1.0),
                      (kv_post(jnp.where(last, 4, 0), c0, phi_v), 18, 0.0, 1.0), (trans[1], 4, 0.1, 0.9))
            return idx

        mark('s6_phase1')
        idx = lax.fori_loop(0, NTILE, kv_tile, jnp.int32(0))
        mark('s7_mid')
        for cp in cp_ffn(0):
            cp.wait()
        last_product[:] = []

        rmax = route()[1]
        first = (idx // T + 1) % NTILE

        def ffn(f0, nf):
            for j in range(nf):
                cols = pl.ds(pl.multiple_of((f0 + j) * 128, 128), 128)
                accs = [jnp.zeros((8, 128), f32)] * 2
                for r in range(8):
                    rows = pl.ds(r * 128, 128)
                    xc = xcol_v[rows, :]
                    if FPIN:
                        zero = pin()
                    for a, w_v in enumerate((wg_v, wu_v)):
                        prod = w_v[f0 + j, rows, :].astype(f32) * xc
                        acc = accs[a] + zero if FPIN else accs[a]
                        for q in range(16):
                            acc = acc + prod[8 * q:8 * q + 8]
                        accs[a] = acc
                    yield
                gate, up = [jnp.sum(acc, axis=0, keepdims=True) for acc in accs]
                hcol = jnp.broadcast_to(gate * jax.nn.sigmoid(gate) * up, (128, 128)).T
                for n in range(8):
                    ycols = pl.ds(n * 128, 128)
                    prod = wd_v[n, cols, :].astype(f32) * hcol
                    acc = y_acc[:, ycols] + pin() if FPIN else y_acc[:, ycols]
                    for q in range(16):
                        acc = acc + prod[8 * q:8 * q + 8]
                    y_acc[:, ycols] = acc
                    if n % 2 == 1:
                        yield

        def tile(j):
            return (first + j) % NTILE

        def q_post(c, res, ob, ready=None):
            phis, nds, outs = {}, {}, {}
            for tick in range(40):
                step, lane = tick // 4, tick % 4
                if ready is not None and step < 4:
                    phis.setdefault(step, []).append(as_bf16(ready[step, :, pl.ds(lane * 128, 128)]))
                elif step < 8:
                    u, a, pr = step // 4, (step // 2) % 2, step % 2
                    phis.setdefault(step, []).append(_dual_softmax(
                        raw_blk(res, a, u * 128 + pr * 64, lane), pin() if SPIN else None).astype(bf16))
                if 1 <= step < 9 and lane == 1:
                    w = step - 1
                    pair = 2 * (2 * c + w // 4 + 4 * ((w // 2) % 2)) + w % 2
                    nds[step - 1] = _dot(kvb_v[pair], jnp.concatenate(phis.pop(step - 1), axis=1))
                if step >= 2 and lane == 0:
                    nd = nds.pop(step - 2)
                    rd = _recip(nd[64:80, :] + 1e-6)
                    outs[step - 2] = jnp.concatenate(
                        [(nd[0:32, :].reshape(4, 8, T) * rd[0:8, :][None]).reshape(32, T),
                         (nd[32:64, :].reshape(4, 8, T) * rd[8:16, :][None]).reshape(32, T)], axis=0)
                    if (step - 2) % 4 == 3:
                        u = (step - 2) // 4
                        o1 = jnp.concatenate([outs.pop(4 * u), outs.pop(4 * u + 1)], axis=0)
                        o2 = jnp.concatenate([outs.pop(4 * u + 2), outs.pop(4 * u + 3)], axis=0)
                        cmb = _rhs_combos(o1[:, :TH], o1[:, TH:], o2[:, :TH], o2[:, TH:])
                        if OTR == 0:
                            for i in range(7):
                                ob[i, :, pl.ds(u * 128, 128)] = pltpu.bitcast(cmb[i].astype(bf16).T, u32)
                        else:
                            for b in range(2):
                                tr = pltpu.bitcast(jnp.concatenate(
                                    [v[:, b * 128:(b + 1) * 128] for v in cmb], axis=0).astype(bf16).T, u32)
                                for i in range(7):
                                    ob[i, pl.ds(b * 64, 64), pl.ds(u * 128, 128)] = tr[:, i * 128:(i + 1) * 128]
                yield

        def out_project(h, oba, obb, res, ks=(0, 1)):
            def prod(i):
                lhs = jnp.concatenate([(oba, obb)[k][i] for k in ks], axis=1)
                m = _dot_nt(as_bf16(lhs), as_bf16(wo_v[h, i, :, pl.ds(ks[0] * 256, len(ks) * 256)]))
                last_product[:] = [m]
                return m

            def emit(a, b, val):
                if isinstance(res, list):
                    res[a][b] = val
                else:
                    res[a, b] = val

            return _strassen(prod, emit)

        def epilogue(t, h, res, part=None, upd=None, done=None):
            n = EROWS
            for a in range(2):
                for b in range(2):
                    cols = pl.ds(h * 512 + a * 256, 256)
                    for q in range(TH // n):
                        r0 = pl.multiple_of(t * T + b * TH + q * n, n)
                        rows = pl.ds(b * TH + q * n, n)
                        mb, rs = st_v[t, 0, rows, :], st_v[t, 1, rows, :] * 0.5
                        if upd is None:
                            mb = mb + pin(n)
                        x = in_v[pl.ds(r0, n), cols].astype(f32)
                        v = (x - jnp.concatenate([mb, mb], axis=1)) * jnp.concatenate([rs, rs], axis=1)
                        if upd is not None:
                            rid = lax.broadcasted_iota(i32, (n, 256), 0)
                            v = v + jnp.where(rid == idx - r0, upd[:, h * 512 + a * 256:h * 512 + (a + 1) * 256], 0.0)
                        g = v + v * jnp.tanh(v)
                        s = res[a][b][q * n:(q + 1) * n]
                        if part is not None:
                            s = s + part[a, b, pl.ds(q * n, n), :]
                        out_v[pl.ds(r0, n), cols] = (x + s * g).astype(bf16)
                        if done is not None and q == TH // n - 1:
                            done(4 * h + 2 * a + b)
                        yield

        NE = 4 * TH // EROWS
        mark('s8_q0')
        fb = NF - (NTILE - 1) * FL
        res0 = None
        _schedule(clock, (q_post(0, raw_v.at[0], oba_v.at[0], phi_v), 40, 0.0, 1.0))

        def q_tile(j, carry):
            last_product[:] = []
            oba = oba_v.at[pl.ds(j, 2)]
            obb = obb_v.at[zero_s[0]]
            xb = xb_v.at[tile(j + 1)]
            for cp in cp_ffn(j + 1):
                cp.wait()
            fg = ffn(j * FL, FL)
            q0, o0, o1 = ([[None, None], [None, None]] for _ in range(3))
            _schedule(clock, (project(a_v.at[2], xb, q0), 7, 0.0, 1.0), (q_post(1, raw_v.at[1], obb_v.at[0]), 40, 0.0, PEND),
                      (fg, FSL[0], 0.1, 1.0))
            _schedule(clock, (out_project(0, oba.at[0], obb, o0), 7, 0.0, 1.0), (q_post(0, q0, oba.at[1]), 40, 0.05, 1.0),
                      (fg, FSL[1], 0.1, 1.0))
            _schedule(clock, (out_project(1, oba.at[0], obb, o1), 7, 0.0, 1.0), (epilogue(tile(j), 0, o0), NE, 0.0, 1.0),
                      (fg, FSL[2], 0.1, 1.0))
            _schedule(clock, (project(a_v.at[3], xb, raw_v.at[1]), 7, 0.0, 1.0), (epilogue(tile(j), 1, o1), NE, 0.0, 1.0),
                      (fg, FSL[3], 0.1, 0.9))
            cp_o(j, tile(j)).start()
            return carry

        mark('s9_phase2')
        lax.fori_loop(0, NTILE - 1, q_tile, 0)
        mark('sa_tail')

        j = NTILE - 1
        rate[0] = 14
        last_product[:] = []
        oba, obb = oba_v.at[j], obb_v.at[zero_s[0]]
        _schedule(clock, (out_project(0, oba, obb, part_v.at[0], (0,)), 7, 0.0, 0.5),
                  (out_project(1, oba, obb, part_v.at[1], (0,)), 7, 0.5, 1.0),
                  (q_post(1, raw_v.at[1], obb_v.at[0]), 40, 0.0, PEND),
                  (ffn(NF - fb, fb), 12 * fb, 0.1, 0.8))
        upd = jnp.sum(y_acc[...], axis=0, keepdims=True) * (0.5 * jax.nn.sigmoid(rmax[0:1, :]))
        o0, o1 = ([[None, None], [None, None]] for _ in range(2))
        t = tile(j)
        send = lambda blk: cp_o_blk(t, blk).start()
        e0 = epilogue(t, 0, o0, part_v.at[0], upd, send)
        e1 = epilogue(t, 1, o1, part_v.at[1], upd, send)
        _schedule(clock, (out_project(0, oba, obb, o0, (1,)), 7, 0.0, 0.5),
                  (out_project(1, oba, obb, o1, (1,)), 7, 0.5, 1.0),
                  (e0, NE, 0.29, 0.57), (e1, NE, 0.79, 1.07))
        mark('sb_outdma')
        for k in range(NTILE - 1):
            cp_o(k, tile(k)).wait()
        for blk in range(8):
            cp_o_blk(t, blk).wait()
        mark(None)

    scratch = [
        pltpu.VMEM((S + T + 4 * D, D), bf16),
        pltpu.VMEM((NTILE + 1, 2, T, 128), f32),
        pltpu.VMEM((NTILE + 1, 7, TH // 2, 512), u32),
        pltpu.VMEM((D, DH), bf16),
        pltpu.VMEM((8, 128), bf16),
        pltpu.VMEM((8, 128, 128), bf16),
        pltpu.VMEM((4, 7, 128 + RR // 2, 512), u32),
        pltpu.VMEM((2, 7, 128, 512), u32),
        pltpu.VMEM((2, 7, 128, 512), u32),
        pltpu.VMEM((NF, D, 128), bf16),
        pltpu.VMEM((NF, D, 128), bf16),
        pltpu.VMEM((D // 128, F, 128), bf16),
        pltpu.VMEM((H // 2 + 4, 64, 128), f32),
        pltpu.VMEM((H // 2 + 4, 128, 128), f32),
        pltpu.VMEM((H // 2 + 4, 80, 128), bf16),
        pltpu.VMEM((NTILE + 1, 8, T), f32),
        pltpu.VMEM((2, 2, 2, 256, TH), f32),
        pltpu.VMEM((4, 64, T), u32),
        pltpu.VMEM((NTILE, 7, TH // 2, 256), u32),
        pltpu.VMEM((2, 7, TH // 2, 256), u32),
        pltpu.VMEM((2, 2, 2, 256, 256), f32),
        pltpu.VMEM((D, 128), f32),
        pltpu.VMEM((8, D), f32),
        pltpu.VMEM((S, D), bf16),
        pltpu.SMEM((1,), i32),
        pltpu.SemaphoreType.DMA((NTILE + 2,)),
        pltpu.SemaphoreType.DMA((11,)),
        pltpu.SemaphoreType.DMA((1,)),
        pltpu.SemaphoreType.DMA((NTILE,)),
        pltpu.SemaphoreType.DMA((1,)),
    ]

    def call(x, wqkv, wphi, wo, wr, wg, wu, wd):
        hbm = pl.BlockSpec(memory_space=pltpu.HBM)
        return pl.pallas_call(
            kernel,
            out_shape=jax.ShapeDtypeStruct((S, D), bf16),
            in_specs=[hbm] * 8,
            out_specs=hbm,
            scratch_shapes=scratch,
            compiler_params=pltpu.CompilerParams(vmem_limit_bytes=120 * 2**20, flags=FLAGS, disable_bounds_checks=NOBC),
            name="hedgehog",
        )(x, wqkv, wphi, wo, wr, wg, wu, wd)

    return call


@jax.jit
def pallas_recurrent_scan__linear_kernel_hedgehog__moe_arch_mod__prompt_kernel(
    A_x: jax.Array,
    A_wqkv: jax.Array,
    A_w_phi: jax.Array,
    A_wo: jax.Array,
    B_x: jax.Array,
    B_w_r: jax.Array,
    B_w_gate: jax.Array,
    B_w_up: jax.Array,
    B_w_down: jax.Array,
):
    del B_x
    out = make_kernel()(
        A_x.reshape(S, D), A_wqkv, A_w_phi.reshape(D, DH), A_wo,
        B_w_r.reshape(8, 128), B_w_gate, B_w_up, B_w_down)
    return out.reshape(1, S, D)
```

```python
import math
import contextlib

import numpy as np

import jax
import jax.numpy as jnp
from jax import lax
import jax.experimental.pallas as pl
import jax.experimental.pallas.tpu as pltpu

S, D, H, DH, F = 2048, 1024, 32, 32, 3584
T = 512
TH = T // 2
NTILE = S // T
NF = F // 128
FG = NF // NTILE
WQ, WK, WV, WO = (S + T + j * D for j in range(4))
LHS_SUMS, RHS_SUMS = (0, 1, 4, 5, 6), (0, 2, 3, 5, 6)
LOG2E = math.log2(math.e)
EPS_BF16 = float(np.float32(1e-5).astype(jnp.bfloat16))
NT_DIMS = (((1,), (1,)), ((), ()))
f32, bf16, i32, u32 = jnp.float32, jnp.bfloat16, jnp.int32, jnp.uint32


def _dot_nt(a, b):
    return lax.dot_general(a, b, NT_DIMS, preferred_element_type=f32)


def _dot(a, b):
    return jnp.dot(a, b, preferred_element_type=f32)


def aligned(i, n):
    return i if isinstance(i, int) else pl.multiple_of(i, n)


def _recip(v):
    r = pl.reciprocal(v, approx=True)
    return r * (2.0 - v * r)


def _unpack(w):
    return [pltpu.unpack_elementwise(w, index=i, packed_dtype=bf16, unpacked_dtype=f32) for i in range(2)]


def _pack(even, odd):
    return pltpu.bitcast(pltpu.pack_elementwise([even, odd], packed_dtype=bf16), u32)


def _lhs_combos(a11, a12, a21, a22):
    return [a11 + a22, a21 + a22, a11, a22, a11 + a12, a21 - a11, a12 - a22]


def _rhs_combos(b11, b12, b21, b22):
    return [b11 + b22, b11, b12 - b22, b21 - b11, b22, b11 + b12, b21 + b22]


class _Quad:
    def __init__(self, v):
        self.v = v

    def __add__(self, o):
        return _Quad([p + q for p, q in zip(self.v, o.v)])

    def __sub__(self, o):
        return _Quad([p - q for p, q in zip(self.v, o.v)])


def _strassen2(prod, emit, order):
    done = {}

    def inner(i):
        out = [None] * 4

        def put(a, b, val):
            out[2 * a + b] = val
        yield from _strassen(lambda j: prod(7 * i + j), put, order)
        done[i] = _Quad(out)

    def put(a, b, quad):
        for k, val in enumerate(quad.v):
            emit(2 * a + k // 2, 2 * b + k % 2, val)

    outer = _strassen(lambda i: done[i], put, order)
    for i in ((0, 3, 4, 6, 2, 1, 5), (2, 4, 0, 6, 3, 1, 5))[order]:
        steps = inner(i)
        for _ in range(6):
            next(steps)
            yield
        for _ in steps:
            pass
        next(outer)
        yield


def _strassen(prod, emit, order=0):
    if order == 0:
        m1 = prod(0)
        yield
        m4 = prod(3)
        c11 = m1 + m4
        yield
        m5 = prod(4)
        c11 = c11 - m5
        yield
        emit(0, 0, c11 + prod(6))
        yield
        m3 = prod(2)
        emit(0, 1, m3 + m5)
        c22 = m1 + m3
        yield
        m2 = prod(1)
        emit(1, 0, m2 + m4)
        c22 = c22 - m2
        yield
        emit(1, 1, c22 + prod(5))
        yield
    else:
        m3 = prod(2)
        yield
        m5 = prod(4)
        emit(0, 1, m3 + m5)
        yield
        m1 = prod(0)
        c11, c22 = m1 - m5, m1 + m3
        yield
        c11 = c11 + prod(6)
        yield
        m4 = prod(3)
        emit(0, 0, c11 + m4)
        yield
        m2 = prod(1)
        emit(1, 0, m2 + m4)
        c22 = c22 - m2
        yield
        emit(1, 1, c22 + prod(5))
        yield


def _schedule(clock, *streams):
    events = []
    for order, (gen, n, a, b) in enumerate(streams):
        for k in range(n):
            events.append((a + (b - a) * k / n, order, k, gen))
    for when, _, _, gen in sorted(events, key=lambda e: e[:3]):
        clock[:] = [when]
        next(gen)


def _dual_softmax(p, zero=None):
    rows = [p[8 * j:8 * j + 8] for j in range(8)]
    if zero is not None:
        rows[0] = rows[0] + zero

    def reduce(vs, op):
        while len(vs) > 1:
            vs = [op(vs[i], vs[i + 1]) for i in range(0, len(vs), 2)]
        v = op(vs[0], pltpu.roll(vs[0], 4, 0))
        return op(v, pltpu.roll(v, 2, 0))

    mx, mn = reduce(rows, jnp.maximum), reduce(rows, jnp.minimum)
    ep = [jnp.exp2(v - mx) for v in rows]
    en = [jnp.exp2(mn - v) for v in rows]
    rp, rn = _recip(reduce(ep, jnp.add)), _recip(reduce(en, jnp.add))
    return jnp.concatenate([v * rp for v in ep] + [v * rn for v in en], axis=0)


def make_kernel(FL=9, ORDER=1, P2END=0.9, B1END=0.6, B2START=0.2, W1=0.58, W2=0.15, W3=0.6, NOBC=True, DSLOT=3, SF=(3, 1), TW=(), TF=False, SAB=(0, 0), SS=(8, 8), SQ=(4, 4), PEND=1.0, FLAGS=None,
                FPIN=True, FINE=True, SPIN=True, EPIN=True, EROWS=32, DMA_ORDER='a0 a1 a2 a3 k0 v0 k1 v1 k2 v2 k3 v3 x1 f0 x2 f1 o0 o1 x3 f2 o2 o3 x4 f3'.split(), PSLOT=(1, 3), A0=0.55, AEND=0.95, SCOPES=False, OTR=0, FSL=(14, 18, 38, 38)):

    stack = []
    def mark(name):
        if not SCOPES: return
        if stack: stack.pop().__exit__(None, None, None)
        if name:
            cm = jax.named_scope(name); cm.__enter__(); stack.append(cm)

    def kernel(x_hbm, wqkv_hbm, wphi_hbm, wo_hbm, wr_hbm, wg_hbm, wu_hbm, wd_hbm,
               out_hbm,
               in_v, st_v, xb_v, xx_v, wphi_v, wr8_v, wr_v, lm_v, a_v, aa_v, b_v, bb_v, wo_v, wg_v, wu_v, wd_v,
               kv_acc, z_acc, kvb_v, best_v, best_i, raw_v, half_v, phi_v, oba_v, obb_v, part_v, xcol_v, y_acc,
               out_v, zero_s, sem_x, sem_w, sem_s, sem_f, sem_o):
        def cp_x(r0, n, sem, src0=None):
            src0 = r0 if src0 is None else src0
            return pltpu.make_async_copy(x_hbm.at[pl.ds(src0, n)], in_v.at[pl.ds(r0, n)], sem_x.at[sem])

        def cp_x0(piece):
            return cp_x((piece % 2) * TH + (piece // 2) * (TH // 2), TH // 2, 0 if piece < 2 else NTILE + 1)

        def cp_xt(t):
            return cp_x(pl.multiple_of(t * T, T), T, t, pl.multiple_of((t % NTILE) * T, T))

        def cp_w(j, c0, n, sem):
            src = wo_hbm.at[:, pl.ds(c0, n)] if j == 3 else wqkv_hbm.at[:, pl.ds(aligned(j * D + c0, 128), n)]
            return pltpu.make_async_copy(src, in_v.at[pl.ds(WQ + j * D, D), pl.ds(c0, n)], sem_w.at[sem])

        def cp_k(c):
            return cp_w(1, c * 256, 256, c)

        def cp_v(c):
            return cp_w(2, c * 256, 256, c if c else 4)

        def cp_fold(t):
            return [cp_w(0, aligned(g * 128, 128), 128, 5 + t) for g in (t, t + 4)]

        def cp_wo(u):
            g = (u // 2) * 4 + u % 2
            return [cp_w(3, aligned(c * 128, 128), 128, 9 + u // 2) for c in (g, g + 2)]

        cp_phi = pltpu.make_async_copy(wphi_hbm, wphi_v, sem_s.at[0])
        cp_wr = pltpu.make_async_copy(wr_hbm, wr8_v, sem_s.at[0])
        def cp_ffn(g):
            cps = []
            for j in range(FG):
                cols = pl.ds(aligned((g * FG + j) * 128, 128), 128)
                for src, dst in ((wg_hbm, wg_v), (wu_hbm, wu_v)):
                    cps.append(pltpu.make_async_copy(src.at[:, cols], dst.at[g * FG + j], sem_f.at[g]))
            rows = pl.ds(aligned(g * FG * 128, 128), FG * 128)
            for n in range(D // 128):
                cps.append(pltpu.make_async_copy(wd_hbm.at[rows, pl.ds(n * 128, 128)], wd_v.at[n, rows], sem_f.at[g]))
            return cps

        def cp_o(k, t):
            rows = pl.ds(pl.multiple_of(t * T, T), T)
            return pltpu.make_async_copy(out_v.at[rows], out_hbm.at[rows], sem_o.at[0])

        def cp_o_blk(t, blk):
            rows = pl.ds(pl.multiple_of(t * T + (blk % 2) * TH, TH), TH)
            cols = pl.ds((blk // 2) * 256, 256)
            return pltpu.make_async_copy(out_v.at[rows, cols], out_hbm.at[rows, cols], sem_o.at[0])

        cp_wr.start()
        cp_phi.start()
        for n, name in enumerate(DMA_ORDER):
            if n == 1:
                cp_wr.wait()
                cp_phi.wait()
            cps = {"a": cp_x0, "k": cp_k, "v": cp_v, "x": cp_xt, "f": cp_fold, "o": cp_wo}[name[0]](int(name[1]))
            for cp in cps if isinstance(cps, list) else [cps]:
                cp.start()

        last_product = []

        clock = [0.0]
        rate = [7]

        def pin(n=8):
            if not last_product:
                return jnp.zeros((n, 128), f32)
            rows, cols = last_product[0].shape[0] // 8, last_product[0].shape[1] // 128
            q = min(int((clock[0] * last_product[1]) % 1.0 * rows * cols + 1e-6), rows * cols - 1)
            m = last_product[0][(q % rows) * 8:(q % rows) * 8 + 8, (q // rows) * 128:(q // rows) * 128 + 128]
            z = pltpu.bitcast(pltpu.bitcast(m, u32) & zero_s[0].astype(u32), f32)
            return z if n == 8 else jnp.concatenate([z] * (n // 8), axis=0)

        def as_bf16(w):
            return pltpu.bitcast(w, bf16)

        def words(ref, *idx):
            return pltpu.bitcast(ref[idx], u32)

        def feature_maps():
            def target(shape):
                s = lax.broadcasted_iota(i32, shape, 0)
                return (s // 16) * 16 + (s % 8) * 2 + (s // 8) % 2

            rho = target((128, DH))
            sel = (((rho % 64) // 8) * 4 + (rho % 8) // 2 == lax.broadcasted_iota(i32, (128, DH), 1)).astype(bf16)
            rho = target((128, 128))
            keep = (rho // 64) * 2 + rho % 2 == lax.broadcasted_iota(i32, (128, 128), 1) // DH
            for g in range(8):
                full = _dot_nt(sel, wphi_v[pl.ds(g * 128, 128), :])
                lm_v[g] = jnp.where(keep, full, 0.0).astype(bf16)

        def operand(chunk):
            if isinstance(chunk, int):
                return (a_v.at[chunk], None) if chunk < 2 else (b_v.at[chunk - 2], bb_v.at[chunk - 2])
            return a_v.at[chunk], None

        def put_lhs(dst, rows, cols, a11, a12, a21, a22):
            cmb = [_lhs_combos(a11[e], a12[e], a21[e], a22[e]) for e in range(2)]
            for i in range(7):
                dst[i, rows, cols] = _pack(cmb[0][i], cmb[1][i])

        def split_again(src, dst, lhs, r, k):
            for i in range(7):
                zero = pltpu.bitcast(pin(), u32)
                quad = [[_unpack(src[i, pl.ds(h * 64 + r * 8, 8), pl.ds(aligned(c * 256 + k * 128, 128), 128)] | zero
                                 if (h, c) in ((0, 0), (1, 1)) else
                                 src[i, pl.ds(h * 64 + r * 8, 8), pl.ds(aligned(c * 256 + k * 128, 128), 128)])
                         for c in range(2)] for h in range(2)]
                if lhs:
                    cmb = [_lhs_combos(quad[0][0][e], quad[0][1][e], quad[1][0][e], quad[1][1][e]) for e in range(2)]
                else:
                    cmb = [_rhs_combos(quad[0][0][e], quad[1][0][e], quad[0][1][e], quad[1][1][e]) for e in range(2)]
                for n, j in enumerate(LHS_SUMS if lhs else RHS_SUMS):
                    dst[5 * i + n, pl.ds(r * 8, 8), pl.ds(aligned(k * 128, 128), 128)] = _pack(cmb[0][j], cmb[1][j])
                yield

        def second(src, dst, lhs, ij):
            i, j = ij // 7, ij % 7
            sums = LHS_SUMS if lhs else RHS_SUMS
            if j in sums:
                return as_bf16(dst[5 * i + sums.index(j)])
            d = int(j == (3 if lhs else 4))
            return as_bf16(src[i, pl.ds(d * 64, 64), pl.ds(d * 256, 256)])

        def w_blocks(base, top, bot, k):
            return [in_v[pl.ds(aligned(base + kh * 512 + k * 128, 128), 128),
                         pl.ds(aligned(g * 128, 128), 128)] for g in (top, bot) for kh in range(2)]

        def prep_fold(base, top, bot, dst, row_of, ks):
            for k in ks:
                blocks = [_dot_nt(lm_v[g], w) for g, w in zip((top, top, bot, bot), w_blocks(base, top, bot, k))]
                for j in range(8):
                    put_lhs(dst, pl.ds(aligned(row_of(j), 8), 8), pl.ds(aligned(k * 128, 128), 128),
                            *[(p[16 * j:16 * j + 8] * LOG2E, p[16 * j + 8:16 * j + 16] * LOG2E) for p in blocks])
                yield

        def prep_transpose(base, top, bot, dst, row_of, fine=False):
            for k in range(4):
                zero = pltpu.bitcast(pin(64), u32)
                blocks = [pltpu.bitcast(as_bf16(pltpu.bitcast(w, u32) | zero).T, u32)
                          for w in w_blocks(base, top, bot, k)]
                for j in range(8):
                    ws = [w[8 * j:8 * j + 8] for w in blocks]
                    if fine:
                        zero = pltpu.bitcast(pin(), u32)
                        ws = [ws[0] | zero, ws[1], ws[2], ws[3] | zero]
                    put_lhs(dst, pl.ds(aligned(row_of(j), 8), 8), pl.ds(k * 128, 128), *[_unpack(w) for w in ws])
                    if fine or j == 7:
                        yield

        def prep_q(u):
            ch, k = u // 2, u % 2
            for half in range(2):
                g = 2 * ch + half
                yield from prep_fold(WQ, g, g + 4, a_v.at[2 + ch], lambda j: half * 64 + 8 * j, (k, k + 2))

        def split_q(u):
            for r in range(8):
                yield from split_again(a_v.at[2 + u // 2 + zero_s[0]], aa_v.at[u // 2], True, r, u % 2)

        def prep_wo(u, base=WO):
            g = (u // 2) * 4 + u % 2
            return prep_transpose(base, g, g + 2, wo_v.at[u // 2], lambda j: (u % 2) * 64 + 8 * j, TF)

        def x_words(r0, c0):
            return _unpack(words(in_v, pl.ds(r0, 16), pl.ds(c0, 128)))

        def ln_stats(t, st):
            for step in range(32):
                pos = (step % 2) * 16 + step // 2
                r0 = pl.multiple_of(t * T + pos * 16, 16)
                x0 = x_words(r0, 0)
                if last_product:
                    zero = pin()
                    x0 = [v + zero for v in x0]
                s1, s2 = [None, None], [None, None]
                for j in range(1, 8):
                    xj = x_words(r0, j * 128)
                    for e in range(2):
                        d = xj[e] - x0[e]
                        s1[e] = d if j == 1 else s1[e] + d
                        s2[e] = d * d if j == 1 else s2[e] + d * d
                for e in range(2):
                    lane_mean = x0[e] + s1[e] * 0.125
                    m = jnp.sum(lane_mean, axis=-1, keepdims=True) * (1.0 / 128)
                    dm = lane_mean - m
                    v = jnp.sum((s2[e] - s1[e] * s1[e] * 0.125) * 0.125 + dm * dm, axis=-1, keepdims=True) * (1.0 / 128)
                    mb = m.astype(bf16).astype(f32)
                    vb = (v.astype(bf16).astype(f32) + EPS_BF16).astype(bf16).astype(f32)
                    rs = 1.0 / jnp.sqrt(vb).astype(bf16).astype(f32)
                    st[0, pl.ds(pos * 16 + e, 8, stride=2), :] = jnp.broadcast_to(mb, (8, 128))
                    st[1, pl.ds(pos * 16 + e, 8, stride=2), :] = jnp.broadcast_to(rs, (8, 128))
                yield

        def ln_apply(t, st, xb, live):
            for step in range(16):
                r0 = [pl.multiple_of(t * T + hf * TH + step * 16 + zero_s[0], 16) for hf in range(2)]
                srow = [[pl.ds(hf * TH + step * 16 + e, 8, stride=2) for e in range(2)] for hf in range(2)]
                mb0 = [[st[0, srow[hf][e], :] for e in range(2)] for hf in range(2)]
                rs = [[st[1, srow[hf][e], :] for e in range(2)] for hf in range(2)]
                score = [[None, None], [None, None]]
                for k in range(4):
                    zero = pin()
                    mb = [[v + zero for v in row] for row in mb0]
                    blk = [[x_words(r0[hf], kh * 512 + k * 128) for kh in range(2)] for hf in range(2)]
                    cmb = []
                    for e in range(2):
                        nb = [[(blk[hf][kh][e] - mb[hf][e]) * rs[hf][e] for kh in range(2)] for hf in range(2)]
                        cmb.append(_rhs_combos(nb[0][0], nb[1][0], nb[0][1], nb[1][1]))
                        for hf in range(2 if live is not None else 0):
                            part = (nb[hf][0] * wr_v[:, pl.ds(k * 128, 128)]
                                    + nb[hf][1] * wr_v[:, pl.ds(512 + k * 128, 128)])
                            score[hf][e] = part if k == 0 else score[hf][e] + part
                    for i in range(7 if xb is not None else 0):
                        xb[i, pl.ds(step * 8, 8), pl.ds(k * 128, 128)] = _pack(cmb[0][i], cmb[1][i])
                    if k == 3 and live is not None:
                        for hf in range(2):
                            for e in range(2):
                                r = jnp.sum(score[hf][e], axis=-1, keepdims=True).astype(bf16).astype(f32)
                                r = jnp.broadcast_to(r, (8, 128))
                                up = jnp.logical_and(r > best_v[hf, e], live)
                                tok = 2 * lax.broadcasted_iota(i32, (8, 128), 0) + (r0[hf] + e)
                                best_v[hf, e] = jnp.where(up, r, best_v[hf, e])
                                best_i[hf, e] = jnp.where(up, tok, best_i[hf, e])
                    yield

        def ln_split(xb, xx):
            for r in range(8):
                for k in range(2):
                    yield from split_again(xb, xx, False, r, k)

        def project(w, x, res, keep=None, twice=False):
            def emit(r, b, val):
                if isinstance(res, list):
                    res[r][b] = val
                else:
                    res[r, b] = val
                if keep is not None:
                    keep[r, b] = val[64:]

            def prod2(ij):
                m = _dot_nt(second(w[0], w[1], True, ij), second(x[0], x[1], False, ij))
                last_product[:] = [m, 49]
                return m

            def once():
                for c in range(2):
                    def prod(i):
                        m = _dot_nt(as_bf16(w[0][i]), as_bf16(x[0][i, pl.ds(c * 64, 64), :]))
                        last_product[:] = [m, 14]
                        return m

                    def put(a, b, val):
                        emit(2 * a, 2 * b + c, val[:128])
                        emit(2 * a + 1, 2 * b + c, val[128:])

                    yield from _strassen(prod, put, ORDER)

            return (_strassen2(prod2, emit, ORDER), 49, 0.0, 1.0) if twice else (once(), 14, 0.0, 1.0)

        def raw_blk(res, r, r0, lane):
            if isinstance(res, list):
                return res[r][lane][r0:r0 + 64]
            return res[r, lane, pl.ds(r0, 64), :]

        keep_kv = lax.broadcasted_iota(i32, (64, 128), 0) // DH == lax.broadcasted_iota(i32, (64, 128), 1) % 2
        keep_z = lax.broadcasted_iota(i32, (16, 128), 0) // 8 == lax.broadcasted_iota(i32, (16, 128), 1) % 2

        def kv_post(c, res, keep=None):
            def accumulate(p, vt, phi):
                kv = kv_acc[p] + _dot_nt(vt, phi)
                kv_acc[p] = kv
                kvb_v[p, pl.ds(0, 64), :] = jnp.where(keep_kv, kv, 0.0).astype(bf16)

            pending = None
            for a in range(2):
                for pr in range(2):
                    p = 4 * c + 2 * a + pr
                    phis, zs = [], z_acc[p]
                    for lane in range(4):
                        phi = _dual_softmax(raw_blk(res, 2 * a + pr, 0, lane), pin())
                        zs = zs + phi
                        phis.append(phi.astype(bf16))
                        if keep is not None:
                            keep[2 * a + pr, :, pl.ds(lane * 128, 128)] = pltpu.bitcast(phis[-1], u32)
                        if lane == 1 and pending:
                            accumulate(*pending)
                        if lane == 3:
                            z_acc[p] = zs
                            zrow = jnp.broadcast_to(jnp.sum(zs.T, axis=0, keepdims=True), (16, 128))
                            kvb_v[p, pl.ds(64, 16), :] = jnp.where(keep_z, zrow, 0.0).astype(bf16)
                            vt = jnp.concatenate([raw_blk(res, 2 * a + pr, 64, l) for l in range(4)], axis=1)
                            pending = (p, vt.astype(bf16), jnp.concatenate(phis, axis=1))
                        yield
            yield
            accumulate(*pending)
            yield

        def route():
            best, tok = best_v[...].reshape(32, 128), best_i[...].reshape(32, 128)
            rmax = jnp.max(best, axis=0, keepdims=True)
            idx = jnp.min(jnp.where(best == rmax, tok, S).astype(f32)).astype(i32)
            return jnp.clip(idx, 0, S - 1), rmax

        def routed_token(idx):
            base = pl.multiple_of((idx // 16) * 16, 16)
            rows = pl.ds(pl.multiple_of(base % T, 16), 16)
            xn = (in_v[pl.ds(base, 16), :].astype(f32) - st_v[idx // T, 0, rows, 0:1]) * st_v[idx // T, 1, rows, 0:1]
            xsel = jnp.where(lax.broadcasted_iota(i32, (16, D), 0) == idx - base, xn, 0.0)
            xsel = jnp.sum(xsel, axis=0, keepdims=True).astype(bf16).astype(f32)
            for j in range(8):
                row = xsel[:, j * 128:(j + 1) * 128] + pin()
                xcol_v[pl.ds(j * 128, 128), :] = jnp.concatenate([row] * 16, axis=0).T
                yield

        mark('s0_init')
        zero_s[0] = 0
        kv_acc[...] = jnp.zeros(kv_acc.shape, f32)
        z_acc[...] = jnp.zeros(z_acc.shape, f32)
        y_acc[...] = jnp.zeros(y_acc.shape, f32)
        best_v[...] = jnp.full(best_v.shape, -jnp.inf, f32)
        for hf in range(2):
            for e in range(2):
                best_i[hf, e] = 2 * lax.broadcasted_iota(i32, (8, 128), 0) + (hf * TH + e)
        w8 = wr8_v[...].astype(f32)
        wr_v[...] = jnp.broadcast_to(jnp.concatenate([w8[j:j + 1, :] for j in range(8)], axis=1), (8, D))
        feature_maps()
        mark('s1_ln0')
        stats, apply = ln_stats(0, st_v.at[0]), ln_apply(0, st_v.at[0], xb_v.at[0], None)
        cp_x0(0).wait()
        cp_x0(1).wait()
        _schedule(clock, (stats, 16, 0.0, 1.0))
        _schedule(clock, (apply, 32, 0.0, 1.0))
        cp_x0(2).wait()
        cp_x0(3).wait()
        _schedule(clock, (stats, 16, 0.0, 1.0))
        _schedule(clock, (apply, 32, 0.0, 1.0))

        def prep_kv(c):
            cp_k(c).wait()
            if c:
                cp_v(c).wait()
            once, twice = operand(c)
            yield from prep_fold(WK, 2 * c, 2 * c + 1, once, lambda j: (j // 4) * 64 + (j % 4) * 8, range(4))
            if not c:
                cp_v(c).wait()
            yield from prep_transpose(WV, 2 * c, 2 * c + 1, once, lambda j: (j // 4) * 64 + 32 + (j % 4) * 8)
            if c in TW:
                for r in range(8):
                    for k in range(2):
                        for _ in split_again(b_v.at[c - 2 + zero_s[0]], twice, True, r, k):
                            pass
                    if r % 2:
                        yield

        def tokens(t):
            return xb_v.at[t], xx_v.at[t]

        mark('s3_prep0')
        _schedule(clock, (prep_kv(0), 8, 0.0, 1.0))
        mark('s4_proj0')
        _schedule(clock, project(operand(0), tokens(0), raw_v.at[0]),
                  (prep_kv(1), 8, W1, 1.0),
                  (ln_apply(0, st_v.at[0], None, True), 64, 0.08, W1))
        _schedule(clock, project(operand(1), tokens(0), raw_v.at[1]),
                  (kv_post(0, raw_v.at[zero_s[0]]), 18, 0.0, 1.0), (prep_kv(2), 12 if 2 in TW else 8, W2, W3), (prep_kv(3), 12 if 3 in TW else 8, W3, 1.0))

        def kv_tile(t, idx):
            last = t == NTILE - 1
            for cp in cp_fold(t) + [cp_xt(t + 1)]:
                cp.wait()

            @pl.when(jnp.logical_and(t > 0, t < 3))
            def _():
                for cp in cp_wo(2 * t - 2) + cp_wo(2 * t - 1):
                    cp.wait()

            if not NOBC:
                for g in range(NTILE):
                    @pl.when(t == g)
                    def _():
                        for cp in cp_ffn(g):
                            cp.start()

            last_product[:] = []
            idx = route()[0]
            xb, xx, st = xb_v.at[pl.ds(t, 2)], xx_v.at[pl.ds(t, 2)], st_v.at[t + 1]
            stats, apply = ln_stats(t + 1, st), ln_apply(t + 1, st, xb.at[1], jnp.logical_not(last))
            split = ln_split(xb_v.at[t + (1 if TW else 0) + zero_s[0]], xx.at[1 if TW else 0])
            fold = prep_q(t)
            trans = [prep_wo(2 * ((t + 1) % 2) + u, jnp.where(t == 0, WV, WO)) for u in range(2)]

            def fetch_ffn():
                for cp in cp_ffn(t):
                    cp.start()
                    yield

            c2, c3, c0 = ([[None] * 4 for _ in range(4)] for _ in range(3))
            _schedule(clock, project(operand(2), (xb.at[0], xx.at[0]), c2, twice=2 in TW),
                      (kv_post(1, raw_v.at[1]), 18, 0.0, 1.0),
                      (stats, 32, 0.0, 1.0), (fold, SF[0], 0.1, 0.9), (split, 7 * SAB[0], 0.02, 1.0),
                      (fetch_ffn(), 2 * FG + 8 if NOBC else 0, 0.05, 0.95))
            _schedule(clock, project(operand(3), (xb.at[0], xx.at[0]), c3, twice=3 in TW),
                      (kv_post(2, c2), 18, 0.0, 1.0), (apply, 64, 0.03, AEND), (fold, SF[1], 0.1, 0.8),
                      (split, 7 * SAB[1], 0.02, 1.0))
            x = tokens(jnp.where(last, (idx // T + 1) % NTILE, t + 1))
            chunk = jnp.where(last, 2, 0)
            again = split_q(t)
            _schedule(clock, project(operand(chunk), x, c0, keep=half_v),
                      (kv_post(3, c3), 18, 0.0, 1.0), (trans[0], 32 if TF else 4, 0.1, 0.9), (routed_token(idx), 8, 0.0, 1.0),
                      (split, 7 * SS[0], 0.02, 1.0), (again, 7 * SQ[0], 0.05, 1.0))
            _schedule(clock, project(operand(chunk + 1), x, raw_v.at[1]),
                      (kv_post(jnp.where(last, 4, 0), c0, phi_v), 18, 0.0, 1.0), (trans[1], 32 if TF else 4, 0.1, 0.9),
                      (split, 7 * SS[1], 0.02, 0.9), (again, 7 * SQ[1], 0.05, 0.9))
            return idx

        mark('s6_phase1')
        idx = lax.fori_loop(0, NTILE, kv_tile, jnp.int32(0))
        mark('s7_mid')
        for cp in cp_ffn(0):
            cp.wait()
        last_product[:] = []

        rmax = route()[1]
        first = (idx // T + 1) % NTILE

        def ffn(f0, nf):
            for j in range(nf):
                cols = pl.ds(pl.multiple_of((f0 + j) * 128, 128), 128)
                accs = [jnp.zeros((8, 128), f32)] * 2
                for r in range(8):
                    rows = pl.ds(r * 128, 128)
                    xc = xcol_v[rows, :]
                    if FPIN:
                        zero = pin()
                    for a, w_v in enumerate((wg_v, wu_v)):
                        prod = w_v[f0 + j, rows, :].astype(f32) * xc
                        acc = accs[a] + zero if FPIN else accs[a]
                        for q in range(16):
                            acc = acc + prod[8 * q:8 * q + 8]
                        accs[a] = acc
                    yield
                gate, up = [jnp.sum(acc, axis=0, keepdims=True) for acc in accs]
                hcol = jnp.broadcast_to(gate * jax.nn.sigmoid(gate) * up, (128, 128)).T
                for n in range(8):
                    ycols = pl.ds(n * 128, 128)
                    prod = wd_v[n, cols, :].astype(f32) * hcol
                    acc = y_acc[:, ycols] + pin() if FPIN else y_acc[:, ycols]
                    for q in range(16):
                        acc = acc + prod[8 * q:8 * q + 8]
                    y_acc[:, ycols] = acc
                    if n % 2 == 1:
                        yield

        def tile(j):
            return (first + j) % NTILE

        def q_post(c, res, ob, ready=None):
            phis, nds, outs = {}, {}, {}
            for tick in range(40):
                step, lane = tick // 4, tick % 4
                if step < 8:
                    u, a, pr = step // 4, (step // 2) % 2, step % 2
                    if ready is not None and pr == 0:
                        phi = as_bf16(ready[2 * a + u, :, pl.ds(lane * 128, 128)])
                    else:
                        phi = _dual_softmax(raw_blk(res, 2 * a + u, 0 if ready is not None else pr * 64, lane),
                                            pin()).astype(bf16)
                    phis.setdefault(step, []).append(phi)
                if 1 <= step < 9 and lane == 1:
                    w = step - 1
                    pair = 2 * (2 * c + w // 4 + 4 * ((w // 2) % 2)) + w % 2
                    nds[step - 1] = _dot(kvb_v[pair], jnp.concatenate(phis.pop(step - 1), axis=1))
                if step >= 2 and lane == 0:
                    nd = nds.pop(step - 2)
                    rd = _recip(nd[64:80, :] + 1e-6)
                    outs[step - 2] = jnp.concatenate(
                        [(nd[0:32, :].reshape(4, 8, T) * rd[0:8, :][None]).reshape(32, T),
                         (nd[32:64, :].reshape(4, 8, T) * rd[8:16, :][None]).reshape(32, T)], axis=0)
                    if (step - 2) % 4 == 3:
                        u = (step - 2) // 4
                        o1 = jnp.concatenate([outs.pop(4 * u), outs.pop(4 * u + 1)], axis=0)
                        o2 = jnp.concatenate([outs.pop(4 * u + 2), outs.pop(4 * u + 3)], axis=0)
                        cmb = _rhs_combos(o1[:, :TH], o1[:, TH:], o2[:, :TH], o2[:, TH:])
                        if OTR == 0:
                            for i in range(7):
                                ob[i, :, pl.ds(u * 128, 128)] = pltpu.bitcast(cmb[i].astype(bf16).T, u32)
                        else:
                            for b in range(2):
                                tr = pltpu.bitcast(jnp.concatenate(
                                    [v[:, b * 128:(b + 1) * 128] for v in cmb], axis=0).astype(bf16).T, u32)
                                for i in range(7):
                                    ob[i, pl.ds(b * 64, 64), pl.ds(u * 128, 128)] = tr[:, i * 128:(i + 1) * 128]
                yield

        def out_project(h, oba, obb, res, ks=(0, 1)):
            def prod(i):
                lhs = jnp.concatenate([(oba, obb)[k][i] for k in ks], axis=1)
                m = _dot_nt(as_bf16(lhs), as_bf16(wo_v[h, i, :, pl.ds(ks[0] * 256, len(ks) * 256)]))
                last_product[:] = [m, rate[0]]
                return m

            def emit(a, b, val):
                if isinstance(res, list):
                    res[a][b] = val
                else:
                    res[a, b] = val

            return _strassen(prod, emit, ORDER)

        def epilogue(t, h, res, part=None, upd=None, done=None):
            n = EROWS
            for a in range(2):
                for b in range(2):
                    cols = pl.ds(h * 512 + a * 256, 256)
                    for q in range(TH // n):
                        r0 = pl.multiple_of(t * T + b * TH + q * n, n)
                        rows = pl.ds(b * TH + q * n, n)
                        mb, rs = st_v[t, 0, rows, :], st_v[t, 1, rows, :] * 0.5
                        if upd is None:
                            mb = mb + pin(n)
                        x = in_v[pl.ds(r0, n), cols].astype(f32)
                        v = (x - jnp.concatenate([mb, mb], axis=1)) * jnp.concatenate([rs, rs], axis=1)
                        if upd is not None:
                            rid = lax.broadcasted_iota(i32, (n, 256), 0)
                            v = v + jnp.where(rid == idx - r0, upd[:, h * 512 + a * 256:h * 512 + (a + 1) * 256], 0.0)
                        g = v + v * jnp.tanh(v)
                        s = res[a][b][q * n:(q + 1) * n]
                        if part is not None:
                            s = s + part[a, b, pl.ds(q * n, n), :]
                        out_v[pl.ds(r0, n), cols] = (x + s * g).astype(bf16)
                        if done is not None and q == TH // n - 1:
                            done(4 * h + 2 * a + b)
                        yield

        NE = 4 * TH // EROWS
        mark('s8_q0')
        fb = NF - (NTILE - 1) * FL
        res0 = None
        _schedule(clock, (q_post(0, half_v, oba_v.at[0], phi_v), 40, 0.0, 1.0))

        def q_tile(j, carry):
            last_product[:] = []
            oba = oba_v.at[pl.ds(j, 2)]
            obb = obb_v.at[zero_s[0]]
            x = tokens(tile(j + 1))
            for cp in cp_ffn(j + 1):
                cp.wait()
            fg = ffn(j * FL, FL)
            q0, o0, o1 = ([[None] * 4 for _ in range(4)] for _ in range(3))
            _schedule(clock, project((a_v.at[2], aa_v.at[0]), x, q0, twice=True), (q_post(1, raw_v.at[1], obb_v.at[0]), 40, 0.0, PEND),
                      (fg, FSL[0], 0.1, 1.0))
            _schedule(clock, (out_project(0, oba.at[0], obb, o0), 7, 0.0, 1.0), (q_post(0, q0, oba.at[1]), 40, 0.05, 1.0),
                      (fg, FSL[1], 0.1, 1.0))
            _schedule(clock, (out_project(1, oba.at[0], obb, o1), 7, 0.0, 1.0), (epilogue(tile(j), 0, o0), NE, 0.0, 1.0),
                      (fg, FSL[2], 0.1, 1.0))
            _schedule(clock, project((a_v.at[3], aa_v.at[1]), x, raw_v.at[1], twice=True), (epilogue(tile(j), 1, o1), NE, 0.0, 1.0),
                      (fg, FSL[3], 0.1, 0.9))
            cp_o(j, tile(j)).start()
            return carry

        mark('s9_phase2')
        lax.fori_loop(0, NTILE - 1, q_tile, 0)
        mark('sa_tail')

        j = NTILE - 1
        rate[0] = 14
        last_product[:] = []
        oba, obb = oba_v.at[j], obb_v.at[zero_s[0]]
        _schedule(clock, (out_project(0, oba, obb, part_v.at[0], (0,)), 7, 0.0, 0.5),
                  (out_project(1, oba, obb, part_v.at[1], (0,)), 7, 0.5, 1.0),
                  (q_post(1, raw_v.at[1], obb_v.at[0]), 40, 0.0, PEND),
                  (ffn(NF - fb, fb), 12 * fb, 0.1, 0.8))
        upd = jnp.sum(y_acc[...], axis=0, keepdims=True) * (0.5 * jax.nn.sigmoid(rmax[:, 0:1]))
        o0, o1 = ([[None, None], [None, None]] for _ in range(2))
        t = tile(j)
        send = lambda blk: cp_o_blk(t, blk).start()
        e0 = epilogue(t, 0, o0, part_v.at[0], upd, send)
        e1 = epilogue(t, 1, o1, part_v.at[1], upd, send)
        _schedule(clock, (out_project(0, oba, obb, o0, (1,)), 7, 0.0, 0.5),
                  (out_project(1, oba, obb, o1, (1,)), 7, 0.5, 1.0),
                  (e0, NE, 0.29, 0.57), (e1, NE, 0.79, 1.07))
        mark('sb_outdma')
        for k in range(NTILE - 1):
            cp_o(k, tile(k)).wait()
        for blk in range(8):
            cp_o_blk(t, blk).wait()
        mark(None)

    scratch = [
        pltpu.VMEM((S + T + 4 * D, D), bf16),
        pltpu.VMEM((NTILE + 1, 2, T, 128), f32),
        pltpu.VMEM((NTILE + 1, 7, 128, 512), u32),
        pltpu.VMEM((NTILE + 1, 35, 64, 256), u32),
        pltpu.VMEM((D, DH), bf16),
        pltpu.VMEM((8, 128), bf16),
        pltpu.VMEM((8, D), f32),
        pltpu.VMEM((8, 128, 128), bf16),
        pltpu.VMEM((4, 7, 128, 512), u32),
        pltpu.VMEM((2, 35, 64, 256), u32),
        pltpu.VMEM((2, 7, 128, 512), u32),
        pltpu.VMEM((2, 35, 64, 256), u32),
        pltpu.VMEM((2, 7, 128, 512), u32),
        pltpu.VMEM((NF, D, 128), bf16),
        pltpu.VMEM((NF, D, 128), bf16),
        pltpu.VMEM((D // 128, F, 128), bf16),
        pltpu.VMEM((H // 2 + 4, 64, 128), f32),
        pltpu.VMEM((H // 2 + 4, 128, 128), f32),
        pltpu.VMEM((H // 2 + 4, 80, 128), bf16),
        pltpu.VMEM((2, 2, 8, 128), f32),
        pltpu.VMEM((2, 2, 8, 128), i32),
        pltpu.VMEM((2, 4, 4, 128, 128), f32),
        pltpu.VMEM((4, 4, 64, 128), f32),
        pltpu.VMEM((4, 64, T), u32),
        pltpu.VMEM((NTILE, 7, TH // 2, 256), u32),
        pltpu.VMEM((2, 7, TH // 2, 256), u32),
        pltpu.VMEM((2, 2, 2, 256, 256), f32),
        pltpu.VMEM((D, 128), f32),
        pltpu.VMEM((8, D), f32),
        pltpu.VMEM((S, D), bf16),
        pltpu.SMEM((1,), i32),
        pltpu.SemaphoreType.DMA((NTILE + 2,)),
        pltpu.SemaphoreType.DMA((11,)),
        pltpu.SemaphoreType.DMA((1,)),
        pltpu.SemaphoreType.DMA((NTILE,)),
        pltpu.SemaphoreType.DMA((1,)),
    ]

    def call(x, wqkv, wphi, wo, wr, wg, wu, wd):
        hbm = pl.BlockSpec(memory_space=pltpu.HBM)
        return pl.pallas_call(
            kernel,
            out_shape=jax.ShapeDtypeStruct((S, D), bf16),
            in_specs=[hbm] * 8,
            out_specs=hbm,
            scratch_shapes=scratch,
            compiler_params=pltpu.CompilerParams(vmem_limit_bytes=120 * 2**20, flags=FLAGS, disable_bounds_checks=NOBC),
            name="hedgehog",
        )(x, wqkv, wphi, wo, wr, wg, wu, wd)

    return call


@jax.jit
def pallas_recurrent_scan__linear_kernel_hedgehog__moe_arch_mod__prompt_kernel(
    A_x: jax.Array,
    A_wqkv: jax.Array,
    A_w_phi: jax.Array,
    A_wo: jax.Array,
    B_x: jax.Array,
    B_w_r: jax.Array,
    B_w_gate: jax.Array,
    B_w_up: jax.Array,
    B_w_down: jax.Array,
):
    del B_x
    out = make_kernel()(
        A_x.reshape(S, D), A_wqkv, A_w_phi.reshape(D, DH), A_wo,
        B_w_r.reshape(8, 128), B_w_gate, B_w_up, B_w_down)
    return out.reshape(1, S, D)
```

```python
import math
import contextlib

import numpy as np

import jax
import jax.numpy as jnp
from jax import lax
import jax.experimental.pallas as pl
import jax.experimental.pallas.tpu as pltpu

S, D, H, DH, F = 2048, 1024, 32, 32, 3584
T = 512
TH = T // 2
NTILE = S // T
NF = F // 128
FG = NF // NTILE
WQ, WK, WV, WO = (S + T + j * D for j in range(4))
LHS_SUMS, RHS_SUMS = (0, 1, 4, 5, 6), (0, 2, 3, 5, 6)
LOG2E = math.log2(math.e)
EPS_BF16 = float(np.float32(1e-5).astype(jnp.bfloat16))
NT_DIMS = (((1,), (1,)), ((), ()))
f32, bf16, i32, u32 = jnp.float32, jnp.bfloat16, jnp.int32, jnp.uint32


def _dot_nt(a, b):
    return lax.dot_general(a, b, NT_DIMS, preferred_element_type=f32)


def _dot(a, b):
    return jnp.dot(a, b, preferred_element_type=f32)


def aligned(i, n):
    return i if isinstance(i, int) else pl.multiple_of(i, n)


def _recip(v):
    r = pl.reciprocal(v, approx=True)
    return r * (2.0 - v * r)


def _wide(w):
    return pltpu.bitcast(w, bf16).astype(f32)


def _narrow(v):
    return pltpu.bitcast(v.astype(bf16), u32)


def _lhs_combos(a11, a12, a21, a22):
    return [a11 + a22, a21 + a22, a11, a22, a11 + a12, a21 - a11, a12 - a22]


def _rhs_combos(b11, b12, b21, b22):
    return [b11 + b22, b11, b12 - b22, b21 - b11, b22, b11 + b12, b21 + b22]


class _Quad:
    def __init__(self, v):
        self.v = v

    def __add__(self, o):
        return _Quad([p + q for p, q in zip(self.v, o.v)])

    def __sub__(self, o):
        return _Quad([p - q for p, q in zip(self.v, o.v)])


def _strassen2(prod, emit, order):
    done = {}

    def inner(i):
        out = [None] * 4

        def put(a, b, val):
            out[2 * a + b] = val
        yield from _strassen(lambda j: prod(7 * i + j), put, order)
        done[i] = _Quad(out)

    def put(a, b, quad):
        for k, val in enumerate(quad.v):
            emit(2 * a + k // 2, 2 * b + k % 2, val)

    outer = _strassen(lambda i: done[i], put, order)
    for i in ((0, 3, 4, 6, 2, 1, 5), (2, 4, 0, 6, 3, 1, 5))[order]:
        steps = inner(i)
        for _ in range(6):
            next(steps)
            yield
        for _ in steps:
            pass
        next(outer)
        yield


def _strassen(prod, emit, order=0):
    if order == 0:
        m1 = prod(0)
        yield
        m4 = prod(3)
        c11 = m1 + m4
        yield
        m5 = prod(4)
        c11 = c11 - m5
        yield
        emit(0, 0, c11 + prod(6))
        yield
        m3 = prod(2)
        emit(0, 1, m3 + m5)
        c22 = m1 + m3
        yield
        m2 = prod(1)
        emit(1, 0, m2 + m4)
        c22 = c22 - m2
        yield
        emit(1, 1, c22 + prod(5))
        yield
    else:
        m3 = prod(2)
        yield
        m5 = prod(4)
        emit(0, 1, m3 + m5)
        yield
        m1 = prod(0)
        c11, c22 = m1 - m5, m1 + m3
        yield
        c11 = c11 + prod(6)
        yield
        m4 = prod(3)
        emit(0, 0, c11 + m4)
        yield
        m2 = prod(1)
        emit(1, 0, m2 + m4)
        c22 = c22 - m2
        yield
        emit(1, 1, c22 + prod(5))
        yield


SKIP = [False]


def _schedule(clock, *streams):
    if SKIP[0]:
        return
    events = []
    for order, (gen, n, a, b) in enumerate(streams):
        for k in range(n):
            events.append((a + (b - a) * k / n, order, k, gen))
    for when, _, _, gen in sorted(events, key=lambda e: e[:3]):
        clock[:] = [when]
        next(gen)


def _dual_softmax(p, zero=None):
    rows = [p[8 * j:8 * j + 8] for j in range(8)]
    if zero is not None:
        rows[0] = rows[0] + zero

    def reduce(vs, op):
        while len(vs) > 1:
            vs = [op(vs[i], vs[i + 1]) for i in range(0, len(vs), 2)]
        v = op(vs[0], pltpu.roll(vs[0], 4, 0))
        return op(v, pltpu.roll(v, 2, 0))

    mx, mn = reduce(rows, jnp.maximum), reduce(rows, jnp.minimum)
    ep = [jnp.exp2(v - mx) for v in rows]
    en = [jnp.exp2(mn - v) for v in rows]
    rp, rn = _recip(reduce(ep, jnp.add)), _recip(reduce(en, jnp.add))
    return jnp.concatenate([v * rp for v in ep] + [v * rn for v in en], axis=0)


PLAN = dict(
    kv=(0.0, 1.0), stats=(0.0, 0.96), apply=(0.015, 0.935), fold=(0.1, 0.9), fold2=(0.06, 0.84), nfold=3,
    trans=(0.1, 0.9), routed=(0.015, 0.92), split=(0.02, 1.0), split2=(0.035, 0.94), nsplit=56,
    again=(0.065, 1.0), again2=(0.01, 0.94), nagain=14, o1=1,
    p1=(0.0, 1.0), p0=(0.065, 1.0), e0=(0.0, 0.985), e1=(0.0, 0.985), nffn=(14, 18, 38),
    f0=(0.14, 0.96), f1=(0.085, 0.985), f2=(0.02, 1.0), f3=(0.0, 0.925), oq=1, oo=0, on=256,
)


def make_kernel(FLAGS=None, FL=9, W0=0.15, W1=0.7, W2=0.15, W3=0.6, TORD=1, NOSEM=False, E0=(0.2, 0.7), E1=(0.7, 1.2),
                TPIN=False, TQ=0.9, NOBC=True, EROWS=32, SCOPES=False, ONLY=None, INTERP=False,
                DMA_ORDER='a0 a1 a2 a3 k0 v0 k1 v1 k2 v2 k3 v3 x1 f0 x2 f1 o0 o1 x3 f2 o2 o3 x4 f3'.split(), **over):
    P = dict(PLAN, **over)
    FPIN = True

    stack = []
    def mark(name):
        if not SCOPES: return
        if stack: stack.pop().__exit__(None, None, None)
        if name:
            cm = jax.named_scope(name); cm.__enter__(); stack.append(cm)

    def kernel(x_hbm, wqkv_hbm, wphi_hbm, wo_hbm, wr_hbm, wg_hbm, wu_hbm, wd_hbm,
               out_hbm,
               in_v, st_v, xb_v, xx_v, wphi_v, wr8_v, wr_v, lm_v, a_v, aa_v, b_v, wo_v, wg_v, wu_v, wd_v,
               kv_acc, z_acc, kvb_v, best_v, best_i, raw_v, half_v, phi_v, oba_v, obb_v, part_v, xcol_v, y_acc,
               out_v, zero_s, sem_x, sem_w, sem_s, sem_f, sem_o):
        def cp_x(r0, n, sem, src0=None):
            src0 = r0 if src0 is None else src0
            return pltpu.make_async_copy(x_hbm.at[pl.ds(src0, n)], in_v.at[pl.ds(r0, n)], sem_x.at[sem])

        def cp_x0(piece):
            return cp_x((piece % 2) * TH + (piece // 2) * (TH // 2), TH // 2, 0 if piece < 2 else NTILE + 1)

        def cp_xt(t):
            return cp_x(pl.multiple_of(t * T, T), T, t, pl.multiple_of((t % NTILE) * T, T))

        def cp_w(j, c0, n, sem):
            src = wo_hbm.at[:, pl.ds(c0, n)] if j == 3 else wqkv_hbm.at[:, pl.ds(aligned(j * D + c0, 128), n)]
            return pltpu.make_async_copy(src, in_v.at[pl.ds(WQ + j * D, D), pl.ds(c0, n)], sem_w.at[sem])

        def cp_k(c):
            return cp_w(1, c * 256, 256, c)

        def cp_v(c):
            return cp_w(2, c * 256, 256, c if c else 4)

        def cp_fold(u):
            cps = []
            for n in range(8):
                r0 = aligned((n // 2) * 256 + (u % 2) * 128, 128)
                cols = pl.ds(aligned((u // 2) * 256 + (n % 2) * 512, 256), 256)
                cps.append(pltpu.make_async_copy(wqkv_hbm.at[pl.ds(r0, 128), cols],
                                                 in_v.at[pl.ds(aligned(WQ + r0, 128), 128), cols], sem_w.at[5 + u]))
            return cps

        def cp_wo(u):
            g = (u // 2) * 4 + u % 2
            return [cp_w(3, aligned(c * 128, 128), 128, 9 + u // 2) for c in (g, g + 2)]

        cp_phi = pltpu.make_async_copy(wphi_hbm, wphi_v, sem_s.at[0])
        cp_wr = pltpu.make_async_copy(wr_hbm, wr8_v, sem_s.at[0])
        def cp_ffn(g):
            cps = []
            for j in range(FG):
                cols = pl.ds(aligned((g * FG + j) * 128, 128), 128)
                for src, dst in ((wg_hbm, wg_v), (wu_hbm, wu_v)):
                    cps.append(pltpu.make_async_copy(src.at[:, cols], dst.at[g * FG + j], sem_f.at[g]))
            rows = pl.ds(aligned(g * FG * 128, 128), FG * 128)
            for n in range(D // 128):
                cps.append(pltpu.make_async_copy(wd_hbm.at[rows, pl.ds(n * 128, 128)], wd_v.at[n, rows], sem_f.at[g]))
            return cps

        def cp_o(k, t):
            rows = pl.ds(pl.multiple_of(t * T, T), T)
            return pltpu.make_async_copy(out_v.at[rows], out_hbm.at[rows], sem_o.at[0])

        def cp_o_blk(t, blk):
            rows = pl.ds(pl.multiple_of(t * T + (blk % 2) * TH, TH), TH)
            cols = pl.ds((blk // 2) * 256, 256)
            return pltpu.make_async_copy(out_v.at[rows, cols], out_hbm.at[rows, cols], sem_o.at[0])

        cp_wr.start()
        cp_phi.start()
        for n, name in enumerate(DMA_ORDER):
            if n == 1:
                cp_wr.wait()
                cp_phi.wait()
            cps = {"a": cp_x0, "k": cp_k, "v": cp_v, "x": cp_xt, "f": cp_fold, "o": cp_wo}[name[0]](int(name[1]))
            for cp in cps if isinstance(cps, list) else [cps]:
                cp.start()

        last_product = []

        clock = [0.0]
        rate = [7]

        def pin(n=8):
            if not last_product:
                return jnp.zeros((n, 128), f32)
            rows, cols = last_product[0].shape[0] // 8, last_product[0].shape[1] // 128
            q = min(int((clock[0] * last_product[1]) % 1.0 * rows * cols + 1e-6), rows * cols - 1)
            m = last_product[0][(q % rows) * 8:(q % rows) * 8 + 8, (q // rows) * 128:(q // rows) * 128 + 128]
            z = pltpu.bitcast(pltpu.bitcast(m, u32) & zero_s[0].astype(u32), f32)
            return z if n == 8 else jnp.concatenate([z] * (n // 8), axis=0)

        def as_bf16(w):
            return pltpu.bitcast(w, bf16)

        def feature_maps():
            rho = lax.broadcasted_iota(i32, (128, DH), 0)
            sel = (((rho % 64) // 8) * 4 + (rho % 8) // 2 == lax.broadcasted_iota(i32, (128, DH), 1)).astype(bf16)
            rho = lax.broadcasted_iota(i32, (128, 128), 0)
            keep = (rho // 64) * 2 + rho % 2 == lax.broadcasted_iota(i32, (128, 128), 1) // DH
            for g in range(8):
                full = _dot_nt(sel, wphi_v[pl.ds(g * 128, 128), :])
                lm_v.at[g][...] = jnp.where(keep, full, 0.0).astype(bf16)

        def operand(chunk):
            return a_v.at[chunk] if chunk < 2 else b_v.at[chunk - 2]

        def put_lhs(dst, rows, cols, *quadrants):
            for i, v in enumerate(_lhs_combos(*quadrants)):
                dst.at[i][rows, cols] = _narrow(v)

        def split_again(src, dst, lhs, r, k):
            for i in range(7):
                zero = pltpu.bitcast(pin(), u32)
                w = [[src[i, pl.ds(h * 64 + r * 8, 8), pl.ds(aligned(c * 256 + k * 128, 128), 128)]
                      for c in range(2)] for h in range(2)]
                q00, q01, q10, q11 = _wide(w[0][0] | zero), _wide(w[0][1]), _wide(w[1][0]), _wide(w[1][1] | zero)
                cmb = _lhs_combos(q00, q01, q10, q11) if lhs else _rhs_combos(q00, q10, q01, q11)
                for n, j in enumerate(LHS_SUMS if lhs else RHS_SUMS):
                    dst.at[5 * i + n][pl.ds(r * 8, 8), pl.ds(aligned(k * 128, 128), 128)] = _narrow(cmb[j])
                yield

        def second(src, dst, lhs, ij):
            i, j = ij // 7, ij % 7
            sums = LHS_SUMS if lhs else RHS_SUMS
            if j in sums:
                return as_bf16(dst[5 * i + sums.index(j)])
            d = int(j == (3 if lhs else 4))
            return as_bf16(src[i, pl.ds(d * 64, 64), pl.ds(d * 256, 256)])

        def w_blocks(base, top, bot, k):
            return [in_v[pl.ds(aligned(base + kh * 512 + k * 128, 128), 128),
                         pl.ds(aligned(g * 128, 128), 128)] for g in (top, bot) for kh in range(2)]

        def prep_fold(base, top, bot, dst, row_of, ks):
            for k in ks:
                blocks = [_dot_nt(lm_v[g], w) for g, w in zip((top, top, bot, bot), w_blocks(base, top, bot, k))]
                for j in range(8):
                    put_lhs(dst, pl.ds(aligned(row_of(j), 8), 8), pl.ds(aligned(k * 128, 128), 128),
                            *[p[16 * j:16 * j + 16] * LOG2E for p in blocks])
                yield

        def prep_transpose(base, top, bot, dst, row_of):
            for k in range(4):
                zero = pltpu.bitcast(pin(64), u32)
                blocks = [as_bf16(pltpu.bitcast(w, u32) | zero).T for w in w_blocks(base, top, bot, k)]
                for j in range(8):
                    put_lhs(dst, pl.ds(aligned(row_of(j), 8), 8), pl.ds(k * 128, 128),
                            *[w[16 * j:16 * j + 16].astype(f32) for w in blocks])
                yield

        def prep_q(u):
            ch, k = u // 2, u % 2
            for half in range(2):
                g = 2 * ch + half
                yield from prep_fold(WQ, g, g + 4, a_v.at[2 + ch], lambda j: half * 64 + 8 * j, (k, k + 2))

        def split_q(u):
            for r in range(8):
                yield from split_again(a_v.at[2 + u // 2 + zero_s[0]], aa_v.at[u // 2], True, r, u % 2)

        def prep_wo(u, base=WO):
            g = (u // 2) * 4 + u % 2
            return prep_transpose(base, g, g + 2, wo_v.at[u // 2], lambda j: (u % 2) * 64 + 8 * j)

        def x_block(r0, c0):
            return in_v[pl.ds(r0, 16), pl.ds(c0, 128)].astype(f32)

        def ln_stats(t, st):
            for step in range(32):
                pos = (step % 2) * 16 + step // 2
                r0 = pl.multiple_of(t * T + pos * 16, 16)
                x0 = x_block(r0, 0) + pin(16)
                s1 = s2 = None
                for j in range(1, 8):
                    d = x_block(r0, j * 128) - x0
                    s1 = d if j == 1 else s1 + d
                    s2 = d * d if j == 1 else s2 + d * d
                lane_mean = x0 + s1 * 0.125
                m = jnp.sum(lane_mean, axis=-1, keepdims=True) * (1.0 / 128)
                dm = lane_mean - m
                v = jnp.sum((s2 - s1 * s1 * 0.125) * 0.125 + dm * dm, axis=-1, keepdims=True) * (1.0 / 128)
                vb = (v.astype(bf16).astype(f32) + EPS_BF16).astype(bf16).astype(f32)
                st[0, pl.ds(pos * 16, 16), :] = jnp.broadcast_to(m.astype(bf16).astype(f32), (16, 128))
                st[1, pl.ds(pos * 16, 16), :] = jnp.broadcast_to(1.0 / jnp.sqrt(vb).astype(bf16).astype(f32), (16, 128))
                yield

        def ln_apply(t, st, xb, live):
            for step in range(16):
                r0 = [pl.multiple_of(t * T + hf * TH + step * 16 + zero_s[0], 16) for hf in range(2)]
                mean = [st[0, pl.ds(hf * TH + step * 16, 16), :] for hf in range(2)]
                scale = [st[1, pl.ds(hf * TH + step * 16, 16), :] for hf in range(2)]
                score = [None, None]
                for k in range(4):
                    zero = pin(16)
                    xn = [[(x_block(r0[hf], kh * 512 + k * 128) - (mean[hf] + zero)) * scale[hf]
                           for kh in range(2)] for hf in range(2)]
                    if xb is not None:
                        for i, v in enumerate(_rhs_combos(xn[0][0], xn[1][0], xn[0][1], xn[1][1])):
                            xb.at[i][pl.ds(step * 8, 8), pl.ds(k * 128, 128)] = _narrow(v)
                    for hf in range(2 if live is not None else 0):
                        part = (xn[hf][0] * wr_v[:, pl.ds(k * 128, 128)]
                                + xn[hf][1] * wr_v[:, pl.ds(512 + k * 128, 128)])
                        score[hf] = part if k == 0 else score[hf] + part
                        if k == 3:
                            r = jnp.sum(score[hf], axis=-1, keepdims=True).astype(bf16).astype(f32)
                            r = jnp.broadcast_to(r, (16, 128))
                            up = jnp.logical_and(r > best_v[hf], live)
                            best_v[hf] = jnp.where(up, r, best_v[hf])
                            best_i[hf] = jnp.where(up, lax.broadcasted_iota(i32, (16, 128), 0) + r0[hf], best_i[hf])
                    yield

        def ln_split(xb, xx):
            for r in range(8):
                for k in range(2):
                    yield from split_again(xb, xx, False, r, k)

        def project(w, x, res, keep=None):
            def emit(r, b, val):
                if isinstance(res, list):
                    res[r][b] = val
                else:
                    res[r, b] = val
                if keep is not None:
                    keep[r, b] = val[64:]

            def prod2(ij):
                m = _dot_nt(second(*w, True, ij), second(*x, False, ij))
                last_product[:] = [m, 49]
                return m

            def once():
                for c in range(2):
                    def prod(i):
                        m = _dot_nt(as_bf16(w[i]), as_bf16(x[i, pl.ds(c * 64, 64), :]))
                        last_product[:] = [m, 14]
                        return m

                    def put(a, b, val):
                        emit(2 * a, 2 * b + c, val[:128])
                        emit(2 * a + 1, 2 * b + c, val[128:])

                    yield from _strassen(prod, put, P["o1"])

            if isinstance(w, tuple):
                return _strassen2(prod2, emit, P["oq"]), 49, 0.0, 1.0
            return once(), 14, 0.0, 1.0

        def project_part(w, x, res, part):
            def prod(i):
                lhs = jnp.concatenate([w[i, pl.ds(h * 64 + part * 32, 32), :] for h in range(2)], axis=0)
                m = _dot_nt(as_bf16(lhs), as_bf16(x[i]))
                last_product[:] = [m, 14]
                return m

            def put(a, b, val):
                for h in range(2):
                    for c in range(2):
                        res[2 * a + h, 2 * b + c, pl.ds(part * 64, 64), :] = val[h * 64:(h + 1) * 64, c * 128:(c + 1) * 128]

            return _strassen(prod, put, P["o1"])

        def raw_blk(res, r, r0, lane):
            if isinstance(res, list):
                return res[r][lane][r0:r0 + 64]
            return res[r, lane, pl.ds(r0, 64), :]

        keep_kv = lax.broadcasted_iota(i32, (64, 128), 0) // DH == lax.broadcasted_iota(i32, (64, 128), 1) % 2
        keep_z = lax.broadcasted_iota(i32, (16, 128), 0) // 8 == lax.broadcasted_iota(i32, (16, 128), 1) % 2

        def kv_post(c, res, keep=None):
            def accumulate(p, vt, phi):
                kv = kv_acc[p] + _dot_nt(vt, phi)
                kv_acc[p] = kv
                kvb_v.at[p][pl.ds(0, 64), :] = jnp.where(keep_kv, kv, 0.0).astype(bf16)

            pending = None
            for a in range(2):
                for pr in range(2):
                    p = 4 * c + 2 * a + pr
                    phis, zs = [], z_acc[p]
                    for lane in range(4):
                        phi = _dual_softmax(raw_blk(res, 2 * a + pr, 0, lane), pin())
                        zs = zs + phi
                        phis.append(phi)
                        if keep is not None:
                            keep.at[2 * a + pr][:, pl.ds(lane * 128, 128)] = _narrow(phi)
                        if lane == 1 and pending:
                            accumulate(*pending)
                        if lane == 3:
                            z_acc[p] = zs
                            zrow = jnp.broadcast_to(jnp.sum(zs.T, axis=0, keepdims=True), (16, 128))
                            kvb_v.at[p][pl.ds(64, 16), :] = jnp.where(keep_z, zrow, 0.0).astype(bf16)
                            vt = jnp.concatenate([raw_blk(res, 2 * a + pr, 64, l) for l in range(4)], axis=1)
                            pending = (p, vt.astype(bf16), jnp.concatenate(phis, axis=1).astype(bf16))
                        yield
            yield
            accumulate(*pending)
            yield

        def route():
            best, tok = best_v[...].reshape(32, 128), best_i[...].reshape(32, 128)
            rmax = jnp.max(best, axis=0, keepdims=True)
            idx = jnp.min(jnp.where(best == rmax, tok, S).astype(f32)).astype(i32)
            return jnp.clip(idx, 0, S - 1), rmax

        def routed_token(idx):
            base = pl.multiple_of((idx // 16) * 16, 16)
            rows = pl.ds(pl.multiple_of(base % T, 16), 16)
            xn = (in_v[pl.ds(base, 16), :].astype(f32) - st_v[idx // T, 0, rows, 0:1]) * st_v[idx // T, 1, rows, 0:1]
            xsel = jnp.where(lax.broadcasted_iota(i32, (16, D), 0) == idx - base, xn, 0.0)
            xsel = jnp.sum(xsel, axis=0, keepdims=True).astype(bf16).astype(f32)
            for j in range(8):
                row = xsel[:, j * 128:(j + 1) * 128] + pin()
                xcol_v[pl.ds(j * 128, 128), :] = jnp.concatenate([row] * 16, axis=0).T
                yield

        SKIP[0] = ONLY is not None
        mark('s0_init')
        zero_s[0] = 0
        kv_acc[...] = jnp.zeros(kv_acc.shape, f32)
        z_acc[...] = jnp.zeros(z_acc.shape, f32)
        y_acc[...] = jnp.zeros(y_acc.shape, f32)
        best_v[...] = jnp.full(best_v.shape, -jnp.inf, f32)
        for hf in range(2):
            best_i[hf] = lax.broadcasted_iota(i32, (16, 128), 0) + hf * TH
        w8 = wr8_v[...].astype(f32)
        wr_v[...] = jnp.broadcast_to(jnp.concatenate([w8[j:j + 1, :] for j in range(8)], axis=1), (16, D))
        feature_maps()
        mark('s1_ln0')
        stats, apply = ln_stats(0, st_v.at[0]), ln_apply(0, st_v.at[0], xb_v.at[0], None)
        cp_x0(0).wait()
        cp_x0(1).wait()
        _schedule(clock, (stats, 16, 0.0, 1.0))
        _schedule(clock, (apply, 32, 0.0, 1.0))
        cp_x0(2).wait()
        cp_x0(3).wait()
        _schedule(clock, (stats, 16, 0.0, 1.0))
        _schedule(clock, (apply, 32, 0.0, 1.0))

        def prep_kv(c):
            cp_k(c).wait()
            if c:
                cp_v(c).wait()
            once = operand(c)
            yield from prep_fold(WK, 2 * c, 2 * c + 1, once, lambda j: (j // 4) * 64 + (j % 4) * 8, range(4))
            if not c:
                cp_v(c).wait()
            yield from prep_transpose(WV, 2 * c, 2 * c + 1, once, lambda j: (j // 4) * 64 + 32 + (j % 4) * 8)

        def tokens(t):
            return xb_v.at[t], xx_v.at[t]

        mark('s3_prep0')
        first_chunk = prep_kv(0)
        _schedule(clock, (first_chunk, 4, 0.0, 1.0))
        mark('s4_proj0')
        _schedule(clock, (project_part(operand(0), xb_v.at[0], raw_v.at[0], 0), 7, 0.0, 0.5),
                  (project_part(operand(0), xb_v.at[0], raw_v.at[0], 1), 7, 0.5, 1.0),
                  (first_chunk, 4, W0, 0.45), (prep_kv(1), 8, W1, 1.0),
                  (ln_apply(0, st_v.at[0], None, True), 64, 0.03, W1))
        _schedule(clock, project(operand(1), xb_v.at[0], raw_v.at[1]),
                  (kv_post(0, raw_v.at[zero_s[0]]), 18, 0.0, 1.0), (prep_kv(2), 8, W2, W3), (prep_kv(3), 8, W3, 1.0))

        def kv_tile(t, idx):
            SKIP[0] = False
            last = t == NTILE - 1
            for cp in cp_fold(t) + [cp_xt(t + 1)]:
                cp.wait()

            @pl.when(jnp.logical_and(t > 0, t < 3))
            def _():
                for cp in cp_wo(2 * t - 2) + cp_wo(2 * t - 1):
                    cp.wait()

            if not NOBC:
                for g in range(NTILE):
                    @pl.when(t == g)
                    def _():
                        for cp in cp_ffn(g):
                            cp.start()

            last_product[:] = []
            idx = route()[0]
            xb, st = xb_v.at[pl.ds(t, 2)], st_v.at[t + 1]
            stats, apply = ln_stats(t + 1, st), ln_apply(t + 1, st, xb.at[1], jnp.logical_not(last))
            split = ln_split(xb.at[0], xx_v.at[t])
            fold = prep_q(t)
            trans = [prep_wo(2 * ((t + 1) % 2) + u, jnp.where(t == 0, WV, WO)) for u in range(2)]

            def fetch_ffn():
                for cp in cp_ffn(t):
                    cp.start()
                    yield

            c2, c3, c0 = ([[None] * 4 for _ in range(4)] for _ in range(3))
            _schedule(clock, project(operand(2), xb.at[0], c2), (kv_post(1, raw_v.at[1]), 18, *P["kv"]),
                      (stats, 32, *P["stats"]), (fold, P["nfold"], *P["fold"]),
                      (fetch_ffn(), 2 * FG + 8 if NOBC else 0, 0.05, 0.95))
            _schedule(clock, project(operand(3), xb.at[0], c3), (kv_post(2, c2), 18, *P["kv"]),
                      (apply, 64, *P["apply"]), (fold, 4 - P["nfold"], *P["fold2"]))
            x = xb_v.at[jnp.where(last, (idx // T + 1) % NTILE, t + 1)]
            chunk = jnp.where(last, 2, 0)
            again = split_q(t)
            _schedule(clock, project(a_v.at[chunk], x, c0, keep=half_v), (kv_post(3, c3), 18, *P["kv"]),
                      (trans[0], 4, *P["trans"]), (routed_token(idx), 8, *P["routed"]),
                      (split, P["nsplit"], *P["split"]), (again, P["nagain"], *P["again"]))
            _schedule(clock, project(a_v.at[chunk + 1], x, raw_v.at[1]),
                      (kv_post(jnp.where(last, 4, 0), c0, phi_v), 18, *P["kv"]), (trans[1], 4, *P["trans"]),
                      (split, 112 - P["nsplit"], *P["split2"]), (again, 56 - P["nagain"], *P["again2"]))
            return idx

        mark('s6_phase1')
        idx = lax.fori_loop(0, NTILE, kv_tile, jnp.int32(0)) if ONLY != 'p2' else route()[0]
        SKIP[0] = ONLY is not None
        mark('s7_mid')
        for cp in cp_ffn(0):
            cp.wait()
        last_product[:] = []

        rmax = route()[1]
        first = (idx // T + 1) % NTILE

        def ffn(f0, nf):
            for j in range(nf):
                cols = pl.ds(pl.multiple_of((f0 + j) * 128, 128), 128)
                accs = [jnp.zeros((8, 128), f32)] * 2
                for r in range(8):
                    rows = pl.ds(r * 128, 128)
                    xc = xcol_v[rows, :]
                    if FPIN:
                        zero = pin()
                    for a, w_v in enumerate((wg_v, wu_v)):
                        prod = w_v[f0 + j, rows, :].astype(f32) * xc
                        acc = accs[a] + zero if FPIN else accs[a]
                        for q in range(16):
                            acc = acc + prod[8 * q:8 * q + 8]
                        accs[a] = acc
                    yield
                gate, up = [jnp.sum(acc, axis=0, keepdims=True) for acc in accs]
                hcol = jnp.broadcast_to(gate * jax.nn.sigmoid(gate) * up, (128, 128)).T
                for n in range(8):
                    ycols = pl.ds(n * 128, 128)
                    prod = wd_v[n, cols, :].astype(f32) * hcol
                    acc = y_acc[:, ycols] + pin() if FPIN else y_acc[:, ycols]
                    for q in range(16):
                        acc = acc + prod[8 * q:8 * q + 8]
                    y_acc[:, ycols] = acc
                    if n % 2 == 1:
                        yield

        def tile(j):
            return (first + j) % NTILE

        def q_post(c, res, ob, ready=None):
            phis, nds, outs = {}, {}, {}
            for tick in range(40):
                step, lane = tick // 4, tick % 4
                if step < 8:
                    u, a, pr = step // 4, (step // 2) % 2, step % 2
                    if ready is not None and pr == 0:
                        phi = None
                    else:
                        phi = _dual_softmax(raw_blk(res, 2 * a + u, 0 if ready is not None else pr * 64, lane), pin())
                    phis.setdefault(step, []).append(phi)
                if 1 <= step < 9 and lane == 1:
                    w = step - 1
                    pair = 2 * (2 * c + w // 4 + 4 * ((w // 2) % 2)) + w % 2
                    phi = phis.pop(w)
                    phi = (as_bf16(ready[2 * ((w // 2) % 2) + w // 4]) if phi[0] is None
                           else jnp.concatenate(phi, axis=1).astype(bf16))
                    nds[w] = _dot(kvb_v[pair], phi)
                if step >= 2 and lane == 0:
                    nd = nds.pop(step - 2)
                    rd = _recip(nd[64:80, :] + 1e-6)
                    outs[step - 2] = jnp.concatenate(
                        [(nd[0:32, :].reshape(4, 8, T) * rd[0:8, :][None]).reshape(32, T),
                         (nd[32:64, :].reshape(4, 8, T) * rd[8:16, :][None]).reshape(32, T)], axis=0)
                    if (step - 2) % 4 == 3:
                        u = (step - 2) // 4
                        o1 = jnp.concatenate([outs.pop(4 * u), outs.pop(4 * u + 1)], axis=0)
                        o2 = jnp.concatenate([outs.pop(4 * u + 2), outs.pop(4 * u + 3)], axis=0)
                        cmb = _rhs_combos(o1[:, :TH], o1[:, TH:], o2[:, :TH], o2[:, TH:])
                        for i in range(7):
                            ob.at[i][:, pl.ds(u * 128, 128)] = pltpu.bitcast(cmb[i].astype(bf16).T, u32)
                yield

        def out_project(h, oba, obb, res, ks=(0, 1), order=P["oo"], n=P["on"]):
            parts = {}
            for c in range(256 // n):
                def prod(i):
                    lhs = jnp.concatenate([(oba, obb)[k][i] for k in ks], axis=1)
                    rhs = wo_v[h, i, pl.ds(c * n // 2, n // 2), pl.ds(ks[0] * 256, len(ks) * 256)]
                    m = _dot_nt(as_bf16(lhs), as_bf16(rhs))
                    last_product[:] = [m, rate[0] * (256 // n)]
                    return m

                def emit(a, b, val):
                    if isinstance(res, list):
                        parts[a, b, c] = val
                        if c == 256 // n - 1:
                            res[a][b] = jnp.concatenate([parts[a, b, cc] for cc in range(256 // n)], axis=1)
                    else:
                        res[a, b, :, pl.ds(c * n, n)] = val

                yield from _strassen(prod, emit, order)

        def epilogue(t, h, res, part=None, upd=None, done=None, order=0):
            n = EROWS
            for a in range(2):
                for b in ((1, 0) if order and a == 0 else (0, 1)):
                    cols = pl.ds(h * 512 + a * 256, 256)
                    for q in range(TH // n):
                        r0 = pl.multiple_of(t * T + b * TH + q * n, n)
                        rows = pl.ds(b * TH + q * n, n)
                        mb, rs = st_v[t, 0, rows, :], st_v[t, 1, rows, :] * 0.5
                        if upd is None or TPIN:
                            mb = mb + pin(n)
                        x = in_v[pl.ds(r0, n), cols].astype(f32)
                        v = (x - jnp.concatenate([mb, mb], axis=1)) * jnp.concatenate([rs, rs], axis=1)
                        if upd is not None:
                            rid = lax.broadcasted_iota(i32, (n, 256), 0)
                            v = v + jnp.where(rid == idx - r0, upd[:, h * 512 + a * 256:h * 512 + (a + 1) * 256], 0.0)
                        g = v + v * jnp.tanh(v)
                        s = res[a][b][q * n:(q + 1) * n]
                        if part is not None:
                            s = s + part[a, b, pl.ds(q * n, n), :]
                        out_v[pl.ds(r0, n), cols] = (x + s * g).astype(bf16)
                        if done is not None and q == TH // n - 1:
                            done(4 * h + 2 * a + b)
                        yield

        NE = 4 * TH // EROWS
        mark('s8_q0')
        fb = NF - (NTILE - 1) * FL
        res0 = None
        _schedule(clock, (q_post(0, half_v, oba_v.at[0], phi_v), 40, 0.0, 1.0))

        def q_tile(j, carry):
            SKIP[0] = False
            last_product[:] = []
            oba = oba_v.at[pl.ds(j, 2)]
            obb = obb_v.at[zero_s[0]]
            x = tokens(tile(j + 1))
            for cp in cp_ffn(j + 1):
                cp.wait()
            fg = ffn(j * FL, FL)
            q0, o0, o1 = ([[None] * 4 for _ in range(4)] for _ in range(3))
            nf, no = P["nffn"], 7 * 256 // P["on"]
            _schedule(clock, project((a_v.at[2], aa_v.at[0]), x, q0),
                      (q_post(1, raw_v.at[1], obb_v.at[0]), 40, *P["p1"]), (fg, nf[0], *P["f0"]))
            _schedule(clock, (out_project(0, oba.at[0], obb, o0), no, 0.0, 1.0),
                      (q_post(0, q0, oba.at[1]), 40, *P["p0"]), (fg, nf[1], *P["f1"]))
            _schedule(clock, (out_project(1, oba.at[0], obb, o1), no, 0.0, 1.0),
                      (epilogue(tile(j), 0, o0), NE, *P["e0"]), (fg, nf[2], *P["f2"]))
            _schedule(clock, project((a_v.at[3], aa_v.at[1]), x, raw_v.at[1]),
                      (epilogue(tile(j), 1, o1), NE, *P["e1"]), (fg, 12 * FL - sum(nf), *P["f3"]))
            cp_o(j, tile(j)).start()
            return carry

        mark('s9_phase2')
        if ONLY != 'p1':
            lax.fori_loop(0, NTILE - 1, q_tile, 0)
        SKIP[0] = ONLY is not None
        if ONLY:
            keep = sum(jnp.sum(pltpu.bitcast(r[(0,) * (len(r.shape) - 2) + (pl.ds(pl.multiple_of(zero_s[0], 16), 16), slice(0, 128))], f32))
                       for r in (xb_v, xx_v, a_v, aa_v, wo_v, kvb_v, raw_v, half_v, phi_v, xcol_v, oba_v, obb_v))
            out_v[0:16, 0:128] = jnp.full((16, 128), keep + jnp.sum(y_acc[...]) + jnp.sum(best_v[...]), f32).astype(bf16)
        mark('sa_tail')

        j = NTILE - 1
        rate[0] = 14
        last_product[:] = []
        oba, obb = oba_v.at[j], obb_v.at[zero_s[0]]
        _schedule(clock, (out_project(0, oba, obb, part_v.at[0], (0,), TORD, 256), 7, 0.0, 0.5),
                  (out_project(1, oba, obb, part_v.at[1], (0,), TORD, 256), 7, 0.5, 1.0),
                  (q_post(1, raw_v.at[1], obb_v.at[0]), 40, 0.0, TQ),
                  (ffn(NF - fb, fb), 12 * fb, 0.1, 0.8))
        upd = jnp.sum(y_acc[...], axis=0, keepdims=True) * (0.5 * jax.nn.sigmoid(rmax[:, 0:1]))
        o0, o1 = ([[None, None], [None, None]] for _ in range(2))
        t = tile(j)
        send = lambda blk: cp_o_blk(t, blk).start()
        e0 = epilogue(t, 0, o0, part_v.at[0], upd, send, TORD)
        e1 = epilogue(t, 1, o1, part_v.at[1], upd, send, TORD)
        _schedule(clock, (out_project(0, oba, obb, o0, (1,), TORD, 256), 7, 0.0, 0.5),
                  (out_project(1, oba, obb, o1, (1,), TORD, 256), 7, 0.5, 1.0),
                  (e0, NE, *E0), (e1, NE, *E1))
        mark('sb_outdma')
        for k in range(NTILE - 1):
            cp_o(k, tile(k)).wait()
        for blk in range(8):
            cp_o_blk(t, blk).wait()
        mark(None)

    scratch = [
        pltpu.VMEM((S + T + 4 * D, D), bf16),
        pltpu.VMEM((NTILE + 1, 2, T, 128), f32),
        pltpu.VMEM((NTILE + 1, 7, 128, 512), u32),
        pltpu.VMEM((NTILE, 35, 64, 256), u32),
        pltpu.VMEM((D, DH), bf16),
        pltpu.VMEM((8, 128), bf16),
        pltpu.VMEM((16, D), f32),
        pltpu.VMEM((8, 128, 128), bf16),
        pltpu.VMEM((4, 7, 128, 512), u32),
        pltpu.VMEM((2, 35, 64, 256), u32),
        pltpu.VMEM((2, 7, 128, 512), u32),
        pltpu.VMEM((2, 7, 128, 512), u32),
        pltpu.VMEM((NF, D, 128), bf16),
        pltpu.VMEM((NF, D, 128), bf16),
        pltpu.VMEM((D // 128, F, 128), bf16),
        pltpu.VMEM((H // 2 + 4, 64, 128), f32),
        pltpu.VMEM((H // 2 + 4, 128, 128), f32),
        pltpu.VMEM((H // 2 + 4, 80, 128), bf16),
        pltpu.VMEM((2, 16, 128), f32),
        pltpu.VMEM((2, 16, 128), i32),
        pltpu.VMEM((2, 4, 4, 128, 128), f32),
        pltpu.VMEM((4, 4, 64, 128), f32),
        pltpu.VMEM((4, 64, T), u32),
        pltpu.VMEM((NTILE, 7, TH // 2, 256), u32),
        pltpu.VMEM((2, 7, TH // 2, 256), u32),
        pltpu.VMEM((2, 2, 2, 256, 256), f32),
        pltpu.VMEM((D, 128), f32),
        pltpu.VMEM((8, D), f32),
        pltpu.VMEM((S, D), bf16),
        pltpu.SMEM((1,), i32),
        pltpu.SemaphoreType.DMA((NTILE + 2,)),
        pltpu.SemaphoreType.DMA((11,)),
        pltpu.SemaphoreType.DMA((1,)),
        pltpu.SemaphoreType.DMA((NTILE,)),
        pltpu.SemaphoreType.DMA((1,)),
    ]

    def call(x, wqkv, wphi, wo, wr, wg, wu, wd):
        hbm = pl.BlockSpec(memory_space=pltpu.HBM)
        return pl.pallas_call(
            kernel,
            out_shape=jax.ShapeDtypeStruct((S, D), bf16),
            in_specs=[hbm] * 8,
            out_specs=hbm,
            scratch_shapes=scratch,
            compiler_params=pltpu.CompilerParams(vmem_limit_bytes=120 * 2**20, flags=FLAGS, disable_bounds_checks=NOBC, disable_semaphore_checks=NOSEM),
            name="hedgehog", interpret=INTERP,
        )(x, wqkv, wphi, wo, wr, wg, wu, wd)

    return call


@jax.jit
def pallas_recurrent_scan__linear_kernel_hedgehog__moe_arch_mod__prompt_kernel(
    A_x: jax.Array,
    A_wqkv: jax.Array,
    A_w_phi: jax.Array,
    A_wo: jax.Array,
    B_x: jax.Array,
    B_w_r: jax.Array,
    B_w_gate: jax.Array,
    B_w_up: jax.Array,
    B_w_down: jax.Array,
):
    del B_x
    out = make_kernel()(
        A_x.reshape(S, D), A_wqkv, A_w_phi.reshape(D, DH), A_wo,
        B_w_r.reshape(8, 128), B_w_gate, B_w_up, B_w_down)
    return out.reshape(1, S, D)
```

```python
import math
import contextlib

import numpy as np

import jax
import jax.numpy as jnp
from jax import lax
import jax.experimental.pallas as pl
import jax.experimental.pallas.tpu as pltpu

S, D, H, DH, F = 2048, 1024, 32, 32, 3584
T = 512
TH = T // 2
NTILE = S // T
NF = F // 128
FG = NF // NTILE
WQ, WK, WV, WO = (S + T + j * D for j in range(4))
LHS_SUMS, RHS_SUMS = (0, 1, 4, 5, 6), (0, 2, 3, 5, 6)
LOG2E = math.log2(math.e)
EPS_BF16 = float(np.float32(1e-5).astype(jnp.bfloat16))
NT_DIMS = (((1,), (1,)), ((), ()))
f32, bf16, i32, u32 = jnp.float32, jnp.bfloat16, jnp.int32, jnp.uint32


def _dot_nt(a, b):
    return lax.dot_general(a, b, NT_DIMS, preferred_element_type=f32)


def _dot(a, b):
    return jnp.dot(a, b, preferred_element_type=f32)


def aligned(i, n):
    return i if isinstance(i, int) else pl.multiple_of(i, n)


def _recip(v):
    r = pl.reciprocal(v, approx=True)
    return r * (2.0 - v * r)


def _wide(w):
    return pltpu.bitcast(w, bf16).astype(f32)


def _narrow(v):
    return pltpu.bitcast(v.astype(bf16), u32)


def _lhs_combos(a11, a12, a21, a22):
    return [a11 + a22, a21 + a22, a11, a22, a11 + a12, a21 - a11, a12 - a22]


def _rhs_combos(b11, b12, b21, b22):
    return [b11 + b22, b11, b12 - b22, b21 - b11, b22, b11 + b12, b21 + b22]


class _Quad:
    def __init__(self, v):
        self.v = v

    def __add__(self, o):
        return _Quad([p + q for p, q in zip(self.v, o.v)])

    def __sub__(self, o):
        return _Quad([p - q for p, q in zip(self.v, o.v)])


def _strassen2(prod, emit, order):
    done = {}

    def inner(i):
        out = [None] * 4

        def put(a, b, val):
            out[2 * a + b] = val
        yield from _strassen(lambda j: prod(7 * i + j), put, order)
        done[i] = _Quad(out)

    def put(a, b, quad):
        for k, val in enumerate(quad.v):
            emit(2 * a + k // 2, 2 * b + k % 2, val)

    outer = _strassen(lambda i: done[i], put, order)
    for i in ((0, 3, 4, 6, 2, 1, 5), (2, 4, 0, 6, 3, 1, 5))[order]:
        steps = inner(i)
        for _ in range(6):
            next(steps)
            yield
        for _ in steps:
            pass
        next(outer)
        yield


def _strassen(prod, emit, order=0):
    if order == 0:
        m1 = prod(0)
        yield
        m4 = prod(3)
        c11 = m1 + m4
        yield
        m5 = prod(4)
        c11 = c11 - m5
        yield
        emit(0, 0, c11 + prod(6))
        yield
        m3 = prod(2)
        emit(0, 1, m3 + m5)
        c22 = m1 + m3
        yield
        m2 = prod(1)
        emit(1, 0, m2 + m4)
        c22 = c22 - m2
        yield
        emit(1, 1, c22 + prod(5))
        yield
    else:
        m3 = prod(2)
        yield
        m5 = prod(4)
        emit(0, 1, m3 + m5)
        yield
        m1 = prod(0)
        c11, c22 = m1 - m5, m1 + m3
        yield
        c11 = c11 + prod(6)
        yield
        m4 = prod(3)
        emit(0, 0, c11 + m4)
        yield
        m2 = prod(1)
        emit(1, 0, m2 + m4)
        c22 = c22 - m2
        yield
        emit(1, 1, c22 + prod(5))
        yield


SKIP = [False]


def _schedule(clock, *streams):
    if SKIP[0]:
        return
    events = []
    for order, (gen, n, a, b) in enumerate(streams):
        for k in range(n):
            events.append((a + (b - a) * k / n, order, k, gen))
    for when, _, _, gen in sorted(events, key=lambda e: e[:3]):
        clock[:] = [when]
        next(gen)


def _dual_softmax(p, zero=None):
    rows = [p[8 * j:8 * j + 8] for j in range(8)]
    if zero is not None:
        rows[0] = rows[0] + zero

    def reduce(vs, op):
        while len(vs) > 1:
            vs = [op(vs[i], vs[i + 1]) for i in range(0, len(vs), 2)]
        v = op(vs[0], pltpu.roll(vs[0], 4, 0))
        return op(v, pltpu.roll(v, 2, 0))

    mx, mn = reduce(rows, jnp.maximum), reduce(rows, jnp.minimum)
    ep = [jnp.exp2(v - mx) for v in rows]
    en = [jnp.exp2(mn - v) for v in rows]
    rp, rn = _recip(reduce(ep, jnp.add)), _recip(reduce(en, jnp.add))
    return jnp.concatenate([v * rp for v in ep] + [v * rn for v in en], axis=0)


PLAN = dict(
    kv=(0.0, 0.92), stats=(0.0, 0.96), apply=(0.015, 0.935), fold=(0.1, 0.9), fold2=(0.06, 0.84), nfold=3,
    trans=(0.085, 0.86), routed=(0.015, 0.945), split=(0.02, 1.0), split2=(0.09, 0.97), nsplit=56,
    again=(0.0, 1.0), again2=(0.0, 0.9), nagain=0, o1=1,
    p1=(0.0, 1.0), p0=(0.065, 1.0), e0=(0.055, 0.96), e1=(0.0, 0.985), nffn=(14, 18, 38),
    f0=(0.125, 0.945), f1=(0.165, 0.945), f2=(0.02, 1.0), f3=(0.0, 0.925), oq=1, oo=1, on=256,
)


def make_kernel(FLAGS=None, FL=9, W0=0.15, W1=0.7, W2=0.15, W3=0.6, TORD=1, NOSEM=False, E0=(0.2, 0.7), E1=(0.7, 1.2),
                TPIN=False, TQ=0.9, NOBC=True, EROWS=32, SCOPES=False, ONLY=None, TW=(2, 3), INTERP=False,
                DMA_ORDER='a0 a1 a2 a3 k0 v0 k1 v1 k2 v2 k3 v3 x1 f0 x2 f1 o0 o1 x3 f2 o2 o3 x4 f3'.split(), **over):
    P = dict(PLAN, **over)
    FPIN = True

    stack = []
    def mark(name):
        if not SCOPES: return
        if stack: stack.pop().__exit__(None, None, None)
        if name:
            cm = jax.named_scope(name); cm.__enter__(); stack.append(cm)

    def kernel(x_hbm, wqkv_hbm, wphi_hbm, wo_hbm, wr_hbm, wg_hbm, wu_hbm, wd_hbm,
               out_hbm,
               in_v, st_v, xb_v, xx_v, wphi_v, wr8_v, wr_v, lm_v, a_v, aa_v, b_v, bb_v, wo_v, wg_v, wu_v, wd_v,
               kv_acc, z_acc, kvb_v, best_v, best_i, raw_v, half_v, phi_v, oba_v, obb_v, part_v, xcol_v, y_acc,
               out_v, zero_s, sem_x, sem_w, sem_s, sem_f, sem_o):
        def cp_x(r0, n, sem, src0=None):
            src0 = r0 if src0 is None else src0
            return pltpu.make_async_copy(x_hbm.at[pl.ds(src0, n)], in_v.at[pl.ds(r0, n)], sem_x.at[sem])

        def cp_x0(piece):
            return cp_x((piece % 2) * TH + (piece // 2) * (TH // 2), TH // 2, 0 if piece < 2 else NTILE + 1)

        def cp_xt(t):
            return cp_x(pl.multiple_of(t * T, T), T, t, pl.multiple_of((t % NTILE) * T, T))

        def cp_w(j, c0, n, sem):
            src = wo_hbm.at[:, pl.ds(c0, n)] if j == 3 else wqkv_hbm.at[:, pl.ds(aligned(j * D + c0, 128), n)]
            return pltpu.make_async_copy(src, in_v.at[pl.ds(WQ + j * D, D), pl.ds(c0, n)], sem_w.at[sem])

        def cp_k(c):
            return cp_w(1, c * 256, 256, c)

        def cp_v(c):
            return cp_w(2, c * 256, 256, c if c else 4)

        def cp_fold(u):
            cps = []
            for n in range(8):
                r0 = aligned((n // 2) * 256 + (u % 2) * 128, 128)
                cols = pl.ds(aligned((u // 2) * 256 + (n % 2) * 512, 256), 256)
                cps.append(pltpu.make_async_copy(wqkv_hbm.at[pl.ds(r0, 128), cols],
                                                 in_v.at[pl.ds(aligned(WQ + r0, 128), 128), cols], sem_w.at[5 + u]))
            return cps

        def cp_wo(u):
            g = (u // 2) * 4 + u % 2
            return [cp_w(3, aligned(c * 128, 128), 128, 9 + u // 2) for c in (g, g + 2)]

        cp_phi = pltpu.make_async_copy(wphi_hbm, wphi_v, sem_s.at[0])
        cp_wr = pltpu.make_async_copy(wr_hbm, wr8_v, sem_s.at[0])
        def cp_ffn(g):
            cps = []
            for j in range(FG):
                cols = pl.ds(aligned((g * FG + j) * 128, 128), 128)
                for src, dst in ((wg_hbm, wg_v), (wu_hbm, wu_v)):
                    cps.append(pltpu.make_async_copy(src.at[:, cols], dst.at[g * FG + j], sem_f.at[g]))
            rows = pl.ds(aligned(g * FG * 128, 128), FG * 128)
            for n in range(D // 128):
                cps.append(pltpu.make_async_copy(wd_hbm.at[rows, pl.ds(n * 128, 128)], wd_v.at[n, rows], sem_f.at[g]))
            return cps

        def cp_o(k, t):
            rows = pl.ds(pl.multiple_of(t * T, T), T)
            return pltpu.make_async_copy(out_v.at[rows], out_hbm.at[rows], sem_o.at[0])

        def cp_o_blk(t, blk):
            rows = pl.ds(pl.multiple_of(t * T + (blk % 2) * TH, TH), TH)
            cols = pl.ds((blk // 2) * 256, 256)
            return pltpu.make_async_copy(out_v.at[rows, cols], out_hbm.at[rows, cols], sem_o.at[0])

        cp_wr.start()
        cp_phi.start()
        for n, name in enumerate(DMA_ORDER):
            if n == 1:
                cp_wr.wait()
                cp_phi.wait()
            cps = {"a": cp_x0, "k": cp_k, "v": cp_v, "x": cp_xt, "f": cp_fold, "o": cp_wo}[name[0]](int(name[1]))
            for cp in cps if isinstance(cps, list) else [cps]:
                cp.start()

        last_product = []

        clock = [0.0]
        rate = [7]

        def pin(n=8):
            if not last_product:
                return jnp.zeros((n, 128), f32)
            rows, cols = last_product[0].shape[0] // 8, last_product[0].shape[1] // 128
            q = min(int((clock[0] * last_product[1]) % 1.0 * rows * cols + 1e-6), rows * cols - 1)
            m = last_product[0][(q % rows) * 8:(q % rows) * 8 + 8, (q // rows) * 128:(q // rows) * 128 + 128]
            z = pltpu.bitcast(pltpu.bitcast(m, u32) & zero_s[0].astype(u32), f32)
            return z if n == 8 else jnp.concatenate([z] * (n // 8), axis=0)

        def as_bf16(w):
            return pltpu.bitcast(w, bf16)

        def feature_maps():
            rho = lax.broadcasted_iota(i32, (128, DH), 0)
            sel = (((rho % 64) // 8) * 4 + (rho % 8) // 2 == lax.broadcasted_iota(i32, (128, DH), 1)).astype(bf16)
            rho = lax.broadcasted_iota(i32, (128, 128), 0)
            keep = (rho // 64) * 2 + rho % 2 == lax.broadcasted_iota(i32, (128, 128), 1) // DH
            for g in range(8):
                full = _dot_nt(sel, wphi_v[pl.ds(g * 128, 128), :])
                lm_v.at[g][...] = jnp.where(keep, full, 0.0).astype(bf16)

        def operand(chunk):
            return a_v.at[chunk] if chunk < 2 else b_v.at[chunk - 2]

        def put_lhs(dst, rows, cols, *quadrants):
            for i, v in enumerate(_lhs_combos(*quadrants)):
                dst.at[i][rows, cols] = _narrow(v)

        def split_again(src, dst, lhs, r, k):
            for i in range(7):
                zero = pltpu.bitcast(pin(), u32)
                w = [[src[i, pl.ds(h * 64 + r * 8, 8), pl.ds(aligned(c * 256 + k * 128, 128), 128)]
                      for c in range(2)] for h in range(2)]
                q00, q01, q10, q11 = _wide(w[0][0] | zero), _wide(w[0][1]), _wide(w[1][0]), _wide(w[1][1] | zero)
                cmb = _lhs_combos(q00, q01, q10, q11) if lhs else _rhs_combos(q00, q10, q01, q11)
                for n, j in enumerate(LHS_SUMS if lhs else RHS_SUMS):
                    dst.at[5 * i + n][pl.ds(r * 8, 8), pl.ds(aligned(k * 128, 128), 128)] = _narrow(cmb[j])
                yield

        def second(src, dst, lhs, ij):
            i, j = ij // 7, ij % 7
            sums = LHS_SUMS if lhs else RHS_SUMS
            if j in sums:
                return as_bf16(dst[5 * i + sums.index(j)])
            d = int(j == (3 if lhs else 4))
            return as_bf16(src[i, pl.ds(d * 64, 64), pl.ds(d * 256, 256)])

        def w_blocks(base, top, bot, k):
            return [in_v[pl.ds(aligned(base + kh * 512 + k * 128, 128), 128),
                         pl.ds(aligned(g * 128, 128), 128)] for g in (top, bot) for kh in range(2)]

        def prep_fold(base, top, bot, dst, row_of, ks):
            for k in ks:
                blocks = [_dot_nt(lm_v[g], w) for g, w in zip((top, top, bot, bot), w_blocks(base, top, bot, k))]
                for j in range(8):
                    put_lhs(dst, pl.ds(aligned(row_of(j), 8), 8), pl.ds(aligned(k * 128, 128), 128),
                            *[p[16 * j:16 * j + 16] * LOG2E for p in blocks])
                yield

        def prep_transpose(base, top, bot, dst, row_of):
            for k in range(4):
                zero = pltpu.bitcast(pin(64), u32)
                blocks = [as_bf16(pltpu.bitcast(w, u32) | zero).T for w in w_blocks(base, top, bot, k)]
                for j in range(8):
                    put_lhs(dst, pl.ds(aligned(row_of(j), 8), 8), pl.ds(k * 128, 128),
                            *[w[16 * j:16 * j + 16].astype(f32) for w in blocks])
                yield

        def prep_q(u):
            ch, k = u // 2, u % 2
            for half in range(2):
                g = 2 * ch + half
                yield from prep_fold(WQ, g, g + 4, a_v.at[2 + ch], lambda j: half * 64 + 8 * j, (k, k + 2))

        def split_q(u):
            for r in range(8):
                yield from split_again(a_v.at[2 + u // 2 + zero_s[0]], aa_v.at[u // 2], True, r, u % 2)

        def prep_wo(u, base=WO):
            g = (u // 2) * 4 + u % 2
            return prep_transpose(base, g, g + 2, wo_v.at[u // 2], lambda j: (u % 2) * 64 + 8 * j)

        def x_block(r0, c0):
            return in_v[pl.ds(r0, 16), pl.ds(c0, 128)].astype(f32)

        def ln_stats(t, st):
            for step in range(32):
                pos = (step % 2) * 16 + step // 2
                r0 = pl.multiple_of(t * T + pos * 16, 16)
                x0 = x_block(r0, 0) + pin(16)
                s1 = s2 = None
                for j in range(1, 8):
                    d = x_block(r0, j * 128) - x0
                    s1 = d if j == 1 else s1 + d
                    s2 = d * d if j == 1 else s2 + d * d
                lane_mean = x0 + s1 * 0.125
                m = jnp.sum(lane_mean, axis=-1, keepdims=True) * (1.0 / 128)
                dm = lane_mean - m
                v = jnp.sum((s2 - s1 * s1 * 0.125) * 0.125 + dm * dm, axis=-1, keepdims=True) * (1.0 / 128)
                vb = (v.astype(bf16).astype(f32) + EPS_BF16).astype(bf16).astype(f32)
                st[0, pl.ds(pos * 16, 16), :] = jnp.broadcast_to(m.astype(bf16).astype(f32), (16, 128))
                st[1, pl.ds(pos * 16, 16), :] = jnp.broadcast_to(1.0 / jnp.sqrt(vb).astype(bf16).astype(f32), (16, 128))
                yield

        def ln_apply(t, st, xb, live):
            for step in range(16):
                r0 = [pl.multiple_of(t * T + hf * TH + step * 16 + zero_s[0], 16) for hf in range(2)]
                mean = [st[0, pl.ds(hf * TH + step * 16, 16), :] for hf in range(2)]
                scale = [st[1, pl.ds(hf * TH + step * 16, 16), :] for hf in range(2)]
                score = [None, None]
                for k in range(4):
                    zero = pin(16)
                    xn = [[(x_block(r0[hf], kh * 512 + k * 128) - (mean[hf] + zero)) * scale[hf]
                           for kh in range(2)] for hf in range(2)]
                    if xb is not None:
                        for i, v in enumerate(_rhs_combos(xn[0][0], xn[1][0], xn[0][1], xn[1][1])):
                            xb.at[i][pl.ds(step * 8, 8), pl.ds(k * 128, 128)] = _narrow(v)
                    for hf in range(2 if live is not None else 0):
                        part = (xn[hf][0] * wr_v[:, pl.ds(k * 128, 128)]
                                + xn[hf][1] * wr_v[:, pl.ds(512 + k * 128, 128)])
                        score[hf] = part if k == 0 else score[hf] + part
                        if k == 3:
                            r = jnp.sum(score[hf], axis=-1, keepdims=True).astype(bf16).astype(f32)
                            r = jnp.broadcast_to(r, (16, 128))
                            up = jnp.logical_and(r > best_v[hf], live)
                            best_v[hf] = jnp.where(up, r, best_v[hf])
                            best_i[hf] = jnp.where(up, lax.broadcasted_iota(i32, (16, 128), 0) + r0[hf], best_i[hf])
                    yield

        def ln_split(xb, xx):
            for r in range(8):
                for k in range(2):
                    yield from split_again(xb, xx, False, r, k)

        def project(w, x, res, keep=None):
            def emit(r, b, val):
                if isinstance(res, list):
                    res[r][b] = val
                else:
                    res[r, b] = val
                if keep is not None:
                    keep[r, b] = val[64:]

            def prod2(ij):
                m = _dot_nt(second(*w, True, ij), second(*x, False, ij))
                last_product[:] = [m, 49]
                return m

            def once():
                for c in range(2):
                    def prod(i):
                        m = _dot_nt(as_bf16(w[i]), as_bf16(x[i, pl.ds(c * 64, 64), :]))
                        last_product[:] = [m, 14]
                        return m

                    def put(a, b, val):
                        emit(2 * a, 2 * b + c, val[:128])
                        emit(2 * a + 1, 2 * b + c, val[128:])

                    yield from _strassen(prod, put, P["o1"])

            if isinstance(w, tuple):
                return _strassen2(prod2, emit, P["oq"]), 49, 0.0, 1.0
            return once(), 14, 0.0, 1.0

        def project_part(w, x, res, part):
            def prod(i):
                lhs = jnp.concatenate([w[i, pl.ds(h * 64 + part * 32, 32), :] for h in range(2)], axis=0)
                m = _dot_nt(as_bf16(lhs), as_bf16(x[i]))
                last_product[:] = [m, 14]
                return m

            def put(a, b, val):
                for h in range(2):
                    for c in range(2):
                        res[2 * a + h, 2 * b + c, pl.ds(part * 64, 64), :] = val[h * 64:(h + 1) * 64, c * 128:(c + 1) * 128]

            return _strassen(prod, put, P["o1"])

        def raw_blk(res, r, r0, lane):
            if isinstance(res, list):
                return res[r][lane][r0:r0 + 64]
            return res[r, lane, pl.ds(r0, 64), :]

        keep_kv = lax.broadcasted_iota(i32, (64, 128), 0) // DH == lax.broadcasted_iota(i32, (64, 128), 1) % 2
        keep_z = lax.broadcasted_iota(i32, (16, 128), 0) // 8 == lax.broadcasted_iota(i32, (16, 128), 1) % 2

        def kv_post(c, res, keep=None):
            def accumulate(p, vt, phi):
                kv = kv_acc[p] + _dot_nt(vt, phi)
                kv_acc[p] = kv
                kvb_v.at[p][pl.ds(0, 64), :] = jnp.where(keep_kv, kv, 0.0).astype(bf16)

            pending = None
            for a in range(2):
                for pr in range(2):
                    p = 4 * c + 2 * a + pr
                    phis, zs = [], z_acc[p]
                    for lane in range(4):
                        phi = _dual_softmax(raw_blk(res, 2 * a + pr, 0, lane), pin())
                        zs = zs + phi
                        phis.append(phi)
                        if keep is not None:
                            keep.at[2 * a + pr][:, pl.ds(lane * 128, 128)] = _narrow(phi)
                        if lane == 1 and pending:
                            accumulate(*pending)
                        if lane == 3:
                            z_acc[p] = zs
                            zrow = jnp.broadcast_to(jnp.sum(zs.T, axis=0, keepdims=True), (16, 128))
                            kvb_v.at[p][pl.ds(64, 16), :] = jnp.where(keep_z, zrow, 0.0).astype(bf16)
                            vt = jnp.concatenate([raw_blk(res, 2 * a + pr, 64, l) for l in range(4)], axis=1)
                            pending = (p, vt.astype(bf16), jnp.concatenate(phis, axis=1).astype(bf16))
                        yield
            yield
            accumulate(*pending)
            yield

        def route():
            best, tok = best_v[...].reshape(32, 128), best_i[...].reshape(32, 128)
            rmax = jnp.max(best, axis=0, keepdims=True)
            idx = jnp.min(jnp.where(best == rmax, tok, S).astype(f32)).astype(i32)
            return jnp.clip(idx, 0, S - 1), rmax

        def routed_token(idx):
            base = pl.multiple_of((idx // 16) * 16, 16)
            rows = pl.ds(pl.multiple_of(base % T, 16), 16)
            xn = (in_v[pl.ds(base, 16), :].astype(f32) - st_v[idx // T, 0, rows, 0:1]) * st_v[idx // T, 1, rows, 0:1]
            xsel = jnp.where(lax.broadcasted_iota(i32, (16, D), 0) == idx - base, xn, 0.0)
            xsel = jnp.sum(xsel, axis=0, keepdims=True).astype(bf16).astype(f32)
            for j in range(8):
                row = xsel[:, j * 128:(j + 1) * 128] + pin()
                xcol_v[pl.ds(j * 128, 128), :] = jnp.concatenate([row] * 16, axis=0).T
                yield

        SKIP[0] = ONLY is not None
        mark('s0_init')
        zero_s[0] = 0
        kv_acc[...] = jnp.zeros(kv_acc.shape, f32)
        z_acc[...] = jnp.zeros(z_acc.shape, f32)
        y_acc[...] = jnp.zeros(y_acc.shape, f32)
        best_v[...] = jnp.full(best_v.shape, -jnp.inf, f32)
        for hf in range(2):
            best_i[hf] = lax.broadcasted_iota(i32, (16, 128), 0) + hf * TH
        w8 = wr8_v[...].astype(f32)
        wr_v[...] = jnp.broadcast_to(jnp.concatenate([w8[j:j + 1, :] for j in range(8)], axis=1), (16, D))
        feature_maps()
        mark('s1_ln0')
        stats, apply = ln_stats(0, st_v.at[0]), ln_apply(0, st_v.at[0], xb_v.at[0], None)
        cp_x0(0).wait()
        cp_x0(1).wait()
        _schedule(clock, (stats, 16, 0.0, 1.0))
        _schedule(clock, (apply, 32, 0.0, 1.0))
        cp_x0(2).wait()
        cp_x0(3).wait()
        _schedule(clock, (stats, 16, 0.0, 1.0))
        _schedule(clock, (apply, 32, 0.0, 1.0))

        def prep_kv(c):
            cp_k(c).wait()
            if c:
                cp_v(c).wait()
            once = operand(c)
            yield from prep_fold(WK, 2 * c, 2 * c + 1, once, lambda j: (j // 4) * 64 + (j % 4) * 8, range(4))
            if not c:
                cp_v(c).wait()
            yield from prep_transpose(WV, 2 * c, 2 * c + 1, once, lambda j: (j // 4) * 64 + 32 + (j % 4) * 8)
            if c in TW:
                for k in range(2):
                    for r in range(8):
                        for _ in split_again(b_v.at[c - 2 + zero_s[0]], bb_v.at[c - 2], True, r, k):
                            pass
                        if r % 2:
                            yield

        def tokens(t):
            return xb_v.at[t], xx_v.at[t]

        mark('s3_prep0')
        first_chunk = prep_kv(0)
        _schedule(clock, (first_chunk, 4, 0.0, 1.0))
        mark('s4_proj0')
        _schedule(clock, (project_part(operand(0), xb_v.at[0], raw_v.at[0], 0), 7, 0.0, 0.5),
                  (project_part(operand(0), xb_v.at[0], raw_v.at[0], 1), 7, 0.5, 1.0),
                  (first_chunk, 4, W0, 0.45), (prep_kv(1), 8, W1, 1.0),
                  (ln_apply(0, st_v.at[0], None, True), 64, 0.03, W1),
                  (ln_split(xb_v.at[zero_s[0]], xx_v.at[0]), 112 if TW else 0, 0.03, 1.0))
        _schedule(clock, project(operand(1), xb_v.at[0], raw_v.at[1]),
                  (kv_post(0, raw_v.at[zero_s[0]]), 18, 0.0, 1.0), (prep_kv(2), 16 if 2 in TW else 8, W2, W3), (prep_kv(3), 16 if 3 in TW else 8, W3, 1.0))

        def kv_tile(t, idx):
            SKIP[0] = False
            last = t == NTILE - 1
            for cp in cp_fold(t) + [cp_xt(t + 1)]:
                cp.wait()

            @pl.when(jnp.logical_and(t > 0, t < 3))
            def _():
                for cp in cp_wo(2 * t - 2) + cp_wo(2 * t - 1):
                    cp.wait()

            if not NOBC:
                for g in range(NTILE):
                    @pl.when(t == g)
                    def _():
                        for cp in cp_ffn(g):
                            cp.start()

            last_product[:] = []
            idx = route()[0]
            xb, st = xb_v.at[pl.ds(t, 2)], st_v.at[t + 1]
            stats, apply = ln_stats(t + 1, st), ln_apply(t + 1, st, xb.at[1], jnp.logical_not(last))
            xx = xx_v.at[pl.ds(t, 2)]
            split = ln_split(xb_v.at[t + 1 + zero_s[0]], xx.at[1]) if TW else ln_split(xb.at[0], xx.at[0])
            slot = lambda c: ((operand(c), bb_v.at[c - 2]), (xb.at[0], xx.at[0])) if c in TW else (operand(c), xb.at[0])
            fold = prep_q(t)
            trans = [prep_wo(2 * ((t + 1) % 2) + u, jnp.where(t == 0, WV, WO)) for u in range(2)]

            def fetch_ffn():
                for cp in cp_ffn(t):
                    cp.start()
                    yield

            c2, c3, c0 = ([[None] * 4 for _ in range(4)] for _ in range(3))
            _schedule(clock, project(*slot(2), c2), (kv_post(1, raw_v.at[1]), 18, *P["kv"]),
                      (stats, 32, *P["stats"]), (fold, P["nfold"], *P["fold"]),
                      (fetch_ffn(), 2 * FG + 8 if NOBC else 0, 0.05, 0.95))
            _schedule(clock, project(*slot(3), c3), (kv_post(2, c2), 18, *P["kv"]),
                      (apply, 64, *P["apply"]), (fold, 4 - P["nfold"], *P["fold2"]))
            x = xb_v.at[jnp.where(last, (idx // T + 1) % NTILE, t + 1)]
            chunk = jnp.where(last, 2, 0)
            again = split_q(t)
            _schedule(clock, project(a_v.at[chunk], x, c0, keep=half_v), (kv_post(3, c3), 18, *P["kv"]),
                      (trans[0], 4, *P["trans"]), (routed_token(idx), 8, *P["routed"]),
                      (split, P["nsplit"], *P["split"]), (again, P["nagain"], *P["again"]))
            _schedule(clock, project(a_v.at[chunk + 1], x, raw_v.at[1]),
                      (kv_post(jnp.where(last, 4, 0), c0, phi_v), 18, *P["kv"]), (trans[1], 4, *P["trans"]),
                      (split, 112 - P["nsplit"], *P["split2"]), (again, 56 - P["nagain"], *P["again2"]))
            return idx

        mark('s6_phase1')
        idx = lax.fori_loop(0, NTILE, kv_tile, jnp.int32(0)) if ONLY != 'p2' else route()[0]
        SKIP[0] = ONLY is not None
        mark('s7_mid')
        for cp in cp_ffn(0):
            cp.wait()
        last_product[:] = []

        rmax = route()[1]
        first = (idx // T + 1) % NTILE

        def ffn(f0, nf):
            for j in range(nf):
                cols = pl.ds(pl.multiple_of((f0 + j) * 128, 128), 128)
                accs = [jnp.zeros((8, 128), f32)] * 2
                for r in range(8):
                    rows = pl.ds(r * 128, 128)
                    xc = xcol_v[rows, :]
                    if FPIN:
                        zero = pin()
                    for a, w_v in enumerate((wg_v, wu_v)):
                        prod = w_v[f0 + j, rows, :].astype(f32) * xc
                        acc = accs[a] + zero if FPIN else accs[a]
                        for q in range(16):
                            acc = acc + prod[8 * q:8 * q + 8]
                        accs[a] = acc
                    yield
                gate, up = [jnp.sum(acc, axis=0, keepdims=True) for acc in accs]
                hcol = jnp.broadcast_to(gate * jax.nn.sigmoid(gate) * up, (128, 128)).T
                for n in range(8):
                    ycols = pl.ds(n * 128, 128)
                    prod = wd_v[n, cols, :].astype(f32) * hcol
                    acc = y_acc[:, ycols] + pin() if FPIN else y_acc[:, ycols]
                    for q in range(16):
                        acc = acc + prod[8 * q:8 * q + 8]
                    y_acc[:, ycols] = acc
                    if n % 2 == 1:
                        yield

        def tile(j):
            return (first + j) % NTILE

        def q_post(c, res, ob, ready=None):
            phis, nds, outs = {}, {}, {}
            for tick in range(40):
                step, lane = tick // 4, tick % 4
                if step < 8:
                    u, a, pr = step // 4, (step // 2) % 2, step % 2
                    if ready is not None and pr == 0:
                        phi = None
                    else:
                        phi = _dual_softmax(raw_blk(res, 2 * a + u, 0 if ready is not None else pr * 64, lane), pin())
                    phis.setdefault(step, []).append(phi)
                if 1 <= step < 9 and lane == 1:
                    w = step - 1
                    pair = 2 * (2 * c + w // 4 + 4 * ((w // 2) % 2)) + w % 2
                    phi = phis.pop(w)
                    phi = (as_bf16(ready[2 * ((w // 2) % 2) + w // 4]) if phi[0] is None
                           else jnp.concatenate(phi, axis=1).astype(bf16))
                    nds[w] = _dot(kvb_v[pair], phi)
                if step >= 2 and lane == 0:
                    nd = nds.pop(step - 2)
                    rd = _recip(nd[64:80, :] + 1e-6)
                    outs[step - 2] = jnp.concatenate(
                        [(nd[0:32, :].reshape(4, 8, T) * rd[0:8, :][None]).reshape(32, T),
                         (nd[32:64, :].reshape(4, 8, T) * rd[8:16, :][None]).reshape(32, T)], axis=0)
                    if (step - 2) % 4 == 3:
                        u = (step - 2) // 4
                        o1 = jnp.concatenate([outs.pop(4 * u), outs.pop(4 * u + 1)], axis=0)
                        o2 = jnp.concatenate([outs.pop(4 * u + 2), outs.pop(4 * u + 3)], axis=0)
                        cmb = _rhs_combos(o1[:, :TH], o1[:, TH:], o2[:, :TH], o2[:, TH:])
                        for i in range(7):
                            ob.at[i][:, pl.ds(u * 128, 128)] = pltpu.bitcast(cmb[i].astype(bf16).T, u32)
                yield

        def out_project(h, oba, obb, res, ks=(0, 1), order=P["oo"], n=P["on"]):
            parts = {}
            for c in range(256 // n):
                def prod(i):
                    lhs = jnp.concatenate([(oba, obb)[k][i] for k in ks], axis=1)
                    rhs = wo_v[h, i, pl.ds(c * n // 2, n // 2), pl.ds(ks[0] * 256, len(ks) * 256)]
                    m = _dot_nt(as_bf16(lhs), as_bf16(rhs))
                    last_product[:] = [m, rate[0] * (256 // n)]
                    return m

                def emit(a, b, val):
                    if isinstance(res, list):
                        parts[a, b, c] = val
                        if c == 256 // n - 1:
                            res[a][b] = jnp.concatenate([parts[a, b, cc] for cc in range(256 // n)], axis=1)
                    else:
                        res[a, b, :, pl.ds(c * n, n)] = val

                yield from _strassen(prod, emit, order)

        def epilogue(t, h, res, part=None, upd=None, done=None, order=0):
            n = EROWS
            for a in range(2):
                for b in ((1, 0) if order and a == 0 else (0, 1)):
                    cols = pl.ds(h * 512 + a * 256, 256)
                    for q in range(TH // n):
                        r0 = pl.multiple_of(t * T + b * TH + q * n, n)
                        rows = pl.ds(b * TH + q * n, n)
                        mb, rs = st_v[t, 0, rows, :], st_v[t, 1, rows, :] * 0.5
                        if upd is None or TPIN:
                            mb = mb + pin(n)
                        x = in_v[pl.ds(r0, n), cols].astype(f32)
                        v = (x - jnp.concatenate([mb, mb], axis=1)) * jnp.concatenate([rs, rs], axis=1)
                        if upd is not None:
                            rid = lax.broadcasted_iota(i32, (n, 256), 0)
                            v = v + jnp.where(rid == idx - r0, upd[:, h * 512 + a * 256:h * 512 + (a + 1) * 256], 0.0)
                        g = v + v * jnp.tanh(v)
                        s = res[a][b][q * n:(q + 1) * n]
                        if part is not None:
                            s = s + part[a, b, pl.ds(q * n, n), :]
                        out_v[pl.ds(r0, n), cols] = (x + s * g).astype(bf16)
                        if done is not None and q == TH // n - 1:
                            done(4 * h + 2 * a + b)
                        yield

        NE = 4 * TH // EROWS
        mark('s8_q0')
        fb = NF - (NTILE - 1) * FL
        res0 = None
        _schedule(clock, (q_post(0, half_v, oba_v.at[0], phi_v), 40, 0.0, 1.0))

        def q_tile(j, carry):
            SKIP[0] = False
            last_product[:] = []
            oba = oba_v.at[pl.ds(j, 2)]
            obb = obb_v.at[zero_s[0]]
            x = tokens(tile(j + 1))
            for cp in cp_ffn(j + 1):
                cp.wait()
            fg = ffn(j * FL, FL)
            q0, o0, o1 = ([[None] * 4 for _ in range(4)] for _ in range(3))
            nf, no = P["nffn"], 7 * 256 // P["on"]
            _schedule(clock, project((a_v.at[2], aa_v.at[0]), x, q0),
                      (q_post(1, raw_v.at[1], obb_v.at[0]), 40, *P["p1"]), (fg, nf[0], *P["f0"]))
            _schedule(clock, (out_project(0, oba.at[0], obb, o0), no, 0.0, 1.0),
                      (q_post(0, q0, oba.at[1]), 40, *P["p0"]), (fg, nf[1], *P["f1"]))
            _schedule(clock, (out_project(1, oba.at[0], obb, o1), no, 0.0, 1.0),
                      (epilogue(tile(j), 0, o0), NE, *P["e0"]), (fg, nf[2], *P["f2"]))
            _schedule(clock, project((a_v.at[3], aa_v.at[1]), x, raw_v.at[1]),
                      (epilogue(tile(j), 1, o1), NE, *P["e1"]), (fg, 12 * FL - sum(nf), *P["f3"]))
            cp_o(j, tile(j)).start()
            return carry

        mark('s9_phase2')
        if ONLY != 'p1':
            lax.fori_loop(0, NTILE - 1, q_tile, 0)
        SKIP[0] = ONLY is not None
        if ONLY:
            keep = sum(jnp.sum(pltpu.bitcast(r[(0,) * (len(r.shape) - 2) + (pl.ds(pl.multiple_of(zero_s[0], 16), 16), slice(0, 128))], f32))
                       for r in (xb_v, xx_v, a_v, aa_v, wo_v, kvb_v, raw_v, half_v, phi_v, xcol_v, oba_v, obb_v))
            out_v[0:16, 0:128] = jnp.full((16, 128), keep + jnp.sum(y_acc[...]) + jnp.sum(best_v[...]), f32).astype(bf16)
        mark('sa_tail')

        j = NTILE - 1
        rate[0] = 14
        last_product[:] = []
        oba, obb = oba_v.at[j], obb_v.at[zero_s[0]]
        _schedule(clock, (out_project(0, oba, obb, part_v.at[0], (0,), TORD, 256), 7, 0.0, 0.5),
                  (out_project(1, oba, obb, part_v.at[1], (0,), TORD, 256), 7, 0.5, 1.0),
                  (q_post(1, raw_v.at[1], obb_v.at[0]), 40, 0.0, TQ),
                  (ffn(NF - fb, fb), 12 * fb, 0.1, 0.8))
        upd = jnp.sum(y_acc[...], axis=0, keepdims=True) * (0.5 * jax.nn.sigmoid(rmax[:, 0:1]))
        o0, o1 = ([[None, None], [None, None]] for _ in range(2))
        t = tile(j)
        send = lambda blk: cp_o_blk(t, blk).start()
        e0 = epilogue(t, 0, o0, part_v.at[0], upd, send, TORD)
        e1 = epilogue(t, 1, o1, part_v.at[1], upd, send, TORD)
        _schedule(clock, (out_project(0, oba, obb, o0, (1,), TORD, 256), 7, 0.0, 0.5),
                  (out_project(1, oba, obb, o1, (1,), TORD, 256), 7, 0.5, 1.0),
                  (e0, NE, *E0), (e1, NE, *E1))
        mark('sb_outdma')
        for k in range(NTILE - 1):
            cp_o(k, tile(k)).wait()
        for blk in range(8):
            cp_o_blk(t, blk).wait()
        mark(None)

    scratch = [
        pltpu.VMEM((S + T + 4 * D, D), bf16),
        pltpu.VMEM((NTILE + 1, 2, T, 128), f32),
        pltpu.VMEM((NTILE + 1, 7, 128, 512), u32),
        pltpu.VMEM((NTILE + 1, 35, 64, 256), u32),
        pltpu.VMEM((D, DH), bf16),
        pltpu.VMEM((8, 128), bf16),
        pltpu.VMEM((16, D), f32),
        pltpu.VMEM((8, 128, 128), bf16),
        pltpu.VMEM((4, 7, 128, 512), u32),
        pltpu.VMEM((2, 35, 64, 256), u32),
        pltpu.VMEM((2, 7, 128, 512), u32),
        pltpu.VMEM((2, 35, 64, 256), u32),
        pltpu.VMEM((2, 7, 128, 512), u32),
        pltpu.VMEM((NF, D, 128), bf16),
        pltpu.VMEM((NF, D, 128), bf16),
        pltpu.VMEM((D // 128, F, 128), bf16),
        pltpu.VMEM((H // 2 + 4, 64, 128), f32),
        pltpu.VMEM((H // 2 + 4, 128, 128), f32),
        pltpu.VMEM((H // 2 + 4, 80, 128), bf16),
        pltpu.VMEM((2, 16, 128), f32),
        pltpu.VMEM((2, 16, 128), i32),
        pltpu.VMEM((2, 4, 4, 128, 128), f32),
        pltpu.VMEM((4, 4, 64, 128), f32),
        pltpu.VMEM((4, 64, T), u32),
        pltpu.VMEM((NTILE, 7, TH // 2, 256), u32),
        pltpu.VMEM((2, 7, TH // 2, 256), u32),
        pltpu.VMEM((2, 2, 2, 256, 256), f32),
        pltpu.VMEM((D, 128), f32),
        pltpu.VMEM((8, D), f32),
        pltpu.VMEM((S, D), bf16),
        pltpu.SMEM((1,), i32),
        pltpu.SemaphoreType.DMA((NTILE + 2,)),
        pltpu.SemaphoreType.DMA((11,)),
        pltpu.SemaphoreType.DMA((1,)),
        pltpu.SemaphoreType.DMA((NTILE,)),
        pltpu.SemaphoreType.DMA((1,)),
    ]

    def call(x, wqkv, wphi, wo, wr, wg, wu, wd):
        hbm = pl.BlockSpec(memory_space=pltpu.HBM)
        return pl.pallas_call(
            kernel,
            out_shape=jax.ShapeDtypeStruct((S, D), bf16),
            in_specs=[hbm] * 8,
            out_specs=hbm,
            scratch_shapes=scratch,
            compiler_params=pltpu.CompilerParams(vmem_limit_bytes=120 * 2**20, flags=FLAGS, disable_bounds_checks=NOBC, disable_semaphore_checks=NOSEM),
            name="hedgehog", interpret=INTERP,
        )(x, wqkv, wphi, wo, wr, wg, wu, wd)

    return call


@jax.jit
def pallas_recurrent_scan__linear_kernel_hedgehog__moe_arch_mod__prompt_kernel(
    A_x: jax.Array,
    A_wqkv: jax.Array,
    A_w_phi: jax.Array,
    A_wo: jax.Array,
    B_x: jax.Array,
    B_w_r: jax.Array,
    B_w_gate: jax.Array,
    B_w_up: jax.Array,
    B_w_down: jax.Array,
):
    del B_x
    out = make_kernel()(
        A_x.reshape(S, D), A_wqkv, A_w_phi.reshape(D, DH), A_wo,
        B_w_r.reshape(8, 128), B_w_gate, B_w_up, B_w_down)
    return out.reshape(1, S, D)
```

```python
import math
import contextlib

import numpy as np

import jax
import jax.numpy as jnp
from jax import lax
import jax.experimental.pallas as pl
import jax.experimental.pallas.tpu as pltpu

S, D, H, DH, F = 2048, 1024, 32, 32, 3584
T = 512
TH = T // 2
NTILE = S // T
NF = F // 128
FG = NF // NTILE
WQ, WK, WV, WO = (S + T + j * D for j in range(4))
LHS_SUMS, RHS_SUMS = (0, 1, 4, 5, 6), (0, 2, 3, 5, 6)
LOG2E = math.log2(math.e)
EPS_BF16 = float(np.float32(1e-5).astype(jnp.bfloat16))
NT_DIMS = (((1,), (1,)), ((), ()))
f32, bf16, i32, u32 = jnp.float32, jnp.bfloat16, jnp.int32, jnp.uint32


def _dot_nt(a, b):
    return lax.dot_general(a, b, NT_DIMS, preferred_element_type=f32)


def _dot(a, b):
    return jnp.dot(a, b, preferred_element_type=f32)


def aligned(i, n):
    return i if isinstance(i, int) else pl.multiple_of(i, n)


def _recip(v):
    r = pl.reciprocal(v, approx=True)
    return r * (2.0 - v * r)


def _wide(w):
    return pltpu.bitcast(w, bf16).astype(f32)


def _narrow(v):
    return pltpu.bitcast(v.astype(bf16), u32)


def _lhs_combos(a11, a12, a21, a22):
    return [a11 + a22, a21 + a22, a11, a22, a11 + a12, a21 - a11, a12 - a22]


def _rhs_combos(b11, b12, b21, b22):
    return [b11 + b22, b11, b12 - b22, b21 - b11, b22, b11 + b12, b21 + b22]


class _Quad:
    def __init__(self, v):
        self.v = v

    def __add__(self, o):
        return _Quad([p + q for p, q in zip(self.v, o.v)])

    def __sub__(self, o):
        return _Quad([p - q for p, q in zip(self.v, o.v)])


def _strassen2(prod, emit, order):
    done = {}

    def inner(i):
        out = [None] * 4

        def put(a, b, val):
            out[2 * a + b] = val
        yield from _strassen(lambda j: prod(7 * i + j), put, order)
        done[i] = _Quad(out)

    def put(a, b, quad):
        for k, val in enumerate(quad.v):
            emit(2 * a + k // 2, 2 * b + k % 2, val)

    outer = _strassen(lambda i: done[i], put, order)
    for i in ((0, 3, 4, 6, 2, 1, 5), (2, 4, 0, 6, 3, 1, 5))[order]:
        steps = inner(i)
        for _ in range(6):
            next(steps)
            yield
        for _ in steps:
            pass
        next(outer)
        yield


def _strassen(prod, emit, order=0):
    if order == 0:
        m1 = prod(0)
        yield
        m4 = prod(3)
        c11 = m1 + m4
        yield
        m5 = prod(4)
        c11 = c11 - m5
        yield
        emit(0, 0, c11 + prod(6))
        yield
        m3 = prod(2)
        emit(0, 1, m3 + m5)
        c22 = m1 + m3
        yield
        m2 = prod(1)
        emit(1, 0, m2 + m4)
        c22 = c22 - m2
        yield
        emit(1, 1, c22 + prod(5))
        yield
    else:
        m3 = prod(2)
        yield
        m5 = prod(4)
        emit(0, 1, m3 + m5)
        yield
        m1 = prod(0)
        c11, c22 = m1 - m5, m1 + m3
        yield
        c11 = c11 + prod(6)
        yield
        m4 = prod(3)
        emit(0, 0, c11 + m4)
        yield
        m2 = prod(1)
        emit(1, 0, m2 + m4)
        c22 = c22 - m2
        yield
        emit(1, 1, c22 + prod(5))
        yield


SKIP = [False]


def _schedule(clock, *streams):
    if SKIP[0]:
        return
    events = []
    for order, (gen, n, a, b) in enumerate(streams):
        for k in range(n):
            events.append((a + (b - a) * k / n, order, k, gen))
    for when, _, _, gen in sorted(events, key=lambda e: e[:3]):
        clock[:] = [when]
        next(gen)


def _dual_softmax(p, zero=None):
    rows = [p[8 * j:8 * j + 8] for j in range(8)]
    if zero is not None:
        rows[0] = rows[0] + zero

    def reduce(vs, op):
        while len(vs) > 1:
            vs = [op(vs[i], vs[i + 1]) for i in range(0, len(vs), 2)]
        v = op(vs[0], pltpu.roll(vs[0], 4, 0))
        return op(v, pltpu.roll(v, 2, 0))

    mx, mn = reduce(rows, jnp.maximum), reduce(rows, jnp.minimum)
    ep = [jnp.exp2(v - mx) for v in rows]
    en = [jnp.exp2(mn - v) for v in rows]
    rp, rn = _recip(reduce(ep, jnp.add)), _recip(reduce(en, jnp.add))
    return jnp.concatenate([v * rp for v in ep] + [v * rn for v in en], axis=0)


PLAN = dict(
    kv=(0.08, 0.905), stats=(0.0, 0.96), apply=(0.015, 0.935), fold=(0.06, 0.915), fold2=(0.075, 0.84), nfold=0,
    trans=(0.085, 0.875), routed=(0.04, 0.89), split=(0.005, 1.0), split2=(0.09, 0.97), nsplit=56,
    again=(0.0, 1.0), again2=(0.0, 0.9), nagain=42, o1=0,
    p1=(0.0, 1.0), p0=(0.065, 1.0), e0=(0.055, 0.96), e1=(0.0, 0.985), nffn=(14, 18, 38),
    f0=(0.125, 0.945), f1=(0.165, 0.945), f2=(0.02, 1.0), f3=(0.0, 0.925), oq=1, oo=1, on=256,
)


def make_kernel(FLAGS=None, FL=9, W0=0.15, WS=0.6, WK0=(0.52, 1.3), W1=0.75, K2=(1.05, 1.3), S2=(1.31, 1.62), K3=(1.5, 1.72), S3=(1.73, 2.0), TORD=1, NOSEM=False, E0=(0.2, 0.7), E1=(0.7, 1.2),
                TPIN=False, TQ=0.9, NOBC=True, EROWS=32, SCOPES=False, ONLY=None, TW=(2, 3), INTERP=False,
                DMA_ORDER='a0 a1 a2 a3 k0 v0 k1 v1 k2 v2 k3 v3 x1 f0 x2 f1 o0 x3 f2 o1 x4 f3'.split(), **over):
    P = dict(PLAN, **over)
    FPIN = True

    stack = []
    def mark(name):
        if not SCOPES: return
        if stack: stack.pop().__exit__(None, None, None)
        if name:
            cm = jax.named_scope(name); cm.__enter__(); stack.append(cm)

    def kernel(x_hbm, wqkv_hbm, wphi_hbm, wo_hbm, wr_hbm, wg_hbm, wu_hbm, wd_hbm,
               out_hbm,
               in_v, st_v, xb_v, xx_v, wphi_v, wr8_v, wr_v, lm_v, a_v, aa_v, b_v, bb_v, wo_v, ffn_v,
               kv_acc, z_acc, kvb_v, best_v, best_i, raw_v, half_v, phi_v, oba_v, obb_v, part_v, xcol_v, y_acc,
               out_v, zero_s, sem_x, sem_w, sem_s, sem_f, sem_o):
        def cp_x(r0, n, sem, src0=None):
            src0 = r0 if src0 is None else src0
            return pltpu.make_async_copy(x_hbm.at[pl.ds(src0, n)], in_v.at[pl.ds(r0, n)], sem_x.at[sem])

        def cp_x0(piece):
            return cp_x((piece % 2) * TH + (piece // 2) * (TH // 2), TH // 2, 0 if piece < 2 else NTILE + 1)

        def cp_xt(t):
            return cp_x(pl.multiple_of(t * T, T), T, t, pl.multiple_of((t % NTILE) * T, T))

        def cp_w(j, c0, n, sem):
            src = wo_hbm.at[:, pl.ds(c0, n)] if j == 3 else wqkv_hbm.at[:, pl.ds(aligned(j * D + c0, 128), n)]
            return pltpu.make_async_copy(src, in_v.at[pl.ds(WQ + j * D, D), pl.ds(c0, n)], sem_w.at[sem])

        def cp_k(c):
            return cp_w(1, c * 256, 256, c)

        def cp_v(c):
            return cp_w(2, c * 256, 256, c if c else 4)

        def start_q(u):
            for n in range(8):
                src = wqkv_hbm.at[pl.ds((n // 2) * 256 + (u % 2) * 128, 128), pl.ds((u // 2) * 256 + (n % 2) * 512, 256)]
                pltpu.make_async_copy(src, in_v.at[pl.ds(WQ + (u // 2) * 512 + (n // 2) * 128, 128),
                                                   pl.ds((u % 2) * 512 + (n % 2) * 256, 256)], sem_w.at[5 + u]).start()

        def q_blocks(u):
            return in_v.at[pl.ds(aligned(WQ + (u // 2) * 512, 512), 512), pl.ds(aligned((u % 2) * 512, 512), 512)]

        def wait_all(filled, sem):
            pltpu.make_async_copy(filled, filled, sem).wait()

        def cp_wo(h):
            return cp_w(3, aligned(h * 512, 512), 512, 9 + h)

        cp_phi = pltpu.make_async_copy(wphi_hbm, wphi_v, sem_s.at[0])
        cp_wr = pltpu.make_async_copy(wr_hbm, wr8_v, sem_s.at[0])
        def start_ffn(g):
            for j in range(FG):
                cols = pl.ds(aligned((g * FG + j) * 128, 128), 128)
                for n, src in enumerate((wg_hbm, wu_hbm)):
                    pltpu.make_async_copy(src.at[:, cols], ffn_v.at[g, pl.ds((n * FG + j) * D, D)], sem_f.at[g]).start()
                    yield
            rows = pl.ds(aligned(g * FG * 128, 128), FG * 128)
            for n in range(D // 128):
                pltpu.make_async_copy(wd_hbm.at[rows, pl.ds(n * 128, 128)],
                                      ffn_v.at[g, pl.ds(2 * FG * D + n * FG * 128, FG * 128)], sem_f.at[g]).start()
                yield

        def cp_o(k, t):
            rows = pl.ds(pl.multiple_of(t * T, T), T)
            return pltpu.make_async_copy(out_v.at[rows], out_hbm.at[rows], sem_o.at[0])

        def cp_o_blk(t, blk):
            rows = pl.ds(pl.multiple_of(t * T + (blk % 2) * TH, TH), TH)
            cols = pl.ds((blk // 2) * 256, 256)
            return pltpu.make_async_copy(out_v.at[rows, cols], out_hbm.at[rows, cols], sem_o.at[0])

        cp_wr.start()
        cp_phi.start()
        for n, name in enumerate(DMA_ORDER):
            if n == 1:
                cp_wr.wait()
                cp_phi.wait()
            if name[0] == "f":
                start_q(int(name[1]))
            else:
                {"a": cp_x0, "k": cp_k, "v": cp_v, "x": cp_xt, "o": cp_wo}[name[0]](int(name[1])).start()

        last_product = []

        clock = [0.0]
        rate = [7]

        def pin(n=8):
            if not last_product:
                return jnp.zeros((n, 128), f32)
            rows, cols = last_product[0].shape[0] // 8, last_product[0].shape[1] // 128
            q = min(int((clock[0] * last_product[1]) % 1.0 * rows * cols + 1e-6), rows * cols - 1)
            m = last_product[0][(q % rows) * 8:(q % rows) * 8 + 8, (q // rows) * 128:(q // rows) * 128 + 128]
            z = pltpu.bitcast(pltpu.bitcast(m, u32) & zero_s[0].astype(u32), f32)
            return z if n == 8 else jnp.concatenate([z] * (n // 8), axis=0)

        def as_bf16(w):
            return pltpu.bitcast(w, bf16)

        def feature_maps():
            rho = lax.broadcasted_iota(i32, (128, DH), 0)
            sel = (((rho % 64) // 8) * 4 + (rho % 8) // 2 == lax.broadcasted_iota(i32, (128, DH), 1)).astype(bf16)
            rho = lax.broadcasted_iota(i32, (128, 128), 0)
            keep = (rho // 64) * 2 + rho % 2 == lax.broadcasted_iota(i32, (128, 128), 1) // DH
            for g in range(8):
                full = _dot_nt(sel, wphi_v[pl.ds(g * 128, 128), :])
                lm_v.at[g][...] = jnp.where(keep, full, 0.0).astype(bf16)

        def operand(chunk):
            return a_v.at[chunk] if chunk < 2 else b_v.at[chunk - 2]

        def put_lhs(dst, rows, cols, *quadrants):
            for i, v in enumerate(_lhs_combos(*quadrants)):
                dst.at[i][rows, cols] = _narrow(v)

        def split_again(src, dst, lhs, r, k):
            for i in range(7):
                zero = pltpu.bitcast(pin(), u32)
                w = [[src[i, pl.ds(h * 64 + r * 8, 8), pl.ds(aligned(c * 256 + k * 128, 128), 128)]
                      for c in range(2)] for h in range(2)]
                q00, q01, q10, q11 = _wide(w[0][0] | zero), _wide(w[0][1]), _wide(w[1][0]), _wide(w[1][1] | zero)
                cmb = _lhs_combos(q00, q01, q10, q11) if lhs else _rhs_combos(q00, q10, q01, q11)
                for n, j in enumerate(LHS_SUMS if lhs else RHS_SUMS):
                    dst.at[5 * i + n][pl.ds(r * 8, 8), pl.ds(aligned(k * 128, 128), 128)] = _narrow(cmb[j])
                yield

        def second(src, dst, lhs, ij):
            i, j = ij // 7, ij % 7
            sums = LHS_SUMS if lhs else RHS_SUMS
            if j in sums:
                return as_bf16(dst[5 * i + sums.index(j)])
            d = int(j == (3 if lhs else 4))
            return as_bf16(src[i, pl.ds(d * 64, 64), pl.ds(d * 256, 256)])

        def w_blocks(base, top, bot, k):
            return [in_v[pl.ds(aligned(base + kh * 512 + k * 128, 128), 128),
                         pl.ds(aligned(g * 128, 128), 128)] for g in (top, bot) for kh in range(2)]

        def prep_fold(blocks_of, top, bot, dst, row_of, ks):
            for k in ks:
                blocks = [_dot_nt(lm_v[g], w) for g, w in zip((top, top, bot, bot), blocks_of(k))]
                for j in range(8):
                    put_lhs(dst, pl.ds(aligned(row_of(j), 8), 8), pl.ds(aligned(k * 128, 128), 128),
                            *[p[16 * j:16 * j + 16] * LOG2E for p in blocks])
                yield

        def prep_transpose(base, top, bot, dst, row_of):
            for k in range(4):
                zero = pltpu.bitcast(pin(64), u32)
                blocks = [as_bf16(pltpu.bitcast(w, u32) | zero).T for w in w_blocks(base, top, bot, k)]
                for j in range(8):
                    put_lhs(dst, pl.ds(aligned(row_of(j), 8), 8), pl.ds(k * 128, 128),
                            *[w[16 * j:16 * j + 16].astype(f32) for w in blocks])
                yield

        def prep_q(u):
            ch, k, w = u // 2, u % 2, q_blocks(u)
            for half in range(2):
                g = 2 * ch + half
                for c in range(2):
                    blocks = [w[pl.ds((2 * kh + c) * 128, 128), pl.ds(a * 256 + half * 128, 128)]
                              for a in range(2) for kh in range(2)]
                    yield from prep_fold(lambda _: blocks, g, g + 4, a_v.at[2 + ch],
                                         lambda j: half * 64 + 8 * j, (k + 2 * c,))

        def split_q(u):
            for r in range(8):
                yield from split_again(a_v.at[2 + u // 2 + zero_s[0]], aa_v.at[u // 2], True, r, u % 2)

        def prep_wo(u, base=WO):
            g = (u // 2) * 4 + u % 2
            return prep_transpose(base, g, g + 2, wo_v.at[u // 2], lambda j: (u % 2) * 64 + 8 * j)

        def x_block(r0, c0):
            return in_v[pl.ds(r0, 16), pl.ds(c0, 128)].astype(f32)

        def ln_stats(t, st):
            for step in range(32):
                pos = (step % 2) * 16 + step // 2
                r0 = pl.multiple_of(t * T + pos * 16, 16)
                x0 = x_block(r0, 0) + pin(16)
                s1 = s2 = None
                for j in range(1, 8):
                    d = x_block(r0, j * 128) - x0
                    s1 = d if j == 1 else s1 + d
                    s2 = d * d if j == 1 else s2 + d * d
                lane_mean = x0 + s1 * 0.125
                m = jnp.sum(lane_mean, axis=-1, keepdims=True) * (1.0 / 128)
                dm = lane_mean - m
                v = jnp.sum((s2 - s1 * s1 * 0.125) * 0.125 + dm * dm, axis=-1, keepdims=True) * (1.0 / 128)
                vb = (v.astype(bf16).astype(f32) + EPS_BF16).astype(bf16).astype(f32)
                st[0, pl.ds(pos * 16, 16), :] = jnp.broadcast_to(m.astype(bf16).astype(f32), (16, 128))
                st[1, pl.ds(pos * 16, 16), :] = jnp.broadcast_to(1.0 / jnp.sqrt(vb).astype(bf16).astype(f32), (16, 128))
                yield

        def ln_apply(t, st, xb, score_too):
            for step in range(16):
                r0 = [pl.multiple_of(t * T + hf * TH + step * 16 + zero_s[0], 16) for hf in range(2)]
                mean = [st[0, pl.ds(hf * TH + step * 16, 16), :] for hf in range(2)]
                scale = [st[1, pl.ds(hf * TH + step * 16, 16), :] for hf in range(2)]
                score = [None, None]
                for k in range(4):
                    zero = pin(16)
                    xn = [[(x_block(r0[hf], kh * 512 + k * 128) - (mean[hf] + zero)) * scale[hf]
                           for kh in range(2)] for hf in range(2)]
                    for i, v in enumerate(_rhs_combos(xn[0][0], xn[1][0], xn[0][1], xn[1][1])):
                        xb.at[i][pl.ds(step * 8, 8), pl.ds(k * 128, 128)] = _narrow(v)
                    for hf in range(2 if score_too else 0):
                        part = (xn[hf][0] * wr_v[:, pl.ds(k * 128, 128)]
                                + xn[hf][1] * wr_v[:, pl.ds(512 + k * 128, 128)])
                        score[hf] = part if k == 0 else score[hf] + part
                        if k == 3:
                            r = jnp.sum(score[hf], axis=-1, keepdims=True).astype(bf16).astype(f32)
                            r = jnp.broadcast_to(r, (16, 128))
                            slot = 2 * (t // NTILE) + hf
                            up = r > best_v[slot]
                            best_v[slot] = jnp.where(up, r, best_v[slot])
                            best_i[slot] = jnp.where(up, lax.broadcasted_iota(i32, (16, 128), 0) + r0[hf] % S, best_i[slot])
                    yield

        def ln_split(xb, xx):
            for r in range(8):
                for k in range(2):
                    yield from split_again(xb, xx, False, r, k)

        def project(w, x, res, keep=None):
            def emit(r, b, val):
                if isinstance(res, list):
                    res[r][b] = val
                else:
                    res[r, b] = val
                if keep is not None:
                    keep[r, b] = val[64:]

            def prod2(ij):
                m = _dot_nt(second(*w, True, ij), second(*x, False, ij))
                last_product[:] = [m, 49]
                return m

            def once():
                for c in range(2):
                    def prod(i):
                        m = _dot_nt(as_bf16(w[i]), as_bf16(x[i, pl.ds(c * 64, 64), :]))
                        last_product[:] = [m, 14]
                        return m

                    def put(a, b, val):
                        emit(2 * a, 2 * b + c, val[:128])
                        emit(2 * a + 1, 2 * b + c, val[128:])

                    yield from _strassen(prod, put, P["o1"])

            if isinstance(w, tuple):
                return _strassen2(prod2, emit, P["oq"]), 49, 0.0, 1.0
            return once(), 14, 0.0, 1.0

        def project_part(w, x, res, part):
            def prod(i):
                lhs = jnp.concatenate([w[i, pl.ds(h * 64 + part * 32, 32), :] for h in range(2)], axis=0)
                m = _dot_nt(as_bf16(lhs), as_bf16(x[i]))
                last_product[:] = [m, 14]
                return m

            def put(a, b, val):
                for h in range(2):
                    for c in range(2):
                        res[2 * a + h, 2 * b + c, pl.ds(part * 64, 64), :] = val[h * 64:(h + 1) * 64, c * 128:(c + 1) * 128]

            return _strassen(prod, put, P["o1"])

        def raw_blk(res, r, r0, lane):
            if isinstance(res, list):
                return res[r][lane][r0:r0 + 64]
            return res[r, lane, pl.ds(r0, 64), :]

        keep_kv = lax.broadcasted_iota(i32, (64, 128), 0) // DH == lax.broadcasted_iota(i32, (64, 128), 1) % 2
        keep_z = lax.broadcasted_iota(i32, (16, 128), 0) // 8 == lax.broadcasted_iota(i32, (16, 128), 1) % 2

        def kv_post(c, res, keep=None, late=False):
            def accumulate(p, quarter, phi):
                vt = jnp.concatenate([raw_blk(res, quarter, 64, l) for l in range(4)], axis=1).astype(bf16)
                kv = kv_acc[p] + _dot_nt(vt, phi)
                kv_acc[p] = kv
                kvb_v.at[p][pl.ds(0, 64), :] = jnp.where(keep_kv, kv, 0.0).astype(bf16)

            pending = []
            for a in range(2):
                for pr in range(2):
                    p = 4 * c + 2 * a + pr
                    phis, zs = [], z_acc[p]
                    for lane in range(4):
                        phi = _dual_softmax(raw_blk(res, 2 * a + pr, 0, lane), pin())
                        zs = zs + phi
                        phis.append(phi)
                        if keep is not None:
                            keep.at[2 * a + pr][:, pl.ds(lane * 128, 128)] = _narrow(phi)
                        if lane == 1 and pending and (a or not late):
                            accumulate(*pending.pop(0))
                        if lane == 3:
                            z_acc[p] = zs
                            zrow = jnp.broadcast_to(jnp.sum(zs.T, axis=0, keepdims=True), (16, 128))
                            kvb_v.at[p][pl.ds(64, 16), :] = jnp.where(keep_z, zrow, 0.0).astype(bf16)
                            pending.append((p, 2 * a + pr, jnp.concatenate(phis, axis=1).astype(bf16)))
                        yield
            yield
            for rest in pending:
                accumulate(*rest)
            yield

        def route():
            best, tok = best_v[...].reshape(64, 128), best_i[...].reshape(64, 128)
            rmax = jnp.max(best, axis=0, keepdims=True)
            idx = jnp.min(jnp.where(best == rmax, tok, S).astype(f32)).astype(i32)
            return jnp.clip(idx, 0, S - 1), rmax

        def routed_token():
            idx = route()[0]
            base = pl.multiple_of((idx // 16) * 16, 16)
            rows = pl.ds(pl.multiple_of(base % T, 16), 16)
            xn = (in_v[pl.ds(base, 16), :].astype(f32) - st_v[idx // T, 0, rows, 0:1]) * st_v[idx // T, 1, rows, 0:1]
            xsel = jnp.where(lax.broadcasted_iota(i32, (16, D), 0) == idx - base, xn, 0.0)
            xsel = jnp.sum(xsel, axis=0, keepdims=True).astype(bf16).astype(f32)
            for j in range(8):
                row = xsel[:, j * 128:(j + 1) * 128] + pin()
                xcol_v[pl.ds(j * 128, 128), :] = jnp.concatenate([row] * 16, axis=0).T
                yield

        SKIP[0] = ONLY is not None
        mark('s0_init')
        zero_s[0] = 0
        kv_acc[...] = jnp.zeros(kv_acc.shape, f32)
        z_acc[...] = jnp.zeros(z_acc.shape, f32)
        y_acc[...] = jnp.zeros(y_acc.shape, f32)
        best_v[...] = jnp.full(best_v.shape, -jnp.inf, f32)
        best_i[...] = jnp.zeros(best_i.shape, i32)
        w8 = wr8_v[...].astype(f32)
        wr_v[...] = jnp.broadcast_to(jnp.concatenate([w8[j:j + 1, :] for j in range(8)], axis=1), (16, D))
        feature_maps()
        mark('s1_ln0')
        stats, apply = ln_stats(0, st_v.at[0]), ln_apply(0, st_v.at[0], xb_v.at[0], False)
        cp_x0(0).wait()
        cp_x0(1).wait()
        _schedule(clock, (stats, 16, 0.0, 1.0))
        _schedule(clock, (apply, 32, 0.0, 1.0))
        cp_x0(2).wait()
        cp_x0(3).wait()
        _schedule(clock, (stats, 16, 0.0, 1.0))
        _schedule(clock, (apply, 32, 0.0, 1.0))

        def prep_kv(c):
            cp_k(c).wait()
            if c:
                cp_v(c).wait()
            once = operand(c)
            yield from prep_fold(lambda k: w_blocks(WK, 2 * c, 2 * c + 1, k), 2 * c, 2 * c + 1, once, lambda j: (j // 4) * 64 + (j % 4) * 8, range(4))
            if not c:
                cp_v(c).wait()
            yield from prep_transpose(WV, 2 * c, 2 * c + 1, once, lambda j: (j // 4) * 64 + 32 + (j % 4) * 8)

        def split_kv(c):
            for k in range(2):
                for r in range(8):
                    yield from split_again(b_v.at[c - 2 + zero_s[0]], bb_v.at[c - 2], True, r, k)

        mark('s3_prep0')
        first_chunk = prep_kv(0)
        _schedule(clock, (first_chunk, 4, 0.0, 1.0))
        mark('s4_proj0')
        next_chunk = project(operand(1), xb_v.at[0], raw_v.at[1])[0]
        _schedule(clock, (project_part(operand(0), xb_v.at[0], raw_v.at[0], 0), 7, 0.0, 0.5),
                  (project_part(operand(0), xb_v.at[0], raw_v.at[0], 1), 7, 0.5, 1.0), (next_chunk, 14, 1.0, 2.0),
                  (first_chunk, 4, W0, 0.45), (ln_split(xb_v.at[zero_s[0]], xx_v.at[0]), 112, 0.03, WS),
                  (kv_post(0, raw_v.at[zero_s[0]], late=True), 18, *WK0),
                  (prep_kv(1), 8, W1, 1.0), (prep_kv(2), 8, *K2), (split_kv(2), 112, *S2), (prep_kv(3), 8, *K3), (split_kv(3), 112, *S3))

        def kv_tile(t, _):
            SKIP[0] = False
            last = t == NTILE - 1
            wait_all(q_blocks(t), sem_w.at[5 + t])
            cp_xt(t + 1).wait()

            @pl.when(jnp.logical_and(t > 0, t < 3))
            def _():
                cp_wo(t - 1).wait()

            if not NOBC:
                for g in range(NTILE):
                    @pl.when(t == g)
                    def _():
                        for _ in start_ffn(g):
                            pass

            last_product[:] = []
            first = (route()[0] // T) % (NTILE - 1) + 1
            xb, st = xb_v.at[pl.ds(t, 2)], st_v.at[t + 1]
            stats, apply = ln_stats(t + 1, st), ln_apply(t + 1, st, xb.at[1], True)
            xx = xx_v.at[pl.ds(t, 2)]
            split = ln_split(xb_v.at[t + 1 + zero_s[0]], xx.at[1]) if TW else ln_split(xb.at[0], xx.at[0])
            slot = lambda c: ((operand(c), bb_v.at[c - 2]), (xb.at[0], xx.at[0])) if c in TW else (operand(c), xb.at[0])
            fold = prep_q(t)
            trans = [prep_wo(2 * ((t + 1) % 2) + u, jnp.where(t == 0, WV, WO)) for u in range(2)]

            c2, c3, c0 = ([[None] * 4 for _ in range(4)] for _ in range(3))
            _schedule(clock, project(*slot(2), c2), (kv_post(1, raw_v.at[1]), 18, *P["kv"]),
                      (stats, 32, *P["stats"]), (fold, P["nfold"], *P["fold"]),
                      (start_ffn(t), 2 * FG + 8 if NOBC else 0, 0.05, 0.95))
            _schedule(clock, project(*slot(3), c3), (kv_post(2, c2), 18, *P["kv"]),
                      (apply, 64, *P["apply"]), (fold, 4 - P["nfold"], *P["fold2"]))
            x = xb_v.at[jnp.where(last, first, t + 1)]
            chunk = jnp.where(last, 2, 0)
            again = split_q(t)
            _schedule(clock, project(a_v.at[chunk], x, c0, keep=half_v), (kv_post(3, c3), 18, *P["kv"]),
                      (trans[0], 4, *P["trans"]), (routed_token(), 8, *P["routed"]),
                      (split, P["nsplit"], *P["split"]), (again, P["nagain"], *P["again"]))
            _schedule(clock, project(a_v.at[chunk + 1], x, raw_v.at[1]),
                      (kv_post(jnp.where(last, 4, 0), c0, phi_v), 18, *P["kv"]), (trans[1], 4, *P["trans"]),
                      (split, 112 - P["nsplit"], *P["split2"]), (again, 56 - P["nagain"], *P["again2"]))
            return first

        mark('s6_phase1')
        first = lax.fori_loop(0, NTILE, kv_tile, jnp.int32(0)) if ONLY != 'p2' else route()[0] // T
        SKIP[0] = ONLY is not None
        mark('s7_mid')
        wait_all(ffn_v.at[0], sem_f.at[0])
        last_product[:] = []

        idx, rmax = route()

        def ffn(f0, nf):
            for j in range(nf):
                group, tile_in_group = ffn_v.at[(f0 + j) // FG], (f0 + j) % FG
                accs = [jnp.zeros((8, 128), f32)] * 2
                for r in range(8):
                    rows = pl.ds(r * 128, 128)
                    xc = xcol_v[rows, :]
                    if FPIN:
                        zero = pin()
                    for a in range(2):
                        w = group[pl.ds(aligned((a * FG + tile_in_group) * D + r * 128, 128), 128), :]
                        prod = w.astype(f32) * xc
                        acc = accs[a] + zero if FPIN else accs[a]
                        for q in range(16):
                            acc = acc + prod[8 * q:8 * q + 8]
                        accs[a] = acc
                    yield
                gate, up = [jnp.sum(acc, axis=0, keepdims=True) for acc in accs]
                hcol = jnp.broadcast_to(gate * jax.nn.sigmoid(gate) * up, (128, 128)).T
                for n in range(8):
                    ycols = pl.ds(n * 128, 128)
                    w = group[pl.ds(aligned(2 * FG * D + (n * FG + tile_in_group) * 128, 128), 128), :]
                    prod = w.astype(f32) * hcol
                    acc = y_acc[:, ycols] + pin() if FPIN else y_acc[:, ycols]
                    for q in range(16):
                        acc = acc + prod[8 * q:8 * q + 8]
                    y_acc[:, ycols] = acc
                    if n % 2 == 1:
                        yield

        final = idx // T
        lo, hi = jnp.minimum(first, final), jnp.maximum(first, final)
        second_tile = jnp.where(lo > 0, 0, jnp.where(hi > 1, 1, 2))
        third_tile = 6 - first - final - second_tile

        def tile(j):
            return jnp.where(j == 0, first, jnp.where(j == 1, second_tile, jnp.where(j == 2, third_tile, final)))

        def q_post(c, res, ob, ready=None):
            phis, nds, outs = {}, {}, {}
            for tick in range(40):
                step, lane = tick // 4, tick % 4
                if step < 8:
                    u, a, pr = step // 4, (step // 2) % 2, step % 2
                    if ready is not None and pr == 0:
                        phi = None
                    else:
                        phi = _dual_softmax(raw_blk(res, 2 * a + u, 0 if ready is not None else pr * 64, lane), pin())
                    phis.setdefault(step, []).append(phi)
                if 1 <= step < 9 and lane == 1:
                    w = step - 1
                    pair = 2 * (2 * c + w // 4 + 4 * ((w // 2) % 2)) + w % 2
                    phi = phis.pop(w)
                    phi = (as_bf16(ready[2 * ((w // 2) % 2) + w // 4]) if phi[0] is None
                           else jnp.concatenate(phi, axis=1).astype(bf16))
                    nds[w] = _dot(kvb_v[pair], phi)
                if step >= 2 and lane == 0:
                    nd = nds.pop(step - 2)
                    rd = _recip(nd[64:80, :] + 1e-6)
                    outs[step - 2] = jnp.concatenate(
                        [(nd[0:32, :].reshape(4, 8, T) * rd[0:8, :][None]).reshape(32, T),
                         (nd[32:64, :].reshape(4, 8, T) * rd[8:16, :][None]).reshape(32, T)], axis=0)
                    if (step - 2) % 4 == 3:
                        u = (step - 2) // 4
                        o1 = jnp.concatenate([outs.pop(4 * u), outs.pop(4 * u + 1)], axis=0)
                        o2 = jnp.concatenate([outs.pop(4 * u + 2), outs.pop(4 * u + 3)], axis=0)
                        cmb = _rhs_combos(o1[:, :TH], o1[:, TH:], o2[:, :TH], o2[:, TH:])
                        for i in range(7):
                            ob.at[i][:, pl.ds(u * 128, 128)] = pltpu.bitcast(cmb[i].astype(bf16).T, u32)
                yield

        def out_project(h, oba, obb, res, ks=(0, 1), order=P["oo"], n=P["on"]):
            parts = {}
            for c in range(256 // n):
                def prod(i):
                    lhs = jnp.concatenate([(oba, obb)[k][i] for k in ks], axis=1)
                    rhs = wo_v[h, i, pl.ds(c * n // 2, n // 2), pl.ds(ks[0] * 256, len(ks) * 256)]
                    m = _dot_nt(as_bf16(lhs), as_bf16(rhs))
                    last_product[:] = [m, rate[0] * (256 // n)]
                    return m

                def emit(a, b, val):
                    if isinstance(res, list):
                        parts[a, b, c] = val
                        if c == 256 // n - 1:
                            res[a][b] = jnp.concatenate([parts[a, b, cc] for cc in range(256 // n)], axis=1)
                    else:
                        res[a, b, :, pl.ds(c * n, n)] = val

                yield from _strassen(prod, emit, order)

        def epilogue(t, h, res, part=None, upd=None, done=None, order=0):
            n = EROWS
            for a in range(2):
                for b in ((1, 0) if order and a == 0 else (0, 1)):
                    cols = pl.ds(h * 512 + a * 256, 256)
                    for q in range(TH // n):
                        r0 = pl.multiple_of(t * T + b * TH + q * n, n)
                        rows = pl.ds(b * TH + q * n, n)
                        mb, rs = st_v[t, 0, rows, :], st_v[t, 1, rows, :] * 0.5
                        if upd is None or TPIN:
                            mb = mb + pin(n)
                        x = in_v[pl.ds(r0, n), cols].astype(f32)
                        v = (x - jnp.concatenate([mb, mb], axis=1)) * jnp.concatenate([rs, rs], axis=1)
                        if upd is not None:
                            rid = lax.broadcasted_iota(i32, (n, 256), 0)
                            v = v + jnp.where(rid == idx - r0, upd[:, h * 512 + a * 256:h * 512 + (a + 1) * 256], 0.0)
                        g = v + v * jnp.tanh(v)
                        s = res[a][b][q * n:(q + 1) * n]
                        if part is not None:
                            s = s + part[a, b, pl.ds(q * n, n), :]
                        out_v[pl.ds(r0, n), cols] = (x + s * g).astype(bf16)
                        if done is not None and q == TH // n - 1:
                            done(4 * h + 2 * a + b)
                        yield

        NE = 4 * TH // EROWS
        mark('s8_q0')
        fb = NF - (NTILE - 1) * FL
        res0 = None
        _schedule(clock, (q_post(0, half_v, oba_v.at[0], phi_v), 40, 0.0, 1.0))

        def q_tile(j, carry):
            SKIP[0] = False
            last_product[:] = []
            oba = oba_v.at[pl.ds(j, 2)]
            obb = obb_v.at[zero_s[0]]
            x = xb_v.at[tile(j + 1)], xx_v.at[tile(j + 1)]
            wait_all(ffn_v.at[j + 1], sem_f.at[j + 1])
            fg = ffn(j * FL, FL)
            q0, o0, o1 = ([[None] * 4 for _ in range(4)] for _ in range(3))
            nf, no = P["nffn"], 7 * 256 // P["on"]
            _schedule(clock, project((a_v.at[2], aa_v.at[0]), x, q0),
                      (q_post(1, raw_v.at[1], obb_v.at[0]), 40, *P["p1"]), (fg, nf[0], *P["f0"]))
            _schedule(clock, (out_project(0, oba.at[0], obb, o0), no, 0.0, 1.0),
                      (q_post(0, q0, oba.at[1]), 40, *P["p0"]), (fg, nf[1], *P["f1"]))
            _schedule(clock, (out_project(1, oba.at[0], obb, o1), no, 0.0, 1.0),
                      (epilogue(tile(j), 0, o0), NE, *P["e0"]), (fg, nf[2], *P["f2"]))
            _schedule(clock, project((a_v.at[3], aa_v.at[1]), x, raw_v.at[1]),
                      (epilogue(tile(j), 1, o1), NE, *P["e1"]), (fg, 12 * FL - sum(nf), *P["f3"]))
            cp_o(j, tile(j)).start()
            return carry

        mark('s9_phase2')
        if ONLY != 'p1':
            lax.fori_loop(0, NTILE - 1, q_tile, 0)
        SKIP[0] = ONLY is not None
        if ONLY:
            keep = sum(jnp.sum(pltpu.bitcast(r[(0,) * (len(r.shape) - 2) + (pl.ds(pl.multiple_of(zero_s[0], 16), 16), slice(0, 128))], f32))
                       for r in (xb_v, xx_v, a_v, aa_v, wo_v, kvb_v, raw_v, half_v, phi_v, xcol_v, oba_v, obb_v))
            out_v[0:16, 0:128] = jnp.full((16, 128), keep + jnp.sum(y_acc[...]) + jnp.sum(best_v[...]), f32).astype(bf16)
        mark('sa_tail')

        j = NTILE - 1
        rate[0] = 14
        last_product[:] = []
        oba, obb = oba_v.at[j], obb_v.at[zero_s[0]]
        _schedule(clock, (out_project(0, oba, obb, part_v.at[0], (0,), TORD, 256), 7, 0.0, 0.5),
                  (out_project(1, oba, obb, part_v.at[1], (0,), TORD, 256), 7, 0.5, 1.0),
                  (q_post(1, raw_v.at[1], obb_v.at[0]), 40, 0.0, TQ),
                  (ffn(NF - fb, fb), 12 * fb, 0.1, 0.8))
        upd = jnp.sum(y_acc[...], axis=0, keepdims=True) * (0.5 * jax.nn.sigmoid(rmax[:, 0:1]))
        o0, o1 = ([[None, None], [None, None]] for _ in range(2))
        t = tile(j)
        send = lambda blk: cp_o_blk(t, blk).start()
        e0 = epilogue(t, 0, o0, part_v.at[0], upd, send, TORD)
        e1 = epilogue(t, 1, o1, part_v.at[1], upd, send, TORD)
        _schedule(clock, (out_project(0, oba, obb, o0, (1,), TORD, 256), 7, 0.0, 0.5),
                  (out_project(1, oba, obb, o1, (1,), TORD, 256), 7, 0.5, 1.0),
                  (e0, NE, *E0), (e1, NE, *E1))
        mark('sb_outdma')
        pltpu.make_async_copy(out_v, out_hbm, sem_o.at[0]).wait()
        mark(None)

    scratch = [
        pltpu.VMEM((S + T + 4 * D, D), bf16),
        pltpu.VMEM((NTILE + 1, 2, T, 128), f32),
        pltpu.VMEM((NTILE + 1, 7, 128, 512), u32),
        pltpu.VMEM((NTILE + 1, 35, 64, 256), u32),
        pltpu.VMEM((D, DH), bf16),
        pltpu.VMEM((8, 128), bf16),
        pltpu.VMEM((16, D), f32),
        pltpu.VMEM((8, 128, 128), bf16),
        pltpu.VMEM((4, 7, 128, 512), u32),
        pltpu.VMEM((2, 35, 64, 256), u32),
        pltpu.VMEM((2, 7, 128, 512), u32),
        pltpu.VMEM((2, 35, 64, 256), u32),
        pltpu.VMEM((2, 7, 128, 512), u32),
        pltpu.VMEM((NTILE, 3 * FG * D, 128), bf16),
        pltpu.VMEM((H // 2 + 4, 64, 128), f32),
        pltpu.VMEM((H // 2 + 4, 128, 128), f32),
        pltpu.VMEM((H // 2 + 4, 80, 128), bf16),
        pltpu.VMEM((4, 16, 128), f32),
        pltpu.VMEM((4, 16, 128), i32),
        pltpu.VMEM((2, 4, 4, 128, 128), f32),
        pltpu.VMEM((4, 4, 64, 128), f32),
        pltpu.VMEM((4, 64, T), u32),
        pltpu.VMEM((NTILE, 7, TH // 2, 256), u32),
        pltpu.VMEM((2, 7, TH // 2, 256), u32),
        pltpu.VMEM((2, 2, 2, 256, 256), f32),
        pltpu.VMEM((D, 128), f32),
        pltpu.VMEM((8, D), f32),
        pltpu.VMEM((S, D), bf16),
        pltpu.SMEM((1,), i32),
        pltpu.SemaphoreType.DMA((NTILE + 2,)),
        pltpu.SemaphoreType.DMA((11,)),
        pltpu.SemaphoreType.DMA((1,)),
        pltpu.SemaphoreType.DMA((NTILE,)),
        pltpu.SemaphoreType.DMA((1,)),
    ]

    def call(x, wqkv, wphi, wo, wr, wg, wu, wd):
        hbm = pl.BlockSpec(memory_space=pltpu.HBM)
        return pl.pallas_call(
            kernel,
            out_shape=jax.ShapeDtypeStruct((S, D), bf16),
            in_specs=[hbm] * 8,
            out_specs=hbm,
            scratch_shapes=scratch,
            compiler_params=pltpu.CompilerParams(vmem_limit_bytes=120 * 2**20, flags=FLAGS, disable_bounds_checks=NOBC, disable_semaphore_checks=NOSEM),
            name="hedgehog", interpret=INTERP,
        )(x, wqkv, wphi, wo, wr, wg, wu, wd)

    return call


@jax.jit
def pallas_recurrent_scan__linear_kernel_hedgehog__moe_arch_mod__prompt_kernel(
    A_x: jax.Array,
    A_wqkv: jax.Array,
    A_w_phi: jax.Array,
    A_wo: jax.Array,
    B_x: jax.Array,
    B_w_r: jax.Array,
    B_w_gate: jax.Array,
    B_w_up: jax.Array,
    B_w_down: jax.Array,
):
    del B_x
    out = make_kernel()(
        A_x.reshape(S, D), A_wqkv, A_w_phi.reshape(D, DH), A_wo,
        B_w_r.reshape(8, 128), B_w_gate, B_w_up, B_w_down)
    return out.reshape(1, S, D)
```

```python
import math
import contextlib

import numpy as np

import jax
import jax.numpy as jnp
from jax import lax
import jax.experimental.pallas as pl
import jax.experimental.pallas.tpu as pltpu

S, D, H, DH, F = 2048, 1024, 32, 32, 3584
T = 512
TH = T // 2
NTILE = S // T
NF = F // 128
FG = NF // NTILE
WQ, WK, WV, WO = (S + T + j * D for j in range(4))
LHS_SUMS, RHS_SUMS = (0, 1, 4, 5, 6), (0, 2, 3, 5, 6)
LOG2E = math.log2(math.e)
EPS_BF16 = float(np.float32(1e-5).astype(jnp.bfloat16))
NT_DIMS = (((1,), (1,)), ((), ()))
f32, bf16, i32, u32 = jnp.float32, jnp.bfloat16, jnp.int32, jnp.uint32


def _dot_nt(a, b):
    return lax.dot_general(a, b, NT_DIMS, preferred_element_type=f32)


def _dot(a, b):
    return jnp.dot(a, b, preferred_element_type=f32)


def aligned(i, n):
    return i if isinstance(i, int) else pl.multiple_of(i, n)


def _recip(v):
    r = pl.reciprocal(v, approx=True)
    return r * (2.0 - v * r)


def _wide(w):
    return pltpu.bitcast(w, bf16).astype(f32)


def _narrow(v):
    return pltpu.bitcast(v.astype(bf16), u32)


def _lhs_combos(a11, a12, a21, a22):
    return [a11 + a22, a21 + a22, a11, a22, a11 + a12, a21 - a11, a12 - a22]


def _rhs_combos(b11, b12, b21, b22):
    return [b11 + b22, b11, b12 - b22, b21 - b11, b22, b11 + b12, b21 + b22]


class _Quad:
    def __init__(self, v):
        self.v = v

    def __add__(self, o):
        return _Quad([p + q for p, q in zip(self.v, o.v)])

    def __sub__(self, o):
        return _Quad([p - q for p, q in zip(self.v, o.v)])


def _strassen2(prod, emit, order):
    done = {}

    def inner(i):
        out = [None] * 4

        def put(a, b, val):
            out[2 * a + b] = val
        yield from _strassen(lambda j: prod(7 * i + j), put, order)
        done[i] = _Quad(out)

    def put(a, b, quad):
        for k, val in enumerate(quad.v):
            emit(2 * a + k // 2, 2 * b + k % 2, val)

    outer = _strassen(lambda i: done[i], put, order)
    for i in ((0, 3, 4, 6, 2, 1, 5), (2, 4, 0, 6, 3, 1, 5))[order]:
        steps = inner(i)
        for _ in range(6):
            next(steps)
            yield
        for _ in steps:
            pass
        next(outer)
        yield


def _strassen(prod, emit, order=0):
    if order == 0:
        m1 = prod(0)
        yield
        m4 = prod(3)
        c11 = m1 + m4
        yield
        m5 = prod(4)
        c11 = c11 - m5
        yield
        emit(0, 0, c11 + prod(6))
        yield
        m3 = prod(2)
        emit(0, 1, m3 + m5)
        c22 = m1 + m3
        yield
        m2 = prod(1)
        emit(1, 0, m2 + m4)
        c22 = c22 - m2
        yield
        emit(1, 1, c22 + prod(5))
        yield
    else:
        m3 = prod(2)
        yield
        m5 = prod(4)
        emit(0, 1, m3 + m5)
        yield
        m1 = prod(0)
        c11, c22 = m1 - m5, m1 + m3
        yield
        c11 = c11 + prod(6)
        yield
        m4 = prod(3)
        emit(0, 0, c11 + m4)
        yield
        m2 = prod(1)
        emit(1, 0, m2 + m4)
        c22 = c22 - m2
        yield
        emit(1, 1, c22 + prod(5))
        yield


SKIP = [False]


def _schedule(clock, *streams):
    if SKIP[0]:
        return
    events = []
    for order, (gen, n, a, b) in enumerate(streams):
        for k in range(n):
            events.append((a + (b - a) * k / n, order, k, gen))
    for when, _, _, gen in sorted(events, key=lambda e: e[:3]):
        clock[:] = [when]
        next(gen)


def _head_reduce(vs, op):
    while len(vs) > 1:
        vs = [op(vs[i], vs[i + 1]) for i in range(0, len(vs), 2)]
    v = op(vs[0], pltpu.roll(vs[0], 4, 0))
    return op(v, pltpu.roll(v, 2, 0))


def _dual_softmax(p, zero):
    rows = [p[8 * j:8 * j + 8] for j in range(8)]
    rows[0] = rows[0] + zero
    mx, mn = _head_reduce(rows, jnp.maximum), _head_reduce(rows, jnp.minimum)
    ep = [jnp.exp2(v - mx) for v in rows]
    en = [jnp.exp2(mn - v) for v in rows]
    rp, rn = _recip(_head_reduce(ep, jnp.add)), _recip(_head_reduce(en, jnp.add))
    return jnp.concatenate([v * rp for v in ep] + [v * rn for v in en], axis=0)


PLAN = dict(
    kv=(0.08, 0.905), stats=(0.0, 0.96), apply=(0.015, 0.935), fold=(0.06, 0.915), fold2=(0.075, 0.84), nfold=4,
    trans=(0.05, 0.645), routed=(0.025, 0.89), split=(0.0, 0.885), split2=(0.42, 1.0), again=(0.12, 0.965), o1=0,
    p1=(0.0, 1.0), p0=(0.0, 1.0), e0=(0.055, 0.96), e1=(0.0, 0.985), nffn=(14, 18, 38),
    f0=(0.0, 0.89), f1=(0.085, 0.985), f2=(0.02, 1.0), f3=(0.0, 0.885), oq=1, oo=1, on=256,
)


def make_kernel(FLAGS=None, FL=9, W0=0.15, WS=0.6, WK0=(0.52, 1.3), W1=0.75, S1=(1.0, 1.3), K2=(1.05, 1.3), S2=(1.31, 1.62), K3=(1.5, 1.72), S3=(1.73, 2.0), TORD=1, NOSEM=False, E0=(0.2, 0.7), E1=(0.7, 1.2),
                TPIN=False, TQ=0.9, NOBC=True, EROWS=32, SCOPES=False, ONLY=None, TW=(2, 3), INTERP=False,
                DMA_ORDER='a0 a1 a2 a3 k0 v0 k1 v1 k2 v2 k3 v3 x1 f0 x2 f1 o0 x3 f2 o1 x4 f3'.split(), **over):
    P = dict(PLAN, **over)
    FPIN = True

    stack = []
    def mark(name):
        if not SCOPES: return
        if stack: stack.pop().__exit__(None, None, None)
        if name:
            cm = jax.named_scope(name); cm.__enter__(); stack.append(cm)

    def kernel(x_hbm, wqkv_hbm, wphi_hbm, wo_hbm, wr_hbm, wg_hbm, wu_hbm, wd_hbm,
               out_hbm,
               in_v, st_v, xb_v, xx_v, wphi_v, wr8_v, wr_v, lm_v, a_v, aa_v, b_v, bb_v, wo_v, ffn_v,
               kv_acc, z_acc, kvb_v, zcol_v, best_v, best_i, raw_v, half_v, phi_v, oba_v, obb_v, part_v, gate_v, xcol_v, y_acc,
               out_v, zero_s, sem_x, sem_w, sem_s, sem_f, sem_o):
        def cp_x(r0, n, sem, src0=None):
            src0 = r0 if src0 is None else src0
            return pltpu.make_async_copy(x_hbm.at[pl.ds(src0, n)], in_v.at[pl.ds(r0, n)], sem_x.at[sem])

        def cp_x0(piece):
            return cp_x((piece % 2) * TH + (piece // 2) * (TH // 2), TH // 2, 0 if piece < 2 else NTILE + 1)

        def cp_xt(t):
            return cp_x(pl.multiple_of(t * T, T), T, t, pl.multiple_of((t % NTILE) * T, T))

        def cp_w(j, c0, n, sem):
            src = wo_hbm.at[:, pl.ds(c0, n)] if j == 3 else wqkv_hbm.at[:, pl.ds(aligned(j * D + c0, 128), n)]
            return pltpu.make_async_copy(src, in_v.at[pl.ds(WQ + j * D, D), pl.ds(c0, n)], sem_w.at[sem])

        def cp_k(c):
            return cp_w(1, c * 256, 256, c)

        def cp_v(c):
            return cp_w(2, c * 256, 256, c if c else 4)

        def start_q(u):
            for n in range(8):
                src = wqkv_hbm.at[pl.ds((n // 2) * 256 + (u % 2) * 128, 128), pl.ds((u // 2) * 256 + (n % 2) * 512, 256)]
                pltpu.make_async_copy(src, in_v.at[pl.ds(WQ + (u // 2) * 512 + (n // 2) * 128, 128),
                                                   pl.ds((u % 2) * 512 + (n % 2) * 256, 256)], sem_x.at[u + 1]).start()

        def q_blocks(u):
            return in_v.at[pl.ds(aligned(WQ + (u // 2) * 512, 512), 512), pl.ds(aligned((u % 2) * 512, 512), 512)]

        def wait_all(filled, sem):
            pltpu.make_async_copy(filled, filled, sem).wait()

        def cp_wo(h):
            cols = pl.ds(aligned(h * 512, 512), 512)
            return pltpu.make_async_copy(wo_hbm.at[:, cols], in_v.at[pl.ds(WO, D), cols], sem_x.at[h + 2])

        cp_phi = pltpu.make_async_copy(wphi_hbm, wphi_v, sem_s.at[0])
        cp_wr = pltpu.make_async_copy(wr_hbm, wr8_v, sem_s.at[0])
        def start_ffn(g):
            for j in range(FG):
                cols = pl.ds(aligned((g * FG + j) * 128, 128), 128)
                for n, src in enumerate((wg_hbm, wu_hbm)):
                    pltpu.make_async_copy(src.at[:, cols], ffn_v.at[g, pl.ds((n * FG + j) * D, D)], sem_f.at[g]).start()
                    yield
            rows = pl.ds(aligned(g * FG * 128, 128), FG * 128)
            for n in range(D // 128):
                pltpu.make_async_copy(wd_hbm.at[rows, pl.ds(n * 128, 128)],
                                      ffn_v.at[g, pl.ds(2 * FG * D + n * FG * 128, FG * 128)], sem_f.at[g]).start()
                yield

        def cp_o(k, t):
            rows = pl.ds(pl.multiple_of(t * T, T), T)
            return pltpu.make_async_copy(out_v.at[rows], out_hbm.at[rows], sem_o.at[0])

        def cp_o_blk(t, blk, half):
            rows = pl.ds(pl.multiple_of(t * T + (blk % 2) * TH + half * 128, 128), 128)
            cols = pl.ds((blk // 2) * 256, 256)
            return pltpu.make_async_copy(out_v.at[rows, cols], out_hbm.at[rows, cols], sem_o.at[0])

        cp_wr.start()
        cp_phi.start()
        for n, name in enumerate(DMA_ORDER):
            if n == 1:
                cp_wr.wait()
                cp_phi.wait()
            if name[0] == "f":
                start_q(int(name[1]))
            else:
                {"a": cp_x0, "k": cp_k, "v": cp_v, "x": cp_xt, "o": cp_wo}[name[0]](int(name[1])).start()

        last_product = []

        clock = [0.0]
        rate = [7]

        def pin(n=8):
            if not last_product:
                return jnp.zeros((n, 128), f32)
            rows, cols = last_product[0].shape[0] // 8, last_product[0].shape[1] // 128
            q = min(int((clock[0] * last_product[1]) % 1.0 * rows * cols + 1e-6), rows * cols - 1)
            m = last_product[0][(q % rows) * 8:(q % rows) * 8 + 8, (q // rows) * 128:(q // rows) * 128 + 128]
            z = pltpu.bitcast(pltpu.bitcast(m, u32) & zero_s[0].astype(u32), f32)
            return z if n == 8 else jnp.concatenate([z] * (n // 8), axis=0)

        def as_bf16(w):
            return pltpu.bitcast(w, bf16)

        def feature_maps():
            rho = lax.broadcasted_iota(i32, (128, DH), 0)
            sel = (((rho % 64) // 8) * 4 + (rho % 8) // 2 == lax.broadcasted_iota(i32, (128, DH), 1)).astype(bf16)
            rho = lax.broadcasted_iota(i32, (128, 128), 0)
            keep = (rho // 64) * 2 + rho % 2 == lax.broadcasted_iota(i32, (128, 128), 1) // DH
            for g in range(8):
                full = _dot_nt(sel, wphi_v[pl.ds(g * 128, 128), :])
                lm_v.at[g][...] = jnp.where(keep, full, 0.0).astype(bf16)

        def operand(chunk):
            return a_v.at[chunk] if chunk < 2 else b_v.at[chunk - 2]

        def put_lhs(dst, rows, cols, *quadrants):
            for i, v in enumerate(_lhs_combos(*quadrants)):
                dst.at[i][rows, cols] = _narrow(v)

        def split_again(src, dst, lhs, r, k):
            for i in range(7):
                zero = pltpu.bitcast(pin(), u32)
                w = [[src[i, pl.ds(h * 64 + r * 8, 8), pl.ds(aligned(c * 256 + k * 128, 128), 128)]
                      for c in range(2)] for h in range(2)]
                q00, q01, q10, q11 = _wide(w[0][0] | zero), _wide(w[0][1]), _wide(w[1][0]), _wide(w[1][1] | zero)
                cmb = _lhs_combos(q00, q01, q10, q11) if lhs else _rhs_combos(q00, q10, q01, q11)
                for n, j in enumerate(LHS_SUMS if lhs else RHS_SUMS):
                    dst.at[5 * i + n][pl.ds(r * 8, 8), pl.ds(aligned(k * 128, 128), 128)] = _narrow(cmb[j])
                yield

        def second(src, dst, lhs, ij):
            i, j = ij // 7, ij % 7
            sums = LHS_SUMS if lhs else RHS_SUMS
            if j in sums:
                return as_bf16(dst[5 * i + sums.index(j)])
            d = int(j == (3 if lhs else 4))
            return as_bf16(src[i, pl.ds(d * 64, 64), pl.ds(d * 256, 256)])

        def w_blocks(base, top, bot, k):
            return [in_v[pl.ds(aligned(base + kh * 512 + k * 128, 128), 128),
                         pl.ds(aligned(g * 128, 128), 128)] for g in (top, bot) for kh in range(2)]

        def prep_fold(blocks_of, top, bot, dst, row_of, ks):
            for k in ks:
                blocks = [_dot_nt(lm_v[g], w) for g, w in zip((top, top, bot, bot), blocks_of(k))]
                for j in range(8):
                    put_lhs(dst, pl.ds(aligned(row_of(j), 8), 8), pl.ds(aligned(k * 128, 128), 128),
                            *[p[16 * j:16 * j + 16] * LOG2E for p in blocks])
                yield

        def prep_transpose(base, top, bot, dst, row_of):
            for k in range(4):
                zero = pltpu.bitcast(pin(64), u32)
                blocks = [as_bf16(pltpu.bitcast(w, u32) | zero).T for w in w_blocks(base, top, bot, k)]
                for j in range(8):
                    put_lhs(dst, pl.ds(aligned(row_of(j), 8), 8), pl.ds(k * 128, 128),
                            *[w[16 * j:16 * j + 16].astype(f32) for w in blocks])
                yield

        def prep_q(u):
            ch, k, w = u // 2, u % 2, q_blocks(u)
            for half in range(2):
                g = 2 * ch + half
                for c in range(2):
                    blocks = [w[pl.ds((2 * kh + c) * 128, 128), pl.ds(a * 256 + half * 128, 128)]
                              for a in range(2) for kh in range(2)]
                    yield from prep_fold(lambda _: blocks, g, g + 4, a_v.at[2 + ch],
                                         lambda j: half * 64 + 8 * j, (k + 2 * c,))

        def split_q(u):
            for r in range(8):
                yield from split_again(a_v.at[2 + u // 2 + zero_s[0]], aa_v.at[1 + u // 2], True, r, u % 2)

        def prep_wo(u, base=WO):
            g = (u // 2) * 4 + u % 2
            return prep_transpose(base, g, g + 2, wo_v.at[u // 2], lambda j: (u % 2) * 64 + 8 * j)

        def x_block(r0, c0):
            return in_v[pl.ds(r0, 16), pl.ds(c0, 128)].astype(f32)

        def ln_stats(t, st):
            for step in range(32):
                pos = (step % 2) * 16 + step // 2
                r0 = pl.multiple_of(t * T + pos * 16, 16)
                x0 = x_block(r0, 0) + pin(16)
                s1 = s2 = None
                for j in range(1, 8):
                    d = x_block(r0, j * 128) - x0
                    s1 = d if j == 1 else s1 + d
                    s2 = d * d if j == 1 else s2 + d * d
                lane_mean = x0 + s1 * 0.125
                m = jnp.sum(lane_mean, axis=-1, keepdims=True) * (1.0 / 128)
                dm = lane_mean - m
                v = jnp.sum((s2 - s1 * s1 * 0.125) * 0.125 + dm * dm, axis=-1, keepdims=True) * (1.0 / 128)
                vb = (v.astype(bf16).astype(f32) + EPS_BF16).astype(bf16).astype(f32)
                st[0, pl.ds(pos * 16, 16), :] = jnp.broadcast_to(m.astype(bf16).astype(f32), (16, 128))
                st[1, pl.ds(pos * 16, 16), :] = jnp.broadcast_to(1.0 / jnp.sqrt(vb).astype(bf16).astype(f32), (16, 128))
                yield

        def ln_apply(t, st, xb, score_too):
            for step in range(16):
                r0 = [pl.multiple_of(t * T + hf * TH + step * 16 + zero_s[0], 16) for hf in range(2)]
                mean = [st[0, pl.ds(hf * TH + step * 16, 16), :] for hf in range(2)]
                scale = [st[1, pl.ds(hf * TH + step * 16, 16), :] for hf in range(2)]
                score = [None, None]
                for k in range(4):
                    zero = pin(16)
                    xn = [[(x_block(r0[hf], kh * 512 + k * 128) - (mean[hf] + zero)) * scale[hf]
                           for kh in range(2)] for hf in range(2)]
                    for i, v in enumerate(_rhs_combos(xn[0][0], xn[1][0], xn[0][1], xn[1][1])):
                        xb.at[i][pl.ds(step * 8, 8), pl.ds(k * 128, 128)] = _narrow(v)
                    for hf in range(2 if score_too else 0):
                        part = (xn[hf][0] * wr_v[:, pl.ds(k * 128, 128)]
                                + xn[hf][1] * wr_v[:, pl.ds(512 + k * 128, 128)])
                        score[hf] = part if k == 0 else score[hf] + part
                        if k == 3:
                            r = jnp.sum(score[hf], axis=-1, keepdims=True).astype(bf16).astype(f32)
                            r = jnp.broadcast_to(r, (16, 128))
                            slot = 2 * (t // NTILE) + hf
                            up = r > best_v[slot]
                            best_v[slot] = jnp.where(up, r, best_v[slot])
                            best_i[slot] = jnp.where(up, lax.broadcasted_iota(i32, (16, 128), 0) + r0[hf] % S, best_i[slot])
                    yield

        def ln_split(xb, xx):
            for r in range(8):
                for k in range(2):
                    yield from split_again(xb, xx, False, r, k)

        def project(w, x, res, keep=None):
            def emit(r, b, val):
                if isinstance(res, list):
                    res[r][b] = val
                else:
                    res[r, b] = val
                if keep is not None:
                    keep[r, b] = val[64:]

            def prod2(ij):
                m = _dot_nt(second(*w, True, ij), second(*x, False, ij))
                last_product[:] = [m, 49]
                return m

            def once():
                for c in range(2):
                    def prod(i):
                        m = _dot_nt(as_bf16(w[i]), as_bf16(x[i, pl.ds(c * 64, 64), :]))
                        last_product[:] = [m, 14]
                        return m

                    def put(a, b, val):
                        emit(2 * a, 2 * b + c, val[:128])
                        emit(2 * a + 1, 2 * b + c, val[128:])

                    yield from _strassen(prod, put, P["o1"])

            if isinstance(w, tuple):
                return _strassen2(prod2, emit, P["oq"]), 49, 0.0, 1.0
            return once(), 14, 0.0, 1.0

        def project_part(w, x, res, part):
            def prod(i):
                lhs = jnp.concatenate([w[i, pl.ds(h * 64 + part * 32, 32), :] for h in range(2)], axis=0)
                m = _dot_nt(as_bf16(lhs), as_bf16(x[i]))
                last_product[:] = [m, 14]
                return m

            def put(a, b, val):
                for h in range(2):
                    for c in range(2):
                        res[2 * a + h, 2 * b + c, pl.ds(part * 64, 64), :] = val[h * 64:(h + 1) * 64, c * 128:(c + 1) * 128]

            return _strassen(prod, put, P["o1"])

        def raw_blk(res, r, r0, lane):
            if isinstance(res, list):
                return res[r][lane][r0:r0 + 64]
            return res[r, lane, pl.ds(r0, 64), :]

        keep_kv = lax.broadcasted_iota(i32, (64, 128), 0) // DH == lax.broadcasted_iota(i32, (64, 128), 1) % 2

        def kv_post(c, res, keep=None, late=False):
            def accumulate(p, quarter, phi):
                vt = jnp.concatenate([raw_blk(res, quarter, 64, l) for l in range(4)], axis=1).astype(bf16)
                kv = kv_acc[p] + _dot_nt(vt, phi)
                kv_acc[p] = kv
                kvb_v.at[p][...] = jnp.where(keep_kv, kv, 0.0).astype(bf16)

            pending = []
            for a in range(2):
                for pr in range(2):
                    p = 4 * c + 2 * a + pr
                    phis, zs = [], z_acc[p]
                    for lane in range(4):
                        phi = _dual_softmax(raw_blk(res, 2 * a + pr, 0, lane), pin())
                        zs = zs + phi
                        phis.append(phi)
                        if keep is not None:
                            keep.at[2 * a + pr][:, pl.ds(lane * 128, 128)] = _narrow(phi)
                        if lane == 1 and pending and (a or not late):
                            accumulate(*pending.pop(0))
                        if lane == 3:
                            z_acc[p] = zs
                            zcol_v[p] = jnp.broadcast_to(jnp.sum(zs, axis=-1, keepdims=True), (128, 128))
                            pending.append((p, 2 * a + pr, jnp.concatenate(phis, axis=1).astype(bf16)))
                        yield
            yield
            for rest in pending:
                accumulate(*rest)
            yield

        def route():
            best, tok = best_v[...].reshape(64, 128), best_i[...].reshape(64, 128)
            rmax = jnp.max(best, axis=0, keepdims=True)
            idx = jnp.min(jnp.where(best == rmax, tok, S).astype(f32)).astype(i32)
            return jnp.clip(idx, 0, S - 1), rmax

        def routed_token():
            idx = route()[0]
            base = pl.multiple_of((idx // 16) * 16, 16)
            rows = pl.ds(pl.multiple_of(base % T, 16), 16)
            xn = (in_v[pl.ds(base, 16), :].astype(f32) - st_v[idx // T, 0, rows, 0:1]) * st_v[idx // T, 1, rows, 0:1]
            xsel = jnp.where(lax.broadcasted_iota(i32, (16, D), 0) == idx - base, xn, 0.0)
            xsel = jnp.sum(xsel, axis=0, keepdims=True).astype(bf16).astype(f32)
            for j in range(8):
                row = xsel[:, j * 128:(j + 1) * 128] + pin()
                xcol_v[pl.ds(j * 128, 128), :] = jnp.concatenate([row] * 16, axis=0).T
                yield

        SKIP[0] = ONLY is not None
        mark('s0_init')
        zero_s[0] = 0
        kv_acc[...] = jnp.zeros(kv_acc.shape, f32)
        z_acc[...] = jnp.zeros(z_acc.shape, f32)
        y_acc[...] = jnp.zeros(y_acc.shape, f32)
        best_v[...] = jnp.full(best_v.shape, -jnp.inf, f32)
        best_i[...] = jnp.zeros(best_i.shape, i32)
        w8 = wr8_v[...].astype(f32)
        wr_v[...] = jnp.broadcast_to(jnp.concatenate([w8[j:j + 1, :] for j in range(8)], axis=1), (16, D))
        feature_maps()
        mark('s1_ln0')
        stats, apply = ln_stats(0, st_v.at[0]), ln_apply(0, st_v.at[0], xb_v.at[0], False)
        cp_x0(0).wait()
        cp_x0(1).wait()
        _schedule(clock, (stats, 16, 0.0, 1.0))
        _schedule(clock, (apply, 32, 0.0, 1.0))
        cp_x0(2).wait()
        cp_x0(3).wait()
        _schedule(clock, (stats, 16, 0.0, 1.0))
        _schedule(clock, (apply, 32, 0.0, 1.0))

        def prep_kv(c):
            cp_k(c).wait()
            if c:
                cp_v(c).wait()
            once = operand(c)
            yield from prep_fold(lambda k: w_blocks(WK, 2 * c, 2 * c + 1, k), 2 * c, 2 * c + 1, once, lambda j: (j // 4) * 64 + (j % 4) * 8, range(4))
            if not c:
                cp_v(c).wait()
            yield from prep_transpose(WV, 2 * c, 2 * c + 1, once, lambda j: (j // 4) * 64 + 32 + (j % 4) * 8)

        def split_kv(c):
            for k in range(2):
                for r in range(8):
                    if c == 1:
                        yield from split_again(a_v.at[1 + zero_s[0]], aa_v.at[0], True, r, k)
                    else:
                        yield from split_again(b_v.at[c - 2 + zero_s[0]], bb_v.at[c - 2], True, r, k)

        mark('s3_prep0')
        first_chunk = prep_kv(0)
        _schedule(clock, (first_chunk, 4, 0.0, 1.0))
        mark('s4_proj0')
        next_chunk = project(operand(1), xb_v.at[0], raw_v.at[1])[0]
        _schedule(clock, (project_part(operand(0), xb_v.at[0], raw_v.at[0], 0), 7, 0.0, 0.5),
                  (project_part(operand(0), xb_v.at[0], raw_v.at[0], 1), 7, 0.5, 1.0), (next_chunk, 14, 1.0, 2.0),
                  (first_chunk, 4, W0, 0.45), (ln_split(xb_v.at[zero_s[0]], xx_v.at[0]), 112, 0.03, WS),
                  (kv_post(0, raw_v.at[zero_s[0]], late=True), 18, *WK0),
                  (prep_kv(1), 8, W1, 1.0), (split_kv(1), 112, *S1), (prep_kv(2), 8, *K2), (split_kv(2), 112, *S2), (prep_kv(3), 8, *K3), (split_kv(3), 112, *S3))

        def kv_tile(t, _):
            SKIP[0] = False
            last = t == NTILE - 1
            wait_all(q_blocks(t), sem_x.at[t + 1])
            cp_xt(t + 1).wait()

            @pl.when(jnp.logical_and(t > 0, t < 3))
            def _():
                cp_wo(t - 1).wait()

            if not NOBC:
                for g in range(NTILE):
                    @pl.when(t == g)
                    def _():
                        for _ in start_ffn(g):
                            pass

            last_product[:] = []
            first = (route()[0] // T) % (NTILE - 1) + 1
            xb, st = xb_v.at[pl.ds(t, 2)], st_v.at[t + 1]
            stats, apply = ln_stats(t + 1, st), ln_apply(t + 1, st, xb.at[1], True)
            xx = xx_v.at[pl.ds(t, 2)]
            split = ln_split(xb_v.at[t + 1 + zero_s[0]], xx.at[1]) if TW else ln_split(xb.at[0], xx.at[0])
            slot = lambda c: ((operand(c), bb_v.at[c - 2]), (xb.at[0], xx.at[0])) if c in TW else (operand(c), xb.at[0])
            fold = prep_q(t)
            trans = [prep_wo(2 * ((t + 1) % 2) + u, jnp.where(t == 0, WV, WO)) for u in range(2)]

            c2, c3, c0 = ([[None] * 4 for _ in range(4)] for _ in range(3))
            _schedule(clock, project(*slot(2), c2), (kv_post(1, raw_v.at[1]), 18, *P["kv"]),
                      (stats, 32, *P["stats"]), (fold, P["nfold"], *P["fold"]),
                      (start_ffn(t), 2 * FG + 8 if NOBC else 0, 0.05, 0.95))
            _schedule(clock, project(*slot(3), c3), (kv_post(2, c2), 18, *P["kv"]),
                      (apply, 64, *P["apply"]), (fold, 4 - P["nfold"], *P["fold2"]))
            nxt, chunk = jnp.where(last, first, t + 1), jnp.where(last, 2, 0)
            again = split_q(t)
            _schedule(clock, project(a_v.at[chunk], xb_v.at[nxt], c0, keep=half_v), (kv_post(3, c3), 18, *P["kv"]),
                      (split, 112, *P["split"]), (again, 56, *P["again"]))
            _schedule(clock, project((a_v.at[chunk + 1], aa_v.at[chunk]), (xb_v.at[nxt], xx_v.at[nxt]), raw_v.at[1]),
                      (kv_post(jnp.where(last, 4, 0), c0, phi_v), 18, *P["kv"]), (trans[0], 4, *P["trans"]),
                      (trans[1], 4, *P["split2"]), (routed_token(), 8, *P["routed"]))
            return first

        mark('s6_phase1')
        first = lax.fori_loop(0, NTILE, kv_tile, jnp.int32(0)) if ONLY != 'p2' else route()[0] // T
        SKIP[0] = ONLY is not None
        mark('s7_mid')
        wait_all(ffn_v.at[0], sem_f.at[0])
        last_product[:] = []

        idx, rmax = route()

        def ffn(f0, nf):
            for j in range(nf):
                group, tile_in_group = ffn_v.at[(f0 + j) // FG], (f0 + j) % FG
                accs = [jnp.zeros((8, 128), f32)] * 2
                for r in range(8):
                    rows = pl.ds(r * 128, 128)
                    xc = xcol_v[rows, :]
                    if FPIN:
                        zero = pin()
                    for a in range(2):
                        w = group[pl.ds(aligned((a * FG + tile_in_group) * D + r * 128, 128), 128), :]
                        prod = w.astype(f32) * xc
                        acc = accs[a] + zero if FPIN else accs[a]
                        for q in range(16):
                            acc = acc + prod[8 * q:8 * q + 8]
                        accs[a] = acc
                    yield
                gate, up = [jnp.sum(acc, axis=0, keepdims=True) for acc in accs]
                hcol = jnp.broadcast_to(gate * jax.nn.sigmoid(gate) * up, (128, 128)).T
                for n in range(8):
                    ycols = pl.ds(n * 128, 128)
                    w = group[pl.ds(aligned(2 * FG * D + (n * FG + tile_in_group) * 128, 128), 128), :]
                    prod = w.astype(f32) * hcol
                    acc = y_acc[:, ycols] + pin() if FPIN else y_acc[:, ycols]
                    for q in range(16):
                        acc = acc + prod[8 * q:8 * q + 8]
                    y_acc[:, ycols] = acc
                    if n % 2 == 1:
                        yield

        final = idx // T
        lo, hi = jnp.minimum(first, final), jnp.maximum(first, final)
        second_tile = jnp.where(lo > 0, 0, jnp.where(hi > 1, 1, 2))
        third_tile = 6 - first - final - second_tile

        def tile(j):
            return jnp.where(j == 0, first, jnp.where(j == 1, second_tile, jnp.where(j == 2, third_tile, final)))

        def q_post(c, res, ob, ready=None):
            even = lax.broadcasted_iota(i32, (8, 128), 0) % 2 == 0

            def pair_of(step):
                return 2 * (2 * c + step // 4 + 4 * ((step // 2) % 2)) + step % 2

            phis, scales, nums, outs = {}, {}, {}, {}
            for tick in range(40):
                step, lane = tick // 4, tick % 4
                if step < 8:
                    u, a, pr = step // 4, (step // 2) % 2, step % 2
                    if ready is not None and pr == 0:
                        phi = _wide(ready[2 * a + u, :, pl.ds(lane * 128, 128)])
                    else:
                        phi = _dual_softmax(raw_blk(res, 2 * a + u, 0 if ready is not None else pr * 64, lane), pin())
                    den = phi * zcol_v[pair_of(step)]
                    inv = _recip(_head_reduce([den[8 * j:8 * j + 8] for j in range(16)], jnp.add) + 1e-6)
                    other = pltpu.roll(inv, 1, 0)
                    phis.setdefault(step, []).append(phi)
                    scales.setdefault(step, []).append((jnp.where(even, inv, other), jnp.where(even, other, inv)))
                if 1 <= step < 9 and lane == 1:
                    phi = jnp.concatenate(phis.pop(step - 1), axis=1).astype(bf16)
                    nums[step - 1] = _dot(kvb_v[pair_of(step - 1)], phi)
                if step >= 2 and lane == 0:
                    num, scale = nums.pop(step - 2), scales.pop(step - 2)
                    scale = [jnp.concatenate([v[head] for v in scale], axis=1) for head in range(2)]
                    outs[step - 2] = num * jnp.concatenate([scale[0]] * 4 + [scale[1]] * 4, axis=0)
                    if (step - 2) % 4 == 3:
                        u = (step - 2) // 4
                        o1 = jnp.concatenate([outs.pop(4 * u), outs.pop(4 * u + 1)], axis=0)
                        o2 = jnp.concatenate([outs.pop(4 * u + 2), outs.pop(4 * u + 3)], axis=0)
                        cmb = _rhs_combos(o1[:, :TH], o1[:, TH:], o2[:, :TH], o2[:, TH:])
                        for i in range(7):
                            ob.at[i][:, pl.ds(u * 128, 128)] = pltpu.bitcast(cmb[i].astype(bf16).T, u32)
                yield

        def out_project(h, oba, obb, res, ks=(0, 1), order=P["oo"], n=P["on"]):
            parts = {}
            for c in range(256 // n):
                def prod(i):
                    lhs = jnp.concatenate([(oba, obb)[k][i] for k in ks], axis=1)
                    rhs = wo_v[h, i, pl.ds(c * n // 2, n // 2), pl.ds(ks[0] * 256, len(ks) * 256)]
                    m = _dot_nt(as_bf16(lhs), as_bf16(rhs))
                    last_product[:] = [m, rate[0] * (256 // n)]
                    return m

                def emit(a, b, val):
                    if isinstance(res, list):
                        parts[a, b, c] = val
                        if c == 256 // n - 1:
                            res[a][b] = jnp.concatenate([parts[a, b, cc] for cc in range(256 // n)], axis=1)
                    else:
                        res[a, b, :, pl.ds(c * n, n)] = val

                yield from _strassen(prod, emit, order)

        def gate(t, a, b, h, q, upd):
            n = EROWS
            r0, rows = pl.multiple_of(t * T + b * TH + q * n, n), pl.ds(b * TH + q * n, n)
            mean, scale = st_v[t, 0, rows, :], st_v[t, 1, rows, :] * 0.5
            if upd is None:
                mean = mean + pin(n)
            x = in_v[pl.ds(r0, n), pl.ds(h * 512 + a * 256, 256)].astype(f32)
            v = (x - jnp.concatenate([mean, mean], axis=1)) * jnp.concatenate([scale, scale], axis=1)
            if upd is not None:
                hit = lax.broadcasted_iota(i32, (n, 256), 0) == idx - r0
                v = v + jnp.where(hit, upd[:, h * 512 + a * 256:h * 512 + (a + 1) * 256], 0.0)
            return x, v + v * jnp.tanh(v)

        def epilogue(t, h, res, part=None, upd=None, done=None, order=0, early=None):
            n = EROWS
            for a in range(2):
                for b in ((1, 0) if order and a == 0 else (0, 1)):
                    for q in range(TH // n):
                        r0, cols = pl.multiple_of(t * T + b * TH + q * n, n), pl.ds(h * 512 + a * 256, 256)
                        if early is not None and (a, b) == (1, 1):
                            x, g = in_v[pl.ds(r0, n), cols].astype(f32), early[pl.ds(q * n, n), :]
                        else:
                            x, g = gate(t, a, b, h, q, upd)
                        s = res[a][b][q * n:(q + 1) * n]
                        if part is not None:
                            s = s + part[a, b, pl.ds(q * n, n), :]
                        out_v[pl.ds(r0, n), cols] = (x + s * g).astype(bf16)
                        if done is not None and (q + 1) * n % 128 == 0:
                            done(4 * h + 2 * a + b, (q + 1) * n // 128 - 1)
                        yield

        NE = 4 * TH // EROWS
        mark('s8_q0')
        fb = NF - (NTILE - 1) * FL
        res0 = None
        _schedule(clock, (q_post(0, half_v, oba_v.at[0], phi_v), 40, 0.0, 1.0))

        def q_tile(j, carry):
            SKIP[0] = False
            last_product[:] = []
            oba = oba_v.at[pl.ds(j, 2)]
            obb = obb_v.at[zero_s[0]]
            x = xb_v.at[tile(j + 1)], xx_v.at[tile(j + 1)]
            wait_all(ffn_v.at[j + 1], sem_f.at[j + 1])
            fg = ffn(j * FL, FL)
            q0, o0, o1 = ([[None] * 4 for _ in range(4)] for _ in range(3))
            nf, no = P["nffn"], 7 * 256 // P["on"]
            _schedule(clock, project((a_v.at[2], aa_v.at[1]), x, q0),
                      (q_post(1, raw_v.at[1], obb_v.at[0]), 40, *P["p1"]), (fg, nf[0], *P["f0"]))
            _schedule(clock, (out_project(0, oba.at[0], obb, o0), no, 0.0, 1.0),
                      (q_post(0, q0, oba.at[1]), 40, *P["p0"]), (fg, nf[1], *P["f1"]))
            _schedule(clock, (out_project(1, oba.at[0], obb, o1), no, 0.0, 1.0),
                      (epilogue(tile(j), 0, o0), NE, *P["e0"]), (fg, nf[2], *P["f2"]))
            _schedule(clock, project((a_v.at[3], aa_v.at[2]), x, raw_v.at[1]),
                      (epilogue(tile(j), 1, o1), NE, *P["e1"]), (fg, 12 * FL - sum(nf), *P["f3"]))
            cp_o(j, tile(j)).start()
            return carry

        mark('s9_phase2')
        if ONLY != 'p1':
            lax.fori_loop(0, NTILE - 1, q_tile, 0)
        SKIP[0] = ONLY is not None
        if ONLY:
            keep = sum(jnp.sum(pltpu.bitcast(r[(0,) * (len(r.shape) - 2) + (pl.ds(pl.multiple_of(zero_s[0], 16), 16), slice(0, 128))], f32))
                       for r in (xb_v, xx_v, a_v, aa_v, wo_v, kvb_v, raw_v, half_v, phi_v, xcol_v, oba_v, obb_v))
            out_v[0:16, 0:128] = jnp.full((16, 128), keep + jnp.sum(y_acc[...]) + jnp.sum(best_v[...]), f32).astype(bf16)
        mark('sa_tail')

        j = NTILE - 1
        rate[0] = 14
        last_product[:] = []
        oba, obb = oba_v.at[j], obb_v.at[zero_s[0]]
        _schedule(clock, (out_project(0, oba, obb, part_v.at[0], (0,), TORD, 256), 7, 0.0, 0.5),
                  (out_project(1, oba, obb, part_v.at[1], (0,), TORD, 256), 7, 0.5, 1.0),
                  (q_post(1, raw_v.at[1], obb_v.at[0]), 40, 0.0, TQ),
                  (ffn(NF - fb, fb), 12 * fb, 0.1, 0.8))
        upd = jnp.sum(y_acc[...], axis=0, keepdims=True) * (0.5 * jax.nn.sigmoid(rmax[:, 0:1]))
        o0, o1 = ([[None, None], [None, None]] for _ in range(2))
        t = tile(j)
        send = lambda blk, half: cp_o_blk(t, blk, half).start()

        def last_gate():
            for q in range(TH // EROWS):
                gate_v[0, pl.ds(q * EROWS, EROWS), :] = gate(t, 1, 1, 1, q, upd)[1]
                yield

        e0 = epilogue(t, 0, o0, part_v.at[0], upd, send, TORD)
        e1 = epilogue(t, 1, o1, part_v.at[1], upd, send, TORD, gate_v.at[zero_s[0]])
        _schedule(clock, (out_project(0, oba, obb, o0, (1,), TORD, 256), 7, 0.0, 0.5),
                  (out_project(1, oba, obb, o1, (1,), TORD, 256), 7, 0.5, 1.0),
                  (e0, NE, *E0), (e1, NE, *E1), (last_gate(), TH // EROWS, 0.0, 0.2))
        mark('sb_outdma')
        pltpu.make_async_copy(out_v, out_hbm, sem_o.at[0]).wait()
        mark(None)

    scratch = [
        pltpu.VMEM((S + T + 4 * D, D), bf16),
        pltpu.VMEM((NTILE + 1, 2, T, 128), f32),
        pltpu.VMEM((NTILE + 1, 7, 128, 512), u32),
        pltpu.VMEM((NTILE + 1, 35, 64, 256), u32),
        pltpu.VMEM((D, DH), bf16),
        pltpu.VMEM((8, 128), bf16),
        pltpu.VMEM((16, D), f32),
        pltpu.VMEM((8, 128, 128), bf16),
        pltpu.VMEM((4, 7, 128, 512), u32),
        pltpu.VMEM((3, 35, 64, 256), u32),
        pltpu.VMEM((2, 7, 128, 512), u32),
        pltpu.VMEM((2, 35, 64, 256), u32),
        pltpu.VMEM((2, 7, 128, 512), u32),
        pltpu.VMEM((NTILE, 3 * FG * D, 128), bf16),
        pltpu.VMEM((H // 2 + 4, 64, 128), f32),
        pltpu.VMEM((H // 2 + 4, 128, 128), f32),
        pltpu.VMEM((H // 2 + 4, 64, 128), bf16),
        pltpu.VMEM((H // 2 + 4, 128, 128), f32),
        pltpu.VMEM((4, 16, 128), f32),
        pltpu.VMEM((4, 16, 128), i32),
        pltpu.VMEM((2, 4, 4, 128, 128), f32),
        pltpu.VMEM((4, 4, 64, 128), f32),
        pltpu.VMEM((4, 64, T), u32),
        pltpu.VMEM((NTILE, 7, TH // 2, 256), u32),
        pltpu.VMEM((2, 7, TH // 2, 256), u32),
        pltpu.VMEM((2, 2, 2, 256, 256), f32),
        pltpu.VMEM((2, 256, 256), f32),
        pltpu.VMEM((D, 128), f32),
        pltpu.VMEM((8, D), f32),
        pltpu.VMEM((S, D), bf16),
        pltpu.SMEM((1,), i32),
        pltpu.SemaphoreType.DMA((NTILE + 2,)),
        pltpu.SemaphoreType.DMA((5,)),
        pltpu.SemaphoreType.DMA((1,)),
        pltpu.SemaphoreType.DMA((NTILE,)),
        pltpu.SemaphoreType.DMA((1,)),
    ]

    def call(x, wqkv, wphi, wo, wr, wg, wu, wd):
        hbm = pl.BlockSpec(memory_space=pltpu.HBM)
        return pl.pallas_call(
            kernel,
            out_shape=jax.ShapeDtypeStruct((S, D), bf16),
            in_specs=[hbm] * 8,
            out_specs=hbm,
            scratch_shapes=scratch,
            compiler_params=pltpu.CompilerParams(vmem_limit_bytes=120 * 2**20, flags=FLAGS, disable_bounds_checks=NOBC, disable_semaphore_checks=NOSEM),
            name="hedgehog", interpret=INTERP,
        )(x, wqkv, wphi, wo, wr, wg, wu, wd)

    return call


@jax.jit
def pallas_recurrent_scan__linear_kernel_hedgehog__moe_arch_mod__prompt_kernel(
    A_x: jax.Array,
    A_wqkv: jax.Array,
    A_w_phi: jax.Array,
    A_wo: jax.Array,
    B_x: jax.Array,
    B_w_r: jax.Array,
    B_w_gate: jax.Array,
    B_w_up: jax.Array,
    B_w_down: jax.Array,
):
    del B_x
    out = make_kernel()(
        A_x.reshape(S, D), A_wqkv, A_w_phi.reshape(D, DH), A_wo,
        B_w_r.reshape(8, 128), B_w_gate, B_w_up, B_w_down)
    return out.reshape(1, S, D)
```

```python
import math

import numpy as np

import jax
import jax.numpy as jnp
from jax import lax
import jax.experimental.pallas as pl
import jax.experimental.pallas.tpu as pltpu

S, D, H, DH, F = 2048, 1024, 32, 32, 3584
T = 512
TH = T // 2
NTILE = S // T
NF = F // 128
FG = NF // NTILE
FL = 9
EROWS = 32
WQ, WK, WV, WO = (S + T + j * D for j in range(4))
LHS_SUMS, RHS_SUMS = (0, 1, 4, 5, 6), (0, 2, 3, 5, 6)
LOG2E = math.log2(math.e)
EPS_BF16 = float(np.float32(1e-5).astype(jnp.bfloat16))
f32, bf16, i32, u32 = jnp.float32, jnp.bfloat16, jnp.int32, jnp.uint32


def _dot_nt(a, b):
    return lax.dot_general(a, b, (((1,), (1,)), ((), ())), preferred_element_type=f32)


def _dot(a, b):
    return jnp.dot(a, b, preferred_element_type=f32)


def _aligned(i, n):
    return i if isinstance(i, int) else pl.multiple_of(i, n)


def _recip(v):
    r = pl.reciprocal(v, approx=True)
    return r * (2.0 - v * r)


def _bf16(words):
    return pltpu.bitcast(words, bf16)


def _wide(words):
    return _bf16(words).astype(f32)


def _narrow(v):
    return pltpu.bitcast(v.astype(bf16), u32)


def _lhs_operands(a11, a12, a21, a22):
    return [a11 + a22, a21 + a22, a11, a22, a11 + a12, a21 - a11, a12 - a22]


def _rhs_operands(b11, b12, b21, b22):
    return [b11 + b22, b11, b12 - b22, b21 - b11, b22, b11 + b12, b21 + b22]


def _strassen(prod, emit):
    m3 = prod(2)
    yield
    m5 = prod(4)
    emit(0, 1, m3 + m5)
    yield
    m1 = prod(0)
    c11, c22 = m1 - m5, m1 + m3
    yield
    c11 = c11 + prod(6)
    yield
    m4 = prod(3)
    emit(0, 0, c11 + m4)
    yield
    m2 = prod(1)
    emit(1, 0, m2 + m4)
    c22 = c22 - m2
    yield
    emit(1, 1, c22 + prod(5))
    yield


class _Quad:
    def __init__(self, blocks):
        self.blocks = blocks

    def __add__(self, other):
        return _Quad([p + q for p, q in zip(self.blocks, other.blocks)])

    def __sub__(self, other):
        return _Quad([p - q for p, q in zip(self.blocks, other.blocks)])


def _strassen_twice(prod, emit):
    done = {}

    def inner(i):
        out = [None] * 4

        def put(a, b, val):
            out[2 * a + b] = val

        yield from _strassen(lambda j: prod(7 * i + j), put)
        done[i] = _Quad(out)

    def put(a, b, quad):
        for k, val in enumerate(quad.blocks):
            emit(2 * a + k // 2, 2 * b + k % 2, val)

    outer = _strassen(lambda i: done[i], put)
    for i in (2, 4, 0, 6, 3, 1, 5):
        steps = inner(i)
        for _ in range(6):
            next(steps)
            yield
        for _ in steps:
            pass
        next(outer)
        yield


def _head_reduce(vs, op):
    while len(vs) > 1:
        vs = [op(vs[i], vs[i + 1]) for i in range(0, len(vs), 2)]
    v = op(vs[0], pltpu.roll(vs[0], 4, 0))
    return op(v, pltpu.roll(v, 2, 0))


def _dual_softmax(p, zero):
    rows = [p[8 * j:8 * j + 8] for j in range(8)]
    rows[0] = rows[0] + zero
    mx, mn = _head_reduce(rows, jnp.maximum), _head_reduce(rows, jnp.minimum)
    ep = [jnp.exp2(v - mx) for v in rows]
    en = [jnp.exp2(mn - v) for v in rows]
    rp, rn = _recip(_head_reduce(ep, jnp.add)), _recip(_head_reduce(en, jnp.add))
    return jnp.concatenate([v * rp for v in ep] + [v * rn for v in en], axis=0)


def _kernel(x_hbm, wqkv_hbm, wphi_hbm, wo_hbm, wr_hbm, wg_hbm, wu_hbm, wd_hbm, out_hbm,
            in_v, st_v, x1_v, x2_v, wphi_v, wr8_v, wr_v, map_v, a1_v, a2_v, b1_v, b2_v, wo_v, ffn_v,
            kv_acc, z_acc, kv_v, z_v, best_v, best_i, raw_v, half_v, phi_v, oa_v, ob_v, part_v,
            gate_v, xcol_v, y_acc, out_v, zero_s, sem_x, sem_w, sem_s, sem_f, sem_o):
    def cp_x(r0, n, sem, src0):
        return pltpu.make_async_copy(x_hbm.at[pl.ds(src0, n)], in_v.at[pl.ds(r0, n)], sem_x.at[sem])

    def cp_x0(piece):
        r0 = (piece % 2) * TH + (piece // 2) * (TH // 2)
        return cp_x(r0, TH // 2, 0 if piece < 2 else NTILE + 1, r0)

    def cp_xt(t):
        return cp_x(_aligned(t * T, T), T, t, _aligned((t % NTILE) * T, T))

    def cp_w(j, c, sem):
        return pltpu.make_async_copy(wqkv_hbm.at[:, pl.ds(j * D + c * 256, 256)],
                                     in_v.at[pl.ds(WQ + j * D, D), pl.ds(c * 256, 256)], sem_w.at[sem])

    def cp_k(c):
        return cp_w(1, c, c)

    def cp_v(c):
        return cp_w(2, c, c if c else 4)

    def start_q(u):
        for n in range(8):
            src = wqkv_hbm.at[pl.ds((n // 2) * 256 + (u % 2) * 128, 128), pl.ds((u // 2) * 256 + (n % 2) * 512, 256)]
            dst = in_v.at[pl.ds(WQ + (u // 2) * 512 + (n // 2) * 128, 128), pl.ds((u % 2) * 512 + (n % 2) * 256, 256)]
            pltpu.make_async_copy(src, dst, sem_x.at[u + 1]).start()

    def q_blocks(u):
        return in_v.at[pl.ds(_aligned(WQ + (u // 2) * 512, 512), 512), pl.ds(_aligned((u % 2) * 512, 512), 512)]

    def cp_wo(h):
        cols = pl.ds(_aligned(h * 512, 512), 512)
        return pltpu.make_async_copy(wo_hbm.at[:, cols], in_v.at[pl.ds(WO, D), cols], sem_x.at[h + 2])

    def start_ffn(g):
        for j in range(FG):
            cols = pl.ds(_aligned((g * FG + j) * 128, 128), 128)
            for n, src in enumerate((wg_hbm, wu_hbm)):
                dst = ffn_v.at[g, pl.ds((n * FG + j) * D, D)]
                pltpu.make_async_copy(src.at[:, cols], dst, sem_f.at[g]).start()
                yield
        rows = pl.ds(_aligned(g * FG * 128, 128), FG * 128)
        for n in range(D // 128):
            dst = ffn_v.at[g, pl.ds(2 * FG * D + n * FG * 128, FG * 128)]
            pltpu.make_async_copy(wd_hbm.at[rows, pl.ds(n * 128, 128)], dst, sem_f.at[g]).start()
            yield

    def wait_all(filled, sem):
        pltpu.make_async_copy(filled, filled, sem).wait()

    def start_out(rows, cols):
        pltpu.make_async_copy(out_v.at[rows, cols], out_hbm.at[rows, cols], sem_o.at[0]).start()

    small = [pltpu.make_async_copy(wr_hbm, wr8_v, sem_s.at[0]), pltpu.make_async_copy(wphi_hbm, wphi_v, sem_s.at[0])]
    for cp in small + [cp_x0(0)]:
        cp.start()
    for cp in small:
        cp.wait()
    for piece in range(1, 4):
        cp_x0(piece).start()
    for c in range(4):
        cp_k(c).start()
        cp_v(c).start()
    for t in range(NTILE):
        cp_xt(t + 1).start()
        start_q(t)
        if t in (1, 2):
            cp_wo(t - 1).start()

    clock, product = [0.0], []

    def schedule(*streams):
        events = [(a + (b - a) * k / n, i, k, gen) for i, (gen, n, a, b) in enumerate(streams) for k in range(n)]
        for when, _, _, gen in sorted(events, key=lambda e: e[:3]):
            clock[:] = [when]
            next(gen)

    def matmul(a, b, per_slot):
        m = _dot_nt(_bf16(a), _bf16(b))
        product[:] = [m, per_slot]
        return m

    def pin(n=8):
        if not product:
            return jnp.zeros((n, 128), f32)
        m, per_slot = product
        rows, cols = m.shape[0] // 8, m.shape[1] // 128
        q = min(int((clock[0] * per_slot) % 1.0 * rows * cols + 1e-6), rows * cols - 1)
        m = m[(q % rows) * 8:(q % rows) * 8 + 8, (q // rows) * 128:(q // rows) * 128 + 128]
        z = pltpu.bitcast(pltpu.bitcast(m, u32) & zero_s[0].astype(u32), f32)
        return z if n == 8 else jnp.concatenate([z] * (n // 8), axis=0)

    def feature_maps():
        r = lax.broadcasted_iota(i32, (128, DH), 0)
        select = (((r % 64) // 8) * 4 + (r % 8) // 2 == lax.broadcasted_iota(i32, (128, DH), 1)).astype(bf16)
        r = lax.broadcasted_iota(i32, (128, 128), 0)
        same_head = (r // 64) * 2 + r % 2 == lax.broadcasted_iota(i32, (128, 128), 1) // DH
        for g in range(8):
            full = _dot_nt(select, wphi_v[pl.ds(g * 128, 128), :])
            map_v.at[g][...] = jnp.where(same_head, full, 0.0).astype(bf16)

    def put_lhs(dst, row, col, quadrants):
        for i, v in enumerate(_lhs_operands(*quadrants)):
            dst.at[i][pl.ds(_aligned(row, 8), 8), pl.ds(_aligned(col, 128), 128)] = _narrow(v)

    def w_blocks(base, top, bottom, k):
        return [in_v[pl.ds(_aligned(base + half * 512 + k * 128, 128), 128), pl.ds(_aligned(g * 128, 128), 128)]
                for g in (top, bottom) for half in range(2)]

    def put_folded(blocks, top, bottom, dst, row_of, k):
        blocks = [_dot_nt(map_v[g], w) for g, w in zip((top, top, bottom, bottom), blocks)]
        for j in range(8):
            put_lhs(dst, row_of(j), k * 128, [p[16 * j:16 * j + 16] * LOG2E for p in blocks])

    def put_transposed(base, top, bottom, dst, row_of):
        for k in range(4):
            zero = pltpu.bitcast(pin(64), u32)
            blocks = [_bf16(pltpu.bitcast(w, u32) | zero).T for w in w_blocks(base, top, bottom, k)]
            for j in range(8):
                put_lhs(dst, row_of(j), k * 128, [w[16 * j:16 * j + 16].astype(f32) for w in blocks])
            yield

    def split_again(once, twice, lhs, r, k):
        for i in range(7):
            zero = pltpu.bitcast(pin(), u32)
            w = [[once[i, pl.ds(a * 64 + r * 8, 8), pl.ds(_aligned(b * 256 + k * 128, 128), 128)]
                  for b in range(2)] for a in range(2)]
            q00, q01, q10, q11 = _wide(w[0][0] | zero), _wide(w[0][1]), _wide(w[1][0]), _wide(w[1][1] | zero)
            sums = _lhs_operands(q00, q01, q10, q11) if lhs else _rhs_operands(q00, q10, q01, q11)
            for n, j in enumerate(LHS_SUMS if lhs else RHS_SUMS):
                twice.at[5 * i + n][pl.ds(r * 8, 8), pl.ds(_aligned(k * 128, 128), 128)] = _narrow(sums[j])
            yield

    def operand(once, twice, lhs, ij):
        i, j = ij // 7, ij % 7
        sums = LHS_SUMS if lhs else RHS_SUMS
        if j in sums:
            return twice[5 * i + sums.index(j)]
        d = int(j == (3 if lhs else 4))
        return once[i, pl.ds(d * 64, 64), pl.ds(d * 256, 256)]

    def prep_kv(c):
        dst = a1_v.at[c] if c < 2 else b1_v.at[c - 2]
        cp_k(c).wait()
        if c:
            cp_v(c).wait()
        for k in range(4):
            put_folded(w_blocks(WK, 2 * c, 2 * c + 1, k), 2 * c, 2 * c + 1, dst,
                       lambda j: (j // 4) * 64 + (j % 4) * 8, k)
            yield
        if not c:
            cp_v(c).wait()
        yield from put_transposed(WV, 2 * c, 2 * c + 1, dst, lambda j: (j // 4) * 64 + 32 + (j % 4) * 8)

    def split_kv(c):
        once, twice = (a1_v.at[1 + zero_s[0]], a2_v.at[0]) if c == 1 else (b1_v.at[c - 2 + zero_s[0]], b2_v.at[c - 2])
        for k in range(2):
            for r in range(8):
                yield from split_again(once, twice, True, r, k)

    def prep_q(u):
        w = q_blocks(u)
        for a in range(2):
            g = 2 * (u // 2) + a
            for c in range(2):
                blocks = [w[pl.ds((2 * half + c) * 128, 128), pl.ds(b * 256 + a * 128, 128)]
                          for b in range(2) for half in range(2)]
                put_folded(blocks, g, g + 4, a1_v.at[2 + u // 2], lambda j: a * 64 + 8 * j, u % 2 + 2 * c)
                yield

    def split_q(u):
        for r in range(8):
            yield from split_again(a1_v.at[2 + u // 2 + zero_s[0]], a2_v.at[1 + u // 2], True, r, u % 2)

    def prep_wo(u, base):
        g = (u // 2) * 4 + u % 2
        return put_transposed(base, g, g + 2, wo_v.at[u // 2], lambda j: (u % 2) * 64 + 8 * j)

    def x_block(r0, n, cols):
        return jnp.concatenate([in_v[pl.ds(pl.multiple_of(r0 + q, 8), 8), cols].astype(f32)
                                for q in range(0, n, 8)], axis=0)

    def ln_stats(t, st):
        for step in range(32):
            pos = ((step % 2) * 16 + step // 2) * 16
            r0 = pl.multiple_of(t * T + pos, 16)
            x0 = x_block(r0, 16, pl.ds(0, 128)) + pin(16)
            s1 = s2 = None
            for j in range(1, 8):
                d = x_block(r0, 16, pl.ds(j * 128, 128)) - x0
                s1 = d if j == 1 else s1 + d
                s2 = d * d if j == 1 else s2 + d * d
            lane_mean = x0 + s1 * 0.125
            mean = jnp.sum(lane_mean, axis=-1, keepdims=True) * (1.0 / 128)
            d = lane_mean - mean
            var = jnp.sum((s2 - s1 * s1 * 0.125) * 0.125 + d * d, axis=-1, keepdims=True) * (1.0 / 128)
            var = (var.astype(bf16).astype(f32) + EPS_BF16).astype(bf16).astype(f32)
            st[0, pl.ds(pos, 16), :] = jnp.broadcast_to(mean.astype(bf16).astype(f32), (16, 128))
            st[1, pl.ds(pos, 16), :] = jnp.broadcast_to(1.0 / jnp.sqrt(var).astype(bf16).astype(f32), (16, 128))
            yield

    def ln_apply(t, st, dst, score_too):
        for step in range(16):
            r0 = [pl.multiple_of(t * T + b * TH + step * 16 + zero_s[0], 16) for b in range(2)]
            mean = [st[0, pl.ds(b * TH + step * 16, 16), :] for b in range(2)]
            scale = [st[1, pl.ds(b * TH + step * 16, 16), :] for b in range(2)]
            score = [None, None]
            for k in range(4):
                zero = pin(16)
                xn = [[(x_block(r0[b], 16, pl.ds(half * 512 + k * 128, 128)) - (mean[b] + zero)) * scale[b]
                       for half in range(2)] for b in range(2)]
                for i, v in enumerate(_rhs_operands(xn[0][0], xn[1][0], xn[0][1], xn[1][1])):
                    dst.at[i][pl.ds(step * 8, 8), pl.ds(k * 128, 128)] = _narrow(v)
                for b in range(2 if score_too else 0):
                    part = xn[b][0] * wr_v[:, pl.ds(k * 128, 128)] + xn[b][1] * wr_v[:, pl.ds(512 + k * 128, 128)]
                    score[b] = part if k == 0 else score[b] + part
                    if k == 3:
                        r = jnp.sum(score[b], axis=-1, keepdims=True).astype(bf16).astype(f32)
                        r = jnp.broadcast_to(r, (16, 128))
                        token = lax.broadcasted_iota(i32, (16, 128), 0) + r0[b] % S
                        slot = 2 * (t // NTILE) + b
                        better = r > best_v[slot]
                        best_v[slot] = jnp.where(better, r, best_v[slot])
                        best_i[slot] = jnp.where(better, token, best_i[slot])
                yield

    def ln_split(once, twice):
        for r in range(8):
            for k in range(2):
                yield from split_again(once, twice, False, r, k)

    def route():
        score, token = best_v[...].reshape(64, 128), best_i[...].reshape(64, 128)
        top = jnp.max(score, axis=0, keepdims=True)
        idx = jnp.min(jnp.where(score == top, token, S).astype(f32)).astype(i32)
        return jnp.clip(idx, 0, S - 1), top

    def routed_token():
        idx = route()[0]
        base = pl.multiple_of((idx // 16) * 16, 16)
        rows = pl.ds(pl.multiple_of(base % T, 16), 16)
        xn = (in_v[pl.ds(base, 16), :].astype(f32) - st_v[idx // T, 0, rows, 0:1]) * st_v[idx // T, 1, rows, 0:1]
        xn = jnp.where(lax.broadcasted_iota(i32, (16, D), 0) == idx - base, xn, 0.0)
        xn = jnp.sum(xn, axis=0, keepdims=True).astype(bf16).astype(f32)
        for j in range(8):
            row = xn[:, j * 128:(j + 1) * 128] + pin()
            xcol_v[pl.ds(j * 128, 128), :] = jnp.concatenate([row] * 16, axis=0).T
            yield

    def ffn(f0, n):
        for j in range(n):
            group, f = ffn_v.at[(f0 + j) // FG], (f0 + j) % FG
            accs = [jnp.zeros((8, 128), f32)] * 2
            for r in range(8):
                x, zero = xcol_v[pl.ds(r * 128, 128), :], pin()
                for a in range(2):
                    prod = group[pl.ds(_aligned((a * FG + f) * D + r * 128, 128), 128), :].astype(f32) * x
                    acc = accs[a] + zero
                    for q in range(16):
                        acc = acc + prod[8 * q:8 * q + 8]
                    accs[a] = acc
                yield
            gate, up = [jnp.sum(acc, axis=0, keepdims=True) for acc in accs]
            hidden = jnp.broadcast_to(gate * jax.nn.sigmoid(gate) * up, (128, 128)).T
            for c in range(8):
                prod = group[pl.ds(_aligned(2 * FG * D + (c * FG + f) * 128, 128), 128), :].astype(f32) * hidden
                acc = y_acc[:, pl.ds(c * 128, 128)] + pin()
                for q in range(16):
                    acc = acc + prod[8 * q:8 * q + 8]
                y_acc[:, pl.ds(c * 128, 128)] = acc
                if c % 2:
                    yield

    def project(w, x, res, keep=None):
        def emit(r, b, val):
            if isinstance(res, list):
                res[r][b] = val
            else:
                res[r, b] = val
            if keep is not None:
                keep[r, b] = val[64:]

        def once():
            for c in range(2):
                def put(a, b, val):
                    emit(2 * a, 2 * b + c, val[:128])
                    emit(2 * a + 1, 2 * b + c, val[128:])

                yield from _strassen(lambda i: matmul(w[i], x[i, pl.ds(c * 64, 64), :], 14), put)

        if isinstance(w, tuple):
            return _strassen_twice(lambda i: matmul(operand(*w, True, i), operand(*x, False, i), 49), emit), 49, 0.0, 1.0
        return once(), 14, 0.0, 1.0

    def project_part(w, x, res, part):
        def prod(i):
            rows = [w[i, pl.ds(a * 64 + part * 32, 32), :] for a in range(2)]
            return matmul(jnp.concatenate(rows, axis=0), x[i], 14)

        def put(a, b, val):
            for r in range(2):
                for c in range(2):
                    res[2 * a + r, 2 * b + c, pl.ds(part * 64, 64), :] = val[r * 64:(r + 1) * 64, c * 128:(c + 1) * 128]

        return _strassen(prod, put)

    def rows_of(res, r, r0, b):
        return res[r][b][r0:r0 + 64] if isinstance(res, list) else res[r, b, pl.ds(r0, 64), :]

    def kv_post(c, res, keep=None, values_late=False):
        same_head = lax.broadcasted_iota(i32, (64, 128), 0) // DH == lax.broadcasted_iota(i32, (64, 128), 1) % 2

        def accumulate(r, phi):
            v = jnp.concatenate([rows_of(res, r, 64, b) for b in range(4)], axis=1).astype(bf16)
            kv = kv_acc[4 * c + r] + _dot_nt(v, phi)
            kv_acc[4 * c + r] = kv
            kv_v.at[4 * c + r][...] = jnp.where(same_head, kv, 0.0).astype(bf16)

        pending = []
        for r in range(4):
            phis, z = [], z_acc[4 * c + r]
            for b in range(4):
                phi = _dual_softmax(rows_of(res, r, 0, b), pin())
                z = z + phi
                phis.append(phi)
                if keep is not None:
                    keep.at[r][:, pl.ds(b * 128, 128)] = _narrow(phi)
                if b == 1 and pending and not values_late:
                    accumulate(*pending.pop(0))
                if b == 3:
                    z_acc[4 * c + r] = z
                    z_v[4 * c + r] = jnp.broadcast_to(jnp.sum(z, axis=-1, keepdims=True), (128, 128))
                    pending.append((r, jnp.concatenate(phis, axis=1).astype(bf16)))
                yield
        yield
        for rest in pending:
            accumulate(*rest)
        yield

    def q_post(c, res, dst, ready=None):
        even = lax.broadcasted_iota(i32, (8, 128), 0) % 2 == 0
        phis, scales, nums, outs = {}, {}, {}, {}

        def pair(step):
            return 2 * (2 * c + step // 4 + 4 * ((step // 2) % 2)) + step % 2

        for tick in range(40):
            step, b = tick // 4, tick % 4
            if step < 8:
                r = 2 * ((step // 2) % 2) + step // 4
                if ready is None:
                    phi = _dual_softmax(rows_of(res, r, (step % 2) * 64, b), pin())
                elif step % 2:
                    phi = _dual_softmax(rows_of(res, r, 0, b), pin())
                else:
                    phi = _wide(ready[r, :, pl.ds(b * 128, 128)])
                den = phi * z_v[pair(step)]
                inv = _recip(_head_reduce([den[8 * j:8 * j + 8] for j in range(16)], jnp.add) + 1e-6)
                other = pltpu.roll(inv, 1, 0)
                phis.setdefault(step, []).append(phi)
                scales.setdefault(step, []).append((jnp.where(even, inv, other), jnp.where(even, other, inv)))
            if 1 <= step < 9 and b == 1:
                phi = jnp.concatenate(phis.pop(step - 1), axis=1).astype(bf16)
                nums[step - 1] = _dot(kv_v[pair(step - 1)], phi)
            if step >= 2 and b == 0:
                scale = scales.pop(step - 2)
                scale = [jnp.concatenate([v[head] for v in scale], axis=1) for head in range(2)]
                outs[step - 2] = nums.pop(step - 2) * jnp.concatenate([scale[0]] * 4 + [scale[1]] * 4, axis=0)
                if (step - 2) % 4 == 3:
                    u = (step - 2) // 4
                    o1 = jnp.concatenate([outs.pop(4 * u), outs.pop(4 * u + 1)], axis=0)
                    o2 = jnp.concatenate([outs.pop(4 * u + 2), outs.pop(4 * u + 3)], axis=0)
                    for i, v in enumerate(_rhs_operands(o1[:, :TH], o1[:, TH:], o2[:, :TH], o2[:, TH:])):
                        dst.at[i][:, pl.ds(u * 128, 128)] = pltpu.bitcast(v.astype(bf16).T, u32)
            yield

    def out_project(h, o, res, ks, per_slot):
        def prod(i):
            lhs = jnp.concatenate([o[k][i] for k in ks], axis=1)
            return matmul(lhs, wo_v[h, i, :, pl.ds(ks[0] * 256, len(ks) * 256)], per_slot)

        def emit(a, b, val):
            if isinstance(res, list):
                res[a][b] = val
            else:
                res[a, b] = val

        return _strassen(prod, emit)

    zero_s[0] = 0
    kv_acc[...] = jnp.zeros(kv_acc.shape, f32)
    z_acc[...] = jnp.zeros(z_acc.shape, f32)
    y_acc[...] = jnp.zeros(y_acc.shape, f32)
    best_v[...] = jnp.full(best_v.shape, -jnp.inf, f32)
    best_i[...] = jnp.zeros(best_i.shape, i32)
    w8 = wr8_v[...].astype(f32)
    wr_v[...] = jnp.broadcast_to(jnp.concatenate([w8[j:j + 1, :] for j in range(8)], axis=1), (16, D))
    feature_maps()
    stats, apply = ln_stats(0, st_v.at[0]), ln_apply(0, st_v.at[0], x1_v.at[0], False)
    for half in range(2):
        cp_x0(2 * half).wait()
        cp_x0(2 * half + 1).wait()
        schedule((stats, 16, 0.0, 1.0))
        schedule((apply, 32, 0.0, 1.0))
    chunk0 = prep_kv(0)
    schedule((chunk0, 4, 0.0, 1.0))
    schedule((project_part(a1_v.at[0], x1_v.at[0], raw_v.at[0], 0), 7, 0.0, 0.5),
             (project_part(a1_v.at[0], x1_v.at[0], raw_v.at[0], 1), 7, 0.5, 1.0),
             (project(a1_v.at[1], x1_v.at[0], raw_v.at[1])[0], 14, 1.0, 2.0),
             (chunk0, 4, 0.15, 0.45), (ln_split(x1_v.at[zero_s[0]], x2_v.at[0]), 112, 0.03, 0.6),
             (kv_post(0, raw_v.at[zero_s[0]], values_late=True), 18, 0.52, 1.3),
             (prep_kv(1), 8, 0.75, 1.0), (split_kv(1), 112, 1.0, 1.3),
             (prep_kv(2), 8, 1.05, 1.3), (split_kv(2), 112, 1.31, 1.62),
             (prep_kv(3), 8, 1.5, 1.72), (split_kv(3), 112, 1.73, 2.0))

    def kv_tile(t, _):
        last = t == NTILE - 1
        wait_all(q_blocks(t), sem_x.at[t + 1])
        cp_xt(t + 1).wait()

        @pl.when(jnp.logical_and(t > 0, t < 3))
        def _():
            cp_wo(t - 1).wait()

        product[:] = []
        first = (route()[0] // T) % (NTILE - 1) + 1
        x1, x2, st = x1_v.at[pl.ds(t, 2)], x2_v.at[pl.ds(t, 2)], st_v.at[t + 1]
        split = ln_split(x1_v.at[t + 1 + zero_s[0]], x2.at[1])
        wo = [prep_wo(2 * ((t + 1) % 2) + u, jnp.where(t == 0, WV, WO)) for u in range(2)]
        c2, c3, c0 = ([[None] * 4 for _ in range(4)] for _ in range(3))
        schedule(project((b1_v.at[0], b2_v.at[0]), (x1.at[0], x2.at[0]), c2),
                 (kv_post(1, raw_v.at[1]), 18, 0.08, 0.905), (ln_stats(t + 1, st), 32, 0.0, 0.96),
                 (start_ffn(t), 2 * FG + 8, 0.05, 0.95))
        schedule(project((b1_v.at[1], b2_v.at[1]), (x1.at[0], x2.at[0]), c3),
                 (kv_post(2, c2), 18, 0.08, 0.905), (ln_apply(t + 1, st, x1.at[1], True), 64, 0.015, 0.935),
                 (prep_q(t), 4, 0.075, 0.76))
        nxt, chunk = jnp.where(last, first, t + 1), jnp.where(last, 2, 0)
        schedule(project(a1_v.at[chunk], x1_v.at[nxt], c0, keep=half_v),
                 (kv_post(3, c3), 18, 0.08, 0.905), (split, 112, 0.0, 0.885), (split_q(t), 56, 0.12, 0.965))
        schedule(project((a1_v.at[chunk + 1], a2_v.at[chunk]), (x1_v.at[nxt], x2_v.at[nxt]), raw_v.at[1]),
                 (kv_post(jnp.where(last, 4, 0), c0, keep=phi_v), 18, 0.08, 0.905),
                 (wo[0], 4, 0.05, 0.645), (wo[1], 4, 0.42, 1.0), (routed_token(), 8, 0.025, 0.89))
        return first

    first = lax.fori_loop(0, NTILE, kv_tile, jnp.int32(0))

    wait_all(ffn_v.at[0], sem_f.at[0])
    product[:] = []
    idx, top_score = route()
    final = idx // T
    lo, hi = jnp.minimum(first, final), jnp.maximum(first, final)
    second = jnp.where(lo > 0, 0, jnp.where(hi > 1, 1, 2))
    third = 6 - first - final - second

    def tile(j):
        return jnp.where(j == 0, first, jnp.where(j == 1, second, jnp.where(j == 2, third, final)))

    def gate(t, h, a, b, q, update):
        r0, rows = pl.multiple_of(t * T + b * TH + q * EROWS, EROWS), pl.ds(b * TH + q * EROWS, EROWS)
        c0 = h * 512 + a * 256
        mean, scale = st_v[t, 0, rows, :], st_v[t, 1, rows, :] * 0.5
        if update is None:
            mean = mean + pin(EROWS)
        x = x_block(r0, EROWS, pl.ds(c0, 256))
        v = (x - jnp.concatenate([mean, mean], axis=1)) * jnp.concatenate([scale, scale], axis=1)
        if update is not None:
            hit = lax.broadcasted_iota(i32, (EROWS, 256), 0) == idx - r0
            v = v + jnp.where(hit, update[:, c0:c0 + 256], 0.0)
        return x, v + v * jnp.tanh(v)

    def epilogue(t, h, res, part=None, update=None, early=None):
        for a, b in ((0, 1), (0, 0), (1, 0), (1, 1)) if part is not None else ((0, 0), (0, 1), (1, 0), (1, 1)):
            for q in range(TH // EROWS):
                r0, cols = pl.multiple_of(t * T + b * TH + q * EROWS, EROWS), pl.ds(h * 512 + a * 256, 256)
                if early is not None and (a, b) == (1, 1):
                    x, g = x_block(r0, EROWS, cols), early[pl.ds(q * EROWS, EROWS), :]
                else:
                    x, g = gate(t, h, a, b, q, update)
                s = res[a][b][q * EROWS:(q + 1) * EROWS]
                if part is not None:
                    s = s + part[a, b, pl.ds(q * EROWS, EROWS), :]
                out_v[pl.ds(r0, EROWS), cols] = (x + s * g).astype(bf16)
                if part is not None and (q + 1) * EROWS % 128 == 0:
                    start_out(pl.ds(pl.multiple_of(t * T + b * TH + (q + 1) * EROWS - 128, 128), 128), cols)
                yield

    steps = 4 * TH // EROWS
    schedule((q_post(0, half_v, oa_v.at[0], ready=phi_v), 40, 0.0, 1.0))

    def q_tile(j, carry):
        product[:] = []
        oa = oa_v.at[pl.ds(j, 2)]
        o = oa.at[0], ob_v.at[zero_s[0]]
        x = x1_v.at[tile(j + 1)], x2_v.at[tile(j + 1)]
        wait_all(ffn_v.at[j + 1], sem_f.at[j + 1])
        hidden = ffn(j * FL, FL)
        q0, s0, s1 = ([[None] * 4 for _ in range(4)] for _ in range(3))
        schedule(project((a1_v.at[2], a2_v.at[1]), x, q0),
                 (q_post(1, raw_v.at[1], ob_v.at[0]), 40, 0.0, 1.0), (hidden, 14, 0.0, 0.89))
        schedule((out_project(0, o, s0, (0, 1), 7), 7, 0.0, 1.0),
                 (q_post(0, q0, oa.at[1]), 40, 0.0, 1.0), (hidden, 18, 0.085, 0.985))
        schedule((out_project(1, o, s1, (0, 1), 7), 7, 0.0, 1.0),
                 (epilogue(tile(j), 0, s0), steps, 0.055, 0.96), (hidden, 38, 0.02, 1.0))
        schedule(project((a1_v.at[3], a2_v.at[2]), x, raw_v.at[1]),
                 (epilogue(tile(j), 1, s1), steps, 0.0, 0.985), (hidden, 12 * FL - 70, 0.0, 0.885))
        start_out(pl.ds(pl.multiple_of(tile(j) * T, T), T), slice(None))
        return carry

    lax.fori_loop(0, NTILE - 1, q_tile, 0)

    product[:] = []
    o = oa_v.at[NTILE - 1], ob_v.at[zero_s[0]]
    rest = NF - (NTILE - 1) * FL
    schedule((out_project(0, o, part_v.at[0], (0,), 14), 7, 0.0, 0.5),
             (out_project(1, o, part_v.at[1], (0,), 14), 7, 0.5, 1.0),
             (q_post(1, raw_v.at[1], ob_v.at[0]), 40, 0.0, 0.9), (ffn(NF - rest, rest), 12 * rest, 0.1, 0.8))
    update = jnp.sum(y_acc[...], axis=0, keepdims=True) * (0.5 * jax.nn.sigmoid(top_score[:, 0:1]))
    s0, s1 = ([[None, None], [None, None]] for _ in range(2))

    def last_gate():
        for q in range(TH // EROWS):
            gate_v[0, pl.ds(q * EROWS, EROWS), :] = gate(final, 1, 1, 1, q, update)[1]
            yield

    schedule((out_project(0, o, s0, (1,), 14), 7, 0.0, 0.5), (out_project(1, o, s1, (1,), 14), 7, 0.5, 1.0),
             (epilogue(final, 0, s0, part_v.at[0], update), steps, 0.2, 0.7),
             (epilogue(final, 1, s1, part_v.at[1], update, gate_v.at[zero_s[0]]), steps, 0.7, 1.2),
             (last_gate(), TH // EROWS, 0.0, 0.2))
    pltpu.make_async_copy(out_v, out_hbm, sem_o.at[0]).wait()


def _call(x, wqkv, wphi, wo, wr, wg, wu, wd, interpret=False):
    scratch = [
        pltpu.VMEM((S + T + 4 * D, D), bf16),
        pltpu.VMEM((NTILE + 1, 2, T, 128), f32),
        pltpu.VMEM((NTILE + 1, 7, 128, 512), u32),
        pltpu.VMEM((NTILE + 1, 35, 64, 256), u32),
        pltpu.VMEM((D, DH), bf16),
        pltpu.VMEM((8, 128), bf16),
        pltpu.VMEM((16, D), f32),
        pltpu.VMEM((8, 128, 128), bf16),
        pltpu.VMEM((4, 7, 128, 512), u32),
        pltpu.VMEM((3, 35, 64, 256), u32),
        pltpu.VMEM((2, 7, 128, 512), u32),
        pltpu.VMEM((2, 35, 64, 256), u32),
        pltpu.VMEM((2, 7, 128, 512), u32),
        pltpu.VMEM((NTILE, 3 * FG * D, 128), bf16),
        pltpu.VMEM((H // 2 + 4, 64, 128), f32),
        pltpu.VMEM((H // 2 + 4, 128, 128), f32),
        pltpu.VMEM((H // 2 + 4, 64, 128), bf16),
        pltpu.VMEM((H // 2 + 4, 128, 128), f32),
        pltpu.VMEM((4, 16, 128), f32),
        pltpu.VMEM((4, 16, 128), i32),
        pltpu.VMEM((2, 4, 4, 128, 128), f32),
        pltpu.VMEM((4, 4, 64, 128), f32),
        pltpu.VMEM((4, 64, T), u32),
        pltpu.VMEM((NTILE, 7, 128, 256), u32),
        pltpu.VMEM((2, 7, 128, 256), u32),
        pltpu.VMEM((2, 2, 2, 256, 256), f32),
        pltpu.VMEM((2, 256, 256), f32),
        pltpu.VMEM((D, 128), f32),
        pltpu.VMEM((8, D), f32),
        pltpu.VMEM((S, D), bf16),
        pltpu.SMEM((1,), i32),
        pltpu.SemaphoreType.DMA((NTILE + 2,)),
        pltpu.SemaphoreType.DMA((5,)),
        pltpu.SemaphoreType.DMA((1,)),
        pltpu.SemaphoreType.DMA((NTILE,)),
        pltpu.SemaphoreType.DMA((1,)),
    ]
    hbm = pl.BlockSpec(memory_space=pltpu.HBM)
    return pl.pallas_call(
        _kernel,
        out_shape=jax.ShapeDtypeStruct((S, D), bf16),
        in_specs=[hbm] * 8,
        out_specs=hbm,
        scratch_shapes=scratch,
        compiler_params=pltpu.CompilerParams(
            vmem_limit_bytes=120 * 2**20, disable_bounds_checks=True, disable_semaphore_checks=True),
        name="hedgehog",
        interpret=interpret,
    )(x, wqkv, wphi, wo, wr, wg, wu, wd)


@jax.jit
def pallas_recurrent_scan__linear_kernel_hedgehog__moe_arch_mod__prompt_kernel(
    A_x: jax.Array,
    A_wqkv: jax.Array,
    A_w_phi: jax.Array,
    A_wo: jax.Array,
    B_x: jax.Array,
    B_w_r: jax.Array,
    B_w_gate: jax.Array,
    B_w_up: jax.Array,
    B_w_down: jax.Array,
):
    del B_x
    out = _call(A_x.reshape(S, D), A_wqkv, A_w_phi.reshape(D, DH), A_wo,
                B_w_r.reshape(8, 128), B_w_gate, B_w_up, B_w_down)
    return out.reshape(1, S, D)
```

```python
import math

import numpy as np

import jax
import jax.numpy as jnp
from jax import lax
import jax.experimental.pallas as pl
import jax.experimental.pallas.tpu as pltpu

S, D, H, DH, F = 2048, 1024, 32, 32, 3584
T = 512
TH = T // 2
NTILE = S // T
NF = F // 128
FG = NF // NTILE
FL = 9
EROWS = 32
WQ, WK, WV, WO = (S + T + j * D for j in range(4))
LHS_SUMS, RHS_SUMS = (0, 1, 4, 5, 6), (0, 2, 3, 5, 6)
LOG2E = math.log2(math.e)
EPS_BF16 = float(np.float32(1e-5).astype(jnp.bfloat16))
f32, bf16, i32, u32 = jnp.float32, jnp.bfloat16, jnp.int32, jnp.uint32


def _dot_nt(a, b):
    return lax.dot_general(a, b, (((1,), (1,)), ((), ())), preferred_element_type=f32)


def _dot(a, b):
    return jnp.dot(a, b, preferred_element_type=f32)


def _aligned(i, n):
    return i if isinstance(i, int) else pl.multiple_of(i, n)


def _recip(v):
    r = pl.reciprocal(v, approx=True)
    return r * (2.0 - v * r)


def _bf16(words):
    return pltpu.bitcast(words, bf16)


def _wide(words):
    return _bf16(words).astype(f32)


def _narrow(v):
    return pltpu.bitcast(v.astype(bf16), u32)


def _lhs_operands(a11, a12, a21, a22):
    return [a11 + a22, a21 + a22, a11, a22, a11 + a12, a21 - a11, a12 - a22]


def _rhs_operands(b11, b12, b21, b22):
    return [b11 + b22, b11, b12 - b22, b21 - b11, b22, b11 + b12, b21 + b22]


def _strassen(prod, emit):
    m3 = prod(2)
    yield
    m5 = prod(4)
    emit(0, 1, m3 + m5)
    yield
    m1 = prod(0)
    c11, c22 = m1 - m5, m1 + m3
    yield
    c11 = c11 + prod(6)
    yield
    m4 = prod(3)
    emit(0, 0, c11 + m4)
    yield
    m2 = prod(1)
    emit(1, 0, m2 + m4)
    c22 = c22 - m2
    yield
    emit(1, 1, c22 + prod(5))
    yield


class _Quad:
    def __init__(self, blocks):
        self.blocks = blocks

    def __add__(self, other):
        return _Quad([p + q for p, q in zip(self.blocks, other.blocks)])

    def __sub__(self, other):
        return _Quad([p - q for p, q in zip(self.blocks, other.blocks)])


def _strassen_twice(prod, emit):
    done = {}

    def inner(i):
        out = [None] * 4

        def put(a, b, val):
            out[2 * a + b] = val

        yield from _strassen(lambda j: prod(7 * i + j), put)
        done[i] = _Quad(out)

    def put(a, b, quad):
        for k, val in enumerate(quad.blocks):
            emit(2 * a + k // 2, 2 * b + k % 2, val)

    outer = _strassen(lambda i: done[i], put)
    for i in (2, 4, 0, 6, 3, 1, 5):
        steps = inner(i)
        for _ in range(6):
            next(steps)
            yield
        for _ in steps:
            pass
        next(outer)
        yield


def _head_reduce(vs, op):
    while len(vs) > 1:
        vs = [op(vs[i], vs[i + 1]) for i in range(0, len(vs), 2)]
    v = op(vs[0], pltpu.roll(vs[0], 4, 0))
    return op(v, pltpu.roll(v, 2, 0))


def _dual_softmax(p, zero):
    rows = [p[8 * j:8 * j + 8] for j in range(8)]
    rows[0] = rows[0] + zero
    mx, mn = _head_reduce(rows, jnp.maximum), _head_reduce(rows, jnp.minimum)
    ep = [jnp.exp2(v - mx) for v in rows]
    en = [jnp.exp2(mn - v) for v in rows]
    rp, rn = _recip(_head_reduce(ep, jnp.add)), _recip(_head_reduce(en, jnp.add))
    return jnp.concatenate([v * rp for v in ep] + [v * rn for v in en], axis=0)


def _kernel(x_hbm, wqkv_hbm, wphi_hbm, wo_hbm, wr_hbm, wg_hbm, wu_hbm, wd_hbm, out_hbm,
            in_v, st_v, x1_v, x2_v, wphi_v, wr8_v, wr_v, map_v, a1_v, a2_v, b1_v, b2_v, wo_v, ffn_v,
            kv_acc, z_acc, kv_v, z_v, best_v, best_i, raw_v, half_v, phi_v, oa_v, ob_v, part_v,
            gate_v, xcol_v, y_acc, out_v, zero_s, sem_x, sem_w, sem_s, sem_f, sem_o):
    def cp_x(r0, n, sem, src0):
        return pltpu.make_async_copy(x_hbm.at[pl.ds(src0, n)], in_v.at[pl.ds(r0, n)], sem_x.at[sem])

    def cp_x0(piece):
        r0 = (piece % 2) * TH + (piece // 2) * (TH // 2)
        return cp_x(r0, TH // 2, 0 if piece < 2 else NTILE + 1, r0)

    def cp_xt(t):
        return cp_x(_aligned(t * T, T), T, t, _aligned((t % NTILE) * T, T))

    def cp_w(j, c, sem):
        return pltpu.make_async_copy(wqkv_hbm.at[:, pl.ds(j * D + c * 256, 256)],
                                     in_v.at[pl.ds(WQ + j * D, D), pl.ds(c * 256, 256)], sem_w.at[sem])

    def cp_k(c):
        return cp_w(1, c, c)

    def cp_v(c):
        return cp_w(2, c, c if c else 4)

    def start_q(u):
        for n in range(8):
            src = wqkv_hbm.at[pl.ds((n // 2) * 256 + (u % 2) * 128, 128), pl.ds((u // 2) * 256 + (n % 2) * 512, 256)]
            dst = in_v.at[pl.ds(WQ + (u // 2) * 512 + (n // 2) * 128, 128), pl.ds((u % 2) * 512 + (n % 2) * 256, 256)]
            pltpu.make_async_copy(src, dst, sem_x.at[u + 1]).start()

    def q_blocks(u):
        return in_v.at[pl.ds(_aligned(WQ + (u // 2) * 512, 512), 512), pl.ds(_aligned((u % 2) * 512, 512), 512)]

    def cp_wo(h):
        cols = pl.ds(_aligned(h * 512, 512), 512)
        return pltpu.make_async_copy(wo_hbm.at[:, cols], in_v.at[pl.ds(WO, D), cols], sem_x.at[h + 2])

    def start_ffn(g):
        for j in range(FG):
            cols = pl.ds(_aligned((g * FG + j) * 128, 128), 128)
            for n, src in enumerate((wg_hbm, wu_hbm)):
                dst = ffn_v.at[g, pl.ds((n * FG + j) * D, D)]
                pltpu.make_async_copy(src.at[:, cols], dst, sem_f.at[g]).start()
                yield
        rows = pl.ds(_aligned(g * FG * 128, 128), FG * 128)
        for n in range(D // 128):
            dst = ffn_v.at[g, pl.ds(2 * FG * D + n * FG * 128, FG * 128)]
            pltpu.make_async_copy(wd_hbm.at[rows, pl.ds(n * 128, 128)], dst, sem_f.at[g]).start()
            yield

    def wait_all(filled, sem):
        pltpu.make_async_copy(filled, filled, sem).wait()

    def start_out(rows, cols):
        pltpu.make_async_copy(out_v.at[rows, cols], out_hbm.at[rows, cols], sem_o.at[0]).start()

    small = [pltpu.make_async_copy(wr_hbm, wr8_v, sem_s.at[0]), pltpu.make_async_copy(wphi_hbm, wphi_v, sem_s.at[0])]
    for cp in small + [cp_x0(0)]:
        cp.start()
    for cp in small:
        cp.wait()
    for piece in range(1, 4):
        cp_x0(piece).start()
    for c in range(4):
        cp_k(c).start()
        cp_v(c).start()
    for t in range(NTILE):
        cp_xt(t + 1).start()
        start_q(t)
        if t in (1, 2):
            cp_wo(t - 1).start()

    clock, product = [0.0], []

    def schedule(*streams):
        events = [(a + (b - a) * k / n, i, k, gen) for i, (gen, n, a, b) in enumerate(streams) for k in range(n)]
        for when, _, _, gen in sorted(events, key=lambda e: e[:3]):
            clock[:] = [when]
            next(gen)

    def matmul(a, b, per_slot):
        m = _dot_nt(_bf16(a), _bf16(b))
        product[:] = [m, per_slot]
        return m

    def pin(n=8):
        if not product:
            return jnp.zeros((n, 128), f32)
        m, per_slot = product
        rows, cols = m.shape[0] // 8, m.shape[1] // 128
        q = min(int((clock[0] * per_slot) % 1.0 * rows * cols + 1e-6), rows * cols - 1)
        m = m[(q % rows) * 8:(q % rows) * 8 + 8, (q // rows) * 128:(q // rows) * 128 + 128]
        z = pltpu.bitcast(pltpu.bitcast(m, u32) & zero_s[0].astype(u32), f32)
        return z if n == 8 else jnp.concatenate([z] * (n // 8), axis=0)

    def feature_maps():
        r = lax.broadcasted_iota(i32, (128, DH), 0)
        select = (((r % 64) // 8) * 4 + (r % 8) // 2 == lax.broadcasted_iota(i32, (128, DH), 1)).astype(bf16)
        r = lax.broadcasted_iota(i32, (128, 128), 0)
        same_head = (r // 64) * 2 + r % 2 == lax.broadcasted_iota(i32, (128, 128), 1) // DH
        for g in range(8):
            full = _dot_nt(select, wphi_v[pl.ds(g * 128, 128), :])
            map_v.at[g][...] = jnp.where(same_head, full, 0.0).astype(bf16)

    def put_lhs(dst, row, col, quadrants):
        for i, v in enumerate(_lhs_operands(*quadrants)):
            dst.at[i][pl.ds(_aligned(row, 8), 8), pl.ds(_aligned(col, 128), 128)] = _narrow(v)

    def w_blocks(base, top, bottom, k):
        return [in_v[pl.ds(_aligned(base + half * 512 + k * 128, 128), 128), pl.ds(_aligned(g * 128, 128), 128)]
                for g in (top, bottom) for half in range(2)]

    def put_folded(blocks, top, bottom, dst, row_of, k):
        blocks = [_dot_nt(map_v[g], w) for g, w in zip((top, top, bottom, bottom), blocks)]
        for j in range(8):
            put_lhs(dst, row_of(j), k * 128, [p[16 * j:16 * j + 16] * LOG2E for p in blocks])

    def put_transposed(base, top, bottom, dst, row_of):
        for k in range(4):
            zero = pltpu.bitcast(pin(), u32)
            blocks = [pltpu.bitcast(w, u32) for w in w_blocks(base, top, bottom, k)]
            blocks = [_bf16(jnp.concatenate([w[:8] | zero, w[8:]], axis=0)).T for w in blocks]
            for j in range(8):
                put_lhs(dst, row_of(j), k * 128, [w[16 * j:16 * j + 16].astype(f32) for w in blocks])
            yield

    def split_again(once, twice, lhs, r, k):
        for i in range(7):
            zero = pltpu.bitcast(pin(), u32)
            w = [[once[i, pl.ds(a * 64 + r * 8, 8), pl.ds(_aligned(b * 256 + k * 128, 128), 128)]
                  for b in range(2)] for a in range(2)]
            q00, q01, q10, q11 = _wide(w[0][0] | zero), _wide(w[0][1]), _wide(w[1][0]), _wide(w[1][1] | zero)
            sums = _lhs_operands(q00, q01, q10, q11) if lhs else _rhs_operands(q00, q10, q01, q11)
            for n, j in enumerate(LHS_SUMS if lhs else RHS_SUMS):
                twice.at[5 * i + n][pl.ds(r * 8, 8), pl.ds(_aligned(k * 128, 128), 128)] = _narrow(sums[j])
            yield

    def operand(once, twice, lhs, ij):
        i, j = ij // 7, ij % 7
        sums = LHS_SUMS if lhs else RHS_SUMS
        if j in sums:
            return twice[5 * i + sums.index(j)]
        d = int(j == (3 if lhs else 4))
        return once[i, pl.ds(d * 64, 64), pl.ds(d * 256, 256)]

    def prep_kv(c):
        dst = a1_v.at[c] if c < 2 else b1_v.at[c - 2]
        cp_k(c).wait()
        if c:
            cp_v(c).wait()
        for k in range(4):
            put_folded(w_blocks(WK, 2 * c, 2 * c + 1, k), 2 * c, 2 * c + 1, dst,
                       lambda j: (j // 4) * 64 + (j % 4) * 8, k)
            yield
        if not c:
            cp_v(c).wait()
        yield from put_transposed(WV, 2 * c, 2 * c + 1, dst, lambda j: (j // 4) * 64 + 32 + (j % 4) * 8)

    def split_kv(c):
        once, twice = (a1_v.at[1 + zero_s[0]], a2_v.at[0]) if c == 1 else (b1_v.at[c - 2 + zero_s[0]], b2_v.at[c - 2])
        for k in range(2):
            for r in range(8):
                yield from split_again(once, twice, True, r, k)

    def prep_q(u):
        w = q_blocks(u)
        for a in range(2):
            g = 2 * (u // 2) + a
            for c in range(2):
                blocks = [w[pl.ds((2 * half + c) * 128, 128), pl.ds(b * 256 + a * 128, 128)]
                          for b in range(2) for half in range(2)]
                put_folded(blocks, g, g + 4, a1_v.at[2 + u // 2], lambda j: a * 64 + 8 * j, u % 2 + 2 * c)
                yield

    def split_q(u):
        for r in range(8):
            yield from split_again(a1_v.at[2 + u // 2 + zero_s[0]], a2_v.at[1 + u // 2], True, r, u % 2)

    def prep_wo(u, base):
        g = (u // 2) * 4 + u % 2
        return put_transposed(base, g, g + 2, wo_v.at[u // 2], lambda j: (u % 2) * 64 + 8 * j)

    def x_block(r0, n, cols):
        return jnp.concatenate([in_v[pl.ds(pl.multiple_of(r0 + q + (zero_s[1] if q % 16 and n == 16 else 0), 8), 8), cols].astype(f32)
                                for q in range(0, n, 8)], axis=0)

    def ln_stats(t, st, batch):
        lane = lax.broadcasted_iota(i32, (16, 128), 1)
        for start in range(0, 32, batch):
            places = [((step % 2) * 16 + step // 2) * 16 for step in range(start, start + batch)]
            means = variances = jnp.ones((16, 128), f32)
            for n, pos in enumerate(places):
                r0 = pl.multiple_of(t * T + pos, 16)
                x0 = x_block(r0, 16, pl.ds(0, 128)) + pin(16)
                s1 = s2 = None
                for j in range(1, 8):
                    d = x_block(r0, 16, pl.ds(j * 128, 128)) - x0
                    s1 = d if j == 1 else s1 + d
                    s2 = d * d if j == 1 else s2 + d * d
                lane_mean = x0 + s1 * 0.125
                mean = jnp.sum(lane_mean, axis=-1, keepdims=True) * (1.0 / 128)
                d = lane_mean - mean
                var = jnp.sum((s2 - s1 * s1 * 0.125) * 0.125 + d * d, axis=-1, keepdims=True)
                variances = jnp.where(lane == n, jnp.broadcast_to(var, (16, 128)), variances)
                means = jnp.where(lane == n, jnp.broadcast_to(mean, (16, 128)), means)
                yield
            means = means.astype(bf16).astype(f32)
            var = ((variances * (1.0 / 128)).astype(bf16).astype(f32) + EPS_BF16).astype(bf16).astype(f32)
            scale = 1.0 / jnp.sqrt(var).astype(bf16).astype(f32)
            for n, pos in enumerate(places):
                for kind, v in enumerate((means, scale)):
                    st[kind, pl.ds(pos, 16), :] = jnp.broadcast_to(v[:, n:n + 1], (16, 128))
                if (n + 1) % (batch // 4) == 0:
                    yield

    def ln_apply(t, st, dst, score_too):
        for step in range(16):
            r0 = [pl.multiple_of(t * T + b * TH + step * 16 + zero_s[0], 16) for b in range(2)]
            mean = [st[0, pl.ds(b * TH + step * 16, 16), :] for b in range(2)]
            scale = [st[1, pl.ds(b * TH + step * 16, 16), :] for b in range(2)]
            score = [None, None]
            for k in range(4):
                zero = pin(16)
                xn = [[(x_block(r0[b], 16, pl.ds(half * 512 + k * 128, 128)) - (mean[b] + zero)) * scale[b]
                       for half in range(2)] for b in range(2)]
                for i, v in enumerate(_rhs_operands(xn[0][0], xn[1][0], xn[0][1], xn[1][1])):
                    dst.at[i][pl.ds(step * 8, 8), pl.ds(k * 128, 128)] = _narrow(v)
                for b in range(2 if score_too else 0):
                    part = xn[b][0] * wr_v[:, pl.ds(k * 128, 128)] + xn[b][1] * wr_v[:, pl.ds(512 + k * 128, 128)]
                    score[b] = part if k == 0 else score[b] + part
                    if k == 3:
                        r = jnp.sum(score[b], axis=-1, keepdims=True).astype(bf16).astype(f32)
                        r = jnp.broadcast_to(r, (16, 128))
                        token = lax.broadcasted_iota(i32, (16, 128), 0) + r0[b] % S
                        slot = 2 * (t // NTILE) + b
                        better = r > best_v[slot]
                        best_v[slot] = jnp.where(better, r, best_v[slot])
                        best_i[slot] = jnp.where(better, token, best_i[slot])
                yield

    def ln_split(once, twice):
        for r in range(8):
            for k in range(2):
                yield from split_again(once, twice, False, r, k)

    def route():
        score, token = best_v[...].reshape(64, 128), best_i[...].reshape(64, 128)
        top = jnp.max(score, axis=0, keepdims=True)
        idx = jnp.min(jnp.where(score == top, token, S).astype(f32)).astype(i32)
        return jnp.clip(idx, 0, S - 1), top

    def routed_token():
        idx = route()[0]
        base = pl.multiple_of((idx // 16) * 16, 16)
        rows = pl.ds(pl.multiple_of(base % T, 16), 16)
        xn = (in_v[pl.ds(base, 16), :].astype(f32) - st_v[idx // T, 0, rows, 0:1]) * st_v[idx // T, 1, rows, 0:1]
        xn = jnp.where(lax.broadcasted_iota(i32, (16, D), 0) == idx - base, xn, 0.0)
        xn = jnp.sum(xn, axis=0, keepdims=True).astype(bf16).astype(f32)
        for j in range(8):
            row = xn[:, j * 128:(j + 1) * 128] + pin()
            xcol_v[pl.ds(j * 128, 128), :] = jnp.concatenate([row] * 16, axis=0).T
            yield

    def ffn(f0, n):
        for j in range(n):
            group, f = ffn_v.at[(f0 + j) // FG], (f0 + j) % FG
            accs = [jnp.zeros((8, 128), f32)] * 2
            for r in range(8):
                x, zero = xcol_v[pl.ds(r * 128, 128), :], pin()
                for a in range(2):
                    prod = group[pl.ds(_aligned((a * FG + f) * D + r * 128, 128), 128), :].astype(f32) * x
                    acc = accs[a] + zero
                    for q in range(16):
                        acc = acc + prod[8 * q:8 * q + 8]
                    accs[a] = acc
                yield
            gate, up = [jnp.sum(acc, axis=0, keepdims=True) for acc in accs]
            hidden = jnp.broadcast_to(gate * jax.nn.sigmoid(gate) * up, (128, 128)).T
            for c in range(8):
                prod = group[pl.ds(_aligned(2 * FG * D + (c * FG + f) * 128, 128), 128), :].astype(f32) * hidden
                acc = y_acc[:, pl.ds(c * 128, 128)] + pin()
                for q in range(16):
                    acc = acc + prod[8 * q:8 * q + 8]
                y_acc[:, pl.ds(c * 128, 128)] = acc
                if c % 2:
                    yield

    def project(w, x, res, keep=None):
        def emit(r, b, val):
            if isinstance(res, list):
                res[r][b] = val
            else:
                res[r, b] = val
            if keep is not None:
                keep[r, b] = val[64:]

        def once():
            for c in range(2):
                def put(a, b, val):
                    emit(2 * a, 2 * b + c, val[:128])
                    emit(2 * a + 1, 2 * b + c, val[128:])

                yield from _strassen(lambda i: matmul(w[i], x[i, pl.ds(c * 64, 64), :], 14), put)

        if isinstance(w, tuple):
            return _strassen_twice(lambda i: matmul(operand(*w, True, i), operand(*x, False, i), 49), emit), 49, 0.0, 1.0
        return once(), 14, 0.0, 1.0

    def project_part(w, x, res, part):
        def prod(i):
            rows = [w[i, pl.ds(a * 64 + part * 32, 32), :] for a in range(2)]
            return matmul(jnp.concatenate(rows, axis=0), x[i], 14)

        def put(a, b, val):
            for r in range(2):
                for c in range(2):
                    res[2 * a + r, 2 * b + c, pl.ds(part * 64, 64), :] = val[r * 64:(r + 1) * 64, c * 128:(c + 1) * 128]

        return _strassen(prod, put)

    def rows_of(res, r, r0, b):
        return res[r][b][r0:r0 + 64] if isinstance(res, list) else res[r, b, pl.ds(r0, 64), :]

    def kv_post(c, res, keep=None, values_late=False):
        same_head = lax.broadcasted_iota(i32, (64, 128), 0) // DH == lax.broadcasted_iota(i32, (64, 128), 1) % 2

        def accumulate(r, phi):
            v = jnp.concatenate([rows_of(res, r, 64, b) for b in range(4)], axis=1).astype(bf16)
            kv = kv_acc[4 * c + r] + _dot_nt(v, phi)
            kv_acc[4 * c + r] = kv
            kv_v.at[4 * c + r][...] = jnp.where(same_head, kv, 0.0).astype(bf16)

        pending = []
        for r in range(4):
            phis, z = [], z_acc[4 * c + r]
            for b in range(4):
                phi = _dual_softmax(rows_of(res, r, 0, b), pin())
                z = z + phi
                phis.append(phi)
                if keep is not None:
                    keep.at[r][:, pl.ds(b * 128, 128)] = _narrow(phi)
                if b == 1 and pending and not values_late:
                    accumulate(*pending.pop(0))
                if b == 3:
                    z_acc[4 * c + r] = z
                    z_v[4 * c + r] = jnp.broadcast_to(jnp.sum(z, axis=-1, keepdims=True), (128, 128))
                    pending.append((r, jnp.concatenate(phis, axis=1).astype(bf16)))
                yield
        yield
        for rest in pending:
            accumulate(*rest)
        yield

    def q_post(c, res, dst, ready=None):
        even = lax.broadcasted_iota(i32, (8, 128), 0) % 2 == 0
        phis, scales, nums, outs = {}, {}, {}, {}

        def pair(step):
            return 2 * (2 * c + step // 4 + 4 * ((step // 2) % 2)) + step % 2

        for tick in range(40):
            step, b = tick // 4, tick % 4
            if step < 8:
                r = 2 * ((step // 2) % 2) + step // 4
                if ready is None:
                    phi = _dual_softmax(rows_of(res, r, (step % 2) * 64, b), pin())
                elif step % 2:
                    phi = _dual_softmax(rows_of(res, r, 0, b), pin())
                else:
                    phi = _wide(ready[r, :, pl.ds(b * 128, 128)])
                den = phi * z_v[pair(step)]
                inv = _recip(_head_reduce([den[8 * j:8 * j + 8] for j in range(16)], jnp.add) + 1e-6)
                other = pltpu.roll(inv, 1, 0)
                phis.setdefault(step, []).append(phi)
                scales.setdefault(step, []).append((jnp.where(even, inv, other), jnp.where(even, other, inv)))
            if 1 <= step < 9 and b == 1:
                phi = jnp.concatenate(phis.pop(step - 1), axis=1).astype(bf16)
                nums[step - 1] = _dot(kv_v[pair(step - 1)], phi)
            if step >= 2 and b == 0:
                scale = scales.pop(step - 2)
                scale = [jnp.concatenate([v[head] for v in scale], axis=1) for head in range(2)]
                outs[step - 2] = nums.pop(step - 2) * jnp.concatenate([scale[0]] * 4 + [scale[1]] * 4, axis=0)
                if (step - 2) % 4 == 3:
                    u = (step - 2) // 4
                    o1 = jnp.concatenate([outs.pop(4 * u), outs.pop(4 * u + 1)], axis=0)
                    o2 = jnp.concatenate([outs.pop(4 * u + 2), outs.pop(4 * u + 3)], axis=0)
                    for i, v in enumerate(_rhs_operands(o1[:, :TH], o1[:, TH:], o2[:, :TH], o2[:, TH:])):
                        dst.at[i][:, pl.ds(u * 128, 128)] = pltpu.bitcast(v.astype(bf16).T, u32)
            yield

    def out_project(h, o, res, ks, per_slot):
        def prod(i):
            lhs = jnp.concatenate([o[k][i] for k in ks], axis=1)
            return matmul(lhs, wo_v[h, i, :, pl.ds(ks[0] * 256, len(ks) * 256)], per_slot)

        def emit(a, b, val):
            if isinstance(res, list):
                res[a][b] = val
            else:
                res[a, b] = val

        return _strassen(prod, emit)

    zero_s[0] = 0
    zero_s[1] = 0
    kv_acc[...] = jnp.zeros(kv_acc.shape, f32)
    z_acc[...] = jnp.zeros(z_acc.shape, f32)
    y_acc[...] = jnp.zeros(y_acc.shape, f32)
    best_v[...] = jnp.full(best_v.shape, -jnp.inf, f32)
    best_i[...] = jnp.zeros(best_i.shape, i32)
    w8 = wr8_v[...].astype(f32)
    wr_v[...] = jnp.broadcast_to(jnp.concatenate([w8[j:j + 1, :] for j in range(8)], axis=1), (16, D))
    feature_maps()
    stats, apply = ln_stats(0, st_v.at[0], 16), ln_apply(0, st_v.at[0], x1_v.at[0], False)
    for half in range(2):
        cp_x0(2 * half).wait()
        cp_x0(2 * half + 1).wait()
        schedule((stats, 20, 0.0, 1.0))
        schedule((apply, 32, 0.0, 1.0))
    chunk0 = prep_kv(0)
    schedule((chunk0, 4, 0.0, 1.0))
    schedule((project_part(a1_v.at[0], x1_v.at[0], raw_v.at[0], 0), 7, 0.0, 0.5),
             (project_part(a1_v.at[0], x1_v.at[0], raw_v.at[0], 1), 7, 0.5, 1.0),
             (project(a1_v.at[1], x1_v.at[0], raw_v.at[1])[0], 14, 1.0, 2.0),
             (chunk0, 4, 0.15, 0.45), (ln_split(x1_v.at[zero_s[0]], x2_v.at[0]), 112, 0.03, 0.6),
             (kv_post(0, raw_v.at[zero_s[0]], values_late=True), 18, 0.52, 1.3),
             (prep_kv(1), 8, 0.75, 1.0), (split_kv(1), 112, 1.02, 1.31),
             (prep_kv(2), 8, 1.05, 1.3), (split_kv(2), 112, 1.31, 1.62),
             (prep_kv(3), 8, 1.5, 1.72), (split_kv(3), 112, 1.73, 2.0))

    def kv_tile(t, _):
        last = t == NTILE - 1
        wait_all(q_blocks(t), sem_x.at[t + 1])
        cp_xt(t + 1).wait()

        @pl.when(jnp.logical_and(t > 0, t < 3))
        def _():
            cp_wo(t - 1).wait()

        product[:] = []
        first = (route()[0] // T) % (NTILE - 1) + 1
        x1, x2, st = x1_v.at[pl.ds(t, 2)], x2_v.at[pl.ds(t, 2)], st_v.at[t + 1]
        split = ln_split(x1_v.at[t + 1 + zero_s[0]], x2.at[1])
        wo = [prep_wo(2 * ((t + 1) % 2) + u, jnp.where(t == 0, WV, WO)) for u in range(2)]
        c2, c3, c0 = ([[None] * 4 for _ in range(4)] for _ in range(3))
        schedule(project((b1_v.at[0], b2_v.at[0]), (x1.at[0], x2.at[0]), c2),
                 (kv_post(1, raw_v.at[1]), 18, 0.068, 0.965), (ln_stats(t + 1, st, 32), 36, 0.0, 0.99),
                 (start_ffn(t), 2 * FG + 8, 0.05, 0.95))
        schedule(project((b1_v.at[1], b2_v.at[1]), (x1.at[0], x2.at[0]), c3),
                 (kv_post(2, c2), 18, 0.08, 0.965), (ln_apply(t + 1, st, x1.at[1], True), 64, 0.015, 0.935),
                 (prep_q(t), 4, 0.0, 0.656))
        nxt, chunk = jnp.where(last, first, t + 1), jnp.where(last, 2, 0)
        schedule(project(a1_v.at[chunk], x1_v.at[nxt], c0, keep=half_v),
                 (kv_post(3, c3), 18, 0.0, 0.917), (split, 112, 0.0, 0.873), (split_q(t), 56, 0.1, 0.942))
        schedule(project((a1_v.at[chunk + 1], a2_v.at[chunk]), (x1_v.at[nxt], x2_v.at[nxt]), raw_v.at[1]),
                 (kv_post(jnp.where(last, 4, 0), c0, keep=phi_v), 18, 0.08, 0.905),
                 (wo[0], 4, 0.05, 0.69), (wo[1], 4, 0.435, 0.985), (routed_token(), 8, 0.025, 0.878))
        return first

    first = lax.fori_loop(0, NTILE, kv_tile, jnp.int32(0))

    wait_all(ffn_v.at[0], sem_f.at[0])
    product[:] = []
    idx, top_score = route()
    final = idx // T
    lo, hi = jnp.minimum(first, final), jnp.maximum(first, final)
    second = jnp.where(lo > 0, 0, jnp.where(hi > 1, 1, 2))
    third = 6 - first - final - second

    def tile(j):
        return jnp.where(j == 0, first, jnp.where(j == 1, second, jnp.where(j == 2, third, final)))

    def gate(t, h, a, b, q, update):
        r0, rows = pl.multiple_of(t * T + b * TH + q * EROWS, EROWS), pl.ds(b * TH + q * EROWS, EROWS)
        c0 = h * 512 + a * 256
        mean, scale = st_v[t, 0, rows, :], st_v[t, 1, rows, :] * 0.5
        if update is None:
            mean = mean + pin(EROWS)
        x = x_block(r0, EROWS, pl.ds(c0, 256))
        v = (x - jnp.concatenate([mean, mean], axis=1)) * jnp.concatenate([scale, scale], axis=1)
        if update is not None:
            hit = lax.broadcasted_iota(i32, (EROWS, 256), 0) == idx - r0
            v = v + jnp.where(hit, update[:, c0:c0 + 256], 0.0)
        return x, v + v * jnp.tanh(v)

    def epilogue(t, h, res, part=None, update=None, early=None):
        for a, b in ((0, 1), (0, 0), (1, 0), (1, 1)) if part is not None else ((0, 0), (0, 1), (1, 0), (1, 1)):
            for q in range(TH // EROWS):
                r0, cols = pl.multiple_of(t * T + b * TH + q * EROWS, EROWS), pl.ds(h * 512 + a * 256, 256)
                if early is not None and (a, b) == (1, 1):
                    x, g = x_block(r0, EROWS, cols), early[pl.ds(q * EROWS, EROWS), :]
                else:
                    x, g = gate(t, h, a, b, q, update)
                s = res[a][b][q * EROWS:(q + 1) * EROWS]
                if part is not None:
                    s = s + part[a, b, pl.ds(q * EROWS, EROWS), :]
                out_v[pl.ds(r0, EROWS), cols] = (x + s * g).astype(bf16)
                if part is not None and (q + 1) * EROWS % 128 == 0:
                    start_out(pl.ds(pl.multiple_of(t * T + b * TH + (q + 1) * EROWS - 128, 128), 128), cols)
                yield

    steps = 4 * TH // EROWS
    schedule((q_post(0, half_v, oa_v.at[0], ready=phi_v), 40, 0.01, 1.0))

    def q_tile(j, carry):
        product[:] = []
        oa = oa_v.at[pl.ds(j, 2)]
        o = oa.at[0], ob_v.at[zero_s[0]]
        x = x1_v.at[tile(j + 1)], x2_v.at[tile(j + 1)]
        wait_all(ffn_v.at[j + 1], sem_f.at[j + 1])
        hidden = ffn(j * FL, FL)
        q0, s0, s1 = ([[None] * 4 for _ in range(4)] for _ in range(3))
        schedule(project((a1_v.at[2], a2_v.at[1]), x, q0),
                 (q_post(1, raw_v.at[1], ob_v.at[0]), 40, 0.0, 1.0), (hidden, 14, 0.0, 0.89))
        schedule((out_project(0, o, s0, (0, 1), 7), 7, 0.0, 1.0),
                 (q_post(0, q0, oa.at[1]), 40, 0.0, 1.0), (hidden, 18, 0.085, 0.985))
        schedule((out_project(1, o, s1, (0, 1), 7), 7, 0.0, 1.0),
                 (epilogue(tile(j), 0, s0), steps, 0.055, 0.96), (hidden, 38, 0.02, 1.0))
        schedule(project((a1_v.at[3], a2_v.at[2]), x, raw_v.at[1]),
                 (epilogue(tile(j), 1, s1), steps, 0.0, 0.985), (hidden, 12 * FL - 70, 0.0, 0.885))
        start_out(pl.ds(pl.multiple_of(tile(j) * T, T), T), slice(None))
        return carry

    lax.fori_loop(0, NTILE - 1, q_tile, 0)

    product[:] = []
    o = oa_v.at[NTILE - 1], ob_v.at[zero_s[0]]
    rest = NF - (NTILE - 1) * FL
    schedule((out_project(0, o, part_v.at[0], (0,), 14), 7, 0.0, 0.5),
             (out_project(1, o, part_v.at[1], (0,), 14), 7, 0.5, 1.0),
             (q_post(1, raw_v.at[1], ob_v.at[0]), 40, 0.0, 0.9), (ffn(NF - rest, rest), 12 * rest, 0.1, 0.8))
    update = jnp.sum(y_acc[...], axis=0, keepdims=True) * (0.5 * jax.nn.sigmoid(top_score[:, 0:1]))
    s0, s1 = ([[None, None], [None, None]] for _ in range(2))

    def last_gate():
        for q in range(TH // EROWS):
            gate_v[0, pl.ds(q * EROWS, EROWS), :] = gate(final, 1, 1, 1, q, update)[1]
            yield

    schedule((out_project(0, o, s0, (1,), 14), 7, 0.0, 0.5), (out_project(1, o, s1, (1,), 14), 7, 0.5, 1.0),
             (epilogue(final, 0, s0, part_v.at[0], update), steps, 0.2, 0.7),
             (epilogue(final, 1, s1, part_v.at[1], update, gate_v.at[zero_s[0]]), steps, 0.69, 1.21),
             (last_gate(), TH // EROWS, 0.0, 0.2))
    pltpu.make_async_copy(out_v, out_hbm, sem_o.at[0]).wait()


def _call(x, wqkv, wphi, wo, wr, wg, wu, wd, interpret=False):
    scratch = [
        pltpu.VMEM((S + T + 4 * D, D), bf16),
        pltpu.VMEM((NTILE + 1, 2, T, 128), f32),
        pltpu.VMEM((NTILE + 1, 7, 128, 512), u32),
        pltpu.VMEM((NTILE + 1, 35, 64, 256), u32),
        pltpu.VMEM((D, DH), bf16),
        pltpu.VMEM((8, 128), bf16),
        pltpu.VMEM((16, D), f32),
        pltpu.VMEM((8, 128, 128), bf16),
        pltpu.VMEM((4, 7, 128, 512), u32),
        pltpu.VMEM((3, 35, 64, 256), u32),
        pltpu.VMEM((2, 7, 128, 512), u32),
        pltpu.VMEM((2, 35, 64, 256), u32),
        pltpu.VMEM((2, 7, 128, 512), u32),
        pltpu.VMEM((NTILE, 3 * FG * D, 128), bf16),
        pltpu.VMEM((H // 2 + 4, 64, 128), f32),
        pltpu.VMEM((H // 2 + 4, 128, 128), f32),
        pltpu.VMEM((H // 2 + 4, 64, 128), bf16),
        pltpu.VMEM((H // 2 + 4, 128, 128), f32),
        pltpu.VMEM((4, 16, 128), f32),
        pltpu.VMEM((4, 16, 128), i32),
        pltpu.VMEM((2, 4, 4, 128, 128), f32),
        pltpu.VMEM((4, 4, 64, 128), f32),
        pltpu.VMEM((4, 64, T), u32),
        pltpu.VMEM((NTILE, 7, 128, 256), u32),
        pltpu.VMEM((2, 7, 128, 256), u32),
        pltpu.VMEM((2, 2, 2, 256, 256), f32),
        pltpu.VMEM((2, 256, 256), f32),
        pltpu.VMEM((D, 128), f32),
        pltpu.VMEM((8, D), f32),
        pltpu.VMEM((S, D), bf16),
        pltpu.SMEM((2,), i32),
        pltpu.SemaphoreType.DMA((NTILE + 2,)),
        pltpu.SemaphoreType.DMA((5,)),
        pltpu.SemaphoreType.DMA((1,)),
        pltpu.SemaphoreType.DMA((NTILE,)),
        pltpu.SemaphoreType.DMA((1,)),
    ]
    hbm = pl.BlockSpec(memory_space=pltpu.HBM)
    return pl.pallas_call(
        _kernel,
        out_shape=jax.ShapeDtypeStruct((S, D), bf16),
        in_specs=[hbm] * 8,
        out_specs=hbm,
        scratch_shapes=scratch,
        compiler_params=pltpu.CompilerParams(
            vmem_limit_bytes=120 * 2**20, disable_bounds_checks=True, disable_semaphore_checks=True),
        name="hedgehog",
        interpret=interpret,
    )(x, wqkv, wphi, wo, wr, wg, wu, wd)


@jax.jit
def pallas_recurrent_scan__linear_kernel_hedgehog__moe_arch_mod__prompt_kernel(
    A_x: jax.Array,
    A_wqkv: jax.Array,
    A_w_phi: jax.Array,
    A_wo: jax.Array,
    B_x: jax.Array,
    B_w_r: jax.Array,
    B_w_gate: jax.Array,
    B_w_up: jax.Array,
    B_w_down: jax.Array,
):
    del B_x
    out = _call(A_x.reshape(S, D), A_wqkv, A_w_phi.reshape(D, DH), A_wo,
                B_w_r.reshape(8, 128), B_w_gate, B_w_up, B_w_down)
    return out.reshape(1, S, D)
```

```python
import math

import numpy as np

import jax
import jax.numpy as jnp
from jax import lax
import jax.experimental.pallas as pl
import jax.experimental.pallas.tpu as pltpu

S, D, H, DH, F = 2048, 1024, 32, 32, 3584
T = 512
TH = T // 2
NTILE = S // T
NF = F // 128
FG = NF // NTILE
FL = 9
EROWS = 32
WQ, WK, WV, WO = (S + T + j * D for j in range(4))
LHS_SUMS, RHS_SUMS = (0, 1, 4, 5, 6), (0, 2, 3, 5, 6)
LOG2E = math.log2(math.e)
EPS_BF16 = float(np.float32(1e-5).astype(jnp.bfloat16))
f32, bf16, i32, u32 = jnp.float32, jnp.bfloat16, jnp.int32, jnp.uint32


def _dot_nt(a, b):
    return lax.dot_general(a, b, (((1,), (1,)), ((), ())), preferred_element_type=f32)


def _dot(a, b):
    return jnp.dot(a, b, preferred_element_type=f32)


def _aligned(i, n):
    return i if isinstance(i, int) else pl.multiple_of(i, n)


def _recip(v):
    r = pl.reciprocal(v, approx=True)
    return r * (2.0 - v * r)


def _bf16(words):
    return pltpu.bitcast(words, bf16)


def _wide(words):
    return _bf16(words).astype(f32)


def _narrow(v):
    return pltpu.bitcast(v.astype(bf16), u32)


def _lhs_operands(a11, a12, a21, a22):
    return [a11 + a22, a21 + a22, a11, a22, a11 + a12, a21 - a11, a12 - a22]


def _rhs_operands(b11, b12, b21, b22):
    return [b11 + b22, b11, b12 - b22, b21 - b11, b22, b11 + b12, b21 + b22]


def _strassen(prod, emit):
    m3 = prod(2)
    yield
    m5 = prod(4)
    emit(0, 1, m3 + m5)
    yield
    m1 = prod(0)
    c11, c22 = m1 - m5, m1 + m3
    yield
    c11 = c11 + prod(6)
    yield
    m4 = prod(3)
    emit(0, 0, c11 + m4)
    yield
    m2 = prod(1)
    emit(1, 0, m2 + m4)
    c22 = c22 - m2
    yield
    emit(1, 1, c22 + prod(5))
    yield


class _Quad:
    def __init__(self, blocks):
        self.blocks = blocks

    def __add__(self, other):
        return _Quad([p + q for p, q in zip(self.blocks, other.blocks)])

    def __sub__(self, other):
        return _Quad([p - q for p, q in zip(self.blocks, other.blocks)])


def _strassen_twice(prod, emit):
    done = {}

    def inner(i):
        out = [None] * 4

        def put(a, b, val):
            out[2 * a + b] = val

        yield from _strassen(lambda j: prod(7 * i + j), put)
        done[i] = _Quad(out)

    def put(a, b, quad):
        for k, val in enumerate(quad.blocks):
            emit(2 * a + k // 2, 2 * b + k % 2, val)

    outer = _strassen(lambda i: done[i], put)
    for i in (2, 4, 0, 6, 3, 1, 5):
        steps = inner(i)
        for _ in range(6):
            next(steps)
            yield
        for _ in steps:
            pass
        next(outer)
        yield


def _head_reduce(vs, op):
    while len(vs) > 1:
        vs = [op(vs[i], vs[i + 1]) for i in range(0, len(vs), 2)]
    v = op(vs[0], pltpu.roll(vs[0], 4, 0))
    return op(v, pltpu.roll(v, 2, 0))


def _dual_softmax(p, zero):
    rows = [p[8 * j:8 * j + 8] for j in range(8)]
    rows[0] = rows[0] + zero
    mx, mn = _head_reduce(rows, jnp.maximum), _head_reduce(rows, jnp.minimum)
    ep = [jnp.exp2(v - mx) for v in rows]
    en = [jnp.exp2(mn - v) for v in rows]
    rp, rn = _recip(_head_reduce(ep, jnp.add)), _recip(_head_reduce(en, jnp.add))
    return jnp.concatenate([v * rp for v in ep] + [v * rn for v in en], axis=0)


def _kernel(x_hbm, wqkv_hbm, wphi_hbm, wo_hbm, wr_hbm, wg_hbm, wu_hbm, wd_hbm, out_hbm,
            in_v, st_v, x1_v, x2_v, wphi_v, wr8_v, wr_v, map_v, a1_v, a2_v, b1_v, b2_v, wo_v, ffn_v,
            kv_acc, z_acc, kv_v, z_v, best_v, best_i, raw_v, half_v, phi_v, oa_v, ob_v, part_v,
            gate_v, xcol_v, y_acc, out_v, zero_s, sem_x, sem_w, sem_q, sem_s, sem_f, sem_o):
    def cp_x(r0, n, sem, src0):
        return pltpu.make_async_copy(x_hbm.at[pl.ds(src0, n)], in_v.at[pl.ds(r0, n)], sem_x.at[sem])

    def cp_x0(piece):
        r0 = (piece % 2) * TH + (piece // 2) * (TH // 2)
        return cp_x(r0, TH // 2, 0 if piece < 2 else NTILE + 1, r0)

    def cp_xt(t):
        return cp_x(_aligned(t * T, T), T, t, _aligned((t % NTILE) * T, T))

    def cp_w(j, c, sem):
        return pltpu.make_async_copy(wqkv_hbm.at[:, pl.ds(j * D + c * 256, 256)],
                                     in_v.at[pl.ds(WQ + j * D, D), pl.ds(c * 256, 256)], sem_w.at[sem])

    def cp_k(c):
        return cp_w(1, c, c)

    def cp_v(c):
        return cp_w(2, c, c if c else 4)

    def start_q(u):
        for n in range(8):
            src = wqkv_hbm.at[pl.ds((n // 2) * 256 + (u % 2) * 128, 128), pl.ds((u // 2) * 256 + (n % 2) * 512, 256)]
            dst = in_v.at[pl.ds(WQ + (u // 2) * 512 + (n // 2) * 128, 128), pl.ds((u % 2) * 512 + (n % 2) * 256, 256)]
            pltpu.make_async_copy(src, dst, sem_q.at[u]).start()

    def q_blocks(u):
        return in_v.at[pl.ds(_aligned(WQ + (u // 2) * 512, 512), 512), pl.ds(_aligned((u % 2) * 512, 512), 512)]

    def cp_wo(h):
        cols = pl.ds(_aligned(h * 512, 512), 512)
        return pltpu.make_async_copy(wo_hbm.at[:, cols], in_v.at[pl.ds(WO, D), cols], sem_q.at[NTILE + h])

    def start_ffn(g):
        for j in range(FG):
            cols = pl.ds(_aligned((g * FG + j) * 128, 128), 128)
            for n, src in enumerate((wg_hbm, wu_hbm)):
                dst = ffn_v.at[g, pl.ds((n * FG + j) * D, D)]
                pltpu.make_async_copy(src.at[:, cols], dst, sem_f.at[g]).start()
                yield
        rows = pl.ds(_aligned(g * FG * 128, 128), FG * 128)
        for n in range(D // 128):
            dst = ffn_v.at[g, pl.ds(2 * FG * D + n * FG * 128, FG * 128)]
            pltpu.make_async_copy(wd_hbm.at[rows, pl.ds(n * 128, 128)], dst, sem_f.at[g]).start()
            yield

    def wait_all(filled, sem):
        pltpu.make_async_copy(filled, filled, sem).wait()

    def start_out(rows, cols):
        pltpu.make_async_copy(out_v.at[rows, cols], out_hbm.at[rows, cols], sem_o.at[0]).start()

    small = [pltpu.make_async_copy(wr_hbm, wr8_v, sem_s.at[0]), pltpu.make_async_copy(wphi_hbm, wphi_v, sem_s.at[0])]
    for cp in small + [cp_x0(0)]:
        cp.start()
    for cp in small:
        cp.wait()
    for piece in range(1, 4):
        cp_x0(piece).start()
    for c in range(4):
        cp_k(c).start()
        cp_v(c).start()
    for t in range(NTILE):
        cp_xt(t + 1).start()
        start_q(t)
        if t in (1, 2):
            cp_wo(t - 1).start()

    clock, product = [0.0], []

    def schedule(*streams):
        events = [(a + (b - a) * k / n, i, k, gen) for i, (gen, n, a, b) in enumerate(streams) for k in range(n)]
        for when, _, _, gen in sorted(events, key=lambda e: e[:3]):
            clock[:] = [when]
            next(gen)

    def matmul(a, b, per_slot):
        m = _dot_nt(_bf16(a), _bf16(b))
        product[:] = [m, per_slot]
        return m

    def pin(n=8):
        if not product:
            return jnp.zeros((n, 128), f32)
        m, per_slot = product
        rows, cols = m.shape[0] // 8, m.shape[1] // 128
        q = min(int((clock[0] * per_slot) % 1.0 * rows * cols + 1e-6), rows * cols - 1)
        m = m[(q % rows) * 8:(q % rows) * 8 + 8, (q // rows) * 128:(q // rows) * 128 + 128]
        z = pltpu.bitcast(pltpu.bitcast(m, u32) & zero_s[0].astype(u32), f32)
        return z if n == 8 else jnp.concatenate([z] * (n // 8), axis=0)

    def feature_maps():
        r = lax.broadcasted_iota(i32, (128, DH), 0)
        select = (((r % 64) // 8) * 4 + (r % 8) // 2 == lax.broadcasted_iota(i32, (128, DH), 1)).astype(bf16)
        r = lax.broadcasted_iota(i32, (128, 128), 0)
        same_head = (r // 64) * 2 + r % 2 == lax.broadcasted_iota(i32, (128, 128), 1) // DH
        for g in range(8):
            full = _dot_nt(select, wphi_v[pl.ds(g * 128, 128), :])
            map_v.at[g][...] = jnp.where(same_head, full, 0.0).astype(bf16)

    def put_lhs(dst, row, col, quadrants):
        for i, v in enumerate(_lhs_operands(*quadrants)):
            dst.at[i][pl.ds(_aligned(row, 8), 8), pl.ds(_aligned(col, 128), 128)] = _narrow(v)

    def w_blocks(base, top, bottom, k):
        return [in_v[pl.ds(_aligned(base + half * 512 + k * 128, 128), 128), pl.ds(_aligned(g * 128, 128), 128)]
                for g in (top, bottom) for half in range(2)]

    def put_folded(blocks, top, bottom, dst, row_of, k):
        blocks = [_dot_nt(map_v[g], w) for g, w in zip((top, top, bottom, bottom), blocks)]
        for j in range(8):
            put_lhs(dst, row_of(j), k * 128, [p[16 * j:16 * j + 16] * LOG2E for p in blocks])

    def put_transposed(base, top, bottom, dst, row_of):
        for k in range(4):
            zero = pltpu.bitcast(pin(), u32)
            blocks = [pltpu.bitcast(w, u32) for w in w_blocks(base, top, bottom, k)]
            blocks = [_bf16(jnp.concatenate([w[:8] | zero, w[8:]], axis=0)).T for w in blocks]
            for j in range(8):
                put_lhs(dst, row_of(j), k * 128, [w[16 * j:16 * j + 16].astype(f32) for w in blocks])
            yield

    def split_again(once, twice, lhs, r, k):
        for i in range(7):
            zero = pltpu.bitcast(pin(), u32)
            w = [[once[i, pl.ds(a * 64 + r * 8, 8), pl.ds(_aligned(b * 256 + k * 128, 128), 128)]
                  for b in range(2)] for a in range(2)]
            q00, q01, q10, q11 = _wide(w[0][0] | zero), _wide(w[0][1]), _wide(w[1][0]), _wide(w[1][1] | zero)
            sums = _lhs_operands(q00, q01, q10, q11) if lhs else _rhs_operands(q00, q10, q01, q11)
            for n, j in enumerate(LHS_SUMS if lhs else RHS_SUMS):
                twice.at[5 * i + n][pl.ds(r * 8, 8), pl.ds(_aligned(k * 128, 128), 128)] = _narrow(sums[j])
            yield

    def operand(once, twice, lhs, ij):
        i, j = ij // 7, ij % 7
        sums = LHS_SUMS if lhs else RHS_SUMS
        if j in sums:
            return twice[5 * i + sums.index(j)]
        d = int(j == (3 if lhs else 4))
        return once[i, pl.ds(d * 64, 64), pl.ds(d * 256, 256)]

    def prep_kv(c):
        dst = a1_v.at[c] if c < 2 else b1_v.at[c - 2]
        cp_k(c).wait()
        if c:
            cp_v(c).wait()
        for k in range(4):
            put_folded(w_blocks(WK, 2 * c, 2 * c + 1, k), 2 * c, 2 * c + 1, dst,
                       lambda j: (j // 4) * 64 + (j % 4) * 8, k)
            yield
        if not c:
            cp_v(c).wait()
        yield from put_transposed(WV, 2 * c, 2 * c + 1, dst, lambda j: (j // 4) * 64 + 32 + (j % 4) * 8)

    def split_kv(c):
        once, twice = (a1_v.at[1 + zero_s[0]], a2_v.at[0]) if c == 1 else (b1_v.at[c - 2 + zero_s[0]], b2_v.at[c - 2])
        for k in range(2):
            for r in range(8):
                yield from split_again(once, twice, True, r, k)

    def prep_q(u):
        w = q_blocks(u)
        for a in range(2):
            g = 2 * (u // 2) + a
            for c in range(2):
                blocks = [w[pl.ds((2 * half + c) * 128, 128), pl.ds(b * 256 + a * 128, 128)]
                          for b in range(2) for half in range(2)]
                put_folded(blocks, g, g + 4, a1_v.at[2 + u // 2], lambda j: a * 64 + 8 * j, u % 2 + 2 * c)
                yield

    def split_q(u):
        for r in range(8):
            yield from split_again(a1_v.at[2 + u // 2 + zero_s[0]], a2_v.at[1 + u // 2], True, r, u % 2)

    def prep_wo(u, base):
        g = (u // 2) * 4 + u % 2
        return put_transposed(base, g, g + 2, wo_v.at[u // 2], lambda j: (u % 2) * 64 + 8 * j)

    def x_block(r0, n, cols):
        return jnp.concatenate([in_v[pl.ds(pl.multiple_of(r0 + q + (zero_s[1] if q % 16 and n == 16 else 0), 8), 8), cols].astype(f32)
                                for q in range(0, n, 8)], axis=0)

    def ln_stats(t, st, batch):
        lane = lax.broadcasted_iota(i32, (16, 128), 1)
        for start in range(0, 32, batch):
            places = [((step % 2) * 16 + step // 2) * 16 for step in range(start, start + batch)]
            means = variances = jnp.ones((16, 128), f32)
            for n, pos in enumerate(places):
                r0 = pl.multiple_of(t * T + pos, 16)
                x0 = x_block(r0, 16, pl.ds(0, 128)) + pin(16)
                s1 = s2 = None
                for j in range(1, 8):
                    d = x_block(r0, 16, pl.ds(j * 128, 128)) - x0
                    s1 = d if j == 1 else s1 + d
                    s2 = d * d if j == 1 else s2 + d * d
                lane_mean = x0 + s1 * 0.125
                mean = jnp.sum(lane_mean, axis=-1, keepdims=True) * (1.0 / 128)
                d = lane_mean - mean
                var = jnp.sum((s2 - s1 * s1 * 0.125) * 0.125 + d * d, axis=-1, keepdims=True)
                variances = jnp.where(lane == n, jnp.broadcast_to(var, (16, 128)), variances)
                means = jnp.where(lane == n, jnp.broadcast_to(mean, (16, 128)), means)
                yield
            means = means.astype(bf16).astype(f32)
            var = ((variances * (1.0 / 128)).astype(bf16).astype(f32) + EPS_BF16).astype(bf16).astype(f32)
            scale = 1.0 / jnp.sqrt(var).astype(bf16).astype(f32)
            for n, pos in enumerate(places):
                for kind, v in enumerate((means, scale)):
                    st[kind, pl.ds(pos, 16), :] = jnp.broadcast_to(v[:, n:n + 1], (16, 128))
                if (n + 1) % (batch // 4) == 0:
                    yield

    def ln_apply(t, st, dst, score_too):
        for step in range(16):
            r0 = [pl.multiple_of(t * T + b * TH + step * 16 + zero_s[0], 16) for b in range(2)]
            mean = [st[0, pl.ds(b * TH + step * 16, 16), :] for b in range(2)]
            scale = [st[1, pl.ds(b * TH + step * 16, 16), :] for b in range(2)]
            score = [None, None]
            for k in range(4):
                zero = pin(16)
                xn = [[(x_block(r0[b], 16, pl.ds(half * 512 + k * 128, 128)) - (mean[b] + zero)) * scale[b]
                       for half in range(2)] for b in range(2)]
                for i, v in enumerate(_rhs_operands(xn[0][0], xn[1][0], xn[0][1], xn[1][1])):
                    dst.at[i][pl.ds(step * 8, 8), pl.ds(k * 128, 128)] = _narrow(v)
                for b in range(2 if score_too else 0):
                    part = xn[b][0] * wr_v[:, pl.ds(k * 128, 128)] + xn[b][1] * wr_v[:, pl.ds(512 + k * 128, 128)]
                    score[b] = part if k == 0 else score[b] + part
                    if k == 3:
                        r = jnp.sum(score[b], axis=-1, keepdims=True).astype(bf16).astype(f32)
                        r = jnp.broadcast_to(r, (16, 128))
                        token = lax.broadcasted_iota(i32, (16, 128), 0) + r0[b] % S
                        slot = 2 * (t // NTILE) + b
                        better = r > best_v[slot]
                        best_v[slot] = jnp.where(better, r, best_v[slot])
                        best_i[slot] = jnp.where(better, token, best_i[slot])
                yield

    def ln_split(once, twice):
        for r in range(8):
            for k in range(2):
                yield from split_again(once, twice, False, r, k)

    def route():
        score, token = best_v[...].reshape(64, 128), best_i[...].reshape(64, 128)
        top = jnp.max(score, axis=0, keepdims=True)
        idx = jnp.min(jnp.where(score == top, token, S).astype(f32)).astype(i32)
        return jnp.clip(idx, 0, S - 1), top

    def routed_token():
        idx = route()[0]
        base = pl.multiple_of((idx // 16) * 16, 16)
        rows = pl.ds(pl.multiple_of(base % T, 16), 16)
        xn = (in_v[pl.ds(base, 16), :].astype(f32) - st_v[idx // T, 0, rows, 0:1]) * st_v[idx // T, 1, rows, 0:1]
        xn = jnp.where(lax.broadcasted_iota(i32, (16, D), 0) == idx - base, xn, 0.0)
        xn = jnp.sum(xn, axis=0, keepdims=True).astype(bf16).astype(f32)
        for j in range(8):
            row = xn[:, j * 128:(j + 1) * 128] + pin()
            xcol_v[pl.ds(j * 128, 128), :] = jnp.concatenate([row] * 16, axis=0).T
            yield

    def ffn(f0, n):
        for j in range(n):
            group, f = ffn_v.at[(f0 + j) // FG], (f0 + j) % FG
            accs = [jnp.zeros((8, 128), f32)] * 2
            for r in range(8):
                x, zero = xcol_v[pl.ds(r * 128, 128), :], pin()
                for a in range(2):
                    prod = group[pl.ds(_aligned((a * FG + f) * D + r * 128, 128), 128), :].astype(f32) * x
                    acc = accs[a] + zero
                    for q in range(16):
                        acc = acc + prod[8 * q:8 * q + 8]
                    accs[a] = acc
                yield
            gate, up = [jnp.sum(acc, axis=0, keepdims=True) for acc in accs]
            hidden = jnp.broadcast_to(gate * jax.nn.sigmoid(gate) * up, (128, 128)).T
            for c in range(8):
                prod = group[pl.ds(_aligned(2 * FG * D + (c * FG + f) * 128, 128), 128), :].astype(f32) * hidden
                acc = y_acc[:, pl.ds(c * 128, 128)] + pin()
                for q in range(16):
                    acc = acc + prod[8 * q:8 * q + 8]
                y_acc[:, pl.ds(c * 128, 128)] = acc
                if c % 2:
                    yield

    def project(w, x, res, keep=None):
        def emit(r, b, val):
            if isinstance(res, list):
                res[r][b] = val
            else:
                res[r, b] = val
            if keep is not None:
                keep[r, b] = val[64:]

        def once():
            for c in range(2):
                def put(a, b, val):
                    emit(2 * a, 2 * b + c, val[:128])
                    emit(2 * a + 1, 2 * b + c, val[128:])

                yield from _strassen(lambda i: matmul(w[i], x[i, pl.ds(c * 64, 64), :], 14), put)

        if isinstance(w, tuple):
            return _strassen_twice(lambda i: matmul(operand(*w, True, i), operand(*x, False, i), 49), emit), 49, 0.0, 1.0
        return once(), 14, 0.0, 1.0

    def project_part(w, x, res, part):
        def prod(i):
            rows = [w[i, pl.ds(a * 64 + part * 32, 32), :] for a in range(2)]
            return matmul(jnp.concatenate(rows, axis=0), x[i], 14)

        def put(a, b, val):
            for r in range(2):
                for c in range(2):
                    res[2 * a + r, 2 * b + c, pl.ds(part * 64, 64), :] = val[r * 64:(r + 1) * 64, c * 128:(c + 1) * 128]

        return _strassen(prod, put)

    def rows_of(res, r, r0, b):
        return res[r][b][r0:r0 + 64] if isinstance(res, list) else res[r, b, pl.ds(r0, 64), :]

    def kv_post(c, res, keep=None, values_late=False):
        same_head = lax.broadcasted_iota(i32, (64, 128), 0) // DH == lax.broadcasted_iota(i32, (64, 128), 1) % 2

        def accumulate(r, phi):
            v = jnp.concatenate([rows_of(res, r, 64, b) for b in range(4)], axis=1).astype(bf16)
            kv = kv_acc[4 * c + r] + _dot_nt(v, phi)
            kv_acc[4 * c + r] = kv
            kv_v.at[4 * c + r][...] = jnp.where(same_head, kv, 0.0).astype(bf16)

        pending = []
        for r in range(4):
            phis, z = [], z_acc[4 * c + r]
            for b in range(4):
                phi = _dual_softmax(rows_of(res, r, 0, b), pin())
                z = z + phi
                phis.append(phi)
                if keep is not None:
                    keep.at[r][:, pl.ds(b * 128, 128)] = _narrow(phi)
                if b == 1 and pending and not values_late:
                    accumulate(*pending.pop(0))
                if b == 3:
                    z_acc[4 * c + r] = z
                    z_v[4 * c + r] = jnp.broadcast_to(jnp.sum(z, axis=-1, keepdims=True), (128, 128))
                    pending.append((r, jnp.concatenate(phis, axis=1).astype(bf16)))
                yield
        yield
        for rest in pending:
            accumulate(*rest)
        yield

    def q_post(c, res, dst, ready=None):
        even = lax.broadcasted_iota(i32, (8, 128), 0) % 2 == 0
        phis, scales, nums, outs = {}, {}, {}, {}

        def pair(step):
            return 2 * (2 * c + step // 4 + 4 * ((step // 2) % 2)) + step % 2

        for tick in range(40):
            step, b = tick // 4, tick % 4
            if step < 8:
                r = 2 * ((step // 2) % 2) + step // 4
                if ready is None:
                    phi = _dual_softmax(rows_of(res, r, (step % 2) * 64, b), pin())
                elif step % 2:
                    phi = _dual_softmax(rows_of(res, r, 0, b), pin())
                else:
                    phi = _wide(ready[r, :, pl.ds(b * 128, 128)])
                den = phi * z_v[pair(step)]
                inv = _recip(_head_reduce([den[8 * j:8 * j + 8] for j in range(16)], jnp.add) + 1e-6)
                other = pltpu.roll(inv, 1, 0)
                phis.setdefault(step, []).append(phi)
                scales.setdefault(step, []).append((jnp.where(even, inv, other), jnp.where(even, other, inv)))
            if 1 <= step < 9 and b == 1:
                phi = jnp.concatenate(phis.pop(step - 1), axis=1).astype(bf16)
                nums[step - 1] = _dot(kv_v[pair(step - 1)], phi)
            if step >= 2 and b == 0:
                scale = scales.pop(step - 2)
                scale = [jnp.concatenate([v[head] for v in scale], axis=1) for head in range(2)]
                outs[step - 2] = nums.pop(step - 2) * jnp.concatenate([scale[0]] * 4 + [scale[1]] * 4, axis=0)
                if (step - 2) % 4 == 3:
                    u = (step - 2) // 4
                    o1 = jnp.concatenate([outs.pop(4 * u), outs.pop(4 * u + 1)], axis=0)
                    o2 = jnp.concatenate([outs.pop(4 * u + 2), outs.pop(4 * u + 3)], axis=0)
                    for i, v in enumerate(_rhs_operands(o1[:, :TH], o1[:, TH:], o2[:, :TH], o2[:, TH:])):
                        dst.at[i][:, pl.ds(u * 128, 128)] = pltpu.bitcast(v.astype(bf16).T, u32)
            yield

    def out_project(h, o, res, ks, per_slot):
        def prod(i):
            lhs = jnp.concatenate([o[k][i] for k in ks], axis=1)
            return matmul(lhs, wo_v[h, i, :, pl.ds(ks[0] * 256, len(ks) * 256)], per_slot)

        def emit(a, b, val):
            if isinstance(res, list):
                res[a][b] = val
            else:
                res[a, b] = val

        return _strassen(prod, emit)

    zero_s[0] = 0
    zero_s[1] = 0
    kv_acc[...] = jnp.zeros(kv_acc.shape, f32)
    z_acc[...] = jnp.zeros(z_acc.shape, f32)
    y_acc[...] = jnp.zeros(y_acc.shape, f32)
    best_v[...] = jnp.full(best_v.shape, -jnp.inf, f32)
    best_i[...] = jnp.zeros(best_i.shape, i32)
    w8 = wr8_v[...].astype(f32)
    wr_v[...] = jnp.broadcast_to(jnp.concatenate([w8[j:j + 1, :] for j in range(8)], axis=1), (16, D))
    feature_maps()
    stats, apply = ln_stats(0, st_v.at[0], 16), ln_apply(0, st_v.at[0], x1_v.at[0], False)
    for half in range(2):
        cp_x0(2 * half).wait()
        cp_x0(2 * half + 1).wait()
        schedule((stats, 20, 0.0, 1.0))
        schedule((apply, 32, 0.0, 1.0))
    chunk0 = prep_kv(0)
    schedule((chunk0, 4, 0.0, 1.0))
    schedule((project_part(a1_v.at[0], x1_v.at[0], raw_v.at[0], 0), 7, 0.0, 0.5),
             (project_part(a1_v.at[0], x1_v.at[0], raw_v.at[0], 1), 7, 0.5, 1.0),
             (project(a1_v.at[1], x1_v.at[0], raw_v.at[1])[0], 14, 1.0, 2.0),
             (chunk0, 4, 0.15, 0.45), (ln_split(x1_v.at[zero_s[0]], x2_v.at[0]), 112, 0.03, 0.6),
             (kv_post(0, raw_v.at[zero_s[0]], values_late=True), 18, 0.52, 1.3),
             (prep_kv(1), 8, 0.74, 0.96), (split_kv(1), 112, 1.02, 1.31),
             (prep_kv(2), 8, 1.05, 1.3), (split_kv(2), 112, 1.31, 1.62),
             (prep_kv(3), 8, 1.49, 1.7), (split_kv(3), 112, 1.73, 2.0))

    def kv_tile(t, _):
        last = t == NTILE - 1
        wait_all(q_blocks(t), sem_q.at[t])
        cp_xt(t + 1).wait()

        @pl.when(jnp.logical_and(t > 0, t < 3))
        def _():
            cp_wo(t - 1).wait()

        product[:] = []
        first = (route()[0] // T) % (NTILE - 1) + 1
        x1, x2, st = x1_v.at[pl.ds(t, 2)], x2_v.at[pl.ds(t, 2)], st_v.at[t + 1]
        split = ln_split(x1_v.at[t + 1 + zero_s[0]], x2.at[1])
        wo = [prep_wo(2 * ((t + 1) % 2) + u, jnp.where(t == 0, WV, WO)) for u in range(2)]
        c2, c3, c0 = ([[None] * 4 for _ in range(4)] for _ in range(3))
        schedule(project((b1_v.at[0], b2_v.at[0]), (x1.at[0], x2.at[0]), c2),
                 (kv_post(1, raw_v.at[1]), 18, 0.068, 0.965), (ln_stats(t + 1, st, 32), 36, 0.0, 0.99),
                 (start_ffn(t), 2 * FG + 8, 0.05, 0.95))
        schedule(project((b1_v.at[1], b2_v.at[1]), (x1.at[0], x2.at[0]), c3),
                 (kv_post(2, c2), 18, 0.08, 0.965), (ln_apply(t + 1, st, x1.at[1], True), 64, 0.015, 0.935),
                 (prep_q(t), 4, 0.0, 0.656))
        nxt, chunk = jnp.where(last, first, t + 1), jnp.where(last, 2, 0)
        schedule(project(a1_v.at[chunk], x1_v.at[nxt], c0, keep=half_v),
                 (kv_post(3, c3), 18, 0.0, 0.917), (split, 112, 0.0, 0.873), (split_q(t), 56, 0.1, 0.942))
        schedule(project((a1_v.at[chunk + 1], a2_v.at[chunk]), (x1_v.at[nxt], x2_v.at[nxt]), raw_v.at[1]),
                 (kv_post(jnp.where(last, 4, 0), c0, keep=phi_v), 18, 0.08, 0.905),
                 (wo[0], 4, 0.05, 0.69), (wo[1], 4, 0.435, 0.985), (routed_token(), 8, 0.025, 0.878))
        return first

    first = lax.fori_loop(0, NTILE, kv_tile, jnp.int32(0))

    wait_all(ffn_v.at[0], sem_f.at[0])
    product[:] = []
    idx, top_score = route()
    final = idx // T
    lo, hi = jnp.minimum(first, final), jnp.maximum(first, final)
    second = jnp.where(lo > 0, 0, jnp.where(hi > 1, 1, 2))
    third = 6 - first - final - second

    def tile(j):
        return jnp.where(j == 0, first, jnp.where(j == 1, second, jnp.where(j == 2, third, final)))

    def gate(t, h, a, b, q, update):
        r0, rows = pl.multiple_of(t * T + b * TH + q * EROWS, EROWS), pl.ds(b * TH + q * EROWS, EROWS)
        c0 = h * 512 + a * 256
        mean, scale = st_v[t, 0, rows, :], st_v[t, 1, rows, :] * 0.5
        if update is None:
            mean = mean + pin(EROWS)
        x = x_block(r0, EROWS, pl.ds(c0, 256))
        v = (x - jnp.concatenate([mean, mean], axis=1)) * jnp.concatenate([scale, scale], axis=1)
        if update is not None:
            hit = lax.broadcasted_iota(i32, (EROWS, 256), 0) == idx - r0
            v = v + jnp.where(hit, update[:, c0:c0 + 256], 0.0)
        return x, v + v * jnp.tanh(v)

    def epilogue(t, h, res, part=None, update=None, early=None):
        for a, b in ((0, 1), (0, 0), (1, 0), (1, 1)) if part is not None else ((0, 0), (0, 1), (1, 0), (1, 1)):
            for q in range(TH // EROWS):
                r0, cols = pl.multiple_of(t * T + b * TH + q * EROWS, EROWS), pl.ds(h * 512 + a * 256, 256)
                if early is not None and (a, b) == (1, 1):
                    x, g = x_block(r0, EROWS, cols), early[pl.ds(q * EROWS, EROWS), :]
                else:
                    x, g = gate(t, h, a, b, q, update)
                s = res[a][b][q * EROWS:(q + 1) * EROWS]
                if part is not None:
                    s = s + part[a, b, pl.ds(q * EROWS, EROWS), :]
                out_v[pl.ds(r0, EROWS), cols] = (x + s * g).astype(bf16)
                if part is not None and (q + 1) * EROWS % 128 == 0:
                    start_out(pl.ds(pl.multiple_of(t * T + b * TH + (q + 1) * EROWS - 128, 128), 128), cols)
                yield

    steps = 4 * TH // EROWS
    schedule((q_post(0, half_v, oa_v.at[0], ready=phi_v), 40, 0.01, 1.0))

    def q_tile(j, carry):
        product[:] = []
        oa = oa_v.at[pl.ds(j, 2)]
        o = oa.at[0], ob_v.at[zero_s[0]]
        x = x1_v.at[tile(j + 1)], x2_v.at[tile(j + 1)]
        wait_all(ffn_v.at[j + 1], sem_f.at[j + 1])
        hidden = ffn(j * FL, FL)
        q0, s0, s1 = ([[None] * 4 for _ in range(4)] for _ in range(3))
        schedule(project((a1_v.at[2], a2_v.at[1]), x, q0),
                 (q_post(1, raw_v.at[1], ob_v.at[0]), 40, 0.0, 1.0), (hidden, 14, 0.0, 0.89))
        schedule((out_project(0, o, s0, (0, 1), 7), 7, 0.0, 1.0),
                 (q_post(0, q0, oa.at[1]), 40, 0.0, 1.0), (hidden, 18, 0.085, 0.985))
        schedule((out_project(1, o, s1, (0, 1), 7), 7, 0.0, 1.0),
                 (epilogue(tile(j), 0, s0), steps, 0.055, 0.96), (hidden, 38, 0.02, 1.0))
        schedule(project((a1_v.at[3], a2_v.at[2]), x, raw_v.at[1]),
                 (epilogue(tile(j), 1, s1), steps, 0.0, 0.985), (hidden, 12 * FL - 70, 0.0, 0.885))
        start_out(pl.ds(pl.multiple_of(tile(j) * T, T), T), slice(None))
        return carry

    lax.fori_loop(0, NTILE - 1, q_tile, 0)

    product[:] = []
    o = oa_v.at[NTILE - 1], ob_v.at[zero_s[0]]
    rest = NF - (NTILE - 1) * FL
    schedule((out_project(0, o, part_v.at[0], (0,), 14), 7, 0.0, 0.5),
             (out_project(1, o, part_v.at[1], (0,), 14), 7, 0.5, 1.0),
             (q_post(1, raw_v.at[1], ob_v.at[0]), 40, 0.0, 0.9), (ffn(NF - rest, rest), 12 * rest, 0.1, 0.8))
    update = jnp.sum(y_acc[...], axis=0, keepdims=True) * (0.5 * jax.nn.sigmoid(top_score[:, 0:1]))
    s0, s1 = ([[None, None], [None, None]] for _ in range(2))

    def last_gate():
        for q in range(TH // EROWS):
            gate_v[0, pl.ds(q * EROWS, EROWS), :] = gate(final, 1, 1, 1, q, update)[1]
            yield

    schedule((out_project(0, o, s0, (1,), 14), 7, 0.0, 0.5), (out_project(1, o, s1, (1,), 14), 7, 0.5, 1.0),
             (epilogue(final, 0, s0, part_v.at[0], update), steps, 0.2, 0.66),
             (epilogue(final, 1, s1, part_v.at[1], update, gate_v.at[zero_s[0]]), steps, 0.69, 1.21),
             (last_gate(), TH // EROWS, 0.0, 0.2))
    pltpu.make_async_copy(out_v, out_hbm, sem_o.at[0]).wait()


def _call(x, wqkv, wphi, wo, wr, wg, wu, wd, interpret=False):
    scratch = [
        pltpu.VMEM((S + T + 4 * D, D), bf16),
        pltpu.VMEM((NTILE + 1, 2, T, 128), f32),
        pltpu.VMEM((NTILE + 1, 7, 128, 512), u32),
        pltpu.VMEM((NTILE + 1, 35, 64, 256), u32),
        pltpu.VMEM((D, DH), bf16),
        pltpu.VMEM((8, 128), bf16),
        pltpu.VMEM((16, D), f32),
        pltpu.VMEM((8, 128, 128), bf16),
        pltpu.VMEM((4, 7, 128, 512), u32),
        pltpu.VMEM((3, 35, 64, 256), u32),
        pltpu.VMEM((2, 7, 128, 512), u32),
        pltpu.VMEM((2, 35, 64, 256), u32),
        pltpu.VMEM((2, 7, 128, 512), u32),
        pltpu.VMEM((NTILE, 3 * FG * D, 128), bf16),
        pltpu.VMEM((H // 2 + 4, 64, 128), f32),
        pltpu.VMEM((H // 2 + 4, 128, 128), f32),
        pltpu.VMEM((H // 2 + 4, 64, 128), bf16),
        pltpu.VMEM((H // 2 + 4, 128, 128), f32),
        pltpu.VMEM((4, 16, 128), f32),
        pltpu.VMEM((4, 16, 128), i32),
        pltpu.VMEM((2, 4, 4, 128, 128), f32),
        pltpu.VMEM((4, 4, 64, 128), f32),
        pltpu.VMEM((4, 64, T), u32),
        pltpu.VMEM((NTILE, 7, 128, 256), u32),
        pltpu.VMEM((2, 7, 128, 256), u32),
        pltpu.VMEM((2, 2, 2, 256, 256), f32),
        pltpu.VMEM((2, 256, 256), f32),
        pltpu.VMEM((D, 128), f32),
        pltpu.VMEM((8, D), f32),
        pltpu.VMEM((S, D), bf16),
        pltpu.SMEM((2,), i32),
        pltpu.SemaphoreType.DMA((NTILE + 2,)),
        pltpu.SemaphoreType.DMA((5,)),
        pltpu.SemaphoreType.DMA((NTILE + 2,)),
        pltpu.SemaphoreType.DMA((1,)),
        pltpu.SemaphoreType.DMA((NTILE,)),
        pltpu.SemaphoreType.DMA((1,)),
    ]
    hbm = pl.BlockSpec(memory_space=pltpu.HBM)
    return pl.pallas_call(
        _kernel,
        out_shape=jax.ShapeDtypeStruct((S, D), bf16),
        in_specs=[hbm] * 8,
        out_specs=hbm,
        scratch_shapes=scratch,
        compiler_params=pltpu.CompilerParams(
            vmem_limit_bytes=120 * 2**20, disable_bounds_checks=True, disable_semaphore_checks=True),
        name="hedgehog",
        interpret=interpret,
    )(x, wqkv, wphi, wo, wr, wg, wu, wd)


@jax.jit
def pallas_recurrent_scan__linear_kernel_hedgehog__moe_arch_mod__prompt_kernel(
    A_x: jax.Array,
    A_wqkv: jax.Array,
    A_w_phi: jax.Array,
    A_wo: jax.Array,
    B_x: jax.Array,
    B_w_r: jax.Array,
    B_w_gate: jax.Array,
    B_w_up: jax.Array,
    B_w_down: jax.Array,
):
    del B_x
    out = _call(A_x.reshape(S, D), A_wqkv, A_w_phi.reshape(D, DH), A_wo,
                B_w_r.reshape(8, 128), B_w_gate, B_w_up, B_w_down)
    return out.reshape(1, S, D)
```

```python
import math

import numpy as np

import jax
import jax.numpy as jnp
from jax import lax
import jax.experimental.pallas as pl
import jax.experimental.pallas.tpu as pltpu

S, D, H, DH, F = 2048, 1024, 32, 32, 3584
T = 512
TH = T // 2
NTILE = S // T
NF = F // 128
FG = NF // NTILE
FL = 9
EROWS = 32
WQ, WK, WV, WO = (S + T + j * D for j in range(4))
LHS_SUMS, RHS_SUMS = (0, 1, 4, 5, 6), (0, 2, 3, 5, 6)
LOG2E = math.log2(math.e)
EPS_BF16 = float(np.float32(1e-5).astype(jnp.bfloat16))
f32, bf16, i32, u32 = jnp.float32, jnp.bfloat16, jnp.int32, jnp.uint32


def _dot_nt(a, b):
    return lax.dot_general(a, b, (((1,), (1,)), ((), ())), preferred_element_type=f32)


def _dot(a, b):
    return jnp.dot(a, b, preferred_element_type=f32)


def _aligned(i, n):
    return i if isinstance(i, int) else pl.multiple_of(i, n)


def _recip(v):
    r = pl.reciprocal(v, approx=True)
    return r * (2.0 - v * r)


def _bf16(words):
    return pltpu.bitcast(words, bf16)


def _wide(words):
    return _bf16(words).astype(f32)


def _narrow(v):
    return pltpu.bitcast(v.astype(bf16), u32)


def _lhs_operands(a11, a12, a21, a22):
    return [a11 + a22, a21 + a22, a11, a22, a11 + a12, a21 - a11, a12 - a22]


def _rhs_operands(b11, b12, b21, b22):
    return [b11 + b22, b11, b12 - b22, b21 - b11, b22, b11 + b12, b21 + b22]


def _strassen(prod, emit):
    m3 = prod(2)
    yield
    m5 = prod(4)
    emit(0, 1, m3 + m5)
    yield
    m1 = prod(0)
    c11, c22 = m1 - m5, m1 + m3
    yield
    c11 = c11 + prod(6)
    yield
    m4 = prod(3)
    emit(0, 0, c11 + m4)
    yield
    m2 = prod(1)
    emit(1, 0, m2 + m4)
    c22 = c22 - m2
    yield
    emit(1, 1, c22 + prod(5))
    yield


class _Quad:
    def __init__(self, blocks):
        self.blocks = blocks

    def __add__(self, other):
        return _Quad([p + q for p, q in zip(self.blocks, other.blocks)])

    def __sub__(self, other):
        return _Quad([p - q for p, q in zip(self.blocks, other.blocks)])


def _strassen_twice(prod, emit):
    done = {}

    def inner(i):
        out = [None] * 4

        def put(a, b, val):
            out[2 * a + b] = val

        yield from _strassen(lambda j: prod(7 * i + j), put)
        done[i] = _Quad(out)

    def put(a, b, quad):
        for k, val in enumerate(quad.blocks):
            emit(2 * a + k // 2, 2 * b + k % 2, val)

    outer = _strassen(lambda i: done[i], put)
    for i in (2, 4, 0, 6, 3, 1, 5):
        steps = inner(i)
        for _ in range(6):
            next(steps)
            yield
        for _ in steps:
            pass
        next(outer)
        yield


def _head_reduce(vs, op):
    while len(vs) > 1:
        vs = [op(vs[i], vs[i + 1]) for i in range(0, len(vs), 2)]
    v = op(vs[0], pltpu.roll(vs[0], 4, 0))
    return op(v, pltpu.roll(v, 2, 0))


def _dual_softmax(p, zero):
    rows = [p[8 * j:8 * j + 8] for j in range(8)]
    rows[0] = rows[0] + zero
    mx, mn = _head_reduce(rows, jnp.maximum), _head_reduce(rows, jnp.minimum)
    ep = [jnp.exp2(v - mx) for v in rows]
    en = [jnp.exp2(mn - v) for v in rows]
    rp, rn = _recip(_head_reduce(ep, jnp.add)), _recip(_head_reduce(en, jnp.add))
    return jnp.concatenate([v * rp for v in ep] + [v * rn for v in en], axis=0)


def _kernel(x_hbm, wqkv_hbm, wphi_hbm, wo_hbm, wr_hbm, wg_hbm, wu_hbm, wd_hbm, out_hbm,
            in_v, st_v, x1_v, x2_v, wphi_v, wr8_v, wr_v, map_v, a1_v, a2_v, b1_v, b2_v, wo_v, ffn_v,
            kv_acc, z_acc, kv_v, z_v, best_v, best_i, raw_v, half_v, phi_v, oa_v, ob_v, part_v,
            gate_v, xcol_v, y_acc, out_v, zero_s, sem_x, sem_w, sem_q, sem_s, sem_f, sem_o):
    def cp_x(r0, n, sem, src0):
        return pltpu.make_async_copy(x_hbm.at[pl.ds(src0, n)], in_v.at[pl.ds(r0, n)], sem_x.at[sem])

    def cp_x0(piece):
        r0 = (piece % 2) * TH + (piece // 2) * (TH // 2)
        return cp_x(r0, TH // 2, 0 if piece < 2 else NTILE + 1, r0)

    def cp_xt(t):
        return cp_x(_aligned(t * T, T), T, t, _aligned((t % NTILE) * T, T))

    def cp_w(j, c, sem):
        return pltpu.make_async_copy(wqkv_hbm.at[:, pl.ds(j * D + c * 256, 256)],
                                     in_v.at[pl.ds(WQ + j * D, D), pl.ds(c * 256, 256)], sem_w.at[sem])

    def cp_k(c):
        return cp_w(1, c, c)

    def cp_v(c):
        return cp_w(2, c, c if c else 4)

    def start_q(u):
        for n in range(8):
            src = wqkv_hbm.at[pl.ds((n // 2) * 256 + (u % 2) * 128, 128), pl.ds((u // 2) * 256 + (n % 2) * 512, 256)]
            dst = in_v.at[pl.ds(WQ + (u // 2) * 512 + (n // 2) * 128, 128), pl.ds((u % 2) * 512 + (n % 2) * 256, 256)]
            pltpu.make_async_copy(src, dst, sem_q.at[u]).start()

    def q_blocks(u):
        return in_v.at[pl.ds(_aligned(WQ + (u // 2) * 512, 512), 512), pl.ds(_aligned((u % 2) * 512, 512), 512)]

    def cp_wo(h):
        cols = pl.ds(_aligned(h * 512, 512), 512)
        return pltpu.make_async_copy(wo_hbm.at[:, cols], in_v.at[pl.ds(WO, D), cols], sem_q.at[NTILE + h])

    def start_ffn(g):
        for j in range(FG):
            cols = pl.ds(_aligned((g * FG + j) * 128, 128), 128)
            for n, src in enumerate((wg_hbm, wu_hbm)):
                dst = ffn_v.at[g, pl.ds((n * FG + j) * D, D)]
                pltpu.make_async_copy(src.at[:, cols], dst, sem_f.at[g]).start()
                yield
        rows = pl.ds(_aligned(g * FG * 128, 128), FG * 128)
        for n in range(D // 128):
            dst = ffn_v.at[g, pl.ds(2 * FG * D + n * FG * 128, FG * 128)]
            pltpu.make_async_copy(wd_hbm.at[rows, pl.ds(n * 128, 128)], dst, sem_f.at[g]).start()
            yield

    def wait_all(filled, sem):
        pltpu.make_async_copy(filled, filled, sem).wait()

    def start_out(rows, cols):
        pltpu.make_async_copy(out_v.at[rows, cols], out_hbm.at[rows, cols], sem_o.at[0]).start()

    small = [pltpu.make_async_copy(wr_hbm, wr8_v, sem_s.at[0]), pltpu.make_async_copy(wphi_hbm, wphi_v, sem_s.at[0])]
    for cp in small + [cp_x0(0)]:
        cp.start()
    for cp in small:
        cp.wait()
    for piece in range(1, 4):
        cp_x0(piece).start()
    for c in range(4):
        cp_k(c).start()
        cp_v(c).start()
    for t in range(NTILE):
        cp_xt(t + 1).start()
        start_q(t)
        if t in (1, 2):
            cp_wo(t - 1).start()

    clock, product = [0.0], []

    def schedule(*streams):
        events = [(a + (b - a) * k / n, i, k, gen) for i, (gen, n, a, b) in enumerate(streams) for k in range(n)]
        for when, _, _, gen in sorted(events, key=lambda e: e[:3]):
            clock[:] = [when]
            next(gen)

    def matmul(a, b, per_slot):
        m = _dot_nt(_bf16(a), _bf16(b))
        product[:] = [m, per_slot]
        return m

    def pin(n=8):
        if not product:
            return jnp.zeros((n, 128), f32)
        m, per_slot = product
        rows, cols = m.shape[0] // 8, m.shape[1] // 128
        q = min(int((clock[0] * per_slot) % 1.0 * rows * cols + 1e-6), rows * cols - 1)
        m = m[(q % rows) * 8:(q % rows) * 8 + 8, (q // rows) * 128:(q // rows) * 128 + 128]
        z = pltpu.bitcast(pltpu.bitcast(m, u32) & zero_s[0].astype(u32), f32)
        return z if n == 8 else jnp.concatenate([z] * (n // 8), axis=0)

    def feature_maps():
        r = lax.broadcasted_iota(i32, (128, DH), 0)
        select = (((r % 64) // 8) * 4 + (r % 8) // 2 == lax.broadcasted_iota(i32, (128, DH), 1)).astype(bf16)
        r = lax.broadcasted_iota(i32, (128, 128), 0)
        same_head = (r // 64) * 2 + r % 2 == lax.broadcasted_iota(i32, (128, 128), 1) // DH
        for g in range(8):
            full = _dot_nt(select, wphi_v[pl.ds(g * 128, 128), :])
            map_v.at[g][...] = jnp.where(same_head, full, 0.0).astype(bf16)

    def put_lhs(dst, row, col, quadrants):
        for i, v in enumerate(_lhs_operands(*quadrants)):
            dst.at[i][pl.ds(_aligned(row, 8), 8), pl.ds(_aligned(col, 128), 128)] = _narrow(v)

    def w_blocks(base, top, bottom, k):
        return [in_v[pl.ds(_aligned(base + half * 512 + k * 128, 128), 128), pl.ds(_aligned(g * 128, 128), 128)]
                for g in (top, bottom) for half in range(2)]

    def put_folded(blocks, top, bottom, dst, row_of, k):
        blocks = [_dot_nt(map_v[g], w) for g, w in zip((top, top, bottom, bottom), blocks)]
        for j in range(8):
            put_lhs(dst, row_of(j), k * 128, [p[16 * j:16 * j + 16] * LOG2E for p in blocks])

    def put_transposed(base, top, bottom, dst, row_of):
        for k in range(4):
            zero = pltpu.bitcast(pin(), u32)
            blocks = [pltpu.bitcast(w, u32) for w in w_blocks(base, top, bottom, k)]
            blocks = [_bf16(jnp.concatenate([w[:8] | zero, w[8:]], axis=0)).T for w in blocks]
            for j in range(8):
                put_lhs(dst, row_of(j), k * 128, [w[16 * j:16 * j + 16].astype(f32) for w in blocks])
            yield

    def split_again(once, twice, lhs, r, k):
        for i in range(7):
            zero = pltpu.bitcast(pin(), u32)
            w = [[once[i, pl.ds(a * 64 + r * 8, 8), pl.ds(_aligned(b * 256 + k * 128, 128), 128)]
                  for b in range(2)] for a in range(2)]
            q00, q01, q10, q11 = _wide(w[0][0] | zero), _wide(w[0][1]), _wide(w[1][0]), _wide(w[1][1] | zero)
            sums = _lhs_operands(q00, q01, q10, q11) if lhs else _rhs_operands(q00, q10, q01, q11)
            for n, j in enumerate(LHS_SUMS if lhs else RHS_SUMS):
                twice.at[5 * i + n][pl.ds(r * 8, 8), pl.ds(_aligned(k * 128, 128), 128)] = _narrow(sums[j])
            yield

    def operand(once, twice, lhs, ij):
        i, j = ij // 7, ij % 7
        sums = LHS_SUMS if lhs else RHS_SUMS
        if j in sums:
            return twice[5 * i + sums.index(j)]
        d = int(j == (3 if lhs else 4))
        return once[i, pl.ds(d * 64, 64), pl.ds(d * 256, 256)]

    def prep_kv(c):
        dst = a1_v.at[c] if c < 2 else b1_v.at[c - 2]
        cp_k(c).wait()
        if c:
            cp_v(c).wait()
        for k in range(4):
            put_folded(w_blocks(WK, 2 * c, 2 * c + 1, k), 2 * c, 2 * c + 1, dst,
                       lambda j: (j // 4) * 64 + (j % 4) * 8, k)
            yield
        if not c:
            cp_v(c).wait()
        yield from put_transposed(WV, 2 * c, 2 * c + 1, dst, lambda j: (j // 4) * 64 + 32 + (j % 4) * 8)

    def split_kv(c):
        once, twice = (a1_v.at[1 + zero_s[0]], a2_v.at[0]) if c == 1 else (b1_v.at[c - 2 + zero_s[0]], b2_v.at[c - 2])
        for k in range(2):
            for r in range(8):
                yield from split_again(once, twice, True, r, k)

    def prep_q(u):
        w = q_blocks(u)
        for a in range(2):
            g = 2 * (u // 2) + a
            for c in range(2):
                blocks = [w[pl.ds((2 * half + c) * 128, 128), pl.ds(b * 256 + a * 128, 128)]
                          for b in range(2) for half in range(2)]
                put_folded(blocks, g, g + 4, a1_v.at[2 + u // 2], lambda j: a * 64 + 8 * j, u % 2 + 2 * c)
                yield

    def split_q(u):
        for r in range(8):
            yield from split_again(a1_v.at[2 + u // 2 + zero_s[0]], a2_v.at[1 + u // 2], True, r, u % 2)

    def prep_wo(u, base):
        g = (u // 2) * 4 + u % 2
        return put_transposed(base, g, g + 2, wo_v.at[u // 2], lambda j: (u % 2) * 64 + 8 * j)

    def x_block(r0, n, cols):
        return jnp.concatenate([in_v[pl.ds(pl.multiple_of(r0 + q + (zero_s[1] if q % 16 and n == 16 else 0), 8), 8), cols].astype(f32)
                                for q in range(0, n, 8)], axis=0)

    def ln_stats(t, st, batch):
        lane = lax.broadcasted_iota(i32, (16, 128), 1)
        for start in range(0, 32, batch):
            places = [((step % 2) * 16 + step // 2) * 16 for step in range(start, start + batch)]
            means = variances = jnp.ones((16, 128), f32)
            for n, pos in enumerate(places):
                r0 = pl.multiple_of(t * T + pos, 16)
                x0 = x_block(r0, 16, pl.ds(0, 128)) + pin(16)
                s1 = s2 = None
                for j in range(1, 8):
                    d = x_block(r0, 16, pl.ds(j * 128, 128)) - x0
                    s1 = d if j == 1 else s1 + d
                    s2 = d * d if j == 1 else s2 + d * d
                lane_mean = x0 + s1 * 0.125
                mean = jnp.sum(lane_mean, axis=-1, keepdims=True) * (1.0 / 128)
                d = lane_mean - mean
                var = jnp.sum((s2 - s1 * s1 * 0.125) * 0.125 + d * d, axis=-1, keepdims=True)
                variances = jnp.where(lane == n, jnp.broadcast_to(var, (16, 128)), variances)
                means = jnp.where(lane == n, jnp.broadcast_to(mean, (16, 128)), means)
                yield
            means = means.astype(bf16).astype(f32)
            var = ((variances * (1.0 / 128)).astype(bf16).astype(f32) + EPS_BF16).astype(bf16).astype(f32)
            scale = 1.0 / jnp.sqrt(var).astype(bf16).astype(f32)
            for n, pos in enumerate(places):
                for kind, v in enumerate((means, scale)):
                    st[kind, pl.ds(pos, 16), :] = jnp.broadcast_to(v[:, n:n + 1], (16, 128))
                if (n + 1) % (batch // 4) == 0:
                    yield

    def ln_apply(t, st, dst, score_too):
        for step in range(16):
            r0 = [pl.multiple_of(t * T + b * TH + step * 16 + zero_s[0], 16) for b in range(2)]
            mean = [st[0, pl.ds(b * TH + step * 16, 16), :] for b in range(2)]
            scale = [st[1, pl.ds(b * TH + step * 16, 16), :] for b in range(2)]
            score = [None, None]
            for k in range(4):
                zero = pin(16)
                xn = [[(x_block(r0[b], 16, pl.ds(half * 512 + k * 128, 128)) - (mean[b] + zero)) * scale[b]
                       for half in range(2)] for b in range(2)]
                for i, v in enumerate(_rhs_operands(xn[0][0], xn[1][0], xn[0][1], xn[1][1])):
                    dst.at[i][pl.ds(step * 8, 8), pl.ds(k * 128, 128)] = _narrow(v)
                for b in range(2 if score_too else 0):
                    part = xn[b][0] * wr_v[:, pl.ds(k * 128, 128)] + xn[b][1] * wr_v[:, pl.ds(512 + k * 128, 128)]
                    score[b] = part if k == 0 else score[b] + part
                    if k == 3:
                        r = jnp.sum(score[b], axis=-1, keepdims=True).astype(bf16).astype(f32)
                        r = jnp.broadcast_to(r, (16, 128))
                        token = lax.broadcasted_iota(i32, (16, 128), 0) + r0[b] % S
                        slot = 2 * (t // NTILE) + b
                        better = r > best_v[slot]
                        best_v[slot] = jnp.where(better, r, best_v[slot])
                        best_i[slot] = jnp.where(better, token, best_i[slot])
                yield

    def ln_split(once, twice):
        for r in range(8):
            for k in range(2):
                yield from split_again(once, twice, False, r, k)

    def route():
        score, token = best_v[...].reshape(64, 128), best_i[...].reshape(64, 128)
        top = jnp.max(score, axis=0, keepdims=True)
        idx = jnp.min(jnp.where(score == top, token, S).astype(f32)).astype(i32)
        return jnp.clip(idx, 0, S - 1), top

    def routed_token():
        idx = route()[0]
        base = pl.multiple_of((idx // 16) * 16, 16)
        rows = pl.ds(pl.multiple_of(base % T, 16), 16)
        xn = (in_v[pl.ds(base, 16), :].astype(f32) - st_v[idx // T, 0, rows, 0:1]) * st_v[idx // T, 1, rows, 0:1]
        xn = jnp.where(lax.broadcasted_iota(i32, (16, D), 0) == idx - base, xn, 0.0)
        xn = jnp.sum(xn, axis=0, keepdims=True).astype(bf16).astype(f32)
        for j in range(8):
            row = xn[:, j * 128:(j + 1) * 128] + pin()
            xcol_v[pl.ds(j * 128, 128), :] = jnp.concatenate([row] * 16, axis=0).T
            yield

    def ffn(f0, n):
        for j in range(n):
            group, f = ffn_v.at[(f0 + j) // FG], (f0 + j) % FG
            accs = [jnp.zeros((8, 128), f32)] * 2
            for r in range(8):
                x, zero = xcol_v[pl.ds(r * 128, 128), :], pin()
                for a in range(2):
                    prod = group[pl.ds(_aligned((a * FG + f) * D + r * 128, 128), 128), :].astype(f32) * x
                    acc = accs[a] + zero
                    for q in range(16):
                        acc = acc + prod[8 * q:8 * q + 8]
                    accs[a] = acc
                yield
            gate, up = [jnp.sum(acc, axis=0, keepdims=True) for acc in accs]
            hidden = jnp.broadcast_to(gate * jax.nn.sigmoid(gate) * up, (128, 128)).T
            for c in range(8):
                prod = group[pl.ds(_aligned(2 * FG * D + (c * FG + f) * 128, 128), 128), :].astype(f32) * hidden
                acc = y_acc[:, pl.ds(c * 128, 128)] + pin()
                for q in range(16):
                    acc = acc + prod[8 * q:8 * q + 8]
                y_acc[:, pl.ds(c * 128, 128)] = acc
                if c % 2:
                    yield

    def project(w, x, res, keep=None):
        def emit(r, b, val):
            if isinstance(res, list):
                res[r][b] = val
            else:
                res[r, b] = val
            if keep is not None:
                keep[r, b] = val[64:]

        def once():
            for c in range(2):
                def put(a, b, val):
                    emit(2 * a, 2 * b + c, val[:128])
                    emit(2 * a + 1, 2 * b + c, val[128:])

                yield from _strassen(lambda i: matmul(w[i], x[i, pl.ds(c * 64, 64), :], 14), put)

        if isinstance(w, tuple):
            return _strassen_twice(lambda i: matmul(operand(*w, True, i), operand(*x, False, i), 49), emit), 49, 0.0, 1.0
        return once(), 14, 0.0, 1.0

    def project_part(w, x, res, part):
        def prod(i):
            rows = [w[i, pl.ds(a * 64 + part * 32, 32), :] for a in range(2)]
            return matmul(jnp.concatenate(rows, axis=0), x[i], 14)

        def put(a, b, val):
            for r in range(2):
                for c in range(2):
                    res[2 * a + r, 2 * b + c, pl.ds(part * 64, 64), :] = val[r * 64:(r + 1) * 64, c * 128:(c + 1) * 128]

        return _strassen(prod, put)

    def rows_of(res, r, r0, b):
        return res[r][b][r0:r0 + 64] if isinstance(res, list) else res[r, b, pl.ds(r0, 64), :]

    def kv_post(c, res, keep=None, values_late=False):
        same_head = lax.broadcasted_iota(i32, (64, 128), 0) // DH == lax.broadcasted_iota(i32, (64, 128), 1) % 2

        sums = {}

        def accumulate(r, b, phi):
            part = _dot_nt(rows_of(res, r, 64, b).astype(bf16), phi.astype(bf16))
            sums[r] = (kv_acc[4 * c + r] if b == 0 else sums[r]) + part
            if b == 3:
                kv_acc[4 * c + r] = sums[r]
                kv_v.at[4 * c + r][...] = jnp.where(same_head, sums.pop(r), 0.0).astype(bf16)

        pending = []
        for r in range(4):
            z = z_acc[4 * c + r]
            for b in range(4):
                phi = _dual_softmax(rows_of(res, r, 0, b), pin())
                z = z + phi
                if keep is not None:
                    keep.at[r][:, pl.ds(b * 128, 128)] = _narrow(phi)
                pending.append((r, b, phi))
                if len(pending) > 3 and not values_late:
                    accumulate(*pending.pop(0))
                if b == 3:
                    z_acc[4 * c + r] = z
                    z_v[4 * c + r] = jnp.broadcast_to(jnp.sum(z, axis=-1, keepdims=True), (128, 128))
                yield
        yield
        for rest in pending:
            accumulate(*rest)
        yield

    def q_post(c, res, dst, ready=None, lag=1):
        even = lax.broadcasted_iota(i32, (8, 128), 0) % 2 == 0
        phis, scales, nums, outs = {}, {}, {}, {}

        def pair(step):
            return 2 * (2 * c + step // 4 + 4 * ((step // 2) % 2)) + step % 2

        for tick in range(40):
            step, b = tick // 4, tick % 4
            if step < 8:
                r = 2 * ((step // 2) % 2) + step // 4
                if ready is None:
                    phi = _dual_softmax(rows_of(res, r, (step % 2) * 64, b), pin())
                elif step % 2:
                    phi = _dual_softmax(rows_of(res, r, 0, b), pin())
                else:
                    phi = _wide(ready[r, :, pl.ds(b * 128, 128)])
                den = phi * z_v[pair(step)]
                inv = _recip(_head_reduce([den[8 * j:8 * j + 8] for j in range(16)], jnp.add) + 1e-6)
                other = pltpu.roll(inv, 1, 0)
                phis.setdefault(step, []).append(phi)
                scales.setdefault(step, []).append((jnp.where(even, inv, other), jnp.where(even, other, inv)))
            if 1 <= step < 9 and b == lag:
                phi = jnp.concatenate(phis.pop(step - 1), axis=1).astype(bf16)
                nums[step - 1] = _dot(kv_v[pair(step - 1)], phi)
            if step >= 2 and b == 0:
                scale = scales.pop(step - 2)
                scale = [jnp.concatenate([v[head] for v in scale], axis=1) for head in range(2)]
                outs[step - 2] = nums.pop(step - 2) * jnp.concatenate([scale[0]] * 4 + [scale[1]] * 4, axis=0)
                if (step - 2) % 4 == 3:
                    u = (step - 2) // 4
                    o1 = jnp.concatenate([outs.pop(4 * u), outs.pop(4 * u + 1)], axis=0)
                    o2 = jnp.concatenate([outs.pop(4 * u + 2), outs.pop(4 * u + 3)], axis=0)
                    for i, v in enumerate(_rhs_operands(o1[:, :TH], o1[:, TH:], o2[:, :TH], o2[:, TH:])):
                        dst.at[i][:, pl.ds(u * 128, 128)] = pltpu.bitcast(v.astype(bf16).T, u32)
            yield

    def out_project(h, o, res, ks, per_slot):
        def prod(i):
            lhs = jnp.concatenate([o[k][i] for k in ks], axis=1)
            return matmul(lhs, wo_v[h, i, :, pl.ds(ks[0] * 256, len(ks) * 256)], per_slot)

        def emit(a, b, val):
            if isinstance(res, list):
                res[a][b] = val
            else:
                res[a, b] = val

        return _strassen(prod, emit)

    zero_s[0] = 0
    zero_s[1] = 0
    kv_acc[...] = jnp.zeros(kv_acc.shape, f32)
    z_acc[...] = jnp.zeros(z_acc.shape, f32)
    y_acc[...] = jnp.zeros(y_acc.shape, f32)
    best_v[...] = jnp.full(best_v.shape, -jnp.inf, f32)
    best_i[...] = jnp.zeros(best_i.shape, i32)
    w8 = wr8_v[...].astype(f32)
    wr_v[...] = jnp.broadcast_to(jnp.concatenate([w8[j:j + 1, :] for j in range(8)], axis=1), (16, D))
    feature_maps()
    stats, apply = ln_stats(0, st_v.at[0], 16), ln_apply(0, st_v.at[0], x1_v.at[0], False)
    for half in range(2):
        cp_x0(2 * half).wait()
        cp_x0(2 * half + 1).wait()
        schedule((stats, 20, 0.0, 1.0))
        schedule((apply, 32, 0.0, 1.0))
    chunk0 = prep_kv(0)
    schedule((chunk0, 4, 0.0, 1.0))
    schedule((project_part(a1_v.at[0], x1_v.at[0], raw_v.at[0], 0), 7, 0.0, 0.5),
             (project_part(a1_v.at[0], x1_v.at[0], raw_v.at[0], 1), 7, 0.5, 1.0),
             (project(a1_v.at[1], x1_v.at[0], raw_v.at[1])[0], 14, 1.0, 2.0),
             (chunk0, 4, 0.15, 0.45), (ln_split(x1_v.at[zero_s[0]], x2_v.at[0]), 112, 0.03, 0.6),
             (kv_post(0, raw_v.at[zero_s[0]], values_late=True), 18, 0.52, 1.3),
             (prep_kv(1), 8, 0.74, 0.96), (split_kv(1), 112, 1.02, 1.31),
             (prep_kv(2), 8, 1.05, 1.3), (split_kv(2), 112, 1.31, 1.62),
             (prep_kv(3), 8, 1.49, 1.7), (split_kv(3), 112, 1.73, 2.0))

    def kv_tile(t, _):
        last = t == NTILE - 1
        wait_all(q_blocks(t), sem_q.at[t])
        cp_xt(t + 1).wait()

        @pl.when(jnp.logical_and(t > 0, t < 3))
        def _():
            cp_wo(t - 1).wait()

        product[:] = []
        first = (route()[0] // T) % (NTILE - 1) + 1
        x1, x2, st = x1_v.at[pl.ds(t, 2)], x2_v.at[pl.ds(t, 2)], st_v.at[t + 1]
        split = ln_split(x1_v.at[t + 1 + zero_s[0]], x2.at[1])
        wo = [prep_wo(2 * ((t + 1) % 2) + u, jnp.where(t == 0, WV, WO)) for u in range(2)]
        c2, c3, c0 = ([[None] * 4 for _ in range(4)] for _ in range(3))
        schedule(project((b1_v.at[0], b2_v.at[0]), (x1.at[0], x2.at[0]), c2),
                 (kv_post(1, raw_v.at[1]), 18, 0.086, 0.893), (ln_stats(t + 1, st, 32), 36, 0.0, 0.912),
                 (start_ffn(t), 2 * FG + 8, 0.23, 0.908))
        schedule(project((b1_v.at[1], b2_v.at[1]), (x1.at[0], x2.at[0]), c3),
                 (kv_post(2, c2), 18, 0.14, 0.953), (ln_apply(t + 1, st, x1.at[1], True), 64, 0.015, 0.935),
                 (prep_q(t), 4, 0.03, 0.668))
        nxt, chunk = jnp.where(last, first, t + 1), jnp.where(last, 2, 0)
        schedule(project(a1_v.at[chunk], x1_v.at[nxt], c0, keep=half_v),
                 (kv_post(3, c3), 18, 0.0, 0.917), (split, 112, 0.0, 0.903), (split_q(t), 56, 0.1, 0.942))
        schedule(project((a1_v.at[chunk + 1], a2_v.at[chunk]), (x1_v.at[nxt], x2_v.at[nxt]), raw_v.at[1]),
                 (kv_post(jnp.where(last, 4, 0), c0, keep=phi_v), 18, 0.05, 0.917),
                 (wo[0], 4, 0.068, 0.612), (wo[1], 4, 0.447, 0.955), (routed_token(), 8, 0.145, 0.896))
        return first

    first = lax.fori_loop(0, NTILE, kv_tile, jnp.int32(0))

    wait_all(ffn_v.at[0], sem_f.at[0])
    product[:] = []
    idx, top_score = route()
    final = idx // T
    lo, hi = jnp.minimum(first, final), jnp.maximum(first, final)
    second = jnp.where(lo > 0, 0, jnp.where(hi > 1, 1, 2))
    third = 6 - first - final - second

    def tile(j):
        return jnp.where(j == 0, first, jnp.where(j == 1, second, jnp.where(j == 2, third, final)))

    def gate(t, h, a, b, q, update):
        r0, rows = pl.multiple_of(t * T + b * TH + q * EROWS, EROWS), pl.ds(b * TH + q * EROWS, EROWS)
        c0 = h * 512 + a * 256
        mean, scale = st_v[t, 0, rows, :], st_v[t, 1, rows, :] * 0.5
        if update is None:
            mean = mean + pin(EROWS)
        x = x_block(r0, EROWS, pl.ds(c0, 256))
        v = (x - jnp.concatenate([mean, mean], axis=1)) * jnp.concatenate([scale, scale], axis=1)
        if update is not None:
            hit = lax.broadcasted_iota(i32, (EROWS, 256), 0) == idx - r0
            v = v + jnp.where(hit, update[:, c0:c0 + 256], 0.0)
        return x, v + v * jnp.tanh(v)

    def epilogue(t, h, res, part=None, update=None, early=None):
        for a, b in ((0, 1), (0, 0), (1, 0), (1, 1)) if part is not None else ((0, 0), (0, 1), (1, 0), (1, 1)):
            for q in range(TH // EROWS):
                r0, cols = pl.multiple_of(t * T + b * TH + q * EROWS, EROWS), pl.ds(h * 512 + a * 256, 256)
                if early is not None and (a, b) == (1, 1):
                    x, g = x_block(r0, EROWS, cols), early[pl.ds(q * EROWS, EROWS), :]
                else:
                    x, g = gate(t, h, a, b, q, update)
                s = res[a][b][q * EROWS:(q + 1) * EROWS]
                if part is not None:
                    s = s + part[a, b, pl.ds(q * EROWS, EROWS), :]
                out_v[pl.ds(r0, EROWS), cols] = (x + s * g).astype(bf16)
                if part is not None and (q + 1) * EROWS % 128 == 0:
                    start_out(pl.ds(pl.multiple_of(t * T + b * TH + (q + 1) * EROWS - 128, 128), 128), cols)
                yield

    steps = 4 * TH // EROWS
    schedule((q_post(0, half_v, oa_v.at[0], ready=phi_v), 40, 0.01, 1.0))

    def q_tile(j, carry):
        product[:] = []
        oa = oa_v.at[pl.ds(j, 2)]
        o = oa.at[0], ob_v.at[zero_s[0]]
        x = x1_v.at[tile(j + 1)], x2_v.at[tile(j + 1)]
        wait_all(ffn_v.at[j + 1], sem_f.at[j + 1])
        hidden = ffn(j * FL, FL)
        q0, s0, s1 = ([[None] * 4 for _ in range(4)] for _ in range(3))
        schedule(project((a1_v.at[2], a2_v.at[1]), x, q0),
                 (q_post(1, raw_v.at[1], ob_v.at[0]), 40, 0.0, 1.0), (hidden, 14, 0.0, 0.89))
        schedule((out_project(0, o, s0, (0, 1), 7), 7, 0.0, 1.0),
                 (q_post(0, q0, oa.at[1]), 40, 0.0, 1.0), (hidden, 18, 0.085, 0.985))
        schedule((out_project(1, o, s1, (0, 1), 7), 7, 0.0, 1.0),
                 (epilogue(tile(j), 0, s0), steps, 0.055, 0.96), (hidden, 38, 0.02, 1.0))
        schedule(project((a1_v.at[3], a2_v.at[2]), x, raw_v.at[1]),
                 (epilogue(tile(j), 1, s1), steps, 0.0, 0.985), (hidden, 12 * FL - 70, 0.0, 0.885))
        start_out(pl.ds(pl.multiple_of(tile(j) * T, T), T), slice(None))
        return carry

    lax.fori_loop(0, NTILE - 1, q_tile, 0)

    product[:] = []
    o = oa_v.at[NTILE - 1], ob_v.at[zero_s[0]]
    rest = NF - (NTILE - 1) * FL
    schedule((out_project(0, o, part_v.at[0], (0,), 14), 7, 0.0, 0.5),
             (out_project(1, o, part_v.at[1], (0,), 14), 7, 0.5, 1.0),
             (q_post(1, raw_v.at[1], ob_v.at[0], lag=2), 40, 0.0, 0.9), (ffn(NF - rest, rest), 12 * rest, 0.1, 0.8))
    update = jnp.sum(y_acc[...], axis=0, keepdims=True) * (0.5 * jax.nn.sigmoid(top_score[:, 0:1]))
    s0, s1 = ([[None, None], [None, None]] for _ in range(2))

    def last_gate():
        for q in range(TH // EROWS):
            gate_v[0, pl.ds(q * EROWS, EROWS), :] = gate(final, 1, 1, 1, q, update)[1]
            yield

    schedule((out_project(0, o, s0, (1,), 14), 7, 0.0, 0.5), (out_project(1, o, s1, (1,), 14), 7, 0.5, 1.0),
             (epilogue(final, 0, s0, part_v.at[0], update), steps, 0.2, 0.66),
             (epilogue(final, 1, s1, part_v.at[1], update, gate_v.at[zero_s[0]]), steps, 0.69, 1.21),
             (last_gate(), TH // EROWS, 0.0, 0.2))
    pltpu.make_async_copy(out_v, out_hbm, sem_o.at[0]).wait()


def _call(x, wqkv, wphi, wo, wr, wg, wu, wd, interpret=False):
    scratch = [
        pltpu.VMEM((S + T + 4 * D, D), bf16),
        pltpu.VMEM((NTILE + 1, 2, T, 128), f32),
        pltpu.VMEM((NTILE + 1, 7, 128, 512), u32),
        pltpu.VMEM((NTILE + 1, 35, 64, 256), u32),
        pltpu.VMEM((D, DH), bf16),
        pltpu.VMEM((8, 128), bf16),
        pltpu.VMEM((16, D), f32),
        pltpu.VMEM((8, 128, 128), bf16),
        pltpu.VMEM((4, 7, 128, 512), u32),
        pltpu.VMEM((3, 35, 64, 256), u32),
        pltpu.VMEM((2, 7, 128, 512), u32),
        pltpu.VMEM((2, 35, 64, 256), u32),
        pltpu.VMEM((2, 7, 128, 512), u32),
        pltpu.VMEM((NTILE, 3 * FG * D, 128), bf16),
        pltpu.VMEM((H // 2 + 4, 64, 128), f32),
        pltpu.VMEM((H // 2 + 4, 128, 128), f32),
        pltpu.VMEM((H // 2 + 4, 64, 128), bf16),
        pltpu.VMEM((H // 2 + 4, 128, 128), f32),
        pltpu.VMEM((4, 16, 128), f32),
        pltpu.VMEM((4, 16, 128), i32),
        pltpu.VMEM((2, 4, 4, 128, 128), f32),
        pltpu.VMEM((4, 4, 64, 128), f32),
        pltpu.VMEM((4, 64, T), u32),
        pltpu.VMEM((NTILE, 7, 128, 256), u32),
        pltpu.VMEM((2, 7, 128, 256), u32),
        pltpu.VMEM((2, 2, 2, 256, 256), f32),
        pltpu.VMEM((2, 256, 256), f32),
        pltpu.VMEM((D, 128), f32),
        pltpu.VMEM((8, D), f32),
        pltpu.VMEM((S, D), bf16),
        pltpu.SMEM((2,), i32),
        pltpu.SemaphoreType.DMA((NTILE + 2,)),
        pltpu.SemaphoreType.DMA((5,)),
        pltpu.SemaphoreType.DMA((NTILE + 2,)),
        pltpu.SemaphoreType.DMA((1,)),
        pltpu.SemaphoreType.DMA((NTILE,)),
        pltpu.SemaphoreType.DMA((1,)),
    ]
    hbm = pl.BlockSpec(memory_space=pltpu.HBM)
    return pl.pallas_call(
        _kernel,
        out_shape=jax.ShapeDtypeStruct((S, D), bf16),
        in_specs=[hbm] * 8,
        out_specs=hbm,
        scratch_shapes=scratch,
        compiler_params=pltpu.CompilerParams(
            vmem_limit_bytes=120 * 2**20, disable_bounds_checks=True, disable_semaphore_checks=True),
        name="hedgehog",
        interpret=interpret,
    )(x, wqkv, wphi, wo, wr, wg, wu, wd)


@jax.jit
def pallas_recurrent_scan__linear_kernel_hedgehog__moe_arch_mod__prompt_kernel(
    A_x: jax.Array,
    A_wqkv: jax.Array,
    A_w_phi: jax.Array,
    A_wo: jax.Array,
    B_x: jax.Array,
    B_w_r: jax.Array,
    B_w_gate: jax.Array,
    B_w_up: jax.Array,
    B_w_down: jax.Array,
):
    del B_x
    out = _call(A_x.reshape(S, D), A_wqkv, A_w_phi.reshape(D, DH), A_wo,
                B_w_r.reshape(8, 128), B_w_gate, B_w_up, B_w_down)
    return out.reshape(1, S, D)
```

```python
import math

import numpy as np

import jax
import jax.numpy as jnp
from jax import lax
import jax.experimental.pallas as pl
import jax.experimental.pallas.tpu as pltpu

S, D, H, DH, F = 2048, 1024, 32, 32, 3584
T = 512
TH = T // 2
NTILE = S // T
NF = F // 128
FG = NF // NTILE
FL = 9
EROWS = 32
WQ, WK, WV, WO = (S + T + j * D for j in range(4))
LHS_SUMS, RHS_SUMS = (0, 1, 4, 5, 6), (0, 2, 3, 5, 6)
LOG2E = math.log2(math.e)
EPS_BF16 = float(np.float32(1e-5).astype(jnp.bfloat16))
f32, bf16, i32, u32 = jnp.float32, jnp.bfloat16, jnp.int32, jnp.uint32


def _dot_nt(a, b):
    return lax.dot_general(a, b, (((1,), (1,)), ((), ())), preferred_element_type=f32)


def _dot(a, b):
    return jnp.dot(a, b, preferred_element_type=f32)


def _aligned(i, n):
    return i if isinstance(i, int) else pl.multiple_of(i, n)


def _recip(v):
    r = pl.reciprocal(v, approx=True)
    return r * (2.0 - v * r)


def _bf16(words):
    return pltpu.bitcast(words, bf16)


def _wide(words):
    return _bf16(words).astype(f32)


def _narrow(v):
    return pltpu.bitcast(v.astype(bf16), u32)


def _lhs_operands(a11, a12, a21, a22):
    return [a11 + a22, a21 + a22, a11, a22, a11 + a12, a21 - a11, a12 - a22]


def _rhs_operands(b11, b12, b21, b22):
    return [b11 + b22, b11, b12 - b22, b21 - b11, b22, b11 + b12, b21 + b22]


def _strassen(prod, emit):
    m3 = prod(2)
    yield
    m5 = prod(4)
    emit(0, 1, m3 + m5)
    yield
    m1 = prod(0)
    c11, c22 = m1 - m5, m1 + m3
    yield
    c11 = c11 + prod(6)
    yield
    m4 = prod(3)
    emit(0, 0, c11 + m4)
    yield
    m2 = prod(1)
    emit(1, 0, m2 + m4)
    c22 = c22 - m2
    yield
    emit(1, 1, c22 + prod(5))
    yield


class _Quad:
    def __init__(self, blocks):
        self.blocks = blocks

    def __add__(self, other):
        return _Quad([p + q for p, q in zip(self.blocks, other.blocks)])

    def __sub__(self, other):
        return _Quad([p - q for p, q in zip(self.blocks, other.blocks)])


def _strassen_twice(prod, emit):
    done = {}

    def inner(i):
        out = [None] * 4

        def put(a, b, val):
            out[2 * a + b] = val

        yield from _strassen(lambda j: prod(7 * i + j), put)
        done[i] = _Quad(out)

    def put(a, b, quad):
        for k, val in enumerate(quad.blocks):
            emit(2 * a + k // 2, 2 * b + k % 2, val)

    outer = _strassen(lambda i: done[i], put)
    for i in (2, 4, 0, 6, 3, 1, 5):
        steps = inner(i)
        for _ in range(6):
            next(steps)
            yield
        for _ in steps:
            pass
        next(outer)
        yield


def _head_reduce(vs, op):
    while len(vs) > 1:
        vs = [op(vs[i], vs[i + 1]) for i in range(0, len(vs), 2)]
    v = op(vs[0], pltpu.roll(vs[0], 4, 0))
    return op(v, pltpu.roll(v, 2, 0))


def _dual_softmax(p, zero):
    rows = [p[8 * j:8 * j + 8] for j in range(8)]
    rows[0] = rows[0] + zero
    mx, mn = _head_reduce(rows, jnp.maximum), _head_reduce(rows, jnp.minimum)
    ep = [jnp.exp2(v - mx) for v in rows]
    en = [jnp.exp2(mn - v) for v in rows]
    rp, rn = _recip(_head_reduce(ep, jnp.add)), _recip(_head_reduce(en, jnp.add))
    return jnp.concatenate([v * rp for v in ep] + [v * rn for v in en], axis=0)


def _kernel(x_hbm, wqkv_hbm, wphi_hbm, wo_hbm, wr_hbm, wg_hbm, wu_hbm, wd_hbm, out_hbm,
            in_v, st_v, x1_v, x2_v, wphi_v, wr8_v, wr_v, map_v, a1_v, a2_v, b1_v, b2_v, wo_v, ffn_v,
            kv_acc, kv_v, z_v, best_v, best_i, raw_v, half_v, phi_v, oa_v, ob_v, part_v,
            gate_v, xcol_v, y_acc, out_v, zero_s, sem_x, sem_w, sem_q, sem_s, sem_f, sem_o):
    def cp_x(r0, n, sem, src0):
        return pltpu.make_async_copy(x_hbm.at[pl.ds(src0, n)], in_v.at[pl.ds(r0, n)], sem_x.at[sem])

    def cp_x0(piece):
        r0 = (piece % 2) * TH + (piece // 2) * (TH // 2)
        return cp_x(r0, TH // 2, 0 if piece < 2 else NTILE + 1, r0)

    def cp_xt(t):
        return cp_x(_aligned(t * T, T), T, t, _aligned((t % NTILE) * T, T))

    def cp_w(j, c, sem):
        return pltpu.make_async_copy(wqkv_hbm.at[:, pl.ds(j * D + c * 256, 256)],
                                     in_v.at[pl.ds(WQ + j * D, D), pl.ds(c * 256, 256)], sem_w.at[sem])

    def cp_k(c):
        return cp_w(1, c, c)

    def cp_v(c):
        return cp_w(2, c, c if c else 4)

    def start_q(u):
        for n in range(8):
            src = wqkv_hbm.at[pl.ds((n // 2) * 256 + (u % 2) * 128, 128), pl.ds((u // 2) * 256 + (n % 2) * 512, 256)]
            dst = in_v.at[pl.ds(WQ + (u // 2) * 512 + (n // 2) * 128, 128), pl.ds((u % 2) * 512 + (n % 2) * 256, 256)]
            pltpu.make_async_copy(src, dst, sem_q.at[u]).start()

    def q_blocks(u):
        return in_v.at[pl.ds(_aligned(WQ + (u // 2) * 512, 512), 512), pl.ds(_aligned((u % 2) * 512, 512), 512)]

    def cp_wo(h):
        cols = pl.ds(_aligned(h * 512, 512), 512)
        return pltpu.make_async_copy(wo_hbm.at[:, cols], in_v.at[pl.ds(WO, D), cols], sem_q.at[NTILE + h])

    def start_ffn(g):
        for j in range(FG):
            cols = pl.ds(_aligned((g * FG + j) * 128, 128), 128)
            for n, src in enumerate((wg_hbm, wu_hbm)):
                dst = ffn_v.at[g, pl.ds((n * FG + j) * D, D)]
                pltpu.make_async_copy(src.at[:, cols], dst, sem_f.at[g]).start()
                yield
        rows = pl.ds(_aligned(g * FG * 128, 128), FG * 128)
        for n in range(D // 128):
            dst = ffn_v.at[g, pl.ds(2 * FG * D + n * FG * 128, FG * 128)]
            pltpu.make_async_copy(wd_hbm.at[rows, pl.ds(n * 128, 128)], dst, sem_f.at[g]).start()
            yield

    def wait_all(filled, sem):
        pltpu.make_async_copy(filled, filled, sem).wait()

    def start_out(rows, cols):
        pltpu.make_async_copy(out_v.at[rows, cols], out_hbm.at[rows, cols], sem_o.at[0]).start()

    small = [pltpu.make_async_copy(wr_hbm, wr8_v, sem_s.at[0]), pltpu.make_async_copy(wphi_hbm, wphi_v, sem_s.at[0])]
    for cp in small + [cp_x0(0)]:
        cp.start()
    for cp in small:
        cp.wait()
    for piece in range(1, 4):
        cp_x0(piece).start()
    for c in range(4):
        cp_k(c).start()
        cp_v(c).start()
    for t in range(NTILE):
        cp_xt(t + 1).start()
        start_q(t)
        if t in (1, 2):
            cp_wo(t - 1).start()

    clock, product = [0.0], []

    def schedule(*streams):
        events = [(a + (b - a) * k / n, i, k, gen) for i, (gen, n, a, b) in enumerate(streams) for k in range(n)]
        for when, _, _, gen in sorted(events, key=lambda e: e[:3]):
            clock[:] = [when]
            next(gen)

    def matmul(a, b, per_slot):
        m = _dot_nt(_bf16(a), _bf16(b))
        product[:] = [m, per_slot]
        return m

    def pin(n=8):
        if not product:
            return jnp.zeros((n, 128), f32)
        m, per_slot = product
        rows, cols = m.shape[0] // 8, m.shape[1] // 128
        q = min(int((clock[0] * per_slot) % 1.0 * rows * cols + 1e-6), rows * cols - 1)
        m = m[(q % rows) * 8:(q % rows) * 8 + 8, (q // rows) * 128:(q // rows) * 128 + 128]
        z = pltpu.bitcast(pltpu.bitcast(m, u32) & zero_s[0].astype(u32), f32)
        return z if n == 8 else jnp.concatenate([z] * (n // 8), axis=0)

    def feature_maps():
        r = lax.broadcasted_iota(i32, (128, DH), 0)
        select = (((r % 64) // 8) * 4 + (r % 8) // 2 == lax.broadcasted_iota(i32, (128, DH), 1)).astype(bf16)
        r = lax.broadcasted_iota(i32, (128, 128), 0)
        same_head = (r // 64) * 2 + r % 2 == lax.broadcasted_iota(i32, (128, 128), 1) // DH
        for g in range(8):
            full = _dot_nt(select, wphi_v[pl.ds(g * 128, 128), :])
            map_v.at[g][...] = jnp.where(same_head, full, 0.0).astype(bf16)

    def put_lhs(dst, row, col, quadrants):
        for i, v in enumerate(_lhs_operands(*quadrants)):
            dst.at[i][pl.ds(_aligned(row, 8), 8), pl.ds(_aligned(col, 128), 128)] = _narrow(v)

    def w_blocks(base, top, bottom, k):
        return [in_v[pl.ds(_aligned(base + half * 512 + k * 128, 128), 128), pl.ds(_aligned(g * 128, 128), 128)]
                for g in (top, bottom) for half in range(2)]

    def put_folded(blocks, top, bottom, dst, row_of, k):
        blocks = [_dot_nt(map_v[g], w) for g, w in zip((top, top, bottom, bottom), blocks)]
        for j in range(8):
            put_lhs(dst, row_of(j), k * 128, [p[16 * j:16 * j + 16] * LOG2E for p in blocks])

    def put_transposed(base, top, bottom, dst, row_of):
        for k in range(4):
            zero = pltpu.bitcast(pin(), u32)
            blocks = [pltpu.bitcast(w, u32) for w in w_blocks(base, top, bottom, k)]
            blocks = [_bf16(jnp.concatenate([w[:8] | zero, w[8:]], axis=0)).T for w in blocks]
            for j in range(8):
                put_lhs(dst, row_of(j), k * 128, [w[16 * j:16 * j + 16].astype(f32) for w in blocks])
            yield

    def split_again(once, twice, lhs, r, k):
        for i in range(7):
            zero = pltpu.bitcast(pin(), u32)
            w = [[once[i, pl.ds(a * 64 + r * 8, 8), pl.ds(_aligned(b * 256 + k * 128, 128), 128)]
                  for b in range(2)] for a in range(2)]
            q00, q01, q10, q11 = _wide(w[0][0] | zero), _wide(w[0][1]), _wide(w[1][0]), _wide(w[1][1] | zero)
            sums = _lhs_operands(q00, q01, q10, q11) if lhs else _rhs_operands(q00, q10, q01, q11)
            for n, j in enumerate(LHS_SUMS if lhs else RHS_SUMS):
                twice.at[5 * i + n][pl.ds(r * 8, 8), pl.ds(_aligned(k * 128, 128), 128)] = _narrow(sums[j])
            yield

    def operand(once, twice, lhs, ij):
        i, j = ij // 7, ij % 7
        sums = LHS_SUMS if lhs else RHS_SUMS
        if j in sums:
            return twice[5 * i + sums.index(j)]
        d = int(j == (3 if lhs else 4))
        return once[i, pl.ds(d * 64, 64), pl.ds(d * 256, 256)]

    def prep_kv(c):
        dst = a1_v.at[c] if c < 2 else b1_v.at[c - 2]
        cp_k(c).wait()
        if c:
            cp_v(c).wait()
        for k in range(4):
            put_folded(w_blocks(WK, 2 * c, 2 * c + 1, k), 2 * c, 2 * c + 1, dst,
                       lambda j: (j // 4) * 64 + (j % 4) * 8, k)
            yield
        if not c:
            cp_v(c).wait()
        yield from put_transposed(WV, 2 * c, 2 * c + 1, dst, lambda j: (j // 4) * 64 + 32 + (j % 4) * 8)

    def split_kv(c):
        once, twice = (a1_v.at[1 + zero_s[0]], a2_v.at[0]) if c == 1 else (b1_v.at[c - 2 + zero_s[0]], b2_v.at[c - 2])
        for k in range(2):
            for r in range(8):
                yield from split_again(once, twice, True, r, k)

    def prep_q(u):
        w = q_blocks(u)
        for a in range(2):
            g = 2 * (u // 2) + a
            for c in range(2):
                blocks = [w[pl.ds((2 * half + c) * 128, 128), pl.ds(b * 256 + a * 128, 128)]
                          for b in range(2) for half in range(2)]
                put_folded(blocks, g, g + 4, a1_v.at[2 + u // 2], lambda j: a * 64 + 8 * j, u % 2 + 2 * c)
                yield

    def split_q(u):
        for r in range(8):
            yield from split_again(a1_v.at[2 + u // 2 + zero_s[0]], a2_v.at[1 + u // 2], True, r, u % 2)

    def prep_wo(u, base):
        g = (u // 2) * 4 + u % 2
        return put_transposed(base, g, g + 2, wo_v.at[u // 2], lambda j: (u % 2) * 64 + 8 * j)

    def x_block(r0, n, cols):
        return jnp.concatenate([in_v[pl.ds(pl.multiple_of(r0 + q + (zero_s[1] if q % 16 and n == 16 else 0), 8), 8), cols].astype(f32)
                                for q in range(0, n, 8)], axis=0)

    def ln_stats(t, st, batch):
        lane = lax.broadcasted_iota(i32, (16, 128), 1)
        for start in range(0, 32, batch):
            places = [((step % 2) * 16 + step // 2) * 16 for step in range(start, start + batch)]
            means = variances = jnp.ones((16, 128), f32)
            for n, pos in enumerate(places):
                r0 = pl.multiple_of(t * T + pos, 16)
                x0 = x_block(r0, 16, pl.ds(0, 128)) + pin(16)
                s1 = s2 = None
                for j in range(1, 8):
                    d = x_block(r0, 16, pl.ds(j * 128, 128)) - x0
                    s1 = d if j == 1 else s1 + d
                    s2 = d * d if j == 1 else s2 + d * d
                lane_mean = x0 + s1 * 0.125
                mean = jnp.sum(lane_mean, axis=-1, keepdims=True) * (1.0 / 128)
                d = lane_mean - mean
                var = jnp.sum((s2 - s1 * s1 * 0.125) * 0.125 + d * d, axis=-1, keepdims=True)
                variances = jnp.where(lane == n, jnp.broadcast_to(var, (16, 128)), variances)
                means = jnp.where(lane == n, jnp.broadcast_to(mean, (16, 128)), means)
                yield
            means = means.astype(bf16).astype(f32)
            var = ((variances * (1.0 / 128)).astype(bf16).astype(f32) + EPS_BF16).astype(bf16).astype(f32)
            scale = 1.0 / jnp.sqrt(var).astype(bf16).astype(f32)
            for n, pos in enumerate(places):
                for kind, v in enumerate((means, scale)):
                    st[kind, pl.ds(pos, 16), :] = jnp.broadcast_to(v[:, n:n + 1], (16, 128))
                if (n + 1) % (batch // 4) == 0:
                    yield

    def ln_apply(t, st, dst, score_too):
        for step in range(16):
            r0 = [pl.multiple_of(t * T + b * TH + step * 16 + zero_s[0], 16) for b in range(2)]
            mean = [st[0, pl.ds(b * TH + step * 16, 16), :] for b in range(2)]
            scale = [st[1, pl.ds(b * TH + step * 16, 16), :] for b in range(2)]
            score = [None, None]
            for k in range(4):
                zero = pin(16)
                xn = [[(x_block(r0[b], 16, pl.ds(half * 512 + k * 128, 128)) - (mean[b] + zero)) * scale[b]
                       for half in range(2)] for b in range(2)]
                for i, v in enumerate(_rhs_operands(xn[0][0], xn[1][0], xn[0][1], xn[1][1])):
                    dst.at[i][pl.ds(step * 8, 8), pl.ds(k * 128, 128)] = _narrow(v)
                for b in range(2 if score_too else 0):
                    part = xn[b][0] * wr_v[:, pl.ds(k * 128, 128)] + xn[b][1] * wr_v[:, pl.ds(512 + k * 128, 128)]
                    score[b] = part if k == 0 else score[b] + part
                    if k == 3:
                        r = jnp.sum(score[b], axis=-1, keepdims=True).astype(bf16).astype(f32)
                        r = jnp.broadcast_to(r, (16, 128))
                        token = lax.broadcasted_iota(i32, (16, 128), 0) + r0[b] % S
                        slot = 2 * (t // NTILE) + b
                        better = r > best_v[slot]
                        best_v[slot] = jnp.where(better, r, best_v[slot])
                        best_i[slot] = jnp.where(better, token, best_i[slot])
                yield

    def ln_split(once, twice):
        for r in range(8):
            for k in range(2):
                yield from split_again(once, twice, False, r, k)

    def route():
        score, token = best_v[...].reshape(64, 128), best_i[...].reshape(64, 128)
        top = jnp.max(score, axis=0, keepdims=True)
        idx = jnp.min(jnp.where(score == top, token, S).astype(f32)).astype(i32)
        return jnp.clip(idx, 0, S - 1), top

    def routed_token():
        idx = route()[0]
        base = pl.multiple_of((idx // 16) * 16, 16)
        rows = pl.ds(pl.multiple_of(base % T, 16), 16)
        xn = (in_v[pl.ds(base, 16), :].astype(f32) - st_v[idx // T, 0, rows, 0:1]) * st_v[idx // T, 1, rows, 0:1]
        xn = jnp.where(lax.broadcasted_iota(i32, (16, D), 0) == idx - base, xn, 0.0)
        xn = jnp.sum(xn, axis=0, keepdims=True).astype(bf16).astype(f32)
        for j in range(8):
            row = xn[:, j * 128:(j + 1) * 128] + pin()
            xcol_v[pl.ds(j * 128, 128), :] = jnp.concatenate([row] * 16, axis=0).T
            yield

    def ffn(f0, n):
        for j in range(n):
            group, f = ffn_v.at[(f0 + j) // FG], (f0 + j) % FG
            accs = [jnp.zeros((8, 128), f32)] * 2
            for r in range(8):
                x, zero = xcol_v[pl.ds(r * 128, 128), :], pin()
                for a in range(2):
                    prod = group[pl.ds(_aligned((a * FG + f) * D + r * 128, 128), 128), :].astype(f32) * x
                    acc = accs[a] + zero
                    for q in range(16):
                        acc = acc + prod[8 * q:8 * q + 8]
                    accs[a] = acc
                yield
            gate, up = [jnp.sum(acc, axis=0, keepdims=True) for acc in accs]
            hidden = jnp.broadcast_to(gate * jax.nn.sigmoid(gate) * up, (128, 128)).T
            for c in range(8):
                prod = group[pl.ds(_aligned(2 * FG * D + (c * FG + f) * 128, 128), 128), :].astype(f32) * hidden
                acc = y_acc[:, pl.ds(c * 128, 128)] + pin()
                for q in range(16):
                    acc = acc + prod[8 * q:8 * q + 8]
                y_acc[:, pl.ds(c * 128, 128)] = acc
                if c % 2:
                    yield

    def project(w, x, res, keep=None):
        def emit(r, b, val):
            if isinstance(res, list):
                res[r][b] = val
            else:
                res[r, b] = val
            if keep is not None:
                keep[r, b] = val[64:]

        def once():
            for c in range(2):
                def put(a, b, val):
                    emit(2 * a, 2 * b + c, val[:128])
                    emit(2 * a + 1, 2 * b + c, val[128:])

                yield from _strassen(lambda i: matmul(w[i], x[i, pl.ds(c * 64, 64), :], 14), put)

        if isinstance(w, tuple):
            return _strassen_twice(lambda i: matmul(operand(*w, True, i), operand(*x, False, i), 49), emit), 49, 0.0, 1.0
        return once(), 14, 0.0, 1.0

    def project_part(w, x, res, part):
        def prod(i):
            rows = [w[i, pl.ds(a * 64 + part * 32, 32), :] for a in range(2)]
            return matmul(jnp.concatenate(rows, axis=0), x[i], 14)

        def put(a, b, val):
            for r in range(2):
                for c in range(2):
                    res[2 * a + r, 2 * b + c, pl.ds(part * 64, 64), :] = val[r * 64:(r + 1) * 64, c * 128:(c + 1) * 128]

        return _strassen(prod, put)

    def rows_of(res, r, r0, b):
        return res[r][b][r0:r0 + 64] if isinstance(res, list) else res[r, b, pl.ds(r0, 64), :]

    def kv_post(c, res, keep=None, values_late=False):
        same_head = lax.broadcasted_iota(i32, (64, 128), 0) // DH == lax.broadcasted_iota(i32, (64, 128), 1) % 2

        sums = {}

        def accumulate(r, b, phi):
            v = jnp.concatenate([rows_of(res, r, 64, b), jnp.ones((16, 128), f32)], axis=0)
            part = _dot_nt(v.astype(bf16), phi.astype(bf16))[:72]
            sums[r] = (kv_acc[4 * c + r] if b == 0 else sums[r]) + part
            if b == 3:
                total = kv_acc[4 * c + r] = sums.pop(r)
                kv_v.at[4 * c + r][...] = jnp.where(same_head, total[:64], 0.0).astype(bf16)
                z_v[4 * c + r] = jnp.concatenate([total[64:]] * 16, axis=0).T

        pending = []
        for r in range(4):
            for b in range(4):
                phi = _dual_softmax(rows_of(res, r, 0, b), pin())
                if keep is not None:
                    keep.at[r][:, pl.ds(b * 128, 128)] = _narrow(phi)
                pending.append((r, b, phi))
                if len(pending) > 3 and not values_late:
                    accumulate(*pending.pop(0))
                yield
        yield
        for rest in pending:
            accumulate(*rest)
        yield

    def q_post(c, res, dst, ready=None, lag=3):
        even = lax.broadcasted_iota(i32, (8, 128), 0) % 2 == 0
        phis, scales, nums, outs = {}, {}, {}, {}

        def pair(step):
            return 2 * (2 * c + step // 4 + 4 * ((step // 2) % 2)) + step % 2

        for tick in range(32 + lag):
            step, b = tick // 4, tick % 4
            if step < 8:
                r = 2 * ((step // 2) % 2) + step // 4
                if ready is None:
                    phi = _dual_softmax(rows_of(res, r, (step % 2) * 64, b), pin())
                elif step % 2:
                    phi = _dual_softmax(rows_of(res, r, 0, b), pin())
                else:
                    phi = _wide(ready[r, :, pl.ds(b * 128, 128)])
                den = phi * z_v[pair(step)]
                inv = _recip(_head_reduce([den[8 * j:8 * j + 8] for j in range(16)], jnp.add) + 1e-6)
                other = pltpu.roll(inv, 1, 0)
                phis[tick] = phi
                scales[tick] = [jnp.where(even, inv, other)] * 4 + [jnp.where(even, other, inv)] * 4
            n = tick - lag
            if 0 <= n < 32:
                num = _dot(kv_v[pair(n // 4)], phis.pop(n).astype(bf16))
                outs[n] = num * jnp.concatenate(scales.pop(n), axis=0)
                if n % 16 == 15:
                    u = n // 16
                    o = [[jnp.concatenate([jnp.concatenate([outs.pop(16 * u + 8 * a + 4 * p + 2 * h + j) for j in range(2)], axis=1)
                                           for p in range(2)], axis=0) for h in range(2)] for a in range(2)]
                    for i, v in enumerate(_rhs_operands(o[0][0], o[0][1], o[1][0], o[1][1])):
                        dst.at[i][:, pl.ds(u * 128, 128)] = pltpu.bitcast(v.astype(bf16).T, u32)
            yield

    def out_project(h, o, res, ks, per_slot):
        def prod(i):
            lhs = jnp.concatenate([o[k][i] for k in ks], axis=1)
            return matmul(lhs, wo_v[h, i, :, pl.ds(ks[0] * 256, len(ks) * 256)], per_slot)

        def emit(a, b, val):
            if isinstance(res, list):
                res[a][b] = val
            else:
                res[a, b] = val

        return _strassen(prod, emit)

    zero_s[0] = 0
    zero_s[1] = 0
    kv_acc[...] = jnp.zeros(kv_acc.shape, f32)
    y_acc[...] = jnp.zeros(y_acc.shape, f32)
    best_v[...] = jnp.full(best_v.shape, -jnp.inf, f32)
    best_i[...] = jnp.zeros(best_i.shape, i32)
    w8 = wr8_v[...].astype(f32)
    wr_v[...] = jnp.broadcast_to(jnp.concatenate([w8[j:j + 1, :] for j in range(8)], axis=1), (16, D))
    feature_maps()
    stats, apply = ln_stats(0, st_v.at[0], 16), ln_apply(0, st_v.at[0], x1_v.at[0], False)
    for half in range(2):
        cp_x0(2 * half).wait()
        cp_x0(2 * half + 1).wait()
        schedule((stats, 20, 0.0, 1.0))
        schedule((apply, 32, 0.0, 1.0))
    chunk0 = prep_kv(0)
    schedule((chunk0, 4, 0.0, 1.0))
    schedule((project_part(a1_v.at[0], x1_v.at[0], raw_v.at[0], 0), 7, 0.0, 0.5),
             (project_part(a1_v.at[0], x1_v.at[0], raw_v.at[0], 1), 7, 0.5, 1.0),
             (project(a1_v.at[1], x1_v.at[0], raw_v.at[1])[0], 14, 1.0, 2.0),
             (chunk0, 4, 0.15, 0.45), (ln_split(x1_v.at[zero_s[0]], x2_v.at[0]), 112, 0.03, 0.6),
             (kv_post(0, raw_v.at[zero_s[0]], values_late=True), 18, 0.52, 1.3),
             (prep_kv(1), 8, 0.74, 0.96), (split_kv(1), 112, 1.02, 1.31),
             (prep_kv(2), 8, 1.05, 1.3), (split_kv(2), 112, 1.31, 1.62),
             (prep_kv(3), 8, 1.49, 1.7), (split_kv(3), 112, 1.73, 2.0))

    def kv_tile(t, _):
        last = t == NTILE - 1
        wait_all(q_blocks(t), sem_q.at[t])
        cp_xt(t + 1).wait()

        @pl.when(jnp.logical_and(t > 0, t < 3))
        def _():
            cp_wo(t - 1).wait()

        product[:] = []
        first = (route()[0] // T) % (NTILE - 1) + 1
        x1, x2, st = x1_v.at[pl.ds(t, 2)], x2_v.at[pl.ds(t, 2)], st_v.at[t + 1]
        split = ln_split(x1_v.at[t + 1 + zero_s[0]], x2.at[1])
        wo = [prep_wo(2 * ((t + 1) % 2) + u, jnp.where(t == 0, WV, WO)) for u in range(2)]
        c2, c3, c0 = ([[None] * 4 for _ in range(4)] for _ in range(3))
        schedule(project((b1_v.at[0], b2_v.at[0]), (x1.at[0], x2.at[0]), c2),
                 (kv_post(1, raw_v.at[1]), 18, 0.074, 0.863), (ln_stats(t + 1, st, 32), 36, 0.0, 0.882),
                 (start_ffn(t), 2 * FG + 8, 0.23, 0.818))
        schedule(project((b1_v.at[1], b2_v.at[1]), (x1.at[0], x2.at[0]), c3),
                 (kv_post(2, c2), 18, 0.092, 0.869), (ln_apply(t + 1, st, x1.at[1], True), 64, 0.015, 0.935),
                 (prep_q(t), 4, 0.042, 0.686))
        nxt, chunk = jnp.where(last, first, t + 1), jnp.where(last, 2, 0)
        schedule(project(a1_v.at[chunk], x1_v.at[nxt], c0, keep=half_v),
                 (kv_post(3, c3), 18, 0.012, 0.887), (split, 112, 0.0, 0.903), (split_q(t), 56, 0.03, 0.972))
        schedule(project((a1_v.at[chunk + 1], a2_v.at[chunk]), (x1_v.at[nxt], x2_v.at[nxt]), raw_v.at[1]),
                 (kv_post(jnp.where(last, 4, 0), c0, keep=phi_v), 18, 0.05, 0.917),
                 (wo[0], 4, 0.08, 0.6), (wo[1], 4, 0.489, 0.937), (routed_token(), 8, 0.145, 0.896))
        return first

    first = lax.fori_loop(0, NTILE, kv_tile, jnp.int32(0))

    wait_all(ffn_v.at[0], sem_f.at[0])
    product[:] = []
    idx, top_score = route()
    final = idx // T
    lo, hi = jnp.minimum(first, final), jnp.maximum(first, final)
    second = jnp.where(lo > 0, 0, jnp.where(hi > 1, 1, 2))
    third = 6 - first - final - second

    def tile(j):
        return jnp.where(j == 0, first, jnp.where(j == 1, second, jnp.where(j == 2, third, final)))

    def gate(t, h, a, b, q, update):
        r0, rows = pl.multiple_of(t * T + b * TH + q * EROWS, EROWS), pl.ds(b * TH + q * EROWS, EROWS)
        c0 = h * 512 + a * 256
        mean, scale = st_v[t, 0, rows, :], st_v[t, 1, rows, :] * 0.5
        if update is None:
            mean = mean + pin(EROWS)
        x = x_block(r0, EROWS, pl.ds(c0, 256))
        v = (x - jnp.concatenate([mean, mean], axis=1)) * jnp.concatenate([scale, scale], axis=1)
        if update is not None:
            hit = lax.broadcasted_iota(i32, (EROWS, 256), 0) == idx - r0
            v = v + jnp.where(hit, update[:, c0:c0 + 256], 0.0)
        return x, v + v * jnp.tanh(v)

    def epilogue(t, h, res, part=None, update=None, early=None):
        for a, b in ((0, 1), (0, 0), (1, 0), (1, 1)) if part is not None else ((0, 0), (0, 1), (1, 0), (1, 1)):
            for q in range(TH // EROWS):
                r0, cols = pl.multiple_of(t * T + b * TH + q * EROWS, EROWS), pl.ds(h * 512 + a * 256, 256)
                if early is not None and (a, b) == (1, 1):
                    x, g = x_block(r0, EROWS, cols), early[pl.ds(q * EROWS, EROWS), :]
                else:
                    x, g = gate(t, h, a, b, q, update)
                s = res[a][b][q * EROWS:(q + 1) * EROWS]
                if part is not None:
                    s = s + part[a, b, pl.ds(q * EROWS, EROWS), :]
                out_v[pl.ds(r0, EROWS), cols] = (x + s * g).astype(bf16)
                if part is not None and (q + 1) * EROWS % 128 == 0:
                    start_out(pl.ds(pl.multiple_of(t * T + b * TH + (q + 1) * EROWS - 128, 128), 128), cols)
                yield

    steps = 4 * TH // EROWS
    schedule((q_post(0, half_v, oa_v.at[0], ready=phi_v), 35, 0.01, 1.0))

    def q_tile(j, carry):
        product[:] = []
        oa = oa_v.at[pl.ds(j, 2)]
        o = oa.at[0], ob_v.at[zero_s[0]]
        x = x1_v.at[tile(j + 1)], x2_v.at[tile(j + 1)]
        wait_all(ffn_v.at[j + 1], sem_f.at[j + 1])
        hidden = ffn(j * FL, FL)
        q0, s0, s1 = ([[None] * 4 for _ in range(4)] for _ in range(3))
        schedule(project((a1_v.at[2], a2_v.at[1]), x, q0),
                 (q_post(1, raw_v.at[1], ob_v.at[0]), 35, 0.012, 0.898), (hidden, 14, 0.072, 0.95))
        schedule((out_project(0, o, s0, (0, 1), 7), 7, 0.0, 1.0),
                 (q_post(0, q0, oa.at[1]), 35, 0.0, 0.988), (hidden, 18, 0.169, 0.97))
        schedule((out_project(1, o, s1, (0, 1), 7), 7, 0.0, 1.0),
                 (epilogue(tile(j), 0, s0), steps, 0.043, 1.0), (hidden, 38, 0.044, 0.97))
        schedule(project((a1_v.at[3], a2_v.at[2]), x, raw_v.at[1]),
                 (epilogue(tile(j), 1, s1), steps, 0.03, 0.853), (hidden, 12 * FL - 70, 0.0, 0.885))
        start_out(pl.ds(pl.multiple_of(tile(j) * T, T), T), slice(None))
        return carry

    lax.fori_loop(0, NTILE - 1, q_tile, 0)

    product[:] = []
    o = oa_v.at[NTILE - 1], ob_v.at[zero_s[0]]
    rest = NF - (NTILE - 1) * FL
    schedule((out_project(0, o, part_v.at[0], (0,), 14), 7, 0.0, 0.5),
             (out_project(1, o, part_v.at[1], (0,), 14), 7, 0.5, 1.0),
             (q_post(1, raw_v.at[1], ob_v.at[0]), 35, 0.0, 0.9), (ffn(NF - rest, rest), 12 * rest, 0.1, 0.8))
    update = jnp.sum(y_acc[...], axis=0, keepdims=True) * (0.5 * jax.nn.sigmoid(top_score[:, 0:1]))
    s0, s1 = ([[None, None], [None, None]] for _ in range(2))

    def last_gate():
        for q in range(TH // EROWS):
            gate_v[0, pl.ds(q * EROWS, EROWS), :] = gate(final, 1, 1, 1, q, update)[1]
            yield

    schedule((out_project(0, o, s0, (1,), 14), 7, 0.0, 0.5), (out_project(1, o, s1, (1,), 14), 7, 0.5, 1.0),
             (epilogue(final, 0, s0, part_v.at[0], update), steps, 0.2, 0.66),
             (epilogue(final, 1, s1, part_v.at[1], update, gate_v.at[zero_s[0]]), steps, 0.69, 1.21),
             (last_gate(), TH // EROWS, 0.0, 0.2))
    pltpu.make_async_copy(out_v, out_hbm, sem_o.at[0]).wait()


def _call(x, wqkv, wphi, wo, wr, wg, wu, wd, interpret=False):
    scratch = [
        pltpu.VMEM((S + T + 4 * D, D), bf16),
        pltpu.VMEM((NTILE + 1, 2, T, 128), f32),
        pltpu.VMEM((NTILE + 1, 7, 128, 512), u32),
        pltpu.VMEM((NTILE + 1, 35, 64, 256), u32),
        pltpu.VMEM((D, DH), bf16),
        pltpu.VMEM((8, 128), bf16),
        pltpu.VMEM((16, D), f32),
        pltpu.VMEM((8, 128, 128), bf16),
        pltpu.VMEM((4, 7, 128, 512), u32),
        pltpu.VMEM((3, 35, 64, 256), u32),
        pltpu.VMEM((2, 7, 128, 512), u32),
        pltpu.VMEM((2, 35, 64, 256), u32),
        pltpu.VMEM((2, 7, 128, 512), u32),
        pltpu.VMEM((NTILE, 3 * FG * D, 128), bf16),
        pltpu.VMEM((H // 2 + 4, 72, 128), f32),
        pltpu.VMEM((H // 2 + 4, 64, 128), bf16),
        pltpu.VMEM((H // 2 + 4, 128, 128), f32),
        pltpu.VMEM((4, 16, 128), f32),
        pltpu.VMEM((4, 16, 128), i32),
        pltpu.VMEM((2, 4, 4, 128, 128), f32),
        pltpu.VMEM((4, 4, 64, 128), f32),
        pltpu.VMEM((4, 64, T), u32),
        pltpu.VMEM((NTILE, 7, 128, 256), u32),
        pltpu.VMEM((2, 7, 128, 256), u32),
        pltpu.VMEM((2, 2, 2, 256, 256), f32),
        pltpu.VMEM((2, 256, 256), f32),
        pltpu.VMEM((D, 128), f32),
        pltpu.VMEM((8, D), f32),
        pltpu.VMEM((S, D), bf16),
        pltpu.SMEM((2,), i32),
        pltpu.SemaphoreType.DMA((NTILE + 2,)),
        pltpu.SemaphoreType.DMA((5,)),
        pltpu.SemaphoreType.DMA((NTILE + 2,)),
        pltpu.SemaphoreType.DMA((1,)),
        pltpu.SemaphoreType.DMA((NTILE,)),
        pltpu.SemaphoreType.DMA((1,)),
    ]
    hbm = pl.BlockSpec(memory_space=pltpu.HBM)
    return pl.pallas_call(
        _kernel,
        out_shape=jax.ShapeDtypeStruct((S, D), bf16),
        in_specs=[hbm] * 8,
        out_specs=hbm,
        scratch_shapes=scratch,
        compiler_params=pltpu.CompilerParams(
            vmem_limit_bytes=120 * 2**20, disable_bounds_checks=True, disable_semaphore_checks=True),
        name="hedgehog",
        interpret=interpret,
    )(x, wqkv, wphi, wo, wr, wg, wu, wd)


@jax.jit
def pallas_recurrent_scan__linear_kernel_hedgehog__moe_arch_mod__prompt_kernel(
    A_x: jax.Array,
    A_wqkv: jax.Array,
    A_w_phi: jax.Array,
    A_wo: jax.Array,
    B_x: jax.Array,
    B_w_r: jax.Array,
    B_w_gate: jax.Array,
    B_w_up: jax.Array,
    B_w_down: jax.Array,
):
    del B_x
    out = _call(A_x.reshape(S, D), A_wqkv, A_w_phi.reshape(D, DH), A_wo,
                B_w_r.reshape(8, 128), B_w_gate, B_w_up, B_w_down)
    return out.reshape(1, S, D)
```

```python
import math

import numpy as np

import jax
import jax.numpy as jnp
from jax import lax
import jax.experimental.pallas as pl
import jax.experimental.pallas.tpu as pltpu

S, D, H, DH, F = 2048, 1024, 32, 32, 3584
T = 512
TH = T // 2
NTILE = S // T
NF = F // 128
FG = NF // NTILE
FL = 9
EROWS = 32
WQ, WK, WV, WO = (S + T + j * D for j in range(4))
LHS_SUMS, RHS_SUMS = (0, 1, 4, 5, 6), (0, 2, 3, 5, 6)
PRODUCT_ORDER = (2, 4, 0, 6, 3, 1, 5)
LOG2E = math.log2(math.e)
EPS_BF16 = float(np.float32(1e-5).astype(jnp.bfloat16))
f32, bf16, i32, u32 = jnp.float32, jnp.bfloat16, jnp.int32, jnp.uint32


def _dot_nt(a, b):
    return lax.dot_general(a, b, (((1,), (1,)), ((), ())), preferred_element_type=f32)


def _dot(a, b):
    return jnp.dot(a, b, preferred_element_type=f32)


def _aligned(i, n):
    return i if isinstance(i, int) else pl.multiple_of(i, n)


def _recip(v):
    r = pl.reciprocal(v, approx=True)
    return r * (2.0 - v * r)


def _bf16(words):
    return pltpu.bitcast(words, bf16)


def _wide(words):
    return _bf16(words).astype(f32)


def _narrow(v):
    return pltpu.bitcast(v.astype(bf16), u32)


def _lhs_operands(a11, a12, a21, a22):
    return [a11 + a22, a21 + a22, a11, a22, a11 + a12, a21 - a11, a12 - a22]


def _rhs_operands(b11, b12, b21, b22):
    return [b11 + b22, b11, b12 - b22, b21 - b11, b22, b11 + b12, b21 + b22]


def _strassen(prod, emit):
    m3 = prod(2)
    yield
    m5 = prod(4)
    emit(0, 1, m3 + m5)
    yield
    m1 = prod(0)
    c11, c22 = m1 - m5, m1 + m3
    yield
    c11 = c11 + prod(6)
    yield
    m4 = prod(3)
    emit(0, 0, c11 + m4)
    yield
    m2 = prod(1)
    emit(1, 0, m2 + m4)
    c22 = c22 - m2
    yield
    emit(1, 1, c22 + prod(5))
    yield


class _Quad:
    def __init__(self, blocks):
        self.blocks = blocks

    def __add__(self, other):
        return _Quad([p + q for p, q in zip(self.blocks, other.blocks)])

    def __sub__(self, other):
        return _Quad([p - q for p, q in zip(self.blocks, other.blocks)])


def _strassen_twice(prod, emit):
    done = {}

    def inner(i):
        out = [None] * 4

        def put(a, b, val):
            out[2 * a + b] = val

        yield from _strassen(lambda j: prod(7 * i + j), put)
        done[i] = _Quad(out)

    def put(a, b, quad):
        for k, val in enumerate(quad.blocks):
            emit(2 * a + k // 2, 2 * b + k % 2, val)

    outer = _strassen(lambda i: done[i], put)
    for i in PRODUCT_ORDER:
        steps = inner(i)
        for _ in range(6):
            next(steps)
            yield
        for _ in steps:
            pass
        next(outer)
        yield


def _head_reduce(vs, op):
    while len(vs) > 1:
        vs = [op(vs[i], vs[i + 1]) for i in range(0, len(vs), 2)]
    v = op(vs[0], pltpu.roll(vs[0], 4, 0))
    return op(v, pltpu.roll(v, 2, 0))


def _dual_softmax(p, zero):
    rows = [p[8 * j:8 * j + 8] for j in range(8)]
    rows[0] = rows[0] + zero
    mx, mn = _head_reduce(rows, jnp.maximum), _head_reduce(rows, jnp.minimum)
    ep = [jnp.exp2(v - mx) for v in rows]
    en = [jnp.exp2(mn - v) for v in rows]
    rp, rn = _recip(_head_reduce(ep, jnp.add)), _recip(_head_reduce(en, jnp.add))
    return jnp.concatenate([v * rp for v in ep] + [v * rn for v in en], axis=0)


def _kernel(x_hbm, wqkv_hbm, wphi_hbm, wo_hbm, wr_hbm, wg_hbm, wu_hbm, wd_hbm, out_hbm,
            in_v, st_v, x1_v, x2_v, wphi_v, wr8_v, wr_v, map_v, a1_v, a2_v, b1_v, b2_v, wo_v, ffn_v,
            kv_acc, kv_v, z_v, best_v, best_i, raw_v, half_v, phi_v, oa_v, ob_v, part_v,
            gate_v, xcol_v, y_acc, out_v, zero_s, sem_x, sem_w, sem_q, sem_s, sem_f, sem_o):
    def cp_x(r0, n, sem, src0):
        return pltpu.make_async_copy(x_hbm.at[pl.ds(src0, n)], in_v.at[pl.ds(r0, n)], sem_x.at[sem])

    def cp_x0(piece):
        r0 = (piece % 2) * TH + (piece // 2) * (TH // 2)
        return cp_x(r0, TH // 2, 0 if piece < 2 else NTILE + 1, r0)

    def cp_xt(t):
        return cp_x(_aligned(t * T, T), T, t, _aligned((t % NTILE) * T, T))

    def cp_w(j, c, sem):
        return pltpu.make_async_copy(wqkv_hbm.at[:, pl.ds(j * D + c * 256, 256)],
                                     in_v.at[pl.ds(WQ + j * D, D), pl.ds(c * 256, 256)], sem_w.at[sem])

    def cp_k(c):
        return cp_w(1, c, c)

    def cp_v(c):
        return cp_w(2, c, c if c else 4)

    def start_q(u):
        for n in range(8):
            src = wqkv_hbm.at[pl.ds((n // 2) * 256 + (u % 2) * 128, 128), pl.ds((u // 2) * 256 + (n % 2) * 512, 256)]
            dst = in_v.at[pl.ds(WQ + (u // 2) * 512 + (n // 2) * 128, 128), pl.ds((u % 2) * 512 + (n % 2) * 256, 256)]
            pltpu.make_async_copy(src, dst, sem_q.at[u]).start()

    def q_blocks(u):
        return in_v.at[pl.ds(_aligned(WQ + (u // 2) * 512, 512), 512), pl.ds(_aligned((u % 2) * 512, 512), 512)]

    def cp_wo(h):
        cols = pl.ds(_aligned(h * 512, 512), 512)
        return pltpu.make_async_copy(wo_hbm.at[:, cols], in_v.at[pl.ds(WO, D), cols], sem_q.at[NTILE + h])

    def start_ffn(g):
        for j in range(FG):
            cols = pl.ds(_aligned((g * FG + j) * 128, 128), 128)
            for n, src in enumerate((wg_hbm, wu_hbm)):
                dst = ffn_v.at[g, pl.ds((n * FG + j) * D, D)]
                pltpu.make_async_copy(src.at[:, cols], dst, sem_f.at[g]).start()
                yield
        rows = pl.ds(_aligned(g * FG * 128, 128), FG * 128)
        for n in range(D // 128):
            dst = ffn_v.at[g, pl.ds(2 * FG * D + n * FG * 128, FG * 128)]
            pltpu.make_async_copy(wd_hbm.at[rows, pl.ds(n * 128, 128)], dst, sem_f.at[g]).start()
            yield

    def wait_all(filled, sem):
        pltpu.make_async_copy(filled, filled, sem).wait()

    def start_out(rows, cols):
        pltpu.make_async_copy(out_v.at[rows, cols], out_hbm.at[rows, cols], sem_o.at[0]).start()

    small = [pltpu.make_async_copy(wr_hbm, wr8_v, sem_s.at[0]), pltpu.make_async_copy(wphi_hbm, wphi_v, sem_s.at[0])]
    for cp in small + [cp_x0(0)]:
        cp.start()
    for cp in small:
        cp.wait()
    for piece in range(1, 4):
        cp_x0(piece).start()
    for c in range(4):
        cp_k(c).start()
        cp_v(c).start()
    for t in range(NTILE):
        cp_xt(t + 1).start()
        start_q(t)
        if t in (1, 2):
            cp_wo(t - 1).start()

    clock, product = [0.0], []

    def schedule(*streams):
        events = [(a + (b - a) * k / n, i, k, gen) for i, (gen, n, a, b) in enumerate(streams) for k in range(n)]
        for when, _, _, gen in sorted(events, key=lambda e: e[:3]):
            clock[:] = [when]
            next(gen)

    def matmul(a, b, per_slot):
        m = _dot_nt(_bf16(a), _bf16(b))
        product[:] = [m, per_slot]
        return m

    def pin(n=8):
        if not product:
            return jnp.zeros((n, 128), f32)
        m, per_slot = product
        rows, cols = m.shape[0] // 8, m.shape[1] // 128
        q = min(int((clock[0] * per_slot) % 1.0 * rows * cols + 1e-6), rows * cols - 1)
        m = m[(q % rows) * 8:(q % rows) * 8 + 8, (q // rows) * 128:(q // rows) * 128 + 128]
        z = pltpu.bitcast(pltpu.bitcast(m, u32) & zero_s[0].astype(u32), f32)
        return z if n == 8 else jnp.concatenate([z] * (n // 8), axis=0)

    def feature_maps():
        r = lax.broadcasted_iota(i32, (128, DH), 0)
        select = (((r % 64) // 8) * 4 + (r % 8) // 2 == lax.broadcasted_iota(i32, (128, DH), 1)).astype(bf16)
        r = lax.broadcasted_iota(i32, (128, 128), 0)
        same_head = (r // 64) * 2 + r % 2 == lax.broadcasted_iota(i32, (128, 128), 1) // DH
        for g in range(8):
            full = _dot_nt(select, wphi_v[pl.ds(g * 128, 128), :])
            map_v.at[g][...] = jnp.where(same_head, full, 0.0).astype(bf16)

    def put_lhs(dst, row, col, quadrants):
        for i, v in enumerate(_lhs_operands(*quadrants)):
            dst.at[i][pl.ds(_aligned(row, 8), 8), pl.ds(_aligned(col, 128), 128)] = _narrow(v)

    def w_blocks(base, top, bottom, k):
        return [in_v[pl.ds(_aligned(base + half * 512 + k * 128, 128), 128), pl.ds(_aligned(g * 128, 128), 128)]
                for g in (top, bottom) for half in range(2)]

    def put_folded(blocks, top, bottom, dst, row_of, k):
        blocks = [_dot_nt(map_v[g], w) for g, w in zip((top, top, bottom, bottom), blocks)]
        for j in range(8):
            put_lhs(dst, row_of(j), k * 128, [p[16 * j:16 * j + 16] * LOG2E for p in blocks])

    def put_transposed(base, top, bottom, dst, row_of):
        for k in range(4):
            zero = pltpu.bitcast(pin(), u32)
            blocks = [pltpu.bitcast(w, u32) for w in w_blocks(base, top, bottom, k)]
            blocks = [_bf16(jnp.concatenate([w[:8] | zero, w[8:]], axis=0)).T for w in blocks]
            for j in range(8):
                put_lhs(dst, row_of(j), k * 128, [w[16 * j:16 * j + 16].astype(f32) for w in blocks])
            yield

    def split_again(once, twice, lhs, i, r, k):
        zero = pltpu.bitcast(pin(), u32)
        w = [[once[i, pl.ds(a * 64 + r * 8, 8), pl.ds(_aligned(b * 256 + k * 128, 128), 128)]
              for b in range(2)] for a in range(2)]
        q00, q01, q10, q11 = _wide(w[0][0] | zero), _wide(w[0][1]), _wide(w[1][0]), _wide(w[1][1] | zero)
        sums = _lhs_operands(q00, q01, q10, q11) if lhs else _rhs_operands(q00, q10, q01, q11)
        for n, j in enumerate(LHS_SUMS if lhs else RHS_SUMS):
            twice[i].at[n][pl.ds(r * 8, 8), pl.ds(_aligned(k * 128, 128), 128)] = _narrow(sums[j])

    def operand(once, twice, lhs, ij):
        i, j = ij // 7, ij % 7
        sums = LHS_SUMS if lhs else RHS_SUMS
        if j in sums:
            return twice[i][sums.index(j)]
        d = int(j == (3 if lhs else 4))
        return once[i, pl.ds(d * 64, 64), pl.ds(d * 256, 256)]

    def per_operand(ref):
        return [ref.at[pl.ds(5 * i, 5)] for i in range(7)]

    def prep_kv(c):
        dst = a1_v.at[c] if c < 2 else b1_v.at[c - 2]
        cp_k(c).wait()
        if c:
            cp_v(c).wait()
        for k in range(4):
            put_folded(w_blocks(WK, 2 * c, 2 * c + 1, k), 2 * c, 2 * c + 1, dst,
                       lambda j: (j // 4) * 64 + (j % 4) * 8, k)
            yield
        if not c:
            cp_v(c).wait()
        yield from put_transposed(WV, 2 * c, 2 * c + 1, dst, lambda j: (j // 4) * 64 + 32 + (j % 4) * 8)

    def split_kv(c):
        once, twice = (a1_v.at[c + zero_s[0]], a2_v.at[c]) if c < 2 else (b1_v.at[c - 2 + zero_s[0]], b2_v.at[c - 2])
        for k in range(2):
            for r in range(8):
                for i in range(7):
                    split_again(once, per_operand(twice), True, i, r, k)
                    yield

    def prep_q(u):
        w = q_blocks(u)
        for a in range(2):
            g = 2 * (u // 2) + a
            for c in range(2):
                blocks = [w[pl.ds((2 * half + c) * 128, 128), pl.ds(b * 256 + a * 128, 128)]
                          for b in range(2) for half in range(2)]
                put_folded(blocks, g, g + 4, a1_v.at[2 + u // 2], lambda j: a * 64 + 8 * j, u % 2 + 2 * c)
                yield

    def split_q(u):
        for r in range(8):
            for i in range(7):
                split_again(a1_v.at[2 + u // 2 + zero_s[0]], per_operand(a2_v.at[2 + u // 2]), True, i, r, u % 2)
                yield

    def prep_wo(u, base):
        g = (u // 2) * 4 + u % 2
        return put_transposed(base, g, g + 2, wo_v.at[u // 2], lambda j: (u % 2) * 64 + 8 * j)

    def x_block(r0, n, cols):
        return jnp.concatenate([in_v[pl.ds(pl.multiple_of(r0 + q + (zero_s[1] if q % 16 and n == 16 else 0), 8), 8), cols].astype(f32)
                                for q in range(0, n, 8)], axis=0)

    def ln_stats(t, st, batch):
        lane = lax.broadcasted_iota(i32, (16, 128), 1)
        for start in range(0, 32, batch):
            places = [((step % 2) * 16 + step // 2) * 16 for step in range(start, start + batch)]
            means = variances = jnp.ones((16, 128), f32)
            for n, pos in enumerate(places):
                r0 = pl.multiple_of(t * T + pos, 16)
                x0 = x_block(r0, 16, pl.ds(0, 128)) + pin(16)
                s1 = s2 = None
                for j in range(1, 8):
                    d = x_block(r0, 16, pl.ds(j * 128, 128)) - x0
                    s1 = d if j == 1 else s1 + d
                    s2 = d * d if j == 1 else s2 + d * d
                lane_mean = x0 + s1 * 0.125
                mean = jnp.sum(lane_mean, axis=-1, keepdims=True) * (1.0 / 128)
                d = lane_mean - mean
                var = jnp.sum((s2 - s1 * s1 * 0.125) * 0.125 + d * d, axis=-1, keepdims=True)
                variances = jnp.where(lane == n, jnp.broadcast_to(var, (16, 128)), variances)
                means = jnp.where(lane == n, jnp.broadcast_to(mean, (16, 128)), means)
                yield
            means = means.astype(bf16).astype(f32)
            var = ((variances * (1.0 / 128)).astype(bf16).astype(f32) + EPS_BF16).astype(bf16).astype(f32)
            scale = 1.0 / jnp.sqrt(var).astype(bf16).astype(f32)
            for n, pos in enumerate(places):
                for kind, v in enumerate((means, scale)):
                    st[kind, pl.ds(pos, 16), :] = jnp.broadcast_to(v[:, n:n + 1], (16, 128))
                if (n + 1) % (batch // 4) == 0:
                    yield

    def ln_apply(t, st, dst, score_too):
        for step in range(16):
            r0 = [pl.multiple_of(t * T + b * TH + step * 16 + zero_s[0], 16) for b in range(2)]
            mean = [st[0, pl.ds(b * TH + step * 16, 16), :] for b in range(2)]
            scale = [st[1, pl.ds(b * TH + step * 16, 16), :] for b in range(2)]
            score = [None, None]
            for k in range(4):
                zero = pin(16)
                xn = [[(x_block(r0[b], 16, pl.ds(half * 512 + k * 128, 128)) - (mean[b] + zero)) * scale[b]
                       for half in range(2)] for b in range(2)]
                for i, v in enumerate(_rhs_operands(xn[0][0], xn[1][0], xn[0][1], xn[1][1])):
                    dst.at[i][pl.ds(step * 8, 8), pl.ds(k * 128, 128)] = _narrow(v)
                for b in range(2 if score_too else 0):
                    part = xn[b][0] * wr_v[:, pl.ds(k * 128, 128)] + xn[b][1] * wr_v[:, pl.ds(512 + k * 128, 128)]
                    score[b] = part if k == 0 else score[b] + part
                    if k == 3:
                        r = jnp.sum(score[b], axis=-1, keepdims=True).astype(bf16).astype(f32)
                        r = jnp.broadcast_to(r, (16, 128))
                        token = lax.broadcasted_iota(i32, (16, 128), 0) + r0[b] % S
                        slot = 2 * (t // NTILE) + b
                        better = r > best_v[slot]
                        best_v[slot] = jnp.where(better, r, best_v[slot])
                        best_i[slot] = jnp.where(better, token, best_i[slot])
                yield

    def ln_split(once, twice):
        for i in PRODUCT_ORDER:
            for r in range(8):
                for k in range(2):
                    split_again(once, twice, False, i, r, k)
                    yield

    def route():
        score, token = best_v[...].reshape(64, 128), best_i[...].reshape(64, 128)
        top = jnp.max(score, axis=0, keepdims=True)
        idx = jnp.min(jnp.where(score == top, token, S).astype(f32)).astype(i32)
        return jnp.clip(idx, 0, S - 1), top

    def routed_token():
        idx = route()[0]
        base = pl.multiple_of((idx // 16) * 16, 16)
        rows = pl.ds(pl.multiple_of(base % T, 16), 16)
        xn = (in_v[pl.ds(base, 16), :].astype(f32) - st_v[idx // T, 0, rows, 0:1]) * st_v[idx // T, 1, rows, 0:1]
        xn = jnp.where(lax.broadcasted_iota(i32, (16, D), 0) == idx - base, xn, 0.0)
        xn = jnp.sum(xn, axis=0, keepdims=True).astype(bf16).astype(f32)
        for j in range(8):
            row = xn[:, j * 128:(j + 1) * 128] + pin()
            xcol_v[pl.ds(j * 128, 128), :] = jnp.concatenate([row] * 16, axis=0).T
            yield

    def ffn(f0, n):
        for j in range(n):
            group, f = ffn_v.at[(f0 + j) // FG], (f0 + j) % FG
            accs = [jnp.zeros((8, 128), f32)] * 2
            for r in range(8):
                x, zero = xcol_v[pl.ds(r * 128, 128), :], pin()
                for a in range(2):
                    prod = group[pl.ds(_aligned((a * FG + f) * D + r * 128, 128), 128), :].astype(f32) * x
                    acc = accs[a] + zero
                    for q in range(16):
                        acc = acc + prod[8 * q:8 * q + 8]
                    accs[a] = acc
                yield
            gate, up = [jnp.sum(acc, axis=0, keepdims=True) for acc in accs]
            hidden = jnp.broadcast_to(gate * jax.nn.sigmoid(gate) * up, (128, 128)).T
            for c in range(8):
                prod = group[pl.ds(_aligned(2 * FG * D + (c * FG + f) * 128, 128), 128), :].astype(f32) * hidden
                acc = y_acc[:, pl.ds(c * 128, 128)] + pin()
                for q in range(16):
                    acc = acc + prod[8 * q:8 * q + 8]
                y_acc[:, pl.ds(c * 128, 128)] = acc
                if c % 2:
                    yield

    def project(w, x, res, keep=None):
        def emit(r, b, val):
            if isinstance(res, list):
                res[r][b] = val
            else:
                res[r, b] = val
            if keep is not None:
                keep[r, b] = val[64:]

        def once():
            for c in range(2):
                def put(a, b, val):
                    emit(2 * a, 2 * b + c, val[:128])
                    emit(2 * a + 1, 2 * b + c, val[128:])

                yield from _strassen(lambda i: matmul(w[i], x[i, pl.ds(c * 64, 64), :], 14), put)

        if isinstance(w, tuple):
            return _strassen_twice(lambda i: matmul(operand(*w, True, i), operand(*x, False, i), 49), emit), 49, 0.0, 1.0
        return once(), 14, 0.0, 1.0

    def project_part(w, x, res, part):
        def prod(i):
            rows = [w[i, pl.ds(a * 64 + part * 32, 32), :] for a in range(2)]
            return matmul(jnp.concatenate(rows, axis=0), x[i], 14)

        def put(a, b, val):
            for r in range(2):
                for c in range(2):
                    res[2 * a + r, 2 * b + c, pl.ds(part * 64, 64), :] = val[r * 64:(r + 1) * 64, c * 128:(c + 1) * 128]

        return _strassen(prod, put)

    def rows_of(res, r, r0, b):
        return res[r][b][r0:r0 + 64] if isinstance(res, list) else res[r, b, pl.ds(r0, 64), :]

    def kv_post(c, res, keep=None, values_late=False):
        same_head = lax.broadcasted_iota(i32, (64, 128), 0) // DH == lax.broadcasted_iota(i32, (64, 128), 1) % 2

        sums = {}

        def accumulate(r, b, phi):
            v = jnp.concatenate([rows_of(res, r, 64, b), jnp.ones((16, 128), f32)], axis=0)
            part = _dot_nt(v.astype(bf16), phi.astype(bf16))[:72]
            sums[r] = (kv_acc[4 * c + r] if b == 0 else sums[r]) + part
            if b == 3:
                total = kv_acc[4 * c + r] = sums.pop(r)
                kv_v.at[4 * c + r][...] = jnp.where(same_head, total[:64], 0.0).astype(bf16)
                z_v[4 * c + r] = jnp.concatenate([total[64:]] * 16, axis=0).T

        pending = []
        for r in range(4):
            for b in range(4):
                phi = _dual_softmax(rows_of(res, r, 0, b), pin())
                if keep is not None:
                    keep.at[r][:, pl.ds(b * 128, 128)] = _narrow(phi)
                pending.append((r, b, phi))
                if len(pending) > 3 and not values_late:
                    accumulate(*pending.pop(0))
                yield
        yield
        for rest in pending:
            accumulate(*rest)
        yield

    def q_post(c, res, dst, ready=None, lag=3):
        even = lax.broadcasted_iota(i32, (8, 128), 0) % 2 == 0
        phis, scales, nums, outs = {}, {}, {}, {}

        def pair(step):
            return 2 * (2 * c + step // 4 + 4 * ((step // 2) % 2)) + step % 2

        for tick in range(32 + lag):
            step, b = tick // 4, tick % 4
            if step < 8:
                r = 2 * ((step // 2) % 2) + step // 4
                if ready is None:
                    phi = _dual_softmax(rows_of(res, r, (step % 2) * 64, b), pin())
                elif step % 2:
                    phi = _dual_softmax(rows_of(res, r, 0, b), pin())
                else:
                    phi = _wide(ready[r, :, pl.ds(b * 128, 128)])
                den = phi * z_v[pair(step)]
                inv = _recip(_head_reduce([den[8 * j:8 * j + 8] for j in range(16)], jnp.add) + 1e-6)
                other = pltpu.roll(inv, 1, 0)
                phis[tick] = phi
                scales[tick] = [jnp.where(even, inv, other)] * 4 + [jnp.where(even, other, inv)] * 4
            n = tick - lag
            if 0 <= n < 32:
                num = _dot(kv_v[pair(n // 4)], phis.pop(n).astype(bf16))
                outs[n] = num * jnp.concatenate(scales.pop(n), axis=0)
                if n % 16 == 15:
                    u = n // 16
                    o = [[jnp.concatenate([jnp.concatenate([outs.pop(16 * u + 8 * a + 4 * p + 2 * h + j) for j in range(2)], axis=1)
                                           for p in range(2)], axis=0) for h in range(2)] for a in range(2)]
                    for i, v in enumerate(_rhs_operands(o[0][0], o[0][1], o[1][0], o[1][1])):
                        dst.at[i][:, pl.ds(u * 128, 128)] = pltpu.bitcast(v.astype(bf16).T, u32)
            yield

    def out_project(h, o, res, ks, per_slot):
        def prod(i):
            lhs = jnp.concatenate([o[k][i] for k in ks], axis=1)
            return matmul(lhs, wo_v[h, i, :, pl.ds(ks[0] * 256, len(ks) * 256)], per_slot)

        def emit(a, b, val):
            if isinstance(res, list):
                res[a][b] = val
            else:
                res[a, b] = val

        return _strassen(prod, emit)

    zero_s[0] = 0
    zero_s[1] = 0
    kv_acc[...] = jnp.zeros(kv_acc.shape, f32)
    y_acc[...] = jnp.zeros(y_acc.shape, f32)
    best_v[...] = jnp.full(best_v.shape, -jnp.inf, f32)
    best_i[...] = jnp.zeros(best_i.shape, i32)
    w8 = wr8_v[...].astype(f32)
    wr_v[...] = jnp.broadcast_to(jnp.concatenate([w8[j:j + 1, :] for j in range(8)], axis=1), (16, D))
    feature_maps()
    stats, apply = ln_stats(0, st_v.at[0], 16), ln_apply(0, st_v.at[0], x1_v.at[0], False)
    for half in range(2):
        cp_x0(2 * half).wait()
        cp_x0(2 * half + 1).wait()
        schedule((stats, 20, 0.0, 1.0))
        schedule((apply, 32, 0.0, 1.0))
    chunk0 = prep_kv(0)
    schedule((chunk0, 4, 0.0, 1.0))
    schedule((project_part(a1_v.at[0], x1_v.at[0], raw_v.at[0], 0), 7, 0.0, 0.5),
             (project_part(a1_v.at[0], x1_v.at[0], raw_v.at[0], 1), 7, 0.5, 1.0),
             (project(a1_v.at[1], x1_v.at[0], raw_v.at[1])[0], 14, 1.0, 2.0),
             (chunk0, 4, 0.15, 0.45), (ln_split(x1_v.at[zero_s[0]], [x.at[0] for x in x2_v]), 112, 0.03, 0.6),
             (kv_post(0, raw_v.at[zero_s[0]], values_late=True), 18, 0.52, 1.3),
             (split_kv(0), 112, 0.47, 0.75), (prep_kv(1), 8, 0.74, 0.96), (split_kv(1), 112, 1.02, 1.31),
             (prep_kv(2), 8, 1.05, 1.3), (split_kv(2), 112, 1.31, 1.64),
             (prep_kv(3), 8, 1.49, 1.7), (split_kv(3), 112, 1.73, 2.0))

    def kv_tile(t, _):
        last = t == NTILE - 1
        wait_all(q_blocks(t), sem_q.at[t])
        cp_xt(t + 1).wait()

        @pl.when(jnp.logical_and(t > 0, t < 3))
        def _():
            cp_wo(t - 1).wait()

        product[:] = []
        first = (route()[0] // T) % (NTILE - 1) + 1
        x1, x2, st = x1_v.at[pl.ds(t, 2)], [x.at[pl.ds(t, 2)] for x in x2_v], st_v.at[t + 1]
        split = ln_split(x1_v.at[t + 1 + zero_s[0]], [x.at[1] for x in x2])
        x = x1.at[0], [x.at[0] for x in x2]
        wo = [prep_wo(2 * ((t + 1) % 2) + u, jnp.where(t == 0, WV, WO)) for u in range(2)]
        c2, c3, c0 = ([[None] * 4 for _ in range(4)] for _ in range(3))
        again = split_q(t)
        schedule(project((b1_v.at[0], per_operand(b2_v.at[0])), x, c2),
                 (kv_post(1, raw_v.at[1]), 18, 0.188, 1.0), (ln_stats(t + 1, st, 32), 36, 0.0, 0.912),
                 (prep_q(t), 4, 0.002, 0.612), (again, 28, 0.55, 1.0), (start_ffn(t), 2 * FG + 8, 0.072, 0.992))
        schedule(project((b1_v.at[1], per_operand(b2_v.at[1])), x, c3),
                 (kv_post(2, c2), 18, 0.032, 0.935), (ln_apply(t + 1, st, x1.at[1], True), 64, 0.0, 0.8),
                 (again, 28, 0.06, 0.77), (split, 24, 0.81, 0.97))
        nxt, chunk = jnp.where(last, first, t + 1), jnp.where(last, 2, 0)
        x = x1_v.at[nxt], [x.at[nxt] for x in x2_v]
        schedule(project((a1_v.at[chunk], per_operand(a2_v.at[chunk])), x, c0, keep=half_v),
                 (kv_post(3, c3), 18, 0.0, 0.905), (split, 88, 0.0, 0.612))
        schedule(project((a1_v.at[chunk + 1], per_operand(a2_v.at[chunk + 1])), x, raw_v.at[1]),
                 (kv_post(jnp.where(last, 4, 0), c0, keep=phi_v), 18, 0.05, 0.905),
                 (wo[0], 4, 0.002, 0.6), (wo[1], 4, 0.525, 0.913), (routed_token(), 8, 0.073, 0.656))
        return first

    first = lax.fori_loop(0, NTILE, kv_tile, jnp.int32(0))

    wait_all(ffn_v.at[0], sem_f.at[0])
    product[:] = []
    idx, top_score = route()
    final = idx // T
    lo, hi = jnp.minimum(first, final), jnp.maximum(first, final)
    second = jnp.where(lo > 0, 0, jnp.where(hi > 1, 1, 2))
    third = 6 - first - final - second

    def tile(j):
        return jnp.where(j == 0, first, jnp.where(j == 1, second, jnp.where(j == 2, third, final)))

    def gate(t, h, a, b, q, update):
        r0, rows = pl.multiple_of(t * T + b * TH + q * EROWS, EROWS), pl.ds(b * TH + q * EROWS, EROWS)
        c0 = h * 512 + a * 256
        mean, scale = st_v[t, 0, rows, :], st_v[t, 1, rows, :] * 0.5
        if update is None:
            mean = mean + pin(EROWS)
        x = x_block(r0, EROWS, pl.ds(c0, 256))
        v = (x - jnp.concatenate([mean, mean], axis=1)) * jnp.concatenate([scale, scale], axis=1)
        if update is not None:
            hit = lax.broadcasted_iota(i32, (EROWS, 256), 0) == idx - r0
            v = v + jnp.where(hit, update[:, c0:c0 + 256], 0.0)
        return x, v + v * jnp.tanh(v)

    def epilogue(t, h, res, part=None, update=None, early=None):
        for a, b in ((0, 1), (0, 0), (1, 0), (1, 1)) if part is not None else ((0, 0), (0, 1), (1, 0), (1, 1)):
            for q in range(TH // EROWS):
                r0, cols = pl.multiple_of(t * T + b * TH + q * EROWS, EROWS), pl.ds(h * 512 + a * 256, 256)
                if early is not None and (a, b) == (1, 1):
                    x, g = x_block(r0, EROWS, cols), early[pl.ds(q * EROWS, EROWS), :]
                else:
                    x, g = gate(t, h, a, b, q, update)
                s = res[a][b][q * EROWS:(q + 1) * EROWS]
                if part is not None:
                    s = s + part[a, b, pl.ds(q * EROWS, EROWS), :]
                out_v[pl.ds(r0, EROWS), cols] = (x + s * g).astype(bf16)
                if part is not None and (q + 1) * EROWS % 128 == 0:
                    start_out(pl.ds(pl.multiple_of(t * T + b * TH + (q + 1) * EROWS - 128, 128), 128), cols)
                yield

    steps = 4 * TH // EROWS
    schedule((q_post(0, half_v, oa_v.at[0], ready=phi_v), 35, 0.01, 1.0))

    def q_tile(j, carry):
        product[:] = []
        oa = oa_v.at[pl.ds(j, 2)]
        o = oa.at[0], ob_v.at[zero_s[0]]
        x = x1_v.at[tile(j + 1)], [x.at[tile(j + 1)] for x in x2_v]
        wait_all(ffn_v.at[j + 1], sem_f.at[j + 1])
        hidden = ffn(j * FL, FL)
        q0, s0, s1 = ([[None] * 4 for _ in range(4)] for _ in range(3))
        schedule(project((a1_v.at[2], per_operand(a2_v.at[2])), x, q0),
                 (q_post(1, raw_v.at[1], ob_v.at[0]), 35, 0.012, 0.898), (hidden, 14, 0.072, 0.95))
        schedule((out_project(0, o, s0, (0, 1), 7), 7, 0.0, 1.0),
                 (q_post(0, q0, oa.at[1]), 35, 0.0, 0.988), (hidden, 18, 0.169, 0.97))
        schedule((out_project(1, o, s1, (0, 1), 7), 7, 0.0, 1.0),
                 (epilogue(tile(j), 0, s0), steps, 0.043, 1.0), (hidden, 38, 0.044, 0.97))
        schedule(project((a1_v.at[3], per_operand(a2_v.at[3])), x, raw_v.at[1]),
                 (epilogue(tile(j), 1, s1), steps, 0.03, 0.853), (hidden, 12 * FL - 70, 0.0, 0.885))
        start_out(pl.ds(pl.multiple_of(tile(j) * T, T), T), slice(None))
        return carry

    lax.fori_loop(0, NTILE - 1, q_tile, 0)

    product[:] = []
    o = oa_v.at[NTILE - 1], ob_v.at[zero_s[0]]
    rest = NF - (NTILE - 1) * FL
    schedule((out_project(0, o, part_v.at[0], (0,), 14), 7, 0.0, 0.5),
             (out_project(1, o, part_v.at[1], (0,), 14), 7, 0.5, 1.0),
             (q_post(1, raw_v.at[1], ob_v.at[0]), 35, 0.0, 0.9), (ffn(NF - rest, rest), 12 * rest, 0.1, 0.8))
    update = jnp.sum(y_acc[...], axis=0, keepdims=True) * (0.5 * jax.nn.sigmoid(top_score[:, 0:1]))
    s0, s1 = ([[None, None], [None, None]] for _ in range(2))

    def last_gate():
        for q in range(TH // EROWS):
            gate_v[0, pl.ds(q * EROWS, EROWS), :] = gate(final, 1, 1, 1, q, update)[1]
            yield

    schedule((out_project(0, o, s0, (1,), 14), 7, 0.0, 0.5), (out_project(1, o, s1, (1,), 14), 7, 0.5, 1.0),
             (epilogue(final, 0, s0, part_v.at[0], update), steps, 0.2, 0.66),
             (epilogue(final, 1, s1, part_v.at[1], update, gate_v.at[zero_s[0]]), steps, 0.69, 1.21),
             (last_gate(), TH // EROWS, 0.0, 0.2))
    pltpu.make_async_copy(out_v, out_hbm, sem_o.at[0]).wait()


def _call(x, wqkv, wphi, wo, wr, wg, wu, wd, interpret=False):
    scratch = [
        pltpu.VMEM((S + T + 4 * D, D), bf16),
        pltpu.VMEM((NTILE + 1, 2, T, 128), f32),
        pltpu.VMEM((NTILE + 1, 7, 128, 512), u32),
        [pltpu.VMEM((NTILE + 1, 5, 64, 256), u32)] * 7,
        pltpu.VMEM((D, DH), bf16),
        pltpu.VMEM((8, 128), bf16),
        pltpu.VMEM((16, D), f32),
        pltpu.VMEM((8, 128, 128), bf16),
        pltpu.VMEM((4, 7, 128, 512), u32),
        pltpu.VMEM((4, 35, 64, 256), u32),
        pltpu.VMEM((2, 7, 128, 512), u32),
        pltpu.VMEM((2, 35, 64, 256), u32),
        pltpu.VMEM((2, 7, 128, 512), u32),
        pltpu.VMEM((NTILE, 3 * FG * D, 128), bf16),
        pltpu.VMEM((H // 2 + 4, 72, 128), f32),
        pltpu.VMEM((H // 2 + 4, 64, 128), bf16),
        pltpu.VMEM((H // 2 + 4, 128, 128), f32),
        pltpu.VMEM((4, 16, 128), f32),
        pltpu.VMEM((4, 16, 128), i32),
        pltpu.VMEM((2, 4, 4, 128, 128), f32),
        pltpu.VMEM((4, 4, 64, 128), f32),
        pltpu.VMEM((4, 64, T), u32),
        pltpu.VMEM((NTILE, 7, 128, 256), u32),
        pltpu.VMEM((2, 7, 128, 256), u32),
        pltpu.VMEM((2, 2, 2, 256, 256), f32),
        pltpu.VMEM((2, 256, 256), f32),
        pltpu.VMEM((D, 128), f32),
        pltpu.VMEM((8, D), f32),
        pltpu.VMEM((S, D), bf16),
        pltpu.SMEM((2,), i32),
        pltpu.SemaphoreType.DMA((NTILE + 2,)),
        pltpu.SemaphoreType.DMA((5,)),
        pltpu.SemaphoreType.DMA((NTILE + 2,)),
        pltpu.SemaphoreType.DMA((1,)),
        pltpu.SemaphoreType.DMA((NTILE,)),
        pltpu.SemaphoreType.DMA((1,)),
    ]
    hbm = pl.BlockSpec(memory_space=pltpu.HBM)
    return pl.pallas_call(
        _kernel,
        out_shape=jax.ShapeDtypeStruct((S, D), bf16),
        in_specs=[hbm] * 8,
        out_specs=hbm,
        scratch_shapes=scratch,
        compiler_params=pltpu.CompilerParams(
            vmem_limit_bytes=120 * 2**20, disable_bounds_checks=True, disable_semaphore_checks=True),
        name="hedgehog",
        interpret=interpret,
    )(x, wqkv, wphi, wo, wr, wg, wu, wd)


@jax.jit
def pallas_recurrent_scan__linear_kernel_hedgehog__moe_arch_mod__prompt_kernel(
    A_x: jax.Array,
    A_wqkv: jax.Array,
    A_w_phi: jax.Array,
    A_wo: jax.Array,
    B_x: jax.Array,
    B_w_r: jax.Array,
    B_w_gate: jax.Array,
    B_w_up: jax.Array,
    B_w_down: jax.Array,
):
    del B_x
    out = _call(A_x.reshape(S, D), A_wqkv, A_w_phi.reshape(D, DH), A_wo,
                B_w_r.reshape(8, 128), B_w_gate, B_w_up, B_w_down)
    return out.reshape(1, S, D)
```
